```python
import jax
import jax.numpy as jnp

def _softmax(x, axis=-1):
    return jax.nn.softmax(x, axis=axis)
def _gelu(x):
    return jax.nn.gelu(x, approximate=True)
def _silu(x):
    return jax.nn.silu(x)
def _sigmoid(x):
    return jax.nn.sigmoid(x)
def _layernorm(x, axis=-1, eps=1e-5):
    m = jnp.mean(x, axis=axis, keepdims=True)
    v = jnp.var(x, axis=axis, keepdims=True)
    return (x - m) / jnp.sqrt(v + eps)
def _scatter_add(tgt, idx, src, axis=0):
    return tgt.at[idx].add(src)
def _segment_sum(src, seg, n):
    return jax.ops.segment_sum(src, seg, n)
class _Rng:
    def __init__(self, key):
        self._k = key
    def _next(self):
        self._k, sub = jax.random.split(self._k)
        return sub
    def normal(self, shape):
        return jax.random.normal(self._next(), shape, dtype=jnp.bfloat16)
    def randint(self, lo, hi, shape):
        return jax.random.randint(self._next(), shape, lo, hi, dtype=jnp.int32)
    def uniform(self, shape, lo=0.0, hi=1.0):
        return jax.random.uniform(self._next(), shape, jnp.bfloat16, lo, hi)
    def permutation(self, n):
        return jax.random.permutation(self._next(), n)


kernel_name = 'concat_heads__sliding_local_dilated__compressed_kv_cla__prompt'

def setup_inputs():
    _rng = _Rng(jax.random.key(int.from_bytes(__import__("os").urandom(4), "little")))
    _w = (lambda a: (lambda t: t.astype(jnp.bfloat16) if jnp.issubdtype(t.dtype, jnp.floating) else t)(jnp.asarray(a)))
    def _A_setup():
        B, S, D = 1, 2048, 1024
        return {
            "x": _w((lambda *s: _rng.normal(s) * 0.05)(B, S, D)),
            "wqkv": _w((lambda *s: _rng.normal(s) * 0.05)(D, 3 * D)),
            "wo": _w((lambda *s: _rng.normal(s) * 0.05)(D, D)),
        }
    _A_in = _A_setup()

    def _B_setup():
        B, H, Sq, Sk, D, M = 1, 32, 2048, 2048, 128, 1024
        Dc = 4 * D
        return {
            "x": _w((lambda *s: _rng.normal(s) * 0.05)(B, Sq, M)),
            "c_kv": _w((lambda *s: _rng.normal(s) * 0.05)(B, Sk, Dc)),
            "w_q": _w((lambda *s: _rng.normal(s) * 0.05)(M, H, D) * (M ** -0.5)),
            "w_uk": _w((lambda *s: _rng.normal(s) * 0.05)(Dc, H, D) * (Dc ** -0.5)),
            "w_uv": _w((lambda *s: _rng.normal(s) * 0.05)(Dc, H, D) * (Dc ** -0.5)),
            "w_o": _w((lambda *s: _rng.normal(s) * 0.05)(H, D, M) * ((H * D) ** -0.5)),
        }
    _B_in = _B_setup()

    return {
        "A_x": _A_in["x"],
        "A_wqkv": _A_in["wqkv"],
        "A_wo": _A_in["wo"],
        "B_x": _B_in["x"],
        "B_c_kv": _B_in["c_kv"],
        "B_w_q": _B_in["w_q"],
        "B_w_uk": _B_in["w_uk"],
        "B_w_uv": _B_in["w_uv"],
        "B_w_o": _B_in["w_o"],
    }

def reference(A_x, A_wqkv, A_wo, B_x, B_c_kv, B_w_q, B_w_uk, B_w_uv, B_w_o):
    def _A_ref(x, wqkv, wo):
        B, S, D = x.shape
        H = 32; Dh = D // H
        W, dil = 8, 2
        qkv = (lambda x, *d: x.transpose(*d))((x @ wqkv).reshape(B, S, 3, H, Dh), 2, 0, 3, 1, 4)
        q, k, v = qkv[0], qkv[1], qkv[2]
        scale = Dh ** -0.5
        pos = jnp.arange(S)
        off = jnp.arange(W) * dil
        idx = pos[:, None] - off[None, :]
        mask = idx >= 0
        idx_c = jnp.where(mask, idx, 0).reshape(-1)
        kg = k[:, :, idx_c, :].reshape(B, H, S, W, Dh)
        vg = v[:, :, idx_c, :].reshape(B, H, S, W, Dh)
        logits = jnp.einsum("bhsd,bhswd->bhsw", q, kg) * scale
        logits = jnp.where(mask[None, None, :, :], logits, -1e9)
        attn = _softmax(logits, axis=-1)
        o = jnp.einsum("bhsw,bhswd->bhsd", attn, vg)
        return (lambda x, *d: x.transpose(*d))(o, 0, 2, 1, 3).reshape(B, S, D) @ wo

    def _B_ref(x, c_kv, w_q, w_uk, w_uv, w_o):
        B, Sq, M = x.shape[0], x.shape[1], x.shape[2]
        Sk = c_kv.shape[1]
        H, D = w_q.shape[1], w_q.shape[2]
        q = jnp.einsum("bqm,mhd->bhqd", x, w_q)
        k = jnp.einsum("bkc,chd->bhkd", c_kv, w_uk)
        v = jnp.einsum("bkc,chd->bhkd", c_kv, w_uv)
        scores = jnp.einsum("bhqd,bhkd->bhqk", q, k) * (D ** -0.5)
        off = Sk - Sq
        qi = jnp.arange(Sq)[:, None]
        kj = jnp.arange(Sk)[None, :]
        cmask = kj <= (qi + off)
        scores = jnp.where(cmask[None, None], scores, -1e9)
        p = _softmax(scores, axis=-1)
        ctx = jnp.einsum("bhqk,bhkd->bhqd", p, v)
        return jnp.einsum("bhqd,hdm->bqm", ctx, w_o)

    a = _A_ref(A_x, A_wqkv, A_wo)
    b = _B_ref(B_x, B_c_kv, B_w_q, B_w_uk, B_w_uv, B_w_o)
    return jnp.concatenate([a, b], axis=-1)
```

```python
import math

import jax
import jax.numpy as jnp
from jax import lax
import jax.experimental.pallas as pl
import jax.experimental.pallas.tpu as pltpu

S = 2048
DM = 1024
DC = 512
NH = 32
NP = NH // 2
T = 128
RB = 256
RA = 128
WIN, DIL = 8, 2
HALO = 16

LOG2E = math.log2(math.e)
SCALE_A = (DM // NH) ** -0.5 * LOG2E
SCALE_B = T ** -0.5 * LOG2E
MASKED = -1e9 * LOG2E

F32, BF16, U32 = jnp.float32, jnp.bfloat16, jnp.uint32


def _dot(a, b):
    return jnp.dot(a, b, preferred_element_type=F32)


def _dot_nt(a, b):
    return lax.dot_general(a, b, (((1,), (1,)), ((), ())), preferred_element_type=F32)


def _cat(xs, axis=1):
    return xs[0] if len(xs) == 1 else jnp.concatenate(xs, axis=axis)


def _tile(x, t):
    return x[:, t * T:(t + 1) * T]


def _words(ref, lead, start, n):
    half = start // 2
    if not isinstance(half, int):
        half = pl.multiple_of(half, 8)
    return ref.bitcast(U32)[(*lead, pl.ds(half, n // 2), slice(None))]


def _load(ref, lead, start, n):
    return pltpu.bitcast(_words(ref, lead, start, n), BF16)


def _split(w):
    return (pltpu.bitcast(w << 16, F32), pltpu.bitcast(w & jnp.uint32(0xFFFF0000), F32))


def _lhs_terms(a11, a12, a21, a22):
    return (a11 + a22, a21 + a22, a11, a22, a11 + a12, a21 - a11, a12 - a22)


def _rhs_terms(b11, b12, b21, b22):
    return (b11 + b22, b11, b12 - b22, b21 - b11, b22, b11 + b12, b21 + b22)


def _combine(m):
    m1, m2, m3, m4, m5, m6, m7 = m
    return (m1 + m4 - m5 + m7, m3 + m5, m2 + m4, m1 - m2 + m3 + m6)


def _kernel(ax_hbm, wqkv_hbm, wo_hbm, bx_hbm, c_hbm, wq_hbm, wuk_hbm, wuv_hbm, wob_hbm,
            out_hbm,
            bx_raw, c_raw, wq_raw, wk_raw, wv_raw, wob_raw, wqkv_raw, wo_raw, ax_raw,
            bx_t, c_t, ctx_t, wob_t, ax_t, wqkv_t, wo_t, o_t, kbuf, vbuf, obuf,
            zero_smem, sem_in, sem_w, sem_out):

    def pair_copies(j, slot):
        g = j % 8
        word = (g // 2) * 4 + g % 2
        wqkv32 = wqkv_hbm.bitcast(U32)
        wo32 = wo_hbm.bitcast(U32)
        xrow = (j // 2) * (2 * RA) + (j % 2) * (RA // 2)
        pairs = [
            (wuk_hbm.bitcast(U32).at[:, j, :], wk_raw.at[slot]),
            (wuv_hbm.bitcast(U32).at[:, j, :], wv_raw.at[slot]),
            (wq_hbm.bitcast(U32).at[:, j, :], wq_raw.at[slot]),
            (wob_hbm.at[pl.ds(2 * j, 2)], wob_raw.at[slot]),
            (wqkv32.at[pl.ds(pl.multiple_of(16 * j, 16), 16), :], wqkv_raw.at[slot, 0]),
            (wqkv32.at[pl.ds(pl.multiple_of(DM // 4 + 16 * j, 16), 16), :], wqkv_raw.at[slot, 1]),
            (wo32.at[:, word, :], wo_raw.at[slot, 0]),
            (wo32.at[:, word + 2, :], wo_raw.at[slot, 1]),
            (ax_hbm.at[pl.ds(pl.multiple_of(xrow, 64), RA // 2), :], ax_raw.at[slot, 0]),
            (ax_hbm.at[pl.ds(pl.multiple_of(xrow + RA, 64), RA // 2), :], ax_raw.at[slot, 1]),
        ]
        return [pltpu.make_async_copy(src, dst, sem_w.at[slot * len(pairs) + n])
                for n, (src, dst) in enumerate(pairs)]

    nchunk = S // (2 * RB)

    def act_copies(c):
        rows = pl.ds(pl.multiple_of(c * 2 * RB, 2 * RB), 2 * RB)
        return (pltpu.make_async_copy(c_hbm.at[rows, :], c_raw.at[rows, :], sem_in.at[2 * c]),
                pltpu.make_async_copy(bx_hbm.at[rows, :], bx_raw.at[rows, :], sem_in.at[2 * c + 1]))

    def out_copy(c, slot):
        rows = pl.ds(pl.multiple_of(c * 2 * RA, 2 * RA), 2 * RA)
        return pltpu.make_async_copy(obuf.at[slot], out_hbm.at[rows, :], sem_out.at[slot])

    class Tokens:
        def __init__(self):
            self.z = zero_smem[0]
            self.zv = jnp.full((8, T), self.z, jnp.int32).astype(U32)
            self.pending = []

        def after(self, ref, lead, delay):
            first, *rest = lead
            self.pending.append([delay, _words(ref, (first + self.z, *rest), 0, 16) & self.zv])

        def lhs(self, ref, lead, start, n):
            w = _words(ref, lead, start, n)
            return self.tie(w)

        def tie(self, w):
            if self.pending and self.pending[0][0] <= 0:
                w = jnp.concatenate([w[:8] | self.pending.pop(0)[1], w[8:]], axis=0)
            for p in self.pending:
                p[0] -= 1
            return pltpu.bitcast(w, BF16)

    for c in range(nchunk):
        for cp in act_copies(c):
            cp.start()
        if c == 0:
            for cp in pair_copies(0, 0):
                cp.start()
    zero_smem[0] = 0
    for t in range(DM // T):
        kbuf[t, pl.ds(2 * RA, HALO), :] = jnp.zeros((HALO, T), F32)
        vbuf[t, pl.ds(2 * RA, HALO), :] = jnp.zeros((HALO, T), F32)

    def prologue(c, carry):
        top = pl.ds(pl.multiple_of(c * 2 * RB, RB), RB)
        bot = pl.ds(pl.multiple_of(c * 2 * RB + RB, RB), RB)
        dst = pl.ds(pl.multiple_of(c * RB, RB), RB)
        for cp, raw, terms in zip(act_copies(c), (c_raw, bx_raw), (c_t, bx_t)):
            cp.wait()
            nt = terms.shape[1]
            for t in range(nt):
                blocks = [raw[rows, pl.ds(col * T, T)].astype(F32)
                          for rows in (top, bot) for col in (t, nt + t)]
                for i, val in enumerate(_lhs_terms(*blocks)):
                    terms[i, t, dst, :] = val.astype(BF16)
        return carry

    lax.fori_loop(0, nchunk, prologue, 0)

    def pair_body(j, carry):
        slot = j % 2
        for cp in pair_copies(j, slot):
            cp.wait()

        @pl.when(j + 1 < NP)
        def _():
            for cp in pair_copies(j + 1, 1 - slot):
                cp.start()

        tok = Tokens()
        causal = (lax.broadcasted_iota(jnp.int32, (T, T), 1)
                  <= lax.broadcasted_iota(jnp.int32, (T, T), 0))

        def pair_terms(raw):
            k = raw.shape[1] // 2
            b11, b12 = _split(raw[slot, pl.ds(0, k), :])
            b21, b22 = _split(raw[slot, pl.ds(k, k), :])
            return [v.astype(BF16) for v in _rhs_terms(b11, b12, b21, b22)]

        wq, wk, wv = pair_terms(wq_raw), pair_terms(wk_raw), pair_terms(wv_raw)
        q, k, v = {}, {}, {}

        def scatter(dst, c, quads):
            for n, val in enumerate(quads):
                for r in range(RB // T):
                    dst[(2 * c + n // 2) * (RB // T) + r, n % 2] = val[r * T:(r + 1) * T].astype(BF16)

        def proj_q(c):
            m = [_dot(_cat([tok.lhs(bx_t, (i, t), c * RB, RB) for t in range(4)]), wq[i])
                 for i in range(7)]
            scatter(q, c, [x * SCALE_B for x in _combine(m)])

        def proj_kv(c):
            mk, mv = [], []
            for i in range(7):
                a = _cat([tok.lhs(c_t, (i, t), c * RB, RB) for t in range(2)])
                mk.append(_dot(a, wk[i]))
                mv.append(_dot(a, wv[i]))
            scatter(k, c, _combine(mk))
            scatter(v, c, _combine(mv))

        scores, ctx = {}, {}

        def score(i, h):
            qi = tok.tie(pltpu.bitcast(q[i, h], U32)) if tok.pending else q[i, h]
            s = _dot_nt(qi, _cat([k[t, h] for t in range(i + 1)], axis=0))
            tiles = [_tile(s, t) for t in range(i + 1)]
            tiles[-1] = jnp.where(causal, tiles[-1], MASKED)
            scores[i, h] = tiles

        def attend(i, h):
            tiles = scores.pop((i, h))
            m = tiles[0]
            for s in tiles[1:]:
                m = jnp.maximum(m, s)
            m = jnp.max(m, axis=1, keepdims=True)
            p = [jnp.exp2(s - m) for s in tiles]
            l = p[0]
            for x in p[1:]:
                l = l + x
            l = jnp.sum(l, axis=1, keepdims=True)
            o = _dot(_cat(p).astype(BF16), _cat([v[t, h] for t in range(i + 1)], axis=0))
            r = pl.reciprocal(l, approx=True)
            ctx[i, h] = o * (r * (2.0 - l * r))
            b = i // 2
            quad = [(2 * b, 0), (2 * b, 1), (2 * b + 1, 0), (2 * b + 1, 1)]
            if all(u in ctx for u in quad):
                for n, val in enumerate(_lhs_terms(*(ctx.pop(u) for u in quad))):
                    ctx_t[n, j, pl.ds(b * RA, RA), :] = val.astype(BF16)
                tok.pending.append(
                    [1, _words(ctx_t, (6, j + tok.z), b * RA, 16) & tok.zv])

        def prep_wob():
            rows = pl.ds(pl.multiple_of(j * T, T), T)
            for n in range(4):
                blocks = [wob_raw[slot, h, :, pl.ds(col * T, T)].astype(F32)
                          for h in range(2) for col in (n, 4 + n)]
                for i, val in enumerate(_rhs_terms(*blocks)):
                    wob_t[i, n, rows, :] = val.astype(BF16)
            tok.pending.append([2, _words(wob_t, (6, 3 + tok.z), j * T, 16) & tok.zv])

        def prep_ax():
            rows = pl.ds(pl.multiple_of(j * (RA // 2), RA // 2), RA // 2)
            for t in range(4):
                blocks = [ax_raw[slot, half, :, pl.ds(col * T, T)].astype(F32)
                          for half in range(2) for col in (t, 4 + t)]
                for i, val in enumerate(_lhs_terms(*blocks)):
                    ax_t[i, t, rows, :] = val.astype(BF16)
            tok.pending.append([2, _words(ax_t, (6, 3 + tok.z), j * (RA // 2), 16) & tok.zv])

        def prep_wo():
            g = j % 8
            lo, hi = _split(wo_raw[slot, 0]), _split(wo_raw[slot, 1])
            for par in range(2):
                start = ((g % 2) * 2 + par) * T + (g // 2) * NH
                rows = pl.ds(pl.multiple_of(start, NH), NH)
                for n in range(4):
                    blocks = (_tile(lo[par], n), _tile(lo[par], 4 + n),
                              _tile(hi[par], n), _tile(hi[par], 4 + n))
                    for i, val in enumerate(_rhs_terms(*blocks)):
                        wo_t[i, n, rows, :] = val.astype(BF16)
            tok.pending.append([2, _words(wo_t, (6, 3 + tok.z), start, 16) & tok.zv])

        def prep_wqkv():
            lane = lax.broadcasted_iota(jnp.int32, (16, T), 1)
            e, grp, sub = lane >> 5, (lane >> 2) & 7, lane & 3
            rows = pl.ds(pl.multiple_of(j * 32, 32), 32)
            for mat in range(3):
                halves = []
                for half in range(2):
                    x = [wqkv_raw[slot, half, :, pl.ds(mat * DM + t * T, T)] for t in range(8)]
                    y = [jnp.take_along_axis(x[t], sub * 32 + e * 8 + ((grp - t) & 7), axis=1)
                         for t in range(8)]
                    u = [y[-s % 8] for s in range(8)]
                    for bit in (1, 2, 4):
                        u = [jnp.where((grp & bit) != 0, u[(s - bit) % 8], u[s]) for s in range(8)]
                    u = [u[0]] + [jnp.take_along_axis(u[t], e * 32 + ((grp + t) & 7) * 4 + sub, axis=1)
                                  for t in range(1, 8)]
                    halves.append([pltpu.bitcast(w, BF16).astype(F32) for w in u])
                for n in range(4):
                    blocks = (halves[0][n], halves[0][4 + n], halves[1][n], halves[1][4 + n])
                    for i, val in enumerate(_rhs_terms(*blocks)):
                        wqkv_t[i, mat * 4 + n, rows, :] = val.astype(BF16)
            tok.pending.append([2, _words(wqkv_t, (6, 11 + tok.z), j * 32, 16) & tok.zv])

        def both(i):
            return [(i, 0), (i, 1)]

        def steady(blocks, waiting):
            for i in blocks:
                for u in both(i):
                    score(*u)
                    waiting.append(u)
                    attend(*waiting.pop(0))

        proj_kv(0)
        prep_wob()
        proj_q(0)
        score(2, 0)
        score(2, 1)
        prep_ax()
        proj_kv(1)
        score(3, 0)
        attend(2, 0)
        prep_wo()
        proj_q(1)
        attend(2, 1)
        score(3, 1)
        attend(3, 0)
        waiting = [(3, 1)]
        steady(range(4, 8), waiting)
        prep_wqkv()
        proj_kv(2)
        proj_q(2)
        steady(range(8, 12), waiting)
        proj_kv(3)
        proj_q(3)
        steady(range(12, 16), waiting)
        for u in both(0) + both(1):
            score(*u)
        for u in waiting + both(0) + both(1):
            attend(*u)
        return carry

    lax.fori_loop(0, NP, pair_body, 0)

    def chunk_body(c, carry):
        slot = c % 2

        @pl.when(c >= 2)
        def _():
            out_copy(c - 2, slot).wait()

        tok = Tokens()
        row0 = c * RA

        for buf in (kbuf, vbuf):
            for t in range(8):
                buf[t, pl.ds(0, HALO), :] = buf[t, pl.ds(2 * RA, HALO), :]
        xs = [_cat([tok.lhs(ax_t, (i, t), row0, RA) for t in range(4)]) for i in range(7)]
        qa = {}
        for mat in (1, 0, 2):
            for n in range(4):
                quads = _combine([_dot(xs[i], _load(wqkv_t, (i, mat * 4 + n), 0, DM // 2))
                                  for i in range(7)])
                for quad, val in enumerate(quads):
                    half, t = quad // 2, (quad % 2) * 4 + n
                    if mat == 0:
                        qa[half, t] = val * SCALE_A
                    else:
                        (kbuf, vbuf)[mat - 1][t, pl.ds(HALO + half * RA, RA), :] = val

        def local_attention(half, r0, n):
            base = HALO + half * RA + r0
            logits = []
            for w in range(WIN):
                rows = pl.ds(base - DIL * w, n)
                acc = qa[half, 0][r0:r0 + n] * kbuf[0, rows, :]
                for t in range(1, 8):
                    acc = acc + qa[half, t][r0:r0 + n] * kbuf[t, rows, :]
                acc = acc + pltpu.roll(acc, 64, 1)
                acc = acc + pltpu.roll(acc, 32, 1)
                if w and half == 0 and r0 < DIL * w:
                    pos = lax.broadcasted_iota(jnp.int32, (n, T), 0) + (c * 2 * RA + r0)
                    acc = jnp.where(pos >= DIL * w, acc, MASKED)
                logits.append(acc)
            m = logits[0]
            for x in logits[1:]:
                m = jnp.maximum(m, x)
            p = [jnp.exp2(x - m) for x in logits]
            l = p[0]
            for x in p[1:]:
                l = l + x
            r = pl.reciprocal(l, approx=True)
            r = r * (2.0 - l * r)
            p = [x * r for x in p]
            out = []
            for t in range(8):
                acc = p[0] * vbuf[t, pl.ds(base, n), :]
                for w in range(1, WIN):
                    acc = acc + p[w] * vbuf[t, pl.ds(base - DIL * w, n), :]
                out.append(acc)
            return out

        piece = 16

        def attention_piece(s):
            r0 = s * piece
            top, bot = local_attention(0, r0, piece), local_attention(1, r0, piece)
            for t in range(4):
                for i, val in enumerate(_lhs_terms(top[t], top[4 + t], bot[t], bot[4 + t])):
                    o_t[i, t, pl.ds(r0, piece), :] = val.astype(BF16)
            tok.pending.append([12, _words(o_t, (6, 3 + tok.z), r0, 16) & tok.zv])

        def write_out(col0, quads):
            for quad, val in enumerate(quads):
                obuf[slot, pl.ds((quad // 2) * RA, RA),
                     pl.ds(col0 + (quad % 2) * (DM // 2), DM // 2)] = val.astype(BF16)

        m = []
        npiece = RA // piece
        done = 0
        for i in range(7):
            while done < min(npiece, (i + 1) * npiece // 6):
                attention_piece(done)
                done += 1
            a = _cat([tok.lhs(ctx_t, (i, j), row0, RA) for j in range(NP)])
            m.append(_cat([_dot(a, _load(wob_t, (i, n), 0, NP * T)) for n in range(4)]))
        write_out(DM, _combine(m))

        m = []
        for i in range(7):
            a = _cat([tok.lhs(o_t, (i, t), 0, RA) for t in range(4)])
            m.append(_cat([_dot(a, _load(wo_t, (i, n), 0, DM // 2)) for n in range(4)]))
        write_out(0, _combine(m))
        out_copy(c, slot).start()
        return carry

    nout = S // (2 * RA)
    lax.fori_loop(0, nout, chunk_body, 0)
    out_copy(nout - 2, 0).wait()
    out_copy(nout - 1, 1).wait()


@jax.jit
def pallas_concat_heads__sliding_local_dilated__compressed_kv_cla__prompt_kernel(
    A_x: jax.Array,
    A_wqkv: jax.Array,
    A_wo: jax.Array,
    B_x: jax.Array,
    B_c_kv: jax.Array,
    B_w_q: jax.Array,
    B_w_uk: jax.Array,
    B_w_uv: jax.Array,
    B_w_o: jax.Array,
):
    vmem = pltpu.VMEM
    scratch = [
        vmem((S, DM), BF16),
        vmem((S, DC), BF16),
        vmem((2, DM, T), U32),
        vmem((2, DC, T), U32),
        vmem((2, DC, T), U32),
        vmem((2, 2, T, DM), BF16),
        vmem((2, 2, 16, 3 * DM), U32),
        vmem((2, 2, NH, DM), U32),
        vmem((2, 2, RA // 2, DM), BF16),
        vmem((7, DM // 2 // T, S // 2, T), BF16),
        vmem((7, DC // 2 // T, S // 2, T), BF16),
        vmem((7, NP, S // 2, T), BF16),
        vmem((7, DM // 2 // T, NP * T, T), BF16),
        vmem((7, DM // 2 // T, S // 2, T), BF16),
        vmem((7, 3 * DM // 2 // T, DM // 2, T), BF16),
        vmem((7, DM // 2 // T, DM // 2, T), BF16),
        vmem((7, DM // 2 // T, RA, T), BF16),
        vmem((DM // T, HALO + 2 * RA, T), F32),
        vmem((DM // T, HALO + 2 * RA, T), F32),
        vmem((2, 2 * RA, 2 * DM), BF16),
        pltpu.SMEM((1,), jnp.int32),
        pltpu.SemaphoreType.DMA((2 * (S // (2 * RB)),)),
        pltpu.SemaphoreType.DMA((20,)),
        pltpu.SemaphoreType.DMA((2,)),
    ]
    out = pl.pallas_call(
        _kernel,
        out_shape=jax.ShapeDtypeStruct((S, 2 * DM), BF16),
        in_specs=[pl.BlockSpec(memory_space=pl.ANY)] * 9,
        out_specs=pl.BlockSpec(memory_space=pl.ANY),
        scratch_shapes=scratch,
        compiler_params=pltpu.CompilerParams(vmem_limit_bytes=120 * 2**20),
    )(
        A_x.reshape(S, DM),
        A_wqkv,
        A_wo.reshape(NH, DM // NH, DM),
        B_x.reshape(S, DM),
        B_c_kv.reshape(S, DC),
        B_w_q,
        B_w_uk,
        B_w_uv,
        B_w_o,
    )
    return out.reshape(1, S, 2 * DM)
```

```python
import functools
import math

import jax
import jax.numpy as jnp
from jax import lax
import jax.experimental.pallas as pl
import jax.experimental.pallas.tpu as pltpu

CFG = {'fw': '10'}
PQ = int(CFG.get('pq', 12)); CTX_DELAY = int(CFG.get('cd', 2)); SK = int(CFG.get('sk', 3))
BORD = CFG.get('bord', 'k'); WD = int(CFG.get('wd', 1)); OSK = int(CFG.get('osk', 3)); WSK = int(CFG.get('wsk', 7)); ASK = int(CFG.get('ask', 2))
WQ = float(CFG.get('wq', 1)); WKV = float(CFG.get('wkv', 1)); WATT = float(CFG.get('watt', 1)); SIDE = float(CFG.get('side', 0.97)); NKV = int(CFG.get('nkv', 20)); TAILF = float(CFG.get('tailf', 0.9))
LT = CFG.get('lt', ''); LTP = int(CFG.get('ltp', 0)); CTP = int(CFG.get('ctp', -1))
FM = CFG.get('fm', 'prev')
G = int(CFG.get('g', 0)); GL = int(CFG.get('gl', 1))
RP = int(CFG.get('rp', 0))
g_ = lambda k, d: int(CFG.get(k, d))
W0, W1, V0, V1, WWIN, VWIN, OSTEP, VCOMB = g_('w0', 500), g_('w1', 3500), g_('v0', 3500), g_('v1', 900), g_('wwin', 600), g_('vwin', 512), g_('ostep', 60), g_('vcomb', 1500)
AWIN, ASTEP, XSPAN = g_('awin', 256), g_('astep', 150), g_('xspan', 4500)
NFS = g_('nfs', 40); FW = g_('fw', 9)
WSPAN = int(CFG.get('wspan', 49)); VSPAN = int(CFG.get('vspan', 24))

S = 2048
DM = 1024
DC = 512
NH = 32
NP = NH // 2
T = 128
CH = 4 * T
NC = S // CH
RO = 64
CO = 4 * RO
NO = S // CO
ROWB = lambda inner, outer: 2 * outer + inner
WIN, DIL = 8, 2
HALO = 16

LOG2E = math.log2(math.e)
SCALE_A = (DM // NH) ** -0.5 * LOG2E
SCALE_B = T ** -0.5 * LOG2E
MASKED = -1e9 * LOG2E

F32, BF16, U32 = jnp.float32, jnp.bfloat16, jnp.uint32
P = functools.partial


def _dot(a, b):
    return jnp.dot(a, b, preferred_element_type=F32)


def _dot_nt(a, b):
    return lax.dot_general(a, b, (((1,), (1,)), ((), ())), preferred_element_type=F32)


def _cat(xs, axis=1):
    return xs[0] if len(xs) == 1 else jnp.concatenate(xs, axis=axis)


def _aligned(x, n):
    return x if isinstance(x, int) else pl.multiple_of(x, n)


def _words(ref, lead, start, n):
    return ref.bitcast(U32)[(*lead, pl.ds(_aligned(start >> 1, 8), n // 2), slice(None))]


def _load(ref, lead, start, n):
    return pltpu.bitcast(_words(ref, lead, start, n), BF16)


def _split(w):
    return (pltpu.bitcast(w << 16, F32), pltpu.bitcast(w & jnp.uint32(0xFFFF0000), F32))


def _or_first(w, tok):
    bits = w if w.dtype == U32 else pltpu.bitcast(w, U32)
    bits = bits | tok if bits.shape[0] == 8 else _cat([bits[:8] | tok, bits[8:]], axis=0)
    return bits if w.dtype == U32 else pltpu.bitcast(bits, w.dtype)


LHS = (((0, 1), (3, 1)), ((2, 1), (3, 1)), ((0, 1),), ((3, 1),),
       ((0, 1), (1, 1)), ((2, 1), (0, -1)), ((1, 1), (3, -1)))
RHS = (((0, 1), (3, 1)), ((0, 1),), ((1, 1), (3, -1)), ((2, 1), (0, -1)),
       ((3, 1),), ((0, 1), (1, 1)), ((2, 1), (3, 1)))
OUT = (((0, 1), (3, 1)), ((2, 1), (3, -1)), ((1, 1), (3, 1)), ((0, 1), (2, 1)),
       ((0, -1), (1, 1)), ((3, 1),), ((0, 1),))


def _term(table, i, quad):
    (n, _), *rest = table[i]
    val = quad(n)
    for n, sign in rest:
        val = val + quad(n) if sign > 0 else val - quad(n)
    return val


def _terms(table, quad):
    blocks = [quad(n) for n in range(4)]
    return [_term(table, i, blocks.__getitem__) for i in range(7)]


def _terms2(table, i, block):
    return _terms(table, lambda n: _term(
        table, i, lambda m: block(2 * (m // 2) + n // 2, 2 * (m % 2) + n % 2)))


def _combine(m):
    out = [None] * 4
    for i in range(7):
        for n, sign in OUT[i]:
            if out[n] is None:
                out[n] = m[i]
            else:
                out[n] = out[n] + m[i] if sign > 0 else out[n] - m[i]
    return out


def _combine2(m):
    inner = [_combine(m[7 * i:7 * i + 7]) for i in range(7)]
    out = [[None] * 4 for _ in range(4)]
    for n in range(4):
        for quad, val in enumerate(_combine([x[n] for x in inner])):
            out[2 * (quad // 2) + n // 2][2 * (quad % 2) + n % 2] = val
    return out


class _Tokens:
    def __init__(self, zero_smem):
        self.z = zero_smem[0]
        self.zv = jnp.full((8, T), self.z, jnp.int32).astype(U32)

    def stored(self, ref, lead, start):
        first, *rest = lead
        if FM == 'lead':
            if ref.dtype == BF16:
                return _words(ref, (first + self.z, *rest), start, 16) & self.zv
            return self.of(ref[(first + self.z, *rest, pl.ds(start, 8), slice(None))])
        bit = self.z & 1
        if FM == 'prev':
            if ref.dtype == BF16:
                return _words(ref, (first - bit, *rest), start, 16) & self.zv
            return self.of(ref[(first, *rest, pl.ds(_aligned(start + 8 * bit, 8), 8), slice(None))])

    def of(self, *vals):
        tok = vals[0]
        for x in vals[1:]:
            tok = tok + x
        return pltpu.bitcast(tok, U32) & self.zv


def _head_pairs(wqkv_hbm, wo_hbm, bx_hbm, c_hbm, wq_hbm, wuk_hbm, wuv_hbm, wob_hbm,
                ctx_t, wob_t, waq_t, wakv_t, wo_t, zero_smem,
                bx_raw, c_raw, wq_raw, wk_raw, wv_raw, wob_raw, wqkv_raw, wo_raw,
                bx_t, c_t, wq_t, wkv_t, sem_in, sem_w):

    def head_copy(n, j, slot):
        src, dst = ((wuk_hbm, wk_raw), (wuv_hbm, wv_raw), (wq_hbm, wq_raw))[n]
        return pltpu.make_async_copy(src.bitcast(U32).at[:, j, :], dst.at[slot], sem_w.at[3 * slot + n])

    def side_copy(n, j, slot):
        if n == 0:
            src = wob_hbm.at[pl.ds(4 * (j >> 1), 4), pl.ds(_aligned((j & 1) * 64, 64), 64), :]
            dst = wob_raw.at[slot]
        else:
            src = wqkv_hbm.bitcast(U32).at[:, pl.ds(_aligned(8 * j, 8), 8), :]
            dst = wqkv_raw.at[slot]
        return pltpu.make_async_copy(src, dst, sem_w.at[6 + 2 * slot + n])

    def wo_copy(word):
        return pltpu.make_async_copy(wo_hbm.bitcast(U32).at[:, word, :], wo_raw.at[word], sem_w.at[10])

    def act_copy(n, c):
        src, dst = ((c_hbm, c_raw), (bx_hbm, bx_raw))[n]
        rows = pl.ds(c * CH, CH)
        return pltpu.make_async_copy(src.at[rows, :], dst.at[rows, :], sem_in.at[2 * c + n])

    def pair_body(j, first=False):
        slot = j & 1
        if not first:
            for n in range(3):
                head_copy(n, j, 1 - slot).wait()
            for n in range(2):
                side_copy(n, j, slot).wait()
            for n in range(3):
                head_copy(n, jnp.minimum(j + 2, NP - 1), slot).start()
            for n in range(2):
                side_copy(n, jnp.minimum(j + 1, NP - 1), 1 - slot).start()
        tok = _Tokens(zero_smem)
        causal = (lax.broadcasted_iota(jnp.int32, (T, T), 1)
                  <= lax.broadcasted_iota(jnp.int32, (T, T), 0))
        jobs, pace = [], dict(period=0, clock=0)

        def background(cycles):
            pace["clock"] += cycles
            token = None
            while jobs and pace["clock"] >= pace["period"]:
                pace["clock"] -= pace["period"]
                new = jobs.pop(0)()
                token = new if token is None else token | new
            return token

        same = 16 * (tok.z & 1) if first and g_('same', 0) else 0

        def lhs(ref, lead, start, n, cycles):
            w = _words(ref, lead, start + same, n)
            parts = []
            for r in range(0, n // 2, 8):
                token = background(cycles)
                parts.append(w[r:r + 8] if token is None else w[r:r + 8] | token)
            return pltpu.bitcast(_cat(parts, axis=0), BF16)

        def store_terms(dst, first_term, lead, row, terms):
            for i, val in enumerate(terms):
                dst[(first_term + i, *lead, pl.ds(_aligned(row, 16), 16), slice(None))] = val.astype(BF16)
            return tok.stored(dst, (first_term + 6, *lead), row)

        def job_wkv(src, i, r):
            def block(row, col):
                raw = (wk_raw, wv_raw)[col % 2]
                return _split(raw[src, pl.ds(_aligned(row * T + r, 16), 16), :])[col // 2]
            return store_terms(wkv_t, 7 * i, (), r, _terms2(RHS, i, block))

        def job_wq(src, r):
            top, bot = _split(wq_raw[src, pl.ds(_aligned(r, 16), 16), :]), _split(wq_raw[src, pl.ds(_aligned(DM // 2 + r, 16), 16), :])
            return store_terms(wq_t, 0, (), r, _terms(RHS, (top + bot).__getitem__))

        def jobs_wkv(src):
            return [P(job_wkv, src, i, r) for r in range(0, T, 16) for i in range(7)]

        def jobs_wq(src):
            return [P(job_wq, src, r) for r in range(0, DM // 2, 16)]

        def job_wob(i, n, r):
            def block(row, col):
                head = 2 * (row % 2) + row // 2
                return wob_raw[slot, head, pl.ds(r, 16), pl.ds((2 * col + n) * T, T)].astype(F32)
            return store_terms(wob_t, 7 * i, (n,), j * 64 + r, _terms2(RHS, i, block))

        def job_wo(i, n):
            odd = (j >> 2) & 1

            def block(row, col):
                even_t, odd_t = _split(wo_raw[4 * (j & 3) + row, pl.ds(_aligned(16 * (j >> 3), 16), 16),
                                              pl.ds((2 * col + n) * T, T)])
                return jnp.where(odd == 1, odd_t, even_t)
            return store_terms(wo_t, 7 * i, (n,), odd * T + (j & 3) * NH + (j >> 3) * 16,
                               _terms2(RHS, i, block))

        permuted = {}

        def job_permute(mat, row):
            lane = lax.broadcasted_iota(jnp.int32, (8, T), 1)
            e, grp, sub = lane >> 5, (lane >> 2) & 7, lane & 3
            x = [wqkv_raw[slot, row, :, pl.ds(mat * DM + t * T, T)] for t in range(8)]
            y = [jnp.take_along_axis(x[t], sub * 32 + e * 8 + ((grp - t) & 7), axis=1)
                 for t in range(8)]
            u = [y[-s % 8] for s in range(8)]
            for bit in (1, 2, 4):
                u = [jnp.where((grp & bit) != 0, u[(s - bit) % 8], u[s]) for s in range(8)]
            u = [u[0]] + [jnp.take_along_axis(u[t], e * 32 + ((grp + t) & 7) * 4 + sub, axis=1)
                          for t in range(1, 8)]
            permuted[mat, row] = u
            return functools.reduce(jnp.bitwise_or, u) & tok.zv

        def column(mat, row, t):
            return pltpu.bitcast(permuted[mat, row][t], BF16).astype(F32)

        def job_waq(half, n):
            terms = _terms(RHS, lambda m: column(0, 2 * (m // 2) + half, 4 * (m % 2) + n))
            return store_terms(waq_t, 0, (n,), half * 2 * T + 16 * j, terms)

        def job_wakv(mat, i, n):
            terms = _terms2(RHS, i, lambda row, col: column(mat, row, 2 * col + n))
            return store_terms(wakv_t, 7 * i, (2 * (mat - 1) + n,), 16 * j, terms)

        jobs_wob = [P(job_wob, i, n, r) for r in range(0, 64, 16) for n in range(2) for i in range(7)]
        jobs_wo = [P(job_wo, i, n) for n in range(2) for i in range(7)]
        jobs_wa = [P(job_permute, 0, row) for row in range(4)]
        jobs_wa += [P(job_waq, half, n) for half in range(2) for n in range(4)]
        for mat in (1, 2):
            jobs_wa += [P(job_permute, mat, row) for row in range(4)]
            jobs_wa += [P(job_wakv, mat, i, n) for n in range(2) for i in range(7)]

        q, k, v = {}, {}, {}

        def job_x(c, t, r):
            terms = _terms(LHS, lambda m: bx_raw[pl.ds(_aligned(c * CH + (m // 2) * 2 * T + r, 16), 16),
                                                 pl.ds((4 * (m % 2) + t) * T, T)].astype(F32))
            return store_terms(bx_t, 0, (t,), c * 2 * T + r, terms)

        def job_c(c, i, r):
            terms = _terms2(LHS, i, lambda row, col: c_raw[
                pl.ds(_aligned(c * CH + row * T + r, 16), 16), pl.ds(col * T, T)].astype(F32))
            return store_terms(c_t, 7 * i, (), c * T + r, terms)

        def jobs_x(c):
            return [P(job_x, c, t, r) for r in range(0, 2 * T, 16) for t in range(4)]

        def jobs_c(c):
            return [P(job_c, c, i, r) for r in range(0, T, 16) for i in range(7)]

        def proj_q(c):
            m = [_dot(_cat([lhs(bx_t, (i, t), c * 2 * T, 2 * T, 4 * WQ) for t in range(4)]),
                      _load(wq_t, (i,), same, DM // 2)) for i in range(7)]
            for n, val in enumerate(_combine(m)):
                val = val * SCALE_B
                for r in range(2):
                    q[4 * c + 2 * (n // 2) + r, n % 2] = val[r * T:(r + 1) * T].astype(BF16)

        def proj_kv(c):
            m = [_dot(lhs(c_t, (i,), c * T, T, 4 * WKV), _load(wkv_t, (i,), same, T)) for i in range(49)]
            for r, row in enumerate(_combine2(m)):
                for n, val in enumerate(row):
                    (k, v)[n % 2][4 * c + r, n // 2] = val.astype(BF16)

        scores, ctx, stored, last = {}, {}, [], []

        def score(i, h):
            tiles = [_dot_nt(q[i, h], k[t, h]) for t in range(i + 1)]
            tiles[-1] = jnp.where(causal, tiles[-1], MASKED)
            scores[i, h] = tiles

        def attend(i, h):
            tiles = scores.pop((i, h))
            m = jnp.max(functools.reduce(jnp.maximum, tiles), axis=1, keepdims=True)
            p = [jnp.exp2(s - m) for s in tiles]
            l = None
            for t in range(i + 1):
                pv = p[t]
                if RP == 1:
                    pv = pv.astype(BF16).astype(F32)
                l = pv if l is None else l + pv
                if G and t > 0 and (t % G == G - 1 or (t == i and GL)):
                    p[t] = jnp.where(l < 0, l, p[t])
            if LT == 'own' and i > 0:
                p[-1] = jnp.where(l < 0, l, p[-1])
            if LT == 'next':
                if last:
                    prev = last.pop()
                    p[LTP if i > LTP else i] = jnp.where(prev < 0, prev, p[LTP if i > LTP else i])
                last.append(l)
            l = jnp.sum(l, axis=1, keepdims=True)
            if stored and stored[0][0] <= 0:
                p[CTP] = _or_first(p[CTP], stored.pop(0)[1])
            for entry in stored:
                entry[0] -= 1
            for t in range(i):
                token = background(64 * WATT)
                if token is not None:
                    p[t] = _or_first(p[t], token)
            o = _dot(p[0].astype(BF16), v[0, h])
            for t in range(1, i + 1):
                o = o + _dot(p[t].astype(BF16), v[t, h])
            r = pl.reciprocal(l, approx=True)
            ctx[i, h] = o * (r * (2.0 - l * r))
            b = i // 2
            quad = [(2 * b, 0), (2 * b, 1), (2 * b + 1, 0), (2 * b + 1, 1)]
            if all(u in ctx for u in quad):
                for n, val in enumerate(_terms(LHS, lambda m: ctx.pop(quad[m]))):
                    ctx_t[n, j, pl.ds(b * T, T), :] = val.astype(BF16)
                if b not in ((7,) if first else (0, 7)):
                    stored.append([CTX_DELAY, tok.stored(ctx_t, (6, j), b * T)])

        def queue(cycles, more):
            pace["period"], pace["clock"] = cycles / len(more), 0
            jobs.extend(more)

        def interleave(x, y):
            order = [((n + 0.5) / len(x), 0, job) for n, job in enumerate(x)]
            order += [((n + 0.5) / len(y), 1, job) for n, job in enumerate(y)]
            return [job for _, _, job in sorted(order, key=lambda e: e[:2])]

        def both(i):
            return [(i, 0), (i, 1)]

        def steady(blocks, waiting, skip=0):
            for i in blocks:
                for u in both(i)[skip:]:
                    score(*u)
                    waiting.append(u)
                    attend(*waiting.pop(0))

        def loop(rows, body):
            def step(x, carry):
                body(16 * x)
            lax.fori_loop(0, rows // 16, step, None)

        def start(*copies):
            for cp in copies:
                cp.start()

        def wait(*copies):
            for cp in copies:
                cp.wait()

        side = interleave(jobs_wob, jobs_wo + jobs_wa)
        q_time, kv_time, tile_time = 1792 * WQ, 1568 * WKV, 64 * WATT
        if first:
            stage = [act_copy(0, 0), head_copy(0, 0, 0), head_copy(1, 0, 0)]
            start(*stage)
            wait(*stage)
            stage = [act_copy(0, 1), act_copy(0, 2)]
            start(*stage)
            loop(T, lambda r: [(job_wkv(0, i, r), job_c(0, i, r)) for i in range(7)])
            proj_kv(0)
            wait(*stage)
            stage = [act_copy(0, 3), act_copy(1, 0), head_copy(2, 0, 0)]
            start(*stage)
            loop(T, lambda r: [job_c(1, i, r) for i in range(7)])
            queue(0.85 * kv_time, jobs_c(2))
            proj_kv(1)
            proj_kv(2)
            wait(*stage)
            stage = [act_copy(1, 1), act_copy(1, 2)]
            start(*stage)
            loop(T, lambda r: [job_c(3, i, r) for i in range(7)])
            queue(0.9 * kv_time, interleave(jobs_wq(0), jobs_x(0)))
            proj_kv(3)
            proj_q(0)
            for u in both(2) + both(3) + both(0) + both(1):
                score(*u)
            for u in both(2) + both(3) + both(0) + both(1):
                attend(*u)
            wait(*stage)
            stage = [act_copy(1, 3), side_copy(0, 0, 0), side_copy(1, 0, 0)]
            stage += [head_copy(n, 1, 1) for n in range(3)]
            start(*stage)
            lax.fori_loop(0, 16, lambda word, carry: wo_copy(word).start(), None)
            loop(2 * T, lambda r: [job_x(1, t, r) for t in range(4)])
            queue(0.9 * (q_time + (2 * sum(range(4, 8)) - 7) * tile_time), jobs_x(2))
            proj_q(1)
            score(4, 0)
            waiting = [(4, 0)]
            steady([4], waiting, 1)
            steady(range(5, 8), waiting)
            proj_q(2)
            steady(range(8, FW), waiting)
            wait(*stage, *[wo_copy(word) for word in range(16)])
            start(*[side_copy(n, 1, 1) for n in range(2)], *[head_copy(n, 2, 0) for n in range(3)])
            queue(0.95 * (2 * sum(range(FW, 12)) + FW - 1 - 11) * tile_time,
                  interleave(jobs_x(3), side[:NFS]))
            steady(range(FW, 12), waiting)
        else:
            queue(SIDE * (3 * q_time + 4 * kv_time + (2 * sum(range(2, 12)) - 11) * tile_time), side)
            proj_kv(0)
            proj_q(0)
            score(2, 0)
            score(2, 1)
            proj_kv(1)
            score(3, 0)
            attend(2, 0)
            proj_q(1)
            attend(2, 1)
            score(3, 1)
            attend(3, 0)
            waiting = [(3, 1)]
            steady(range(4, 8), waiting)
            proj_kv(2)
            proj_q(2)
            steady(range(8, 12), waiting)
            proj_kv(3)
        assert not jobs, len(jobs)
        more = jobs_wkv(1 - slot)
        queue(1792 * WQ * 0.95, more[:NKV])
        proj_q(3)
        assert not jobs, len(jobs)
        queue(TAILF * tile_time * (11 + 2 * (12 + 13 + 14)),
              interleave(more[NKV:] + (side[NFS:] if first else []), jobs_wq(1 - slot)))
        steady(range(12, 16), waiting)
        assert not jobs, len(jobs)
        small = [] if first else both(0) + both(1)
        for u in small:
            score(*u)
        for u in waiting + small:
            attend(*u)

    if CFG.get('only') != '1':
        if True:
            pair_body(0, first=True)
    def it(j, carry):
        if True:
            pair_body(j)
    if CFG.get('only') != 'f': lax.fori_loop(1, NP, it, None)
    for n in range(3):
        head_copy(n, NP - 1, (NP - 1) % 2).wait()
    for n in range(2):
        side_copy(n, NP - 1, NP % 2).wait()


def _outputs(ax_hbm, out_hbm, ctx_t, wob_t, waq_t, wakv_t, wo_t, zero_smem,
             ax_raw, ax_t, o_t, kbuf, vbuf, qbuf, acc, obuf, sem_ax, sem_out):

    def ax_copy(c, slot):
        rows = pl.ds(_aligned(c * CO, CO), CO)
        return pltpu.make_async_copy(ax_hbm.at[rows, :], ax_raw.at[slot], sem_ax.at[slot])

    def out_copy(c, slot):
        rows = pl.ds(_aligned(c * CO, CO), CO)
        return pltpu.make_async_copy(obuf.at[slot], out_hbm.at[rows, :], sem_out.at[slot])

    def store_ax(src, i, n, r):
        def block(row, col):
            return ax_raw[src, pl.ds(row * RO + r, 16), pl.ds((2 * col + n) * T, T)].astype(F32)
        outer = [_term(LHS, i, lambda m: block(2 * (m // 2) + x // 2, 2 * (m % 2) + x % 2))
                 for x in range(4)]
        for x, val in enumerate(_terms(LHS, outer.__getitem__) + outer[1:3]):
            ax_t[9 * i + x, n, pl.ds(r, 16), :] = val.astype(BF16)

    ax_jobs = [(i, n, r) for n in range(2) for r in range(0, RO, 16) for i in range(7)]

    ax_copy(0, 0).start()
    ax_copy(1, 1).start()
    for buf in (kbuf, vbuf):
        for t in range(8):
            buf[t, pl.ds(CO, HALO), :] = jnp.zeros((HALO, T), F32)
    ax_copy(0, 0).wait()
    for job in ax_jobs:
        store_ax(0, *job)

    small, medium, large = RO, 4 * RO, 4 * RO
    costs = [small] * 49 + [medium] * 14 + [small] * 49 + [large] * 42 + [small] * 49 + [large] * 7
    starts = [sum(costs[:n]) for n in range(len(costs) + 1)]
    t_q, t_v, t_b, t_o, t_last = (starts[n] for n in (49, 63, 112, 154, 203))

    def chunk_body(c, carry):
        slot = c & 1

        @pl.when(c >= 2)
        def _():
            out_copy(c - 2, slot).wait()

        ax_copy(c, 1 - slot).wait()
        ax_copy(jnp.minimum(c + 2, NO - 1), slot).start()
        tok = _Tokens(zero_smem)

        plan, due, clock = {}, {}, [0]

        def schedule(job, begin, end, release=True):
            first = max([clock[0]] + [n for n in range(len(costs)) if starts[n + 1] <= begin])
            last = min(n for n in range(len(costs)) if starts[n] >= end)
            plan.setdefault(first, []).append((job, last, release))

        def step(a, w):
            n = clock[0]
            clock[0] += 1
            for x, token in enumerate(due.pop(n, [])):
                a[x % len(a)] = _or_first(a[x % len(a)], token)
            a = [x.astype(BF16) if x.dtype == F32 else pltpu.bitcast(x, BF16) for x in a]
            res = [None] * len(w)
            for x in range(len(a)):
                for y in range(len(w)):
                    d = _dot(a[x], w[y](x))
                    res[y] = d if res[y] is None else res[y] + d
            return n, res

        def finish(n, res):
            token = None
            for job, last, release in plan.pop(n, []):
                if release and token is None:
                    token = tok.of(res[0][:8])
                due.setdefault(last, []).append(job(token) if release else job())
            return res

        for buf in (kbuf, vbuf):
            for t in range(8):
                buf[t, pl.ds(0, HALO), :] = buf[t, pl.ds(CO, HALO), :]

        def project2(lhs_t, stride, rhs_t, tile0, write, begin, end):
            m = []

            def recombine(y, r):
                blocks = _combine2([x[y][r:r + 8] for x in m])
                return write(blocks, y, r)

            slabs = [(y, r) for r in range(0, RO, 8) for y in range(2)]
            for x, slab in enumerate(slabs):
                schedule(P(recombine, *slab), begin, begin + (end - begin) * (x + 1) // len(slabs), False)
            for i in range(49):
                n, res = step([_words(lhs_t, (stride * (i // 7) + i % 7, x), 0, RO) for x in range(2)],
                              [P(lambda y, x: _load(rhs_t, (i, tile0 + y), x * T, T), y) for y in range(2)])
                m.append(res)
                finish(n, res)

        def write_rows(buf, blocks, y, r):
            for row in range(4):
                for col in range(4):
                    buf[2 * col + y, pl.ds(HALO + row * RO + r, 8), :] = blocks[row][col]
            return tok.of(*[x for row in blocks for x in row])

        project2(ax_t, 9, wakv_t, 0, P(write_rows, kbuf), t_q, t_v - 300)

        def write_q(m, half, y):
            vals = [val * SCALE_A for val in _combine([x[y] for x in m])]
            for quad, val in enumerate(vals):
                qbuf[4 * (quad % 2) + y, pl.ds((2 * (quad // 2) + half) * RO, RO), :] = val
            return tok.of(*[val[r:r + 8] for val in vals for r in range(0, RO, 8)])

        for half in range(2):
            m = []
            done = t_q + (t_v - t_q) * (half + 1) // 2
            for y in range(4):
                schedule(P(write_q, m, half, y), done, done + 200 + 100 * y, False)
            for i in range(7):
                a = [_words(ax_t, (9 * i + x, n), 0, RO) for x in ((2, 7), (8, 3))[half] for n in range(2)]
                n, res = step(a, [P(lambda y, x: _load(waq_t, (i, y), x * T, T), y) for y in range(4)])
                m.append(res)
                finish(n, res)

        att = {}

        def job_weights(row, r, release):
            base = HALO + row * RO + r
            qs = [_or_first(qbuf[t, pl.ds(row * RO + r, 8), :], release) for t in range(8)]
            logits = []
            for w in range(WIN):
                rows = pl.ds(base - DIL * w, 8)
                x = functools.reduce(jnp.add, [qs[t] * kbuf[t, rows, :] for t in range(8)])
                x = x + pltpu.roll(x, 64, 1)
                x = x + pltpu.roll(x, 32, 1)
                if row == 0 and r < DIL * w:
                    pos = lax.broadcasted_iota(jnp.int32, (8, T), 0) + (c * CO + r)
                    x = jnp.where(pos >= DIL * w, x, MASKED)
                logits.append(x)
            m = functools.reduce(jnp.maximum, logits)
            p = [jnp.exp2(x - m) for x in logits]
            l = functools.reduce(jnp.add, p)
            inv = pl.reciprocal(l, approx=True)
            inv = inv * (2.0 - l * inv)
            att[row, r] = [x * inv for x in p]
            return tok.of(*att[row, r])

        def job_values(row, r, release):
            base = HALO + row * RO + r
            p = [_or_first(x, release) for x in att[row, r]]
            att[row, r] = [
                functools.reduce(jnp.add, [p[w] * vbuf[t, pl.ds(base - DIL * w, 8), :]
                                           for w in range(WIN)])
                for t in range(8)]
            return tok.of(*att[row, r])

        def job_o(n, r, i):
            def block(row, col):
                return _cat([att[row, r][2 * col + n], att[row, r + 8][2 * col + n]], axis=0)
            for x, val in enumerate(_terms2(LHS, i, block)):
                o_t[7 * i + x, n, pl.ds(r, 16), :] = val.astype(BF16)
            return tok.stored(o_t, (7 * i + 6, n), r)

        groups = [(row, r + x) for r in range(0, RO, 16) for row in range(4) for x in (0, 8)]
        w0, w1 = t_v + W0, t_b + W1
        v0, v1 = t_b + V0, t_o - V1
        for g, (row, r) in enumerate(groups):
            begin = w0 + (w1 - w0) * g // len(groups)
            schedule(P(job_weights, row, r), begin, begin + WWIN)
            begin = max(v0 + (v1 - v0) * g // len(groups), begin + WWIN)
            schedule(P(job_values, row, r), begin, begin + VWIN)
            if g % 8 == 7:
                for x, (n, i) in enumerate((n, i) for n in range(2) for i in range(7)):
                    schedule(P(job_o, n, r - 8, i), begin, min(begin + VWIN + OSTEP * (x + 1), t_o), False)
        project2(ax_t, 9, wakv_t, 2, P(write_rows, vbuf), t_b, t_b + VCOMB)

        touched = set()

        def project_b(i):
            m = []

            def accumulate(y, inner):
                val = _combine([x[y] for x in m])[inner]
                token = None
                for outer, sign in OUT[i]:
                    row, col = 2 * (inner // 2) + outer // 2, 2 * (2 * (outer % 2) + inner % 2) + y
                    rows = pl.ds(row * RO, RO)
                    total = val
                    if (outer, inner, y) in touched:
                        total = acc[col, rows, :] + val if sign > 0 else acc[col, rows, :] - val
                    touched.add((outer, inner, y))
                    if any(outer == n for x in range(i + 1, 7) for n, _ in OUT[x]):
                        acc[col, rows, :] = total
                        token = tok.stored(acc, (col,), row * RO)
                    else:
                        obuf[slot, rows, pl.ds(DM + col * T, T)] = total.astype(BF16)
                        if token is None:
                            token = tok.of(*[total[r:r + 8] for r in range(0, RO, 8)])
                return token

            parts = [(y, inner) for y in range(2) for inner in range(4)]
            done = starts[clock[0] + 7]
            if i < 6:
                for x, part in enumerate(parts):
                    schedule(P(accumulate, *part), done, done + AWIN + ASTEP * x, False)
            for n in range(7):
                def quad(kt, x):
                    return (i, 2 * kt + x % 2), (2 * c + x // 2) * RO
                if len(LHS[n]) == 1:
                    a = [_words(ctx_t, *quad(kt, LHS[n][0][0]), RO) for kt in range(8)]
                else:
                    a = [_term(LHS, n, lambda x: _load(ctx_t, *quad(kt, x), RO).astype(F32))
                         for kt in range(8)]
                idx, res = step(a, [P(lambda y, x: _load(wob_t, (7 * i + n, y), x * T, T), y)
                                    for y in range(2)])
                m.append(res)
                finish(idx, res)
            if i == 6:
                for part in parts:
                    accumulate(*part)

        for i in range(6):
            project_b(i)

        def job_ax(i, n, r):
            store_ax(1 - slot, i, n, r)
            return tok.stored(ax_t, (9 * i + 8, n), r)

        for x, job in enumerate(ax_jobs):
            schedule(P(job_ax, *job), t_o, t_o + 100 + (XSPAN - 100) * (x + 1) // len(ax_jobs), False)

        halves = {}

        def write_out(blocks, y, r):
            if r % 16 == 0:
                halves[y] = blocks
            else:
                for row in range(4):
                    for col in range(4):
                        val = _cat([halves[y][row][col], blocks[row][col]], axis=0)
                        obuf[slot, pl.ds(row * RO + r - 8, 16), pl.ds((2 * col + y) * T, T)] = val.astype(BF16)
            return tok.of(*[x for row in blocks for x in row])

        project2(o_t, 7, wo_t, 0, write_out, t_last, starts[-2])
        project_b(6)
        assert not plan and not due, (plan, due)
        out_copy(c, slot).start()
        return carry

    def it(c, carry):
        if True:
            chunk_body(c, carry)
    lax.fori_loop(0, NO, it, None)
    ax_copy(NO - 1, (NO - 1) % 2).wait()
    out_copy(NO - 2, 0).wait()
    out_copy(NO - 1, 1).wait()


def _kernel(ax_hbm, wqkv_hbm, wo_hbm, bx_hbm, c_hbm, wq_hbm, wuk_hbm, wuv_hbm, wob_hbm,
            out_hbm, ctx_t, wob_t, waq_t, wakv_t, wo_t, zero_smem, idle_sem):

    @pl.when(pl.semaphore_read(idle_sem) == 0)
    def _():
        zero_smem[0] = 0

    vmem, dma = pltpu.VMEM, pltpu.SemaphoreType.DMA
    shared = (ctx_t, wob_t, waq_t, wakv_t, wo_t, zero_smem)
    if CFG.get('only') != '2': pl.run_scoped(
        P(_head_pairs, wqkv_hbm, wo_hbm, bx_hbm, c_hbm, wq_hbm, wuk_hbm, wuv_hbm, wob_hbm, *shared),
        vmem((S, DM), BF16),
        vmem((S, DC), BF16),
        vmem((2, DM, T), U32),
        vmem((2, DC, T), U32),
        vmem((2, DC, T), U32),
        vmem((2, 4, 64, DM), BF16),
        vmem((2, 4, 8, 3 * DM), U32),
        vmem((16, NH, DM), U32),
        vmem((7, 4, S // 2, T), BF16),
        vmem((49, S // 4, T), BF16),
        vmem((7, DM // 2, T), BF16),
        vmem((49, T, T), BF16),
        dma((2 * NC,)), dma((11,)))
    if CFG.get('only') in ('1', 'f'):
        def fin(buf, sem):
            z = zero_smem[0]
            val = ctx_t[z, z, pl.ds(0, 16), :]
            for ref in (wob_t, waq_t, wakv_t, wo_t):
                val = val + ref[z, z, pl.ds(z * 16, 16), :]
            buf[...] = val
            cp = pltpu.make_async_copy(buf, out_hbm.at[pl.ds(0, 16), pl.ds(0, T)], sem)
            cp.start(); cp.wait()
        pl.run_scoped(fin, vmem((16, T), BF16), dma(()))
        return
    pl.run_scoped(
        P(_outputs, ax_hbm, out_hbm, *shared),
        vmem((2, CO, DM), BF16),
        vmem((63, 2, RO, T), BF16),
        vmem((49, 2, RO, T), BF16),
        vmem((8, HALO + CO, T), F32),
        vmem((8, HALO + CO, T), F32),
        vmem((8, CO, T), F32),
        vmem((8, CO, T), F32),
        vmem((2, CO, 2 * DM), BF16),
        dma((2,)), dma((2,)))


@jax.jit
def pallas_concat_heads__sliding_local_dilated__compressed_kv_cla__prompt_kernel(
    A_x: jax.Array,
    A_wqkv: jax.Array,
    A_wo: jax.Array,
    B_x: jax.Array,
    B_c_kv: jax.Array,
    B_w_q: jax.Array,
    B_w_uk: jax.Array,
    B_w_uv: jax.Array,
    B_w_o: jax.Array,
):
    vmem = pltpu.VMEM
    out = pl.pallas_call(
        _kernel,
        out_shape=jax.ShapeDtypeStruct((S, 2 * DM), BF16),
        in_specs=[pl.BlockSpec(memory_space=pl.ANY)] * 9,
        out_specs=pl.BlockSpec(memory_space=pl.ANY),
        scratch_shapes=[
            vmem((7, NP, S // 2, T), BF16),
            vmem((49, 2, DM, T), BF16),
            vmem((7, 4, DM // 2, T), BF16),
            vmem((49, 4, 2 * T, T), BF16),
            vmem((49, 2, 2 * T, T), BF16),
            pltpu.SMEM((1,), jnp.int32),
            pltpu.SemaphoreType.REGULAR,
        ],
        compiler_params=pltpu.CompilerParams(vmem_limit_bytes=124 * 2**20, disable_bounds_checks=CFG.get('nb', '1') == '1'),
    )(
        A_x.reshape(S, DM),
        A_wqkv.reshape(4, DM // 4, 3 * DM),
        A_wo.reshape(NH, DM // NH, DM),
        B_x.reshape(S, DM),
        B_c_kv.reshape(S, DC),
        B_w_q,
        B_w_uk,
        B_w_uv,
        B_w_o,
    )
    return out.reshape(1, S, 2 * DM)
```

```python
import functools
import math

import jax
import jax.numpy as jnp
from jax import lax
import jax.experimental.pallas as pl
import jax.experimental.pallas.tpu as pltpu

CFG = {'x': '1'}
PQ = int(CFG.get('pq', 12)); CTX_DELAY = int(CFG.get('cd', 2)); SK = int(CFG.get('sk', 3))
BORD = CFG.get('bord', 'k'); WD = int(CFG.get('wd', 1)); OSK = int(CFG.get('osk', 3)); WSK = int(CFG.get('wsk', 7)); ASK = int(CFG.get('ask', 2))
WQ = float(CFG.get('wq', 1)); WKV = float(CFG.get('wkv', 1)); WATT = float(CFG.get('watt', 1)); SIDE = float(CFG.get('side', 0.97)); NKV = int(CFG.get('nkv', 20)); TAILF = float(CFG.get('tailf', 0.9))
LT = CFG.get('lt', ''); LTP = int(CFG.get('ltp', 0)); CTP = int(CFG.get('ctp', -1))
FM = CFG.get('fm', 'prev')
G = int(CFG.get('g', 0)); GL = int(CFG.get('gl', 1))
RP = int(CFG.get('rp', 0))
g_ = lambda k, d: int(CFG.get(k, d))
W0, W1, V0, V1, WWIN, VWIN, OSTEP, VCOMB = g_('w0', 500), g_('w1', 3500), g_('v0', 3500), g_('v1', 900), g_('wwin', 600), g_('vwin', 512), g_('ostep', 60), g_('vcomb', 1500)
AWIN, ASTEP, XSPAN = g_('awin', 256), g_('astep', 150), g_('xspan', 4500)
NFS = g_('nfs', 40); FW = g_('fw', 10)
REL = g_('rel', 0); RQ = g_('rq', 2); RKV = g_('rkv', 12); END = CFG.get('end', 'a'); L7 = g_('l7', 0)
SUBR = g_('sub', 128); FAST = g_('fast', 0)
WSPAN = int(CFG.get('wspan', 49)); VSPAN = int(CFG.get('vspan', 24))

S = 2048
DM = 1024
DC = 512
NH = 32
NP = NH // 2
T = 128
CH = 4 * T
NC = S // CH
RO = 64
CO = 4 * RO
NO = S // CO
ROWB = lambda inner, outer: 2 * outer + inner
WIN, DIL = 8, 2
HALO = 16

LOG2E = math.log2(math.e)
SCALE_A = (DM // NH) ** -0.5 * LOG2E
SCALE_B = T ** -0.5 * LOG2E
MASKED = -1e9 * LOG2E
SAFE_SUM = 2.0 ** 40

F32, BF16, U32 = jnp.float32, jnp.bfloat16, jnp.uint32
P = functools.partial


def _dot(a, b):
    return jnp.dot(a, b, preferred_element_type=F32)


def _dot_nt(a, b):
    return lax.dot_general(a, b, (((1,), (1,)), ((), ())), preferred_element_type=F32)


def _cat(xs, axis=1):
    return xs[0] if len(xs) == 1 else jnp.concatenate(xs, axis=axis)


def _aligned(x, n):
    return x if isinstance(x, int) else pl.multiple_of(x, n)


def _words(ref, lead, start, n):
    return ref.bitcast(U32)[(*lead, pl.ds(_aligned(start >> 1, 8), n // 2), slice(None))]


def _load(ref, lead, start, n):
    return pltpu.bitcast(_words(ref, lead, start, n), BF16)


def _split(w):
    return (pltpu.bitcast(w << 16, F32), pltpu.bitcast(w & jnp.uint32(0xFFFF0000), F32))


def _fold(op, x):
    return functools.reduce(op, [x[r:r + 8] for r in range(0, x.shape[0], 8)])


def _or_first(w, tok):
    bits = w if w.dtype == U32 else pltpu.bitcast(w, U32)
    bits = bits | tok if bits.shape[0] == 8 else _cat([bits[:8] | tok, bits[8:]], axis=0)
    return bits if w.dtype == U32 else pltpu.bitcast(bits, w.dtype)


LHS = (((0, 1), (3, 1)), ((2, 1), (3, 1)), ((0, 1),), ((3, 1),),
       ((0, 1), (1, 1)), ((2, 1), (0, -1)), ((1, 1), (3, -1)))
RHS = (((0, 1), (3, 1)), ((0, 1),), ((1, 1), (3, -1)), ((2, 1), (0, -1)),
       ((3, 1),), ((0, 1), (1, 1)), ((2, 1), (3, 1)))
OUT = (((0, 1), (3, 1)), ((2, 1), (3, -1)), ((1, 1), (3, 1)), ((0, 1), (2, 1)),
       ((0, -1), (1, 1)), ((3, 1),), ((0, 1),))


def _term(table, i, quad):
    (n, _), *rest = table[i]
    val = quad(n)
    for n, sign in rest:
        val = val + quad(n) if sign > 0 else val - quad(n)
    return val


def _terms(table, quad):
    blocks = [quad(n) for n in range(4)]
    return [_term(table, i, blocks.__getitem__) for i in range(7)]


def _terms2(table, i, block):
    return _terms(table, lambda n: _term(
        table, i, lambda m: block(2 * (m // 2) + n // 2, 2 * (m % 2) + n % 2)))


def _combine(m):
    out = [None] * 4
    for i in range(7):
        for n, sign in OUT[i]:
            if out[n] is None:
                out[n] = m[i]
            else:
                out[n] = out[n] + m[i] if sign > 0 else out[n] - m[i]
    return out


def _combine2(m):
    inner = [_combine(m[7 * i:7 * i + 7]) for i in range(7)]
    out = [[None] * 4 for _ in range(4)]
    for n in range(4):
        for quad, val in enumerate(_combine([x[n] for x in inner])):
            out[2 * (quad // 2) + n // 2][2 * (quad % 2) + n % 2] = val
    return out


class _Tokens:
    def __init__(self, zero_smem):
        self.z = zero_smem[0]
        self.zv = jnp.full((8, T), self.z, jnp.int32).astype(U32)

    def stored(self, ref, lead, start):
        first, *rest = lead
        if FM == 'lead':
            if ref.dtype == BF16:
                return _words(ref, (first + self.z, *rest), start, 16) & self.zv
            return self.of(ref[(first + self.z, *rest, pl.ds(start, 8), slice(None))])
        bit = self.z & 1
        if FM == 'prev':
            if ref.dtype == BF16:
                return _words(ref, (first - bit, *rest), start, 16) & self.zv
            return self.of(ref[(first, *rest, pl.ds(_aligned(start + 8 * bit, 8), 8), slice(None))])

    def of(self, *vals):
        tok = vals[0]
        for x in vals[1:]:
            tok = tok + x
        return pltpu.bitcast(tok, U32) & self.zv


def _head_pairs(wqkv_hbm, wo_hbm, bx_hbm, c_hbm, wq_hbm, wuk_hbm, wuv_hbm, wob_hbm, prefetch_ax,
                ctx_t, wob_t, waq_t, wakv_t, wo_t, zero_smem,
                bx_raw, c_raw, wq_raw, wk_raw, wv_raw, wob_raw, wqkv_raw, wo_raw,
                bx_t, c_t, wq_t, wkv_t, guard, sem_in, sem_w):
    guard[...] = jnp.zeros(guard.shape, F32)

    def head_copy(n, j, slot):
        src, dst = ((wuk_hbm, wk_raw), (wuv_hbm, wv_raw), (wq_hbm, wq_raw))[n]
        return pltpu.make_async_copy(src.bitcast(U32).at[:, j, :], dst.at[slot], sem_w.at[3 * slot + n])

    def side_copy(n, j, slot):
        if n == 0:
            src = wob_hbm.at[pl.ds(4 * (j >> 1), 4), pl.ds(_aligned((j & 1) * 64, 64), 64), :]
            dst = wob_raw.at[slot]
        else:
            src = wqkv_hbm.bitcast(U32).at[:, pl.ds(_aligned(8 * j, 8), 8), :]
            dst = wqkv_raw.at[slot]
        return pltpu.make_async_copy(src, dst, sem_w.at[6 + 2 * slot + n])

    def wo_copy(word):
        return pltpu.make_async_copy(wo_hbm.bitcast(U32).at[:, word, :], wo_raw.at[word], sem_w.at[10])

    def act_copy(n, c):
        src, dst = ((c_hbm, c_raw), (bx_hbm, bx_raw))[n]
        rows = pl.ds(c * CH, CH)
        return pltpu.make_async_copy(src.at[rows, :], dst.at[rows, :], sem_in.at[2 * c + n])

    def exact_pairs(qkv, ctx):
        def block(i):
            return pl.ds(pl.multiple_of(i * T, T), T)

        def head(h, carry):
            def weight(raw):
                even, odd = _split(raw[0])
                return jnp.where(h == 0, even, odd).astype(BF16)
            wk, wv, wq = weight(wk_raw), weight(wv_raw), weight(wq_raw)

            def project(i, carry):
                qkv[0, block(i), :] = (_dot(bx_raw[block(i), :], wq) * SCALE_B).astype(BF16)
                qkv[1, block(i), :] = _dot(c_raw[block(i), :], wk).astype(BF16)
                qkv[2, block(i), :] = _dot(c_raw[block(i), :], wv).astype(BF16)
            lax.fori_loop(0, S // T, project, None)

            def attend(i, carry):
                def scores(t):
                    row = lax.broadcasted_iota(jnp.int32, (T, T), 0) + i * T
                    col = lax.broadcasted_iota(jnp.int32, (T, T), 1) + t * T
                    return jnp.where(col <= row, _dot_nt(qkv[0, block(i), :], qkv[1, block(t), :]), MASKED)

                m = lax.fori_loop(
                    0, i + 1, lambda t, m: jnp.maximum(m, jnp.max(scores(t), axis=1, keepdims=True)),
                    jnp.full((T, 1), -jnp.inf, F32))

                def accumulate(t, carry):
                    l, o = carry
                    p = jnp.exp2(scores(t) - m)
                    return (l + jnp.sum(p, axis=1, keepdims=True),
                            o + _dot(p.astype(BF16), qkv[2, block(t), :]))
                l, o = lax.fori_loop(0, i + 1, accumulate,
                                     (jnp.zeros((T, 1), F32), jnp.zeros((T, T), F32)))
                ctx[h, block(i), :] = o / l
            lax.fori_loop(0, S // T, attend, None)

        def pair(j, carry):
            for n in range(3):
                head_copy(n, j, 0).start()
            for n in range(3):
                head_copy(n, j, 0).wait()
            lax.fori_loop(0, 2, head, None)

            def store(b, carry):
                for n, val in enumerate(_terms(LHS, lambda m: ctx[m % 2, block(2 * b + m // 2), :])):
                    ctx_t[n, j, block(b), :] = val.astype(BF16)
            lax.fori_loop(0, S // T // 2, store, None)

        lax.fori_loop(0, NP, pair, None)

    def pair_body(j, first=False):
        slot = j & 1
        if not first:
            for n in range(3):
                head_copy(n, j, 1 - slot).wait()
            for n in range(2):
                side_copy(n, j, slot).wait()
            for n in range(3):
                head_copy(n, jnp.minimum(j + 2, NP - 1), slot).start()
            for n in range(2):
                side_copy(n, jnp.minimum(j + 1, NP - 1), 1 - slot).start()
        tok = _Tokens(zero_smem)
        causal = (lax.broadcasted_iota(jnp.int32, (T, T), 1)
                  <= lax.broadcasted_iota(jnp.int32, (T, T), 0))
        jobs, pace = [], dict(period=0, clock=0)

        def background(cycles, recent):
            pace["clock"] += cycles
            token = None
            while jobs and pace["clock"] >= pace["period"]:
                pace["clock"] -= pace["period"]
                pace["release"] = None if recent is None or not REL else tok.of(recent[:8])
                new = jobs.pop(0)()
                pace["release"] = None
                token = new if token is None else token | new
            return token

        def released(x):
            if pace.get("release") is None:
                return x
            bits = x if x.dtype == U32 else pltpu.bitcast(x, U32)
            bits = _cat([bits[r:r + 8] | pace["release"] for r in range(0, bits.shape[0], 8)], axis=0)
            return bits if x.dtype == U32 else pltpu.bitcast(bits, x.dtype)

        same = 0

        def lhs(ref, lead, start, n, cycles, recent):
            w = _words(ref, lead, start, n)
            parts = []
            for r in range(0, n // 2, 8):
                token = background(cycles, recent)
                parts.append(w[r:r + 8] if token is None else w[r:r + 8] | token)
            return pltpu.bitcast(_cat(parts, axis=0), BF16)

        def store_terms(dst, first_term, lead, row, terms):
            for i, val in enumerate(terms):
                dst[(first_term + i, *lead, pl.ds(_aligned(row, 16), 16), slice(None))] = val.astype(BF16)
            return tok.stored(dst, (first_term + 6, *lead), row)

        def job_wkv(src, i, r):
            def block(row, col):
                raw = (wk_raw, wv_raw)[col % 2]
                return _split(released(raw[src, pl.ds(_aligned(row * T + r, 16), 16), :]))[col // 2]
            return store_terms(wkv_t, 7 * i, (), r, _terms2(RHS, i, block))

        def job_wq(src, r):
            top, bot = _split(released(wq_raw[src, pl.ds(_aligned(r, 16), 16), :])), _split(released(wq_raw[src, pl.ds(_aligned(DM // 2 + r, 16), 16), :]))
            return store_terms(wq_t, 0, (), r, _terms(RHS, (top + bot).__getitem__))

        def jobs_wkv(src):
            return [P(job_wkv, src, i, r) for r in range(0, T, 16) for i in range(7)]

        def jobs_wq(src):
            return [P(job_wq, src, r) for r in range(0, DM // 2, 16)]

        def job_wob(i, n, r):
            def block(row, col):
                head = 2 * (row % 2) + row // 2
                return released(wob_raw[slot, head, pl.ds(r, 16), pl.ds((2 * col + n) * T, T)].astype(F32))
            return store_terms(wob_t, 7 * i, (n,), j * 64 + r, _terms2(RHS, i, block))

        def job_wo(i, n):
            odd = (j >> 2) & 1

            def block(row, col):
                even_t, odd_t = _split(released(wo_raw[4 * (j & 3) + row, pl.ds(_aligned(16 * (j >> 3), 16), 16),
                                              pl.ds((2 * col + n) * T, T)]))
                return jnp.where(odd == 1, odd_t, even_t)
            return store_terms(wo_t, 7 * i, (n,), odd * T + (j & 3) * NH + (j >> 3) * 16,
                               _terms2(RHS, i, block))

        permuted = {}

        def job_permute(mat, row):
            lane = lax.broadcasted_iota(jnp.int32, (8, T), 1)
            e, grp, sub = lane >> 5, (lane >> 2) & 7, lane & 3
            x = [released(wqkv_raw[slot, row, :, pl.ds(mat * DM + t * T, T)]) for t in range(8)]
            y = [jnp.take_along_axis(x[t], sub * 32 + e * 8 + ((grp - t) & 7), axis=1)
                 for t in range(8)]
            u = [y[-s % 8] for s in range(8)]
            for bit in (1, 2, 4):
                u = [jnp.where((grp & bit) != 0, u[(s - bit) % 8], u[s]) for s in range(8)]
            u = [u[0]] + [jnp.take_along_axis(u[t], e * 32 + ((grp + t) & 7) * 4 + sub, axis=1)
                          for t in range(1, 8)]
            permuted[mat, row] = u
            return functools.reduce(jnp.bitwise_or, u) & tok.zv

        def column(mat, row, t):
            return pltpu.bitcast(released(permuted[mat, row][t]), BF16).astype(F32)

        def job_waq(half, n):
            terms = _terms(RHS, lambda m: column(0, 2 * (m // 2) + half, 4 * (m % 2) + n))
            return store_terms(waq_t, 0, (n,), half * 2 * T + 16 * j, terms)

        def job_wakv(mat, i, n):
            terms = _terms2(RHS, i, lambda row, col: column(mat, row, 2 * col + n))
            return store_terms(wakv_t, 7 * i, (2 * (mat - 1) + n,), 16 * j, terms)

        jobs_wob = [P(job_wob, i, n, r) for r in range(0, 64, 16) for n in range(2) for i in range(7)]
        jobs_wo = [P(job_wo, i, n) for n in range(2) for i in range(7)]
        jobs_wa = [P(job_permute, 0, row) for row in range(4)]
        jobs_wa += [P(job_waq, half, n) for half in range(2) for n in range(4)]
        for mat in (1, 2):
            jobs_wa += [P(job_permute, mat, row) for row in range(4)]
            jobs_wa += [P(job_wakv, mat, i, n) for n in range(2) for i in range(7)]

        q, k, v, latest = {}, {}, {}, [None]

        def job_x(c, t, r):
            terms = _terms(LHS, lambda m: bx_raw[pl.ds(_aligned(c * CH + (m // 2) * 2 * T + r, 16), 16),
                                                 pl.ds((4 * (m % 2) + t) * T, T)].astype(F32))
            return store_terms(bx_t, 0, (t,), c * 2 * T + r, terms)

        def job_c(c, i, r):
            terms = _terms2(LHS, i, lambda row, col: c_raw[
                pl.ds(_aligned(c * CH + row * T + r, 16), 16), pl.ds(col * T, T)].astype(F32))
            return store_terms(c_t, 7 * i, (), c * T + r, terms)

        def jobs_x(c):
            return [P(job_x, c, t, r) for r in range(0, 2 * T, 16) for t in range(4)]

        def jobs_c(c):
            return [P(job_c, c, i, r) for r in range(0, T, 16) for i in range(7)]

        def proj_q(c):
            m = []
            for i in range(7):
                recent = m[i - RQ] if i >= RQ else latest[0]
                m.append(_dot(_cat([lhs(bx_t, (i, t), c * 2 * T, 2 * T, 4 * WQ, recent) for t in range(4)]),
                              _load(wq_t, (i,), same, DM // 2)))
            latest[0] = m[-2]
            for n, val in enumerate(_combine(m)):
                val = val * SCALE_B
                for r in range(2):
                    q[4 * c + 2 * (n // 2) + r, n % 2] = val[r * T:(r + 1) * T].astype(BF16)

        def proj_kv(c):
            m = []
            for i in range(49):
                recent = m[i - RKV] if i >= RKV else latest[0]
                m.append(_dot(lhs(c_t, (i,), c * T, T, 4 * WKV, recent), _load(wkv_t, (i,), same, T)))
            latest[0] = m[-RKV]
            for r, row in enumerate(_combine2(m)):
                for n, val in enumerate(row):
                    (k, v)[n % 2][4 * c + r, n // 2] = val.astype(BF16)

        scores, ctx, stored, spread, checks = {}, {}, [], {}, []

        def score(i, h):
            tiles = [_dot_nt(q[i, h], k[t, h]) for t in range(i + 1)]
            tiles[-1] = jnp.where(causal, tiles[-1], MASKED)
            scores[i, h] = tiles

        def attend(i, h):
            tiles = scores.pop((i, h))
            p = [jnp.exp2(s) for s in tiles]
            l = jnp.sum(functools.reduce(jnp.add, p), axis=1, keepdims=True)
            if stored and stored[0][0] <= 0:
                p[CTP] = _or_first(p[CTP], stored.pop(0)[1])
            for entry in stored:
                entry[0] -= 1
            for t in range(i):
                token = background(64 * WATT, None)
                if token is not None:
                    p[t] = _or_first(p[t], token)
            o = _dot(p[0].astype(BF16), v[0, h])
            for t in range(1, i + 1):
                o = o + _dot(p[t].astype(BF16), v[t, h])
            latest[0] = tiles[-1]
            r = pl.reciprocal(l, approx=True)
            ctx[i, h] = o * (r * (2.0 - l * r))
            spread[i, h] = _fold(jnp.maximum, jnp.broadcast_to(l + r, (T, T)))
            b = i // 2
            quad = [(2 * b, 0), (2 * b, 1), (2 * b + 1, 0), (2 * b + 1, 1)]
            if all(u in ctx for u in quad):
                terms = _terms(LHS, lambda m: ctx.pop(quad[m]))
                for n, val in enumerate(terms):
                    ctx_t[n, j, pl.ds(b * T, T), :] = val.astype(BF16)
                checks.append((_fold(jnp.add, terms[0] + terms[5] + terms[6]),
                               functools.reduce(jnp.maximum, [spread.pop(u) for u in quad])))
                if b not in ((7,) if first else (0,) if L7 else (0, 7)):
                    stored.append([0 if b == 7 else CTX_DELAY, tok.stored(ctx_t, (6, j), b * T) | tok.of(*checks[-1])])

        def queue(cycles, more):
            pace["period"], pace["clock"] = cycles / max(len(more), 1), 0
            jobs.extend(more)

        def interleave(x, y):
            order = [((n + 0.5) / len(x), 0, job) for n, job in enumerate(x)]
            order += [((n + 0.5) / max(len(y), 1), 1, job) for n, job in enumerate(y)]
            return [job for _, _, job in sorted(order, key=lambda e: e[:2])]

        def both(i):
            return [(i, 0), (i, 1)]

        def steady(blocks, waiting, skip=0):
            for i in blocks:
                for u in both(i)[skip:]:
                    score(*u)
                    waiting.append(u)
                    attend(*waiting.pop(0))

        def loop(rows, body):
            def step(x, carry):
                body(16 * x)
            lax.fori_loop(0, rows // 16, step, None)

        def start(*copies):
            for cp in copies:
                cp.start()

        def wait(*copies):
            for cp in copies:
                cp.wait()

        side = interleave(jobs_wob, jobs_wo + jobs_wa)
        q_time, kv_time, tile_time = 1792 * WQ, 1568 * WKV, 64 * WATT
        if first:
            stage = [act_copy(0, 0), head_copy(0, 0, 0), head_copy(1, 0, 0)]
            start(*stage)
            wait(*stage)
            stage = [act_copy(0, 1), act_copy(0, 2)]
            start(*stage)
            loop(T, lambda r: [(job_wkv(0, i, r), job_c(0, i, r)) for i in range(7)])
            proj_kv(0)
            wait(*stage)
            stage = [act_copy(0, 3), act_copy(1, 0), head_copy(2, 0, 0)]
            start(*stage)
            loop(T, lambda r: [job_c(1, i, r) for i in range(7)])
            queue(0.85 * kv_time, jobs_c(2))
            proj_kv(1)
            proj_kv(2)
            wait(*stage)
            stage = [act_copy(1, 1), act_copy(1, 2)]
            start(*stage)
            loop(T, lambda r: [job_c(3, i, r) for i in range(7)])
            queue(0.9 * kv_time, interleave(jobs_wq(0), jobs_x(0)))
            proj_kv(3)
            proj_q(0)
            for u in both(2) + both(3) + both(0) + both(1):
                score(*u)
            for u in both(2) + both(3) + both(0) + both(1):
                attend(*u)
            wait(*stage)
            stage = [act_copy(1, 3), side_copy(0, 0, 0), side_copy(1, 0, 0)]
            stage += [head_copy(n, 1, 1) for n in range(3)]
            start(*stage)
            lax.fori_loop(0, 16, lambda word, carry: wo_copy(word).start(), None)
            loop(2 * T, lambda r: [job_x(1, t, r) for t in range(4)])
            queue(0.9 * (q_time + (2 * sum(range(4, 8)) - 7) * tile_time), jobs_x(2))
            proj_q(1)
            score(4, 0)
            waiting = [(4, 0)]
            steady([4], waiting, 1)
            steady(range(5, 8), waiting)
            proj_q(2)
            steady(range(8, FW), waiting)
            wait(*stage, *[wo_copy(word) for word in range(16)])
            start(*[side_copy(n, 1, 1) for n in range(2)], *[head_copy(n, 2, 0) for n in range(3)])
            prefetch_ax()
            queue(0.95 * (2 * sum(range(FW, 12)) + FW - 1 - 11) * tile_time,
                  interleave(jobs_x(3), side[:NFS]))
            steady(range(FW, 12), waiting)
        else:
            if END == 'a':
                queue(SIDE * (3 * q_time + 4 * kv_time + (2 * sum(range(2, 12)) - 11) * tile_time), side)
                proj_kv(0)
                proj_q(0)
                score(2, 0)
                score(2, 1)
                proj_kv(1)
                score(3, 0)
                attend(2, 0)
                proj_q(1)
                attend(2, 1)
                score(3, 1)
                attend(3, 0)
                waiting = [(3, 1)]
                steady(range(4, 8), waiting)
            else:
                nq = 3 if END == 'b' else 2
                queue(SIDE * (nq * q_time + 4 * kv_time + (2 * sum(range(4, 12)) - 11) * tile_time), side)
                proj_kv(0)
                if END == 'b':
                    proj_q(1)
                    proj_kv(1)
                    score(4, 0)
                    proj_q(0)
                else:
                    proj_q(1)
                    proj_kv(1)
                    score(4, 0)
                waiting = [(4, 0)]
                steady([4], waiting, 1)
                steady(range(5, 8), waiting)
            proj_kv(2)
            proj_q(2)
            steady(range(8, 12), waiting)
            proj_kv(3)
        assert not jobs, len(jobs)
        more = jobs_wkv(1 - slot)
        queue(1792 * WQ * 0.95, more[:NKV])
        proj_q(3)
        assert not jobs, len(jobs)
        late_q = END == 'c' and not first
        queue(TAILF * tile_time * (11 + 2 * (12 + 13 + 14)),
              interleave(more[NKV:], (side[NFS:] if first else []) + ([] if late_q else jobs_wq(1 - slot))))
        steady(range(12, 16), waiting)
        assert not jobs, len(jobs)
        if late_q:
            proj_q(0)
            queue(0.9 * tile_time * (15 + 2 * (3 + 2 + 1)), jobs_wq(1 - slot))
        small = [] if first else both(0) + both(1) if END == 'a' else both(3) + both(2) + both(1) + both(0)
        for u in small:
            score(*u)
        for u in waiting + small:
            attend(*u)
        assert not jobs, len(jobs)
        guard[0] = functools.reduce(jnp.add, [x for x, _ in checks], guard[0])
        guard[1] = functools.reduce(jnp.maximum, [x for _, x in checks], guard[1])

    if CFG.get('only') != '1':
        if True:
            pair_body(0, first=True)
    def it(j, carry):
        if True:
            pair_body(j)
    if CFG.get('only') != 'f': lax.fori_loop(1, NP, it, None)
    for n in range(3):
        head_copy(n, NP - 1, (NP - 1) % 2).wait()
    for n in range(2):
        side_copy(n, NP - 1, NP % 2).wait()

    safe = jnp.logical_and(jnp.abs(guard[0]) < jnp.inf, guard[1] < SAFE_SUM)

    @pl.when(jnp.max(jnp.where(safe, 0.0, 1.0)) > 0.0)
    def _():
        pl.run_scoped(exact_pairs, pltpu.VMEM((3, S, T), BF16), pltpu.VMEM((2, S, T), F32))


def _outputs(ax_hbm, out_hbm, ctx_t, wob_t, waq_t, wakv_t, wo_t, zero_smem,
             ax_raw, sem_ax, ax_t, o_t, kbuf, vbuf, qbuf, acc, obuf, sem_out):

    def ax_copy(c, slot):
        rows = pl.ds(_aligned(c * CO, CO), CO)
        return pltpu.make_async_copy(ax_hbm.at[rows, :], ax_raw.at[slot], sem_ax.at[slot])

    def out_copy(c, slot):
        rows = pl.ds(_aligned(c * CO, CO), CO)
        return pltpu.make_async_copy(obuf.at[slot], out_hbm.at[rows, :], sem_out.at[slot])

    def store_ax(src, i, n, r):
        def block(row, col):
            return ax_raw[src, pl.ds(row * RO + r, 16), pl.ds((2 * col + n) * T, T)].astype(F32)
        outer = [_term(LHS, i, lambda m: block(2 * (m // 2) + x // 2, 2 * (m % 2) + x % 2))
                 for x in range(4)]
        for x, val in enumerate(_terms(LHS, outer.__getitem__) + outer[1:3]):
            ax_t[9 * i + x, n, pl.ds(r, 16), :] = val.astype(BF16)

    ax_jobs = [(i, n, r) for n in range(2) for r in range(0, RO, 16) for i in range(7)]

    for buf in (kbuf, vbuf):
        for t in range(8):
            buf[t, pl.ds(CO, HALO), :] = jnp.zeros((HALO, T), F32)
    ax_copy(0, 0).wait()
    for job in ax_jobs:
        store_ax(0, *job)

    small, medium, large = RO, 4 * RO, 4 * RO
    costs = [small] * 49 + [medium] * 14 + [small] * 49 + [large] * 42 + [small] * 49 + [large] * 7
    starts = [sum(costs[:n]) for n in range(len(costs) + 1)]
    t_q, t_v, t_b, t_o, t_last = (starts[n] for n in (49, 63, 112, 154, 203))

    def chunk_body(c, carry):
        slot = c & 1

        @pl.when(c >= 2)
        def _():
            out_copy(c - 2, slot).wait()

        ax_copy(c, 1 - slot).wait()
        ax_copy(jnp.minimum(c + 2, NO - 1), slot).start()
        tok = _Tokens(zero_smem)

        plan, due, clock = {}, {}, [0]

        def schedule(job, begin, end, release=True):
            first = max([clock[0]] + [n for n in range(len(costs)) if starts[n + 1] <= begin])
            last = min(n for n in range(len(costs)) if starts[n] >= end)
            plan.setdefault(first, []).append((job, last, release))

        def step(a, w):
            n = clock[0]
            clock[0] += 1
            for x, token in enumerate(due.pop(n, [])):
                a[x % len(a)] = _or_first(a[x % len(a)], token)
            a = [x.astype(BF16) if x.dtype == F32 else pltpu.bitcast(x, BF16) for x in a]
            res = [None] * len(w)
            for x in range(len(a)):
                for y in range(len(w)):
                    d = _dot(a[x], w[y](x))
                    res[y] = d if res[y] is None else res[y] + d
            return n, res

        def finish(n, res):
            token = None
            for job, last, release in plan.pop(n, []):
                if release and token is None:
                    token = tok.of(res[0][:8])
                due.setdefault(last, []).append(job(token) if release else job())
            return res

        for buf in (kbuf, vbuf):
            for t in range(8):
                buf[t, pl.ds(0, HALO), :] = buf[t, pl.ds(CO, HALO), :]

        def project2(lhs_t, stride, rhs_t, tile0, write, begin, end):
            m = []

            def recombine(y, r):
                blocks = _combine2([x[y][r:r + 8] for x in m])
                return write(blocks, y, r)

            slabs = [(y, r) for r in range(0, RO, 8) for y in range(2)]
            for x, slab in enumerate(slabs):
                schedule(P(recombine, *slab), begin, begin + (end - begin) * (x + 1) // len(slabs), False)
            for i in range(49):
                n, res = step([_words(lhs_t, (stride * (i // 7) + i % 7, x), 0, RO) for x in range(2)],
                              [P(lambda y, x: _load(rhs_t, (i, tile0 + y), x * T, T), y) for y in range(2)])
                m.append(res)
                finish(n, res)

        def write_rows(buf, blocks, y, r):
            for row in range(4):
                for col in range(4):
                    buf[2 * col + y, pl.ds(HALO + row * RO + r, 8), :] = blocks[row][col]
            return tok.of(*[x for row in blocks for x in row])

        project2(ax_t, 9, wakv_t, 0, P(write_rows, kbuf), t_q, t_v - 300)

        def write_q(m, half, y):
            vals = [val * SCALE_A for val in _combine([x[y] for x in m])]
            for quad, val in enumerate(vals):
                qbuf[4 * (quad % 2) + y, pl.ds((2 * (quad // 2) + half) * RO, RO), :] = val
            return tok.of(*[val[r:r + 8] for val in vals for r in range(0, RO, 8)])

        for half in range(2):
            m = []
            done = t_q + (t_v - t_q) * (half + 1) // 2
            for y in range(4):
                schedule(P(write_q, m, half, y), done, done + 200 + 100 * y, False)
            for i in range(7):
                a = [_words(ax_t, (9 * i + x, n), 0, RO) for x in ((2, 7), (8, 3))[half] for n in range(2)]
                n, res = step(a, [P(lambda y, x: _load(waq_t, (i, y), x * T, T), y) for y in range(4)])
                m.append(res)
                finish(n, res)

        att = {}

        def job_weights(row, r, release):
            base = HALO + row * RO + r
            qs = [_or_first(qbuf[t, pl.ds(row * RO + r, 8), :], release) for t in range(8)]
            logits = []
            for w in range(WIN):
                rows = pl.ds(base - DIL * w, 8)
                x = functools.reduce(jnp.add, [qs[t] * kbuf[t, rows, :] for t in range(8)])
                x = x + pltpu.roll(x, 64, 1)
                x = x + pltpu.roll(x, 32, 1)
                if row == 0 and r < DIL * w:
                    pos = lax.broadcasted_iota(jnp.int32, (8, T), 0) + (c * CO + r)
                    x = jnp.where(pos >= DIL * w, x, MASKED)
                logits.append(x)
            m = functools.reduce(jnp.maximum, logits)
            p = [jnp.exp2(x - m) for x in logits]
            l = functools.reduce(jnp.add, p)
            inv = pl.reciprocal(l, approx=True)
            inv = inv * (2.0 - l * inv)
            att[row, r] = [x * inv for x in p]
            return tok.of(*att[row, r])

        def job_values(row, r, release):
            base = HALO + row * RO + r
            p = [_or_first(x, release) for x in att[row, r]]
            att[row, r] = [
                functools.reduce(jnp.add, [p[w] * vbuf[t, pl.ds(base - DIL * w, 8), :]
                                           for w in range(WIN)])
                for t in range(8)]
            return tok.of(*att[row, r])

        def job_o(n, r, i):
            def block(row, col):
                return _cat([att[row, r][2 * col + n], att[row, r + 8][2 * col + n]], axis=0)
            for x, val in enumerate(_terms2(LHS, i, block)):
                o_t[7 * i + x, n, pl.ds(r, 16), :] = val.astype(BF16)
            return tok.stored(o_t, (7 * i + 6, n), r)

        groups = [(row, r + x) for r in range(0, RO, 16) for row in range(4) for x in (0, 8)]
        w0, w1 = t_v + W0, t_b + W1
        v0, v1 = t_b + V0, t_o - V1
        for g, (row, r) in enumerate(groups):
            begin = w0 + (w1 - w0) * g // len(groups)
            schedule(P(job_weights, row, r), begin, begin + WWIN)
            begin = max(v0 + (v1 - v0) * g // len(groups), begin + WWIN)
            schedule(P(job_values, row, r), begin, begin + VWIN)
            if g % 8 == 7:
                for x, (n, i) in enumerate((n, i) for n in range(2) for i in range(7)):
                    schedule(P(job_o, n, r - 8, i), begin, min(begin + VWIN + OSTEP * (x + 1), t_o), False)
        project2(ax_t, 9, wakv_t, 2, P(write_rows, vbuf), t_b, t_b + VCOMB)

        touched = set()

        def project_b(i):
            m = []

            def accumulate(y, inner):
                val = _combine([x[y] for x in m])[inner]
                token = None
                for outer, sign in OUT[i]:
                    row, col = 2 * (outer // 2) + inner // 2, 2 * (2 * (outer % 2) + inner % 2) + y
                    rows = pl.ds(row * RO, RO)
                    total = val
                    if (outer, inner, y) in touched:
                        total = acc[col, rows, :] + val if sign > 0 else acc[col, rows, :] - val
                    touched.add((outer, inner, y))
                    if any(outer == n for x in range(i + 1, 7) for n, _ in OUT[x]):
                        acc[col, rows, :] = total
                        token = tok.stored(acc, (col,), row * RO)
                    else:
                        obuf[slot, rows, pl.ds(DM + col * T, T)] = total.astype(BF16)
                        if token is None:
                            token = tok.of(*[total[r:r + 8] for r in range(0, RO, 8)])
                return token

            parts = [(y, inner) for y in range(2) for inner in range(4)]
            done = starts[clock[0] + 7]
            if i < 6:
                for x, part in enumerate(parts):
                    schedule(P(accumulate, *part), done, done + AWIN + ASTEP * x, False)
            for n in range(7):
                def quad(kt, x):
                    return (i, 2 * kt + x % 2), (2 * c + x // 2) * RO
                if len(LHS[n]) == 1:
                    a = [_words(ctx_t, *quad(kt, LHS[n][0][0]), RO) for kt in range(8)]
                else:
                    a = [_term(LHS, n, lambda x: _load(ctx_t, *quad(kt, x), RO).astype(F32))
                         for kt in range(8)]
                idx, res = step(a, [P(lambda y, x: _load(wob_t, (7 * i + n, y), x * T, T), y)
                                    for y in range(2)])
                m.append(res)
                finish(idx, res)
            if i == 6:
                for part in parts:
                    accumulate(*part)

        for i in range(6):
            project_b(i)

        def job_ax(i, n, r):
            store_ax(1 - slot, i, n, r)
            return tok.stored(ax_t, (9 * i + 8, n), r)

        for x, job in enumerate(ax_jobs):
            schedule(P(job_ax, *job), t_o, t_o + 100 + (XSPAN - 100) * (x + 1) // len(ax_jobs), False)

        halves = {}

        def write_out(blocks, y, r):
            if r % 16 == 0:
                halves[y] = blocks
            else:
                for row in range(4):
                    for col in range(4):
                        val = _cat([halves[y][row][col], blocks[row][col]], axis=0)
                        obuf[slot, pl.ds(row * RO + r - 8, 16), pl.ds((2 * col + y) * T, T)] = val.astype(BF16)
            return tok.of(*[x for row in blocks for x in row])

        project2(o_t, 7, wo_t, 0, write_out, t_last, starts[-2])
        project_b(6)
        assert not plan and not due, (plan, due)
        out_copy(c, slot).start()
        return carry

    def it(c, carry):
        if True:
            chunk_body(c, carry)
    lax.fori_loop(0, NO, it, None)
    ax_copy(NO - 1, (NO - 1) % 2).wait()
    out_copy(NO - 2, 0).wait()
    out_copy(NO - 1, 1).wait()


def _kernel(ax_hbm, wqkv_hbm, wo_hbm, bx_hbm, c_hbm, wq_hbm, wuk_hbm, wuv_hbm, wob_hbm,
            out_hbm, ctx_t, wob_t, waq_t, wakv_t, wo_t, zero_smem, idle_sem, ax_raw, sem_ax):

    @pl.when(pl.semaphore_read(idle_sem) == 0)
    def _():
        zero_smem[0] = 0

    vmem, dma = pltpu.VMEM, pltpu.SemaphoreType.DMA

    def prefetch_ax():
        for c in range(2):
            pltpu.make_async_copy(ax_hbm.at[pl.ds(c * CO, CO), :], ax_raw.at[c], sem_ax.at[c]).start()

    shared = (ctx_t, wob_t, waq_t, wakv_t, wo_t, zero_smem)
    if CFG.get('only') != '2': pl.run_scoped(
        P(_head_pairs, wqkv_hbm, wo_hbm, bx_hbm, c_hbm, wq_hbm, wuk_hbm, wuv_hbm, wob_hbm, prefetch_ax, *shared),
        vmem((S, DM), BF16),
        vmem((S, DC), BF16),
        vmem((2, DM, T), U32),
        vmem((2, DC, T), U32),
        vmem((2, DC, T), U32),
        vmem((2, 4, 64, DM), BF16),
        vmem((2, 4, 8, 3 * DM), U32),
        vmem((16, NH, DM), U32),
        vmem((7, 4, S // 2, T), BF16),
        vmem((49, S // 4, T), BF16),
        vmem((7, DM // 2, T), BF16),
        vmem((49, T, T), BF16),
        vmem((2, 8, T), F32),
        dma((2 * NC,)), dma((11,)))
    if CFG.get('only') in ('1', 'f'):
        def fin(buf, sem):
            z = zero_smem[0]
            val = ctx_t[z, z, pl.ds(0, 16), :]
            for ref in (wob_t, waq_t, wakv_t, wo_t):
                val = val + ref[z, z, pl.ds(z * 16, 16), :]
            buf[...] = val
            cp = pltpu.make_async_copy(buf, out_hbm.at[pl.ds(0, 16), pl.ds(0, T)], sem)
            cp.start(); cp.wait()
        pl.run_scoped(fin, vmem((16, T), BF16), dma(()))
        return
    pl.run_scoped(
        P(_outputs, ax_hbm, out_hbm, *shared, ax_raw, sem_ax),
        vmem((63, 2, RO, T), BF16),
        vmem((49, 2, RO, T), BF16),
        vmem((8, HALO + CO, T), F32),
        vmem((8, HALO + CO, T), F32),
        vmem((8, CO, T), F32),
        vmem((8, CO, T), F32),
        vmem((2, CO, 2 * DM), BF16),
        dma((2,)))


@jax.jit
def pallas_concat_heads__sliding_local_dilated__compressed_kv_cla__prompt_kernel(
    A_x: jax.Array,
    A_wqkv: jax.Array,
    A_wo: jax.Array,
    B_x: jax.Array,
    B_c_kv: jax.Array,
    B_w_q: jax.Array,
    B_w_uk: jax.Array,
    B_w_uv: jax.Array,
    B_w_o: jax.Array,
):
    vmem = pltpu.VMEM
    out = pl.pallas_call(
        _kernel,
        out_shape=jax.ShapeDtypeStruct((S, 2 * DM), BF16),
        in_specs=[pl.BlockSpec(memory_space=pl.ANY)] * 9,
        out_specs=pl.BlockSpec(memory_space=pl.ANY),
        scratch_shapes=[
            vmem((7, NP, S // 2, T), BF16),
            vmem((49, 2, DM, T), BF16),
            vmem((7, 4, DM // 2, T), BF16),
            vmem((49, 4, 2 * T, T), BF16),
            vmem((49, 2, 2 * T, T), BF16),
            pltpu.SMEM((1,), jnp.int32),
            pltpu.SemaphoreType.REGULAR,
            vmem((2, CO, DM), BF16),
            pltpu.SemaphoreType.DMA((2,)),
        ],
        compiler_params=pltpu.CompilerParams(vmem_limit_bytes=124 * 2**20, disable_bounds_checks=CFG.get('nb', '1') == '1'),
    )(
        A_x.reshape(S, DM),
        A_wqkv.reshape(4, DM // 4, 3 * DM),
        A_wo.reshape(NH, DM // NH, DM),
        B_x.reshape(S, DM),
        B_c_kv.reshape(S, DC),
        B_w_q,
        B_w_uk,
        B_w_uv,
        B_w_o,
    )
    return out.reshape(1, S, 2 * DM)
```

```python
import functools
import math

import jax
import jax.numpy as jnp
from jax import lax
import jax.experimental.pallas as pl
import jax.experimental.pallas.tpu as pltpu

CFG = {'x': '1'}
PQ = int(CFG.get('pq', 12)); CTX_DELAY = int(CFG.get('cd', 3)); SK = int(CFG.get('sk', 3))
BORD = CFG.get('bord', 'k'); WD = int(CFG.get('wd', 1)); OSK = int(CFG.get('osk', 3)); WSK = int(CFG.get('wsk', 7)); ASK = int(CFG.get('ask', 2))
WQ = float(CFG.get('wq', 1)); WKV = float(CFG.get('wkv', 1)); WATT = float(CFG.get('watt', 1.5)); SIDE = float(CFG.get('side', 0.85)); NKV = int(CFG.get('nkv', 30)); TAILF = float(CFG.get('tailf', 0.9))
LT = CFG.get('lt', ''); LTP = int(CFG.get('ltp', 0)); CTP = int(CFG.get('ctp', -1))
FM = CFG.get('fm', 'prev')
G = int(CFG.get('g', 0)); GL = int(CFG.get('gl', 1))
RP = int(CFG.get('rp', 0))
g_ = lambda k, d: int(CFG.get(k, d))
W0, W1, V0, V1, WWIN, VWIN, OSTEP, VCOMB = g_('w0', 300), g_('w1', 3500), g_('v0', 2500), g_('v1', 700), g_('wwin', 600), g_('vwin', 300), g_('ostep', 60), g_('vcomb', 1500)
AWIN, ASTEP, XSPAN = g_('awin', 256), g_('astep', 150), g_('xspan', 4500)
NFS = g_('nfs', 40); FW = g_('fw', 9); WO1 = g_('wo1', 2)
REL = g_('rel', 0); RQ = g_('rq', 2); RKV = g_('rkv', 12); END = CFG.get('end', 'a'); L7 = g_('l7', 0)
SUBR = g_('sub', 128); FAST = g_('fast', 0)
LAG0 = g_('lag0', 99); LAG1 = g_('lag1', 5); E2 = g_('e2', 6); E3 = g_('e3', 12)
FQ = float(CFG.get('fq', 0.98))
WSPAN = int(CFG.get('wspan', 49)); VSPAN = int(CFG.get('vspan', 24))

S = 2048
DM = 1024
DC = 512
NH = 32
NP = NH // 2
T = 128
CH = 4 * T
NC = S // CH
RO = 64
CO = 4 * RO
NO = S // CO
ROWB = lambda inner, outer: 2 * outer + inner
WIN, DIL = 8, 2
HALO = 16

LOG2E = math.log2(math.e)
SCALE_A = (DM // NH) ** -0.5 * LOG2E
SCALE_B = T ** -0.5 * LOG2E
MASKED = -1e9 * LOG2E
SAFE_SUM = 2.0 ** 40

F32, BF16, U32 = jnp.float32, jnp.bfloat16, jnp.uint32
P = functools.partial


def _dot(a, b):
    return jnp.dot(a, b, preferred_element_type=F32)


def _dot_nt(a, b):
    return lax.dot_general(a, b, (((1,), (1,)), ((), ())), preferred_element_type=F32)


def _cat(xs, axis=1):
    return xs[0] if len(xs) == 1 else jnp.concatenate(xs, axis=axis)


def _aligned(x, n):
    return x if isinstance(x, int) else pl.multiple_of(x, n)


def _words(ref, lead, start, n):
    return ref.bitcast(U32)[(*lead, pl.ds(_aligned(start >> 1, 8), n // 2), slice(None))]


def _load(ref, lead, start, n):
    return pltpu.bitcast(_words(ref, lead, start, n), BF16)


def _split(w):
    return (pltpu.bitcast(w << 16, F32), pltpu.bitcast(w & jnp.uint32(0xFFFF0000), F32))


def _fold(op, x):
    return functools.reduce(op, [x[r:r + 8] for r in range(0, x.shape[0], 8)])


def _or_first(w, tok):
    bits = w if w.dtype == U32 else pltpu.bitcast(w, U32)
    bits = bits | tok if bits.shape[0] == 8 else _cat([bits[:8] | tok, bits[8:]], axis=0)
    return bits if w.dtype == U32 else pltpu.bitcast(bits, w.dtype)


LHS = (((0, 1), (3, 1)), ((2, 1), (3, 1)), ((0, 1),), ((3, 1),),
       ((0, 1), (1, 1)), ((2, 1), (0, -1)), ((1, 1), (3, -1)))
RHS = (((0, 1), (3, 1)), ((0, 1),), ((1, 1), (3, -1)), ((2, 1), (0, -1)),
       ((3, 1),), ((0, 1), (1, 1)), ((2, 1), (3, 1)))
OUT = (((0, 1), (3, 1)), ((2, 1), (3, -1)), ((1, 1), (3, 1)), ((0, 1), (2, 1)),
       ((0, -1), (1, 1)), ((3, 1),), ((0, 1),))


def _term(table, i, quad):
    (n, _), *rest = table[i]
    val = quad(n)
    for n, sign in rest:
        val = val + quad(n) if sign > 0 else val - quad(n)
    return val


def _terms(table, quad):
    blocks = [quad(n) for n in range(4)]
    return [_term(table, i, blocks.__getitem__) for i in range(7)]


def _terms2(table, i, block):
    return _terms(table, lambda n: _term(
        table, i, lambda m: block(2 * (m // 2) + n // 2, 2 * (m % 2) + n % 2)))


def _combine(m):
    out = [None] * 4
    for i in range(7):
        for n, sign in OUT[i]:
            if out[n] is None:
                out[n] = m[i]
            else:
                out[n] = out[n] + m[i] if sign > 0 else out[n] - m[i]
    return out


def _combine2(m):
    inner = [_combine(m[7 * i:7 * i + 7]) for i in range(7)]
    out = [[None] * 4 for _ in range(4)]
    for n in range(4):
        for quad, val in enumerate(_combine([x[n] for x in inner])):
            out[2 * (quad // 2) + n // 2][2 * (quad % 2) + n % 2] = val
    return out


class _Tokens:
    def __init__(self, zero_smem):
        self.z = zero_smem[0]
        self.zv = jnp.full((8, T), self.z, jnp.int32).astype(U32)

    def stored(self, ref, lead, start):
        first, *rest = lead
        if FM == 'lead':
            if ref.dtype == BF16:
                return _words(ref, (first + self.z, *rest), start, 16) & self.zv
            return self.of(ref[(first + self.z, *rest, pl.ds(start, 8), slice(None))])
        bit = self.z & 1
        if FM == 'prev':
            if ref.dtype == BF16:
                return _words(ref, (first - bit, *rest), start, 16) & self.zv
            return self.of(ref[(first, *rest, pl.ds(_aligned(start + 8 * bit, 8), 8), slice(None))])

    def of(self, *vals):
        tok = vals[0]
        for x in vals[1:]:
            tok = tok + x
        return pltpu.bitcast(tok, U32) & self.zv


def _head_pairs(wqkv_hbm, wo_hbm, bx_hbm, c_hbm, wq_hbm, wuk_hbm, wuv_hbm, wob_hbm, prefetch_ax,
                ctx_t, wob_t, waq_t, wakv_t, wo_t, zero_smem,
                bx_raw, c_raw, wq_raw, wk_raw, wv_raw, wob_raw, wqkv_raw, wo_raw,
                bx_t, c_t, wq_t, wkv_t, guard, sem_in, sem_w):
    guard[...] = jnp.zeros(guard.shape, F32)

    def head_copy(n, j, slot):
        src, dst = ((wuk_hbm, wk_raw), (wuv_hbm, wv_raw), (wq_hbm, wq_raw))[n]
        return pltpu.make_async_copy(src.bitcast(U32).at[:, j, :], dst.at[slot], sem_w.at[3 * slot + n])

    def side_copy(n, j, slot):
        if n == 0:
            src = wob_hbm.at[pl.ds(4 * (j >> 1), 4), pl.ds(_aligned((j & 1) * 64, 64), 64), :]
            dst = wob_raw.at[slot]
        else:
            src = wqkv_hbm.bitcast(U32).at[:, pl.ds(_aligned(8 * j, 8), 8), :]
            dst = wqkv_raw.at[slot]
        return pltpu.make_async_copy(src, dst, sem_w.at[6 + 2 * slot + n])

    def wo_copy(word):
        return pltpu.make_async_copy(wo_hbm.bitcast(U32).at[:, word, :], wo_raw.at[word], sem_w.at[10])

    def act_copy(n, c):
        src, dst = ((c_hbm, c_raw), (bx_hbm, bx_raw))[n]
        rows = pl.ds(c * CH, CH)
        return pltpu.make_async_copy(src.at[rows, :], dst.at[rows, :], sem_in.at[2 * c + n])

    def exact_pairs(qkv, ctx):
        def block(i):
            return pl.ds(pl.multiple_of(i * T, T), T)

        def head(h, carry):
            def weight(raw):
                even, odd = _split(raw[0])
                return jnp.where(h == 0, even, odd).astype(BF16)
            wk, wv, wq = weight(wk_raw), weight(wv_raw), weight(wq_raw)

            def project(i, carry):
                qkv[0, block(i), :] = (_dot(bx_raw[block(i), :], wq) * SCALE_B).astype(BF16)
                qkv[1, block(i), :] = _dot(c_raw[block(i), :], wk).astype(BF16)
                qkv[2, block(i), :] = _dot(c_raw[block(i), :], wv).astype(BF16)
            lax.fori_loop(0, S // T, project, None)

            def attend(i, carry):
                def scores(t):
                    row = lax.broadcasted_iota(jnp.int32, (T, T), 0) + i * T
                    col = lax.broadcasted_iota(jnp.int32, (T, T), 1) + t * T
                    return jnp.where(col <= row, _dot_nt(qkv[0, block(i), :], qkv[1, block(t), :]), MASKED)

                m = lax.fori_loop(
                    0, i + 1, lambda t, m: jnp.maximum(m, jnp.max(scores(t), axis=1, keepdims=True)),
                    jnp.full((T, 1), -jnp.inf, F32))

                def accumulate(t, carry):
                    l, o = carry
                    p = jnp.exp2(scores(t) - m)
                    return (l + jnp.sum(p, axis=1, keepdims=True),
                            o + _dot(p.astype(BF16), qkv[2, block(t), :]))
                l, o = lax.fori_loop(0, i + 1, accumulate,
                                     (jnp.zeros((T, 1), F32), jnp.zeros((T, T), F32)))
                ctx[h, block(i), :] = o / l
            lax.fori_loop(0, S // T, attend, None)

        def pair(j, carry):
            for n in range(3):
                head_copy(n, j, 0).start()
            for n in range(3):
                head_copy(n, j, 0).wait()
            lax.fori_loop(0, 2, head, None)

            def store(b, carry):
                for n, val in enumerate(_terms(LHS, lambda m: ctx[m % 2, block(2 * b + m // 2), :])):
                    ctx_t[n, j, block(b), :] = val.astype(BF16)
            lax.fori_loop(0, S // T // 2, store, None)

        lax.fori_loop(0, NP, pair, None)

    def pair_body(j, first=False):
        slot = j & 1
        if not first:
            for n in range(3):
                head_copy(n, j, 1 - slot).wait()
            for n in range(2):
                side_copy(n, j, slot).wait()
            for n in range(3):
                head_copy(n, jnp.minimum(j + 2, NP - 1), slot).start()
            for n in range(2):
                side_copy(n, jnp.minimum(j + 1, NP - 1), 1 - slot).start()
        tok = _Tokens(zero_smem)
        causal = (lax.broadcasted_iota(jnp.int32, (T, T), 1)
                  <= lax.broadcasted_iota(jnp.int32, (T, T), 0))
        jobs, pace = [], dict(period=0, clock=0)

        def background(cycles, recent):
            pace["clock"] += cycles
            token = None
            while jobs and pace["clock"] >= pace["period"]:
                pace["clock"] -= pace["period"]
                pace["release"] = None if recent is None or not REL else tok.of(recent[:8])
                new = jobs.pop(0)()
                pace["release"] = None
                token = new if token is None else token | new
            return token

        def released(x):
            if pace.get("release") is None:
                return x
            bits = x if x.dtype == U32 else pltpu.bitcast(x, U32)
            bits = _cat([bits[r:r + 8] | pace["release"] for r in range(0, bits.shape[0], 8)], axis=0)
            return bits if x.dtype == U32 else pltpu.bitcast(bits, x.dtype)

        same = 0

        def lhs(ref, lead, start, n, cycles, recent):
            w = _words(ref, lead, start, n)
            parts = []
            for r in range(0, n // 2, 8):
                token = background(cycles, recent)
                parts.append(w[r:r + 8] if token is None else w[r:r + 8] | token)
            return pltpu.bitcast(_cat(parts, axis=0), BF16)

        def store_terms(dst, first_term, lead, row, terms):
            for i, val in enumerate(terms):
                dst[(first_term + i, *lead, pl.ds(_aligned(row, 16), 16), slice(None))] = val.astype(BF16)
            return tok.stored(dst, (first_term + 6, *lead), row)

        def job_wkv(src, i, r):
            def block(row, col):
                raw = (wk_raw, wv_raw)[col % 2]
                return _split(released(raw[src, pl.ds(_aligned(row * T + r, 16), 16), :]))[col // 2]
            return store_terms(wkv_t, 7 * i, (), r, _terms2(RHS, i, block))

        def job_wq(src, r):
            top, bot = _split(released(wq_raw[src, pl.ds(_aligned(r, 16), 16), :])), _split(released(wq_raw[src, pl.ds(_aligned(DM // 2 + r, 16), 16), :]))
            return store_terms(wq_t, 0, (), r, _terms(RHS, (top + bot).__getitem__))

        def jobs_wkv(src):
            return [P(job_wkv, src, i, r) for r in range(0, T, 16) for i in range(7)]

        def jobs_wq(src):
            return [P(job_wq, src, r) for r in range(0, DM // 2, 16)]

        def job_wob(i, n, r):
            def block(row, col):
                head = 2 * (row % 2) + row // 2
                return released(wob_raw[slot, head, pl.ds(r, 16), pl.ds((2 * col + n) * T, T)].astype(F32))
            return store_terms(wob_t, 7 * i, (n,), j * 64 + r, _terms2(RHS, i, block))

        def job_wo(i, n):
            odd = (j >> 2) & 1

            def block(row, col):
                even_t, odd_t = _split(released(wo_raw[4 * (j & 3) + row, pl.ds(_aligned(16 * (j >> 3), 16), 16),
                                              pl.ds((2 * col + n) * T, T)]))
                return jnp.where(odd == 1, odd_t, even_t)
            return store_terms(wo_t, 7 * i, (n,), odd * T + (j & 3) * NH + (j >> 3) * 16,
                               _terms2(RHS, i, block))

        permuted = {}

        def job_permute(mat, row):
            lane = lax.broadcasted_iota(jnp.int32, (8, T), 1)
            e, grp, sub = lane >> 5, (lane >> 2) & 7, lane & 3
            x = [released(wqkv_raw[slot, row, :, pl.ds(mat * DM + t * T, T)]) for t in range(8)]
            y = [jnp.take_along_axis(x[t], sub * 32 + e * 8 + ((grp - t) & 7), axis=1)
                 for t in range(8)]
            u = [y[-s % 8] for s in range(8)]
            for bit in (1, 2, 4):
                u = [jnp.where((grp & bit) != 0, u[(s - bit) % 8], u[s]) for s in range(8)]
            u = [u[0]] + [jnp.take_along_axis(u[t], e * 32 + ((grp + t) & 7) * 4 + sub, axis=1)
                          for t in range(1, 8)]
            permuted[mat, row] = u
            return functools.reduce(jnp.bitwise_or, u) & tok.zv

        def column(mat, row, t):
            return pltpu.bitcast(released(permuted[mat, row][t]), BF16).astype(F32)

        def job_waq(half, n):
            terms = _terms(RHS, lambda m: column(0, 2 * (m // 2) + half, 4 * (m % 2) + n))
            return store_terms(waq_t, 0, (n,), half * 2 * T + 16 * j, terms)

        def job_wakv(mat, i, n):
            terms = _terms2(RHS, i, lambda row, col: column(mat, row, 2 * col + n))
            return store_terms(wakv_t, 7 * i, (2 * (mat - 1) + n,), 16 * j, terms)

        jobs_wob = [P(job_wob, i, n, r) for r in range(0, 64, 16) for n in range(2) for i in range(7)]
        jobs_wo = [P(job_wo, i, n) for n in range(2) for i in range(7)]
        jobs_wa = [P(job_permute, 0, row) for row in range(4)]
        jobs_wa += [P(job_waq, half, n) for half in range(2) for n in range(4)]
        for mat in (1, 2):
            jobs_wa += [P(job_permute, mat, row) for row in range(4)]
            jobs_wa += [P(job_wakv, mat, i, n) for n in range(2) for i in range(7)]

        q, k, v, latest = {}, {}, {}, [None]

        def job_x(c, t, r):
            terms = _terms(LHS, lambda m: bx_raw[pl.ds(_aligned(c * CH + (m // 2) * 2 * T + r, 16), 16),
                                                 pl.ds((4 * (m % 2) + t) * T, T)].astype(F32))
            return store_terms(bx_t, 0, (t,), c * 2 * T + r, terms)

        def job_c(c, i, r):
            terms = _terms2(LHS, i, lambda row, col: c_raw[
                pl.ds(_aligned(c * CH + row * T + r, 16), 16), pl.ds(col * T, T)].astype(F32))
            return store_terms(c_t, 7 * i, (), c * T + r, terms)

        def jobs_x(c):
            return [P(job_x, c, t, r) for r in range(0, 2 * T, 16) for t in range(4)]

        def jobs_c(c):
            return [P(job_c, c, i, r) for r in range(0, T, 16) for i in range(7)]

        def proj_q(c):
            m = []
            for i in range(7):
                recent = m[i - RQ] if i >= RQ else latest[0]
                m.append(_dot(_cat([lhs(bx_t, (i, t), c * 2 * T, 2 * T, 4 * WQ, recent) for t in range(4)]),
                              _load(wq_t, (i,), same, DM // 2)))
            latest[0] = m[-2]
            for n, val in enumerate(_combine(m)):
                val = val * SCALE_B
                for r in range(2):
                    q[4 * c + 2 * (n // 2) + r, n % 2] = val[r * T:(r + 1) * T].astype(BF16)

        def proj_kv(c):
            m = []
            for i in range(49):
                recent = m[i - RKV] if i >= RKV else latest[0]
                m.append(_dot(lhs(c_t, (i,), c * T, T, 4 * WKV, recent), _load(wkv_t, (i,), same, T)))
            latest[0] = m[-RKV]
            for r, row in enumerate(_combine2(m)):
                for n, val in enumerate(row):
                    (k, v)[n % 2][4 * c + r, n // 2] = val.astype(BF16)

        scores, ctx, stored, spread, checks = {}, {}, [], {}, []

        def score(i, h):
            tiles = [_dot_nt(q[i, h], k[t, h]) for t in range(i + 1)]
            tiles[-1] = jnp.where(causal, tiles[-1], MASKED)
            scores[i, h] = tiles

        def attend(i, h):
            tiles = scores.pop((i, h))
            p = [jnp.exp2(s) for s in tiles]
            l = jnp.sum(functools.reduce(jnp.add, p), axis=1, keepdims=True)
            if stored and stored[0][0] <= 0:
                p[CTP] = _or_first(p[CTP], stored.pop(0)[1])
            for entry in stored:
                entry[0] -= 1
            for t in range(i):
                token = background(64 * WATT, None)
                if token is not None:
                    p[t] = _or_first(p[t], token)
            o = _dot(p[0].astype(BF16), v[0, h])
            for t in range(1, i + 1):
                o = o + _dot(p[t].astype(BF16), v[t, h])
            latest[0] = tiles[-1]
            r = pl.reciprocal(l, approx=True)
            ctx[i, h] = o * (r * (2.0 - l * r))
            spread[i, h] = _fold(jnp.maximum, jnp.broadcast_to(l + r, (T, T)))
            b = i // 2
            quad = [(2 * b, 0), (2 * b, 1), (2 * b + 1, 0), (2 * b + 1, 1)]
            if all(u in ctx for u in quad):
                terms = _terms(LHS, lambda m: ctx.pop(quad[m]))
                for n, val in enumerate(terms):
                    ctx_t[n, j, pl.ds(b * T, T), :] = val.astype(BF16)
                checks.append((_fold(jnp.add, terms[0] + terms[5] + terms[6]),
                               functools.reduce(jnp.maximum, [spread.pop(u) for u in quad])))
                if b not in ((7,) if first else (0,) if L7 else (0, 7)):
                    stored.append([L7 - 1 if b == 7 else CTX_DELAY, tok.stored(ctx_t, (6, j), b * T) | tok.of(*checks[-1])])

        def flush():
            while jobs:
                jobs.pop(0)()

        def queue(cycles, more):
            pace["period"], pace["clock"] = cycles / max(len(more), 1), 0
            jobs.extend(more)

        def interleave(x, y):
            order = [((n + 0.5) / len(x), 0, job) for n, job in enumerate(x)]
            order += [((n + 0.5) / max(len(y), 1), 1, job) for n, job in enumerate(y)]
            return [job for _, _, job in sorted(order, key=lambda e: e[:2])]

        def both(i):
            return [(i, 0), (i, 1)]

        def lag(i):
            return 0 if i >= LAG0 else 1 if i >= LAG1 else 2

        def steady(blocks, waiting, skip=0):
            for i in blocks:
                for u in both(i)[skip:]:
                    score(*u)
                    waiting.append(u)
                    while len(waiting) > lag(i):
                        attend(*waiting.pop(0))

        def loop(rows, body):
            def step(x, carry):
                body(16 * x)
            lax.fori_loop(0, rows // 16, step, None)

        def start(*copies):
            for cp in copies:
                cp.start()

        def wait(*copies):
            for cp in copies:
                cp.wait()

        late_q = END == 'c' and not first
        side = interleave(jobs_wob, jobs_wo + jobs_wa)
        q_time, kv_time, tile_time = 1792 * WQ, 1568 * WKV, 64 * WATT
        if first:
            def plain(raw, c, weights):
                def operand():
                    rows = []
                    for r in range(c * CH, (c + 1) * CH, 32):
                        part = raw[pl.ds(r, 32), :]
                        token = background(8 * (raw.shape[1] // T), None)
                        if token is not None:
                            part = _cat([_or_first(part[:, :2 * T], _cat([token, token])), part[:, 2 * T:]])
                        rows.append(part)
                    return _cat(rows, axis=0)
                return [_dot(operand(), w) for w in weights]

            def plain_kv(c):
                for n, val in enumerate(plain(c_raw, c, wkv)):
                    for r in range(4):
                        (k, v)[n // 2][4 * c + r, n % 2] = val[r * T:(r + 1) * T].astype(BF16)

            def plain_q(c):
                for h, val in enumerate(plain(bx_raw, c, wq)):
                    for r in range(4):
                        q[4 * c + r, h] = (val[r * T:(r + 1) * T] * SCALE_B).astype(BF16)

            stage = [act_copy(0, 0), head_copy(0, 0, 0), head_copy(1, 0, 0)]
            start(*stage)
            wait(*stage)
            stage = [act_copy(0, 1), act_copy(0, 2)]
            start(*stage)
            wkv = [w.astype(BF16) for raw in (wk_raw, wv_raw) for w in _split(raw[0])]
            queue(FQ * 2048, jobs_c(0))
            plain_kv(0)
            flush()
            wait(*stage)
            stage = [act_copy(0, 3), act_copy(1, 0), head_copy(2, 0, 0)]
            start(*stage)
            queue(FQ * 4096, jobs_c(1) + jobs_c(2))
            plain_kv(1)
            plain_kv(2)
            flush()
            wait(*stage)
            stage = [act_copy(1, 1), act_copy(1, 2)]
            start(*stage)
            wq = [w.astype(BF16) for w in _split(wq_raw[0])]
            queue(FQ * 4096, jobs_c(3) + jobs_x(0))
            plain_kv(3)
            plain_q(0)
            for u in both(2) + both(3) + both(0) + both(1):
                score(*u)
            for u in both(2) + both(3) + both(0) + both(1):
                attend(*u)
            flush()
            wait(*stage)
            stage = [act_copy(1, 3), side_copy(0, 0, 0), side_copy(1, 0, 0)]
            stage += [head_copy(n, 1, 1) for n in range(3)]
            start(*stage)
            lax.fori_loop(0, WO1, lambda word, carry: wo_copy(word).start(), None)
            queue(FQ * (4096 + (2 * sum(range(4, FW)) - FW + 1) * tile_time), jobs_x(1) + jobs_x(2))
            plain_q(1)
            waiting = []
            steady(range(4, 8), waiting)
            plain_q(2)
            steady(range(8, FW), waiting)
            flush()
            wait(*stage)
            start(*[wo_copy(word) for word in range(WO1, 16)])
            start(*[side_copy(n, 1, 1) for n in range(2)], *[head_copy(n, 2, 0) for n in range(3)])
            queue(FQ * (2048 + (2 * sum(range(FW, 14)) + FW - 1) * tile_time),
                  interleave(jobs_x(3) + interleave(jobs_wob, jobs_wa), jobs_wkv(1) + jobs_wq(1)))
            steady(range(FW, 12), waiting)
            plain_q(3)
            steady(range(12, 14), waiting)
            flush()
            wait(*[wo_copy(word) for word in range(16)])
            prefetch_ax()
            queue(FQ * 40 * tile_time, jobs_wo)
            steady(range(14, 16), waiting)
            flush()
        else:
            if END == 'a':
                queue(SIDE * (3 * q_time + 4 * kv_time + (2 * sum(range(2, 12)) - 11) * tile_time), side)
                proj_kv(0)
                proj_q(0)
                score(2, 0)
                score(2, 1)
                proj_kv(1)
                score(3, 0)
                attend(2, 0)
                proj_q(1)
                attend(2, 1)
                score(3, 1)
                attend(3, 0)
                waiting = [(3, 1)]
                steady(range(4, E2), waiting)
            else:
                nq = 3 if END == 'b' else 2
                queue(SIDE * (nq * q_time + 4 * kv_time + (2 * sum(range(4, 12)) - 11) * tile_time), side)
                proj_kv(0)
                if END == 'b':
                    proj_q(1)
                    proj_kv(1)
                    score(4, 0)
                    proj_q(0)
                else:
                    proj_q(1)
                    proj_kv(1)
                    score(4, 0)
                waiting = [(4, 0)]
                steady([4], waiting, 1)
                steady(range(5, 8), waiting)
            proj_kv(2)
            steady(range(E2, 8), waiting)
            proj_q(2)
            steady(range(8, E3), waiting)
            proj_kv(3)
            steady(range(E3, 12), waiting)
            flush()
            more = jobs_wkv(1 - slot)
            queue(1792 * WQ * 0.95, more[:NKV])
            proj_q(3)
            flush()
            queue(TAILF * tile_time * (11 + 2 * (12 + 13 + 14)),
                  interleave(more[NKV:], ([] if late_q else jobs_wq(1 - slot))))
            steady(range(12, 16), waiting)
            flush()
        if late_q:
            proj_q(0)
            queue(0.9 * tile_time * (15 + 2 * (3 + 2 + 1)), jobs_wq(1 - slot))
        small = [] if first else both(0) + both(1) if END == 'a' else both(3) + both(2) + both(1) + both(0)
        for u in small:
            score(*u)
        for u in waiting + small:
            attend(*u)
        assert not jobs, len(jobs)
        guard[0] = functools.reduce(jnp.add, [x for x, _ in checks], guard[0])
        guard[1] = functools.reduce(jnp.maximum, [x for _, x in checks], guard[1])

    if CFG.get('only') != '1':
        if True:
            pair_body(0, first=True)
    def it(j, carry):
        if True:
            pair_body(j)
    if CFG.get('only') != 'f': lax.fori_loop(1, NP, it, None)
    for n in range(3):
        head_copy(n, NP - 1, (NP - 1) % 2).wait()
    for n in range(2):
        side_copy(n, NP - 1, NP % 2).wait()

    safe = jnp.logical_and(jnp.abs(guard[0]) < jnp.inf, guard[1] < SAFE_SUM)

    @pl.when(jnp.max(jnp.where(safe, 0.0, 1.0)) > 0.0)
    def _():
        pl.run_scoped(exact_pairs, pltpu.VMEM((3, S, T), BF16), pltpu.VMEM((2, S, T), F32))


def _outputs(ax_hbm, out_hbm, ctx_t, wob_t, waq_t, wakv_t, wo_t, zero_smem,
             ax_raw, sem_ax, ax_t, o_t, kbuf, vbuf, qbuf, acc, obuf, sem_out):

    def ax_copy(c, slot):
        rows = pl.ds(_aligned(c * CO, CO), CO)
        return pltpu.make_async_copy(ax_hbm.at[rows, :], ax_raw.at[slot], sem_ax.at[slot])

    def out_copy(c, slot):
        rows = pl.ds(_aligned(c * CO, CO), CO)
        return pltpu.make_async_copy(obuf.at[slot], out_hbm.at[rows, :], sem_out.at[slot])

    def store_ax(src, i, n, r):
        def block(row, col):
            return ax_raw[src, pl.ds(row * RO + r, 16), pl.ds((2 * col + n) * T, T)].astype(F32)
        outer = [_term(LHS, i, lambda m: block(2 * (m // 2) + x // 2, 2 * (m % 2) + x % 2))
                 for x in range(4)]
        for x, val in enumerate(_terms(LHS, outer.__getitem__) + outer[1:3]):
            ax_t[9 * i + x, n, pl.ds(r, 16), :] = val.astype(BF16)

    ax_jobs = [(i, n, r) for n in range(2) for r in range(0, RO, 16) for i in range(7)]

    for buf in (kbuf, vbuf):
        for t in range(8):
            buf[t, pl.ds(CO, HALO), :] = jnp.zeros((HALO, T), F32)
    ax_copy(0, 0).wait()
    for job in ax_jobs:
        store_ax(0, *job)

    small, medium, large = RO, 4 * RO, 4 * RO
    costs = [small] * 49 + [medium] * 14 + [small] * 49 + [large] * 42 + [small] * 49 + [large] * 7
    starts = [sum(costs[:n]) for n in range(len(costs) + 1)]
    t_q, t_v, t_b, t_o, t_last = (starts[n] for n in (49, 63, 112, 154, 203))

    def chunk_body(c, carry):
        slot = c & 1

        @pl.when(c >= 2)
        def _():
            out_copy(c - 2, slot).wait()

        ax_copy(c, 1 - slot).wait()
        ax_copy(jnp.minimum(c + 2, NO - 1), slot).start()
        tok = _Tokens(zero_smem)

        plan, due, clock = {}, {}, [0]

        def schedule(job, begin, end, release=True):
            first = max([clock[0]] + [n for n in range(len(costs)) if starts[n + 1] <= begin])
            last = min(n for n in range(len(costs)) if starts[n] >= end)
            plan.setdefault(first, []).append((job, last, release))

        def step(a, w):
            n = clock[0]
            clock[0] += 1
            for x, token in enumerate(due.pop(n, [])):
                a[x % len(a)] = _or_first(a[x % len(a)], token)
            a = [x.astype(BF16) if x.dtype == F32 else pltpu.bitcast(x, BF16) for x in a]
            res = [None] * len(w)
            for x in range(len(a)):
                for y in range(len(w)):
                    d = _dot(a[x], w[y](x))
                    res[y] = d if res[y] is None else res[y] + d
            return n, res

        def finish(n, res):
            token = None
            for job, last, release in plan.pop(n, []):
                if release and token is None:
                    token = tok.of(res[0][:8])
                due.setdefault(last, []).append(job(token) if release else job())
            return res

        for buf in (kbuf, vbuf):
            for t in range(8):
                buf[t, pl.ds(0, HALO), :] = buf[t, pl.ds(CO, HALO), :]

        def project2(lhs_t, stride, rhs_t, tile0, write, begin, end):
            m = []

            def recombine(y, r):
                blocks = _combine2([x[y][r:r + 8] for x in m])
                return write(blocks, y, r)

            slabs = [(y, r) for r in range(0, RO, 8) for y in range(2)]
            for x, slab in enumerate(slabs):
                schedule(P(recombine, *slab), begin, begin + (end - begin) * (x + 1) // len(slabs), False)
            for i in range(49):
                n, res = step([_words(lhs_t, (stride * (i // 7) + i % 7, x), 0, RO) for x in range(2)],
                              [P(lambda y, x: _load(rhs_t, (i, tile0 + y), x * T, T), y) for y in range(2)])
                m.append(res)
                finish(n, res)

        def write_rows(buf, blocks, y, r):
            for row in range(4):
                for col in range(4):
                    buf[2 * col + y, pl.ds(HALO + row * RO + r, 8), :] = blocks[row][col]
            return tok.of(*[x for row in blocks for x in row])

        project2(ax_t, 9, wakv_t, 0, P(write_rows, kbuf), t_q, t_v - 300)

        def write_q(m, half, y):
            vals = [val * SCALE_A for val in _combine([x[y] for x in m])]
            for quad, val in enumerate(vals):
                qbuf[4 * (quad % 2) + y, pl.ds((2 * (quad // 2) + half) * RO, RO), :] = val
            return tok.of(*[val[r:r + 8] for val in vals for r in range(0, RO, 8)])

        for half in range(2):
            m = []
            done = t_q + (t_v - t_q) * (half + 1) // 2
            for y in range(4):
                schedule(P(write_q, m, half, y), done, done + 200 + 100 * y, False)
            for i in range(7):
                a = [_words(ax_t, (9 * i + x, n), 0, RO) for x in ((2, 7), (8, 3))[half] for n in range(2)]
                n, res = step(a, [P(lambda y, x: _load(waq_t, (i, y), x * T, T), y) for y in range(4)])
                m.append(res)
                finish(n, res)

        att = {}

        def job_weights(row, r, release):
            base = HALO + row * RO + r
            qs = [_or_first(qbuf[t, pl.ds(row * RO + r, 8), :], release) for t in range(8)]
            logits = []
            for w in range(WIN):
                rows = pl.ds(base - DIL * w, 8)
                x = functools.reduce(jnp.add, [qs[t] * kbuf[t, rows, :] for t in range(8)])
                x = x + pltpu.roll(x, 64, 1)
                x = x + pltpu.roll(x, 32, 1)
                if row == 0 and r < DIL * w:
                    pos = lax.broadcasted_iota(jnp.int32, (8, T), 0) + (c * CO + r)
                    x = jnp.where(pos >= DIL * w, x, MASKED)
                logits.append(x)
            m = functools.reduce(jnp.maximum, logits)
            p = [jnp.exp2(x - m) for x in logits]
            l = functools.reduce(jnp.add, p)
            inv = pl.reciprocal(l, approx=True)
            inv = inv * (2.0 - l * inv)
            att[row, r] = [x * inv for x in p]
            return tok.of(*att[row, r])

        def job_values(row, r, release):
            base = HALO + row * RO + r
            p = [_or_first(x, release) for x in att[row, r]]
            att[row, r] = [
                functools.reduce(jnp.add, [p[w] * vbuf[t, pl.ds(base - DIL * w, 8), :]
                                           for w in range(WIN)])
                for t in range(8)]
            return tok.of(*att[row, r])

        def job_o(n, r, i):
            def block(row, col):
                return _cat([att[row, r][2 * col + n], att[row, r + 8][2 * col + n]], axis=0)
            for x, val in enumerate(_terms2(LHS, i, block)):
                o_t[7 * i + x, n, pl.ds(r, 16), :] = val.astype(BF16)
            return tok.stored(o_t, (7 * i + 6, n), r)

        groups = [(row, r + x) for r in range(0, RO, 16) for row in range(4) for x in (0, 8)]
        w0, w1 = t_v + W0, t_b + W1
        v0, v1 = t_b + V0, t_o - V1
        for g, (row, r) in enumerate(groups):
            begin = w0 + (w1 - w0) * g // len(groups)
            schedule(P(job_weights, row, r), begin, begin + WWIN)
            begin = max(v0 + (v1 - v0) * g // len(groups), begin + WWIN)
            schedule(P(job_values, row, r), begin, begin + VWIN)
            if g % 8 == 7:
                for x, (n, i) in enumerate((n, i) for n in range(2) for i in range(7)):
                    schedule(P(job_o, n, r - 8, i), begin, min(begin + VWIN + OSTEP * (x + 1), t_o), False)
        project2(ax_t, 9, wakv_t, 2, P(write_rows, vbuf), t_b, t_b + VCOMB)

        touched = set()

        def project_b(i):
            m = []

            def accumulate(y, inner):
                val = _combine([x[y] for x in m])[inner]
                token = None
                for outer, sign in OUT[i]:
                    row, col = 2 * (outer // 2) + inner // 2, 2 * (2 * (outer % 2) + inner % 2) + y
                    rows = pl.ds(row * RO, RO)
                    total = val
                    if (outer, inner, y) in touched:
                        total = acc[col, rows, :] + val if sign > 0 else acc[col, rows, :] - val
                    touched.add((outer, inner, y))
                    if any(outer == n for x in range(i + 1, 7) for n, _ in OUT[x]):
                        acc[col, rows, :] = total
                        token = tok.stored(acc, (col,), row * RO)
                    else:
                        obuf[slot, rows, pl.ds(DM + col * T, T)] = total.astype(BF16)
                        if token is None:
                            token = tok.of(*[total[r:r + 8] for r in range(0, RO, 8)])
                return token

            parts = [(y, inner) for y in range(2) for inner in range(4)]
            done = starts[clock[0] + 7]
            if i < 6:
                for x, part in enumerate(parts):
                    schedule(P(accumulate, *part), done, done + AWIN + ASTEP * x, False)
            for n in range(7):
                def quad(kt, x):
                    return (i, 2 * kt + x % 2), (2 * c + x // 2) * RO
                if len(LHS[n]) == 1:
                    a = [_words(ctx_t, *quad(kt, LHS[n][0][0]), RO) for kt in range(8)]
                else:
                    a = [_term(LHS, n, lambda x: _load(ctx_t, *quad(kt, x), RO).astype(F32))
                         for kt in range(8)]
                idx, res = step(a, [P(lambda y, x: _load(wob_t, (7 * i + n, y), x * T, T), y)
                                    for y in range(2)])
                m.append(res)
                finish(idx, res)
            if i == 6:
                for part in parts:
                    accumulate(*part)

        for i in range(6):
            project_b(i)

        def job_ax(i, n, r):
            store_ax(1 - slot, i, n, r)
            return tok.stored(ax_t, (9 * i + 8, n), r)

        for x, job in enumerate(ax_jobs):
            schedule(P(job_ax, *job), t_o, t_o + 100 + (XSPAN - 100) * (x + 1) // len(ax_jobs), False)

        halves = {}

        def write_out(blocks, y, r):
            if r % 16 == 0:
                halves[y] = blocks
            else:
                for row in range(4):
                    for col in range(4):
                        val = _cat([halves[y][row][col], blocks[row][col]], axis=0)
                        obuf[slot, pl.ds(row * RO + r - 8, 16), pl.ds((2 * col + y) * T, T)] = val.astype(BF16)
            return tok.of(*[x for row in blocks for x in row])

        project2(o_t, 7, wo_t, 0, write_out, t_last, starts[-2])
        project_b(6)
        assert not plan and not due, (plan, due)
        out_copy(c, slot).start()
        return carry

    def it(c, carry):
        if True:
            chunk_body(c, carry)
    lax.fori_loop(0, NO, it, None)
    ax_copy(NO - 1, (NO - 1) % 2).wait()
    out_copy(NO - 2, 0).wait()
    out_copy(NO - 1, 1).wait()


def _kernel(ax_hbm, wqkv_hbm, wo_hbm, bx_hbm, c_hbm, wq_hbm, wuk_hbm, wuv_hbm, wob_hbm,
            out_hbm, ctx_t, wob_t, waq_t, wakv_t, wo_t, zero_smem, idle_sem, ax_raw, sem_ax):

    @pl.when(pl.semaphore_read(idle_sem) == 0)
    def _():
        zero_smem[0] = 0

    vmem, dma = pltpu.VMEM, pltpu.SemaphoreType.DMA

    def prefetch_ax():
        for c in range(2):
            pltpu.make_async_copy(ax_hbm.at[pl.ds(c * CO, CO), :], ax_raw.at[c], sem_ax.at[c]).start()

    shared = (ctx_t, wob_t, waq_t, wakv_t, wo_t, zero_smem)
    if CFG.get('only') != '2': pl.run_scoped(
        P(_head_pairs, wqkv_hbm, wo_hbm, bx_hbm, c_hbm, wq_hbm, wuk_hbm, wuv_hbm, wob_hbm, prefetch_ax, *shared),
        vmem((S, DM), BF16),
        vmem((S, DC), BF16),
        vmem((2, DM, T), U32),
        vmem((2, DC, T), U32),
        vmem((2, DC, T), U32),
        vmem((2, 4, 64, DM), BF16),
        vmem((2, 4, 8, 3 * DM), U32),
        vmem((16, NH, DM), U32),
        vmem((7, 4, S // 2, T), BF16),
        vmem((49, S // 4, T), BF16),
        vmem((7, DM // 2, T), BF16),
        vmem((49, T, T), BF16),
        vmem((2, 8, T), F32),
        dma((2 * NC,)), dma((11,)))
    if CFG.get('only') in ('1', 'f'):
        def fin(buf, sem):
            z = zero_smem[0]
            val = ctx_t[z, z, pl.ds(0, 16), :]
            for ref in (wob_t, waq_t, wakv_t, wo_t):
                val = val + ref[z, z, pl.ds(z * 16, 16), :]
            buf[...] = val
            cp = pltpu.make_async_copy(buf, out_hbm.at[pl.ds(0, 16), pl.ds(0, T)], sem)
            cp.start(); cp.wait()
        pl.run_scoped(fin, vmem((16, T), BF16), dma(()))
        return
    pl.run_scoped(
        P(_outputs, ax_hbm, out_hbm, *shared, ax_raw, sem_ax),
        vmem((63, 2, RO, T), BF16),
        vmem((49, 2, RO, T), BF16),
        vmem((8, HALO + CO, T), F32),
        vmem((8, HALO + CO, T), F32),
        vmem((8, CO, T), F32),
        vmem((8, CO, T), F32),
        vmem((2, CO, 2 * DM), BF16),
        dma((2,)))


@jax.jit
def pallas_concat_heads__sliding_local_dilated__compressed_kv_cla__prompt_kernel(
    A_x: jax.Array,
    A_wqkv: jax.Array,
    A_wo: jax.Array,
    B_x: jax.Array,
    B_c_kv: jax.Array,
    B_w_q: jax.Array,
    B_w_uk: jax.Array,
    B_w_uv: jax.Array,
    B_w_o: jax.Array,
):
    vmem = pltpu.VMEM
    out = pl.pallas_call(
        _kernel,
        out_shape=jax.ShapeDtypeStruct((S, 2 * DM), BF16),
        in_specs=[pl.BlockSpec(memory_space=pl.ANY)] * 9,
        out_specs=pl.BlockSpec(memory_space=pl.ANY),
        scratch_shapes=[
            vmem((7, NP, S // 2, T), BF16),
            vmem((49, 2, DM, T), BF16),
            vmem((7, 4, DM // 2, T), BF16),
            vmem((49, 4, 2 * T, T), BF16),
            vmem((49, 2, 2 * T, T), BF16),
            pltpu.SMEM((1,), jnp.int32),
            pltpu.SemaphoreType.REGULAR,
            vmem((2, CO, DM), BF16),
            pltpu.SemaphoreType.DMA((2,)),
        ],
        compiler_params=pltpu.CompilerParams(vmem_limit_bytes=124 * 2**20, disable_bounds_checks=CFG.get('nb', '1') == '1',
            flags={'lp': {'XLA_TPU_FORCE_LP_LLO_SCHEDULER': True}, 'ev': {'XLA_TPU_EVENLY_DISTRIBUTE_CRITICAL_NODES': True}, 'rd': {'XLA_TPU_RESCHEDULE_DMA_DONES': True}, '': None}[CFG.get('fl', '')]),
    )(
        A_x.reshape(S, DM),
        A_wqkv.reshape(4, DM // 4, 3 * DM),
        A_wo.reshape(NH, DM // NH, DM),
        B_x.reshape(S, DM),
        B_c_kv.reshape(S, DC),
        B_w_q,
        B_w_uk,
        B_w_uv,
        B_w_o,
    )
    return out.reshape(1, S, 2 * DM)
```

```python
import functools
import math

import jax
import jax.numpy as jnp
from jax import lax
import jax.experimental.pallas as pl
import jax.experimental.pallas.tpu as pltpu

CFG = {'jw': '16', 'wq': '0', 'cd': '12', 'tailf': '0.9', 'end': 'n', 'e2': '8', 'nkv': '8', 'e3': '10', 'wkv': '0.2'}
PQ = int(CFG.get('pq', 12)); CTX_DELAY = int(CFG.get('cd', 12)); SK = int(CFG.get('sk', 3))
BORD = CFG.get('bord', 'k'); WD = int(CFG.get('wd', 1)); OSK = int(CFG.get('osk', 3)); WSK = int(CFG.get('wsk', 7)); ASK = int(CFG.get('ask', 2))
WQ = float(CFG.get('wq', 0)); WKV = float(CFG.get('wkv', 0)); WATT = float(CFG.get('watt', 1)); SIDE = float(CFG.get('side', 0.95)); NKV = int(CFG.get('nkv', 0)); TAILF = float(CFG.get('tailf', 0.9))
LT = CFG.get('lt', ''); LTP = int(CFG.get('ltp', 0)); CTP = int(CFG.get('ctp', -1))
FM = CFG.get('fm', 'prev')
G = int(CFG.get('g', 0)); GL = int(CFG.get('gl', 1))
RP = int(CFG.get('rp', 0))
g_ = lambda k, d: int(CFG.get(k, d))
W0, W1, V0, V1, WWIN, VWIN, OSTEP, VCOMB = g_('w0', 300), g_('w1', 3500), g_('v0', 2500), g_('v1', 700), g_('wwin', 600), g_('vwin', 300), g_('ostep', 60), g_('vcomb', 1500)
AWIN, ASTEP, XSPAN = g_('awin', 256), g_('astep', 150), g_('xspan', 4500)
NFS = g_('nfs', 40); FW = g_('fw', 9); WO1 = g_('wo1', 2)
REL = g_('rel', 1); RQ = g_('rq', 2); RKV = g_('rkv', 12); END = CFG.get('end', 'a'); L7 = g_('l7', 0)
SUBR = g_('sub', 128); FAST = g_('fast', 0)
LAG0 = g_('lag0', 99); LAG1 = g_('lag1', 5); E2 = g_('e2', 6); E3 = g_('e3', 12)
FQ = float(CFG.get('fq', 0.98))
GROUP = g_('grp', 1); DEPTH = g_('dep', 3); UD = g_('ud', 0); E1 = g_('e1', 0)
JW = g_('jw', 5)
WSPAN = int(CFG.get('wspan', 49)); VSPAN = int(CFG.get('vspan', 24))

S = 2048
DM = 1024
DC = 512
NH = 32
NP = NH // 2
T = 128
CH = 4 * T
NC = S // CH
RO = 64
CO = 4 * RO
NO = S // CO
ROWB = lambda inner, outer: 2 * outer + inner
WIN, DIL = 8, 2
HALO = 16

LOG2E = math.log2(math.e)
SCALE_A = (DM // NH) ** -0.5 * LOG2E
SCALE_B = T ** -0.5 * LOG2E
MASKED = -1e9 * LOG2E
SAFE_SUM = 2.0 ** 40

F32, BF16, U32 = jnp.float32, jnp.bfloat16, jnp.uint32
P = functools.partial


def _dot(a, b):
    return jnp.dot(a, b, preferred_element_type=F32)


def _dot_nt(a, b):
    return lax.dot_general(a, b, (((1,), (1,)), ((), ())), preferred_element_type=F32)


def _cat(xs, axis=1):
    return xs[0] if len(xs) == 1 else jnp.concatenate(xs, axis=axis)


def _aligned(x, n):
    return x if isinstance(x, int) else pl.multiple_of(x, n)


def _words(ref, lead, start, n):
    return ref.bitcast(U32)[(*lead, pl.ds(_aligned(start >> 1, 8), n // 2), slice(None))]


def _load(ref, lead, start, n):
    return pltpu.bitcast(_words(ref, lead, start, n), BF16)


def _split(w):
    return (pltpu.bitcast(w << 16, F32), pltpu.bitcast(w & jnp.uint32(0xFFFF0000), F32))


def _fold(op, x):
    return functools.reduce(op, [x[r:r + 8] for r in range(0, x.shape[0], 8)])


def _or_first(w, tok):
    bits = w if w.dtype == U32 else pltpu.bitcast(w, U32)
    bits = bits | tok if bits.shape[0] == 8 else _cat([bits[:8] | tok, bits[8:]], axis=0)
    return bits if w.dtype == U32 else pltpu.bitcast(bits, w.dtype)


LHS = (((0, 1), (3, 1)), ((2, 1), (3, 1)), ((0, 1),), ((3, 1),),
       ((0, 1), (1, 1)), ((2, 1), (0, -1)), ((1, 1), (3, -1)))
RHS = (((0, 1), (3, 1)), ((0, 1),), ((1, 1), (3, -1)), ((2, 1), (0, -1)),
       ((3, 1),), ((0, 1), (1, 1)), ((2, 1), (3, 1)))
OUT = (((0, 1), (3, 1)), ((2, 1), (3, -1)), ((1, 1), (3, 1)), ((0, 1), (2, 1)),
       ((0, -1), (1, 1)), ((3, 1),), ((0, 1),))


def _term(table, i, quad):
    (n, _), *rest = table[i]
    val = quad(n)
    for n, sign in rest:
        val = val + quad(n) if sign > 0 else val - quad(n)
    return val


def _terms(table, quad):
    blocks = [quad(n) for n in range(4)]
    return [_term(table, i, blocks.__getitem__) for i in range(7)]


def _terms2(table, i, block):
    return _terms(table, lambda n: _term(
        table, i, lambda m: block(2 * (m // 2) + n // 2, 2 * (m % 2) + n % 2)))


def _combine(m):
    out = [None] * 4
    for i in range(7):
        for n, sign in OUT[i]:
            if out[n] is None:
                out[n] = m[i]
            else:
                out[n] = out[n] + m[i] if sign > 0 else out[n] - m[i]
    return out


def _combine2(m):
    inner = [_combine(m[7 * i:7 * i + 7]) for i in range(7)]
    out = [[None] * 4 for _ in range(4)]
    for n in range(4):
        for quad, val in enumerate(_combine([x[n] for x in inner])):
            out[2 * (quad // 2) + n // 2][2 * (quad % 2) + n % 2] = val
    return out


class _Tokens:
    def __init__(self, zero_smem):
        self.z = zero_smem[0]
        self.zv = jnp.full((8, T), self.z, jnp.int32).astype(U32)

    def stored(self, ref, lead, start):
        first, *rest = lead
        if FM == 'lead':
            if ref.dtype == BF16:
                return _words(ref, (first + self.z, *rest), start, 16) & self.zv
            return self.of(ref[(first + self.z, *rest, pl.ds(start, 8), slice(None))])
        bit = self.z & 1
        if FM == 'prev':
            if ref.dtype == BF16:
                return _words(ref, (first - bit, *rest), start, 16) & self.zv
            return self.of(ref[(first, *rest, pl.ds(_aligned(start + 8 * bit, 8), 8), slice(None))])

    def of(self, *vals):
        tok = vals[0]
        for x in vals[1:]:
            tok = tok + x
        return pltpu.bitcast(tok, U32) & self.zv


def _head_pairs(wqkv_hbm, wo_hbm, bx_hbm, c_hbm, wq_hbm, wuk_hbm, wuv_hbm, wob_hbm, prefetch_ax,
                ctx_t, wob_t, waq_t, wakv_t, wo_t, zero_smem,
                bx_raw, c_raw, wq_raw, wk_raw, wv_raw, wob_raw, wqkv_raw, wo_raw,
                bx_t, c_t, wq_t, wkv_t, guard, sem_in, sem_w):
    guard[...] = jnp.zeros(guard.shape, F32)

    def head_copy(n, j, slot):
        src, dst = ((wuk_hbm, wk_raw), (wuv_hbm, wv_raw), (wq_hbm, wq_raw))[n]
        return pltpu.make_async_copy(src.bitcast(U32).at[:, j, :], dst.at[slot], sem_w.at[3 * slot + n])

    def side_copy(n, j, slot):
        if n == 0:
            src = wob_hbm.at[pl.ds(4 * (j >> 1), 4), pl.ds(_aligned((j & 1) * 64, 64), 64), :]
            dst = wob_raw.at[slot]
        else:
            src = wqkv_hbm.bitcast(U32).at[:, pl.ds(_aligned(8 * j, 8), 8), :]
            dst = wqkv_raw.at[slot]
        return pltpu.make_async_copy(src, dst, sem_w.at[6 + 2 * slot + n])

    def wo_copy(word):
        return pltpu.make_async_copy(wo_hbm.bitcast(U32).at[:, word, :], wo_raw.at[word], sem_w.at[10])

    def act_copy(n, c):
        src, dst = ((c_hbm, c_raw), (bx_hbm, bx_raw))[n]
        rows = pl.ds(c * CH, CH)
        return pltpu.make_async_copy(src.at[rows, :], dst.at[rows, :], sem_in.at[2 * c + n])

    def exact_pairs(qkv, ctx):
        def block(i):
            return pl.ds(pl.multiple_of(i * T, T), T)

        def head(h, carry):
            def weight(raw):
                even, odd = _split(raw[0])
                return jnp.where(h == 0, even, odd).astype(BF16)
            wk, wv, wq = weight(wk_raw), weight(wv_raw), weight(wq_raw)

            def project(i, carry):
                qkv[0, block(i), :] = (_dot(bx_raw[block(i), :], wq) * SCALE_B).astype(BF16)
                qkv[1, block(i), :] = _dot(c_raw[block(i), :], wk).astype(BF16)
                qkv[2, block(i), :] = _dot(c_raw[block(i), :], wv).astype(BF16)
            lax.fori_loop(0, S // T, project, None)

            def attend(i, carry):
                def scores(t):
                    row = lax.broadcasted_iota(jnp.int32, (T, T), 0) + i * T
                    col = lax.broadcasted_iota(jnp.int32, (T, T), 1) + t * T
                    return jnp.where(col <= row, _dot_nt(qkv[0, block(i), :], qkv[1, block(t), :]), MASKED)

                m = lax.fori_loop(
                    0, i + 1, lambda t, m: jnp.maximum(m, jnp.max(scores(t), axis=1, keepdims=True)),
                    jnp.full((T, 1), -jnp.inf, F32))

                def accumulate(t, carry):
                    l, o = carry
                    p = jnp.exp2(scores(t) - m)
                    return (l + jnp.sum(p, axis=1, keepdims=True),
                            o + _dot(p.astype(BF16), qkv[2, block(t), :]))
                l, o = lax.fori_loop(0, i + 1, accumulate,
                                     (jnp.zeros((T, 1), F32), jnp.zeros((T, T), F32)))
                ctx[h, block(i), :] = o / l
            lax.fori_loop(0, S // T, attend, None)

        def pair(j, carry):
            for n in range(3):
                head_copy(n, j, 0).start()
            for n in range(3):
                head_copy(n, j, 0).wait()
            lax.fori_loop(0, 2, head, None)

            def store(b, carry):
                for n, val in enumerate(_terms(LHS, lambda m: ctx[m % 2, block(2 * b + m // 2), :])):
                    ctx_t[n, j, block(b), :] = val.astype(BF16)
            lax.fori_loop(0, S // T // 2, store, None)

        lax.fori_loop(0, NP, pair, None)

    def pair_body(j, first=False):
        slot = j & 1
        if not first:
            for n in range(3):
                head_copy(n, j, 1 - slot).wait()
            for n in range(2):
                side_copy(n, j, slot).wait()
            for n in range(3):
                head_copy(n, jnp.minimum(j + 2, NP - 1), slot).start()
            for n in range(2):
                side_copy(n, jnp.minimum(j + 1, NP - 1), 1 - slot).start()
        tok = _Tokens(zero_smem)
        causal = (lax.broadcasted_iota(jnp.int32, (T, T), 1)
                  <= lax.broadcasted_iota(jnp.int32, (T, T), 0))
        jobs, pace = [], dict(period=0, clock=0)

        def background(cycles, recent):
            pace["clock"] += cycles
            token = None
            while jobs and pace["clock"] >= pace["period"]:
                pace["clock"] -= pace["period"]
                pace["release"] = None if recent is None or not REL else tok.of(recent[:8])
                new = jobs.pop(0)()
                pace["release"] = None
                token = new if token is None else token | new
            return token

        def released(x):
            if pace.get("release") is None:
                return x
            bits = x if x.dtype == U32 else pltpu.bitcast(x, U32)
            bits = _cat([bits[r:r + 8] | pace["release"] for r in range(0, bits.shape[0], 8)], axis=0)
            return bits if x.dtype == U32 else pltpu.bitcast(bits, x.dtype)

        same = 0

        def lhs(ref, lead, start, n, cycles, recent):
            w = _words(ref, lead, start, n)
            parts = []
            for r in range(0, n // 2, 8):
                token = background(cycles, None)
                parts.append(w[r:r + 8] if token is None else w[r:r + 8] | token)
            return pltpu.bitcast(_cat(parts, axis=0), BF16)

        def store_terms(dst, first_term, lead, row, terms):
            for i, val in enumerate(terms):
                dst[(first_term + i, *lead, pl.ds(_aligned(row, 16), 16), slice(None))] = val.astype(BF16)
            return tok.stored(dst, (first_term + 6, *lead), row)

        def job_wkv(src, i, r):
            def block(row, col):
                raw = (wk_raw, wv_raw)[col % 2]
                return _split(released(raw[src, pl.ds(_aligned(row * T + r, 16), 16), :]))[col // 2]
            return store_terms(wkv_t, 7 * i, (), r, _terms2(RHS, i, block))

        def job_wq(src, r):
            top, bot = _split(released(wq_raw[src, pl.ds(_aligned(r, 16), 16), :])), _split(released(wq_raw[src, pl.ds(_aligned(DM // 2 + r, 16), 16), :]))
            return store_terms(wq_t, 0, (), r, _terms(RHS, (top + bot).__getitem__))

        def jobs_wkv(src):
            return [P(job_wkv, src, i, r) for r in range(0, T, 16) for i in range(7)]

        def jobs_wq(src):
            return [P(job_wq, src, r) for r in range(0, DM // 2, 16)]

        def job_wob(i, n, r):
            def block(row, col):
                head = 2 * (row % 2) + row // 2
                return released(wob_raw[slot, head, pl.ds(r, 16), pl.ds((2 * col + n) * T, T)].astype(F32))
            return store_terms(wob_t, 7 * i, (n,), j * 64 + r, _terms2(RHS, i, block))

        def job_wo(i, n):
            odd = (j >> 2) & 1

            def block(row, col):
                even_t, odd_t = _split(released(wo_raw[4 * (j & 3) + row, pl.ds(_aligned(16 * (j >> 3), 16), 16),
                                              pl.ds((2 * col + n) * T, T)]))
                return jnp.where(odd == 1, odd_t, even_t)
            return store_terms(wo_t, 7 * i, (n,), odd * T + (j & 3) * NH + (j >> 3) * 16,
                               _terms2(RHS, i, block))

        permuted = {}

        def job_permute(mat, row):
            lane = lax.broadcasted_iota(jnp.int32, (8, T), 1)
            e, grp, sub = lane >> 5, (lane >> 2) & 7, lane & 3
            x = [released(wqkv_raw[slot, row, :, pl.ds(mat * DM + t * T, T)]) for t in range(8)]
            y = [jnp.take_along_axis(x[t], sub * 32 + e * 8 + ((grp - t) & 7), axis=1)
                 for t in range(8)]
            u = [y[-s % 8] for s in range(8)]
            for bit in (1, 2, 4):
                u = [jnp.where((grp & bit) != 0, u[(s - bit) % 8], u[s]) for s in range(8)]
            u = [u[0]] + [jnp.take_along_axis(u[t], e * 32 + ((grp + t) & 7) * 4 + sub, axis=1)
                          for t in range(1, 8)]
            permuted[mat, row] = u
            return functools.reduce(jnp.bitwise_or, u) & tok.zv

        def column(mat, row, t):
            return pltpu.bitcast(released(permuted[mat, row][t]), BF16).astype(F32)

        def job_waq(half, n):
            terms = _terms(RHS, lambda m: column(0, 2 * (m // 2) + half, 4 * (m % 2) + n))
            return store_terms(waq_t, 0, (n,), half * 2 * T + 16 * j, terms)

        def job_wakv(mat, i, n):
            terms = _terms2(RHS, i, lambda row, col: column(mat, row, 2 * col + n))
            return store_terms(wakv_t, 7 * i, (2 * (mat - 1) + n,), 16 * j, terms)

        jobs_wob = [P(job_wob, i, n, r) for r in range(0, 64, 16) for n in range(2) for i in range(7)]
        jobs_wo = [P(job_wo, i, n) for n in range(2) for i in range(7)]
        jobs_wa = [P(job_permute, 0, row) for row in range(4)]
        jobs_wa += [P(job_waq, half, n) for half in range(2) for n in range(4)]
        for mat in (1, 2):
            jobs_wa += [P(job_permute, mat, row) for row in range(4)]
            jobs_wa += [P(job_wakv, mat, i, n) for n in range(2) for i in range(7)]

        q, k, v, latest = {}, {}, {}, [None]

        def job_x(c, t, r):
            terms = _terms(LHS, lambda m: bx_raw[pl.ds(_aligned(c * CH + (m // 2) * 2 * T + r, 16), 16),
                                                 pl.ds((4 * (m % 2) + t) * T, T)].astype(F32))
            return store_terms(bx_t, 0, (t,), c * 2 * T + r, terms)

        def job_c(c, i, r):
            terms = _terms2(LHS, i, lambda row, col: c_raw[
                pl.ds(_aligned(c * CH + row * T + r, 16), 16), pl.ds(col * T, T)].astype(F32))
            return store_terms(c_t, 7 * i, (), c * T + r, terms)

        def jobs_x(c):
            return [P(job_x, c, t, r) for r in range(0, 2 * T, 16) for t in range(4)]

        def jobs_c(c):
            return [P(job_c, c, i, r) for r in range(0, T, 16) for i in range(7)]

        def proj_q(c):
            m = []
            for i in range(7):
                recent = m[i - RQ] if i >= RQ else latest[0]
                m.append(_dot(_cat([lhs(bx_t, (i, t), c * 2 * T, 2 * T, 4 * WQ, recent) for t in range(4)]),
                              _load(wq_t, (i,), same, DM // 2)))
            latest[0] = m[-2]
            for n, val in enumerate(_combine(m)):
                val = val * SCALE_B
                for r in range(2):
                    q[4 * c + 2 * (n // 2) + r, n % 2] = val[r * T:(r + 1) * T].astype(BF16)

        def proj_kv(c):
            m = []
            for i in range(49):
                recent = m[i - RKV] if i >= RKV else latest[0]
                m.append(_dot(lhs(c_t, (i,), c * T, T, 4 * WKV, recent), _load(wkv_t, (i,), same, T)))
            latest[0] = m[-RKV]
            for r, row in enumerate(_combine2(m)):
                for n, val in enumerate(row):
                    (k, v)[n % 2][4 * c + r, n // 2] = val.astype(BF16)

        scores, ctx, stored, spread, checks = {}, {}, [], {}, []

        partial, ready = {}, []

        def finish_unit(i, h):
            l, o = partial.pop((i, h))
            l = jnp.sum(l, axis=1, keepdims=True)
            r = pl.reciprocal(l, approx=True)
            ctx[i, h] = o * (r * (2.0 - l * r))
            spread[i, h] = _fold(jnp.maximum, jnp.broadcast_to(l + r, (T, T)))
            b = i // 2
            quad = [(2 * b, 0), (2 * b, 1), (2 * b + 1, 0), (2 * b + 1, 1)]
            if all(u in ctx for u in quad):
                terms = _terms(LHS, lambda m: ctx.pop(quad[m]))
                for n, val in enumerate(terms):
                    ctx_t[n, j, pl.ds(b * T, T), :] = val.astype(BF16)
                checks.append((_fold(jnp.add, terms[0] + terms[5] + terms[6]),
                               functools.reduce(jnp.maximum, [spread.pop(u) for u in quad])))
                stored.append([CTX_DELAY, tok.stored(ctx_t, (6, j), b * T) | tok.of(*checks[-1])])
            elif UD:
                stored.append([UD, tok.of(_fold(jnp.add, ctx[i, h]))])

        def weigh(group):
            for x, (i, h, t, p) in enumerate(group):
                l, o = partial.get((i, h), (None, None))
                l = p if l is None else l + p
                if G and x % G == G - 1 and t > 0:
                    p = jnp.where(l < 0, l, p)
                token = background(64 * WATT, p if REL else None)
                if REL and token is not None:
                    stored.append([JW, token])
                    token = None
                if x == 0:
                    for entry in stored:
                        entry[0] -= 1
                    for entry in [e for e in stored if e[0] <= 0]:
                        stored[:] = [e for e in stored if e is not entry]
                        token = entry[1] if token is None else token | entry[1]
                if token is not None:
                    p = _or_first(p, token)
                d = _dot(p.astype(BF16), v[t, h])
                partial[i, h] = (l, d if o is None else o + d)
                if t == i:
                    finish_unit(i, h)

        def attention(blocks, drain=False):
            items = leftover + [(i, h, t) for i in blocks for h in range(2) for t in range(i + 1)]
            leftover.clear()
            while len(items) >= (1 if drain else GROUP):
                group, items = items[:GROUP], items[GROUP:]
                tiles = []
                for i, h, t in group:
                    s = _dot_nt(q[i, h], k[t, h])
                    if t == i:
                        s = jnp.where(causal, s, MASKED)
                    tiles.append((i, h, t, jnp.exp2(s)))
                ready.append(tiles)
                if len(ready) > DEPTH:
                    weigh(ready.pop(0))
            leftover.extend(items)
            while drain and ready:
                weigh(ready.pop(0))

        leftover = []

        def flush():
            while jobs:
                jobs.pop(0)()

        def queue(cycles, more):
            pace["period"], pace["clock"] = cycles / max(len(more), 1), 0
            jobs.extend(more)

        def interleave(x, y):
            order = [((n + 0.5) / len(x), 0, job) for n, job in enumerate(x)]
            order += [((n + 0.5) / max(len(y), 1), 1, job) for n, job in enumerate(y)]
            return [job for _, _, job in sorted(order, key=lambda e: e[:2])]

        def loop(rows, body):
            def step(x, carry):
                body(16 * x)
            lax.fori_loop(0, rows // 16, step, None)

        def start(*copies):
            for cp in copies:
                cp.start()

        def wait(*copies):
            for cp in copies:
                cp.wait()

        late_q = END == 'c' and not first
        side = interleave(jobs_wob, jobs_wo + jobs_wa)
        q_time, kv_time, tile_time = 1792 * WQ, 1568 * WKV, 64 * WATT
        if first:
            def plain(raw, c, weights):
                def operand():
                    rows = []
                    for r in range(c * CH, (c + 1) * CH, 32):
                        part = raw[pl.ds(r, 32), :]
                        token = background(8 * (raw.shape[1] // T), None)
                        if token is not None:
                            part = _cat([_or_first(part[:, :2 * T], _cat([token, token])), part[:, 2 * T:]])
                        rows.append(part)
                    return _cat(rows, axis=0)
                return [_dot(operand(), w) for w in weights]

            def plain_kv(c):
                for n, val in enumerate(plain(c_raw, c, wkv)):
                    for r in range(4):
                        (k, v)[n // 2][4 * c + r, n % 2] = val[r * T:(r + 1) * T].astype(BF16)

            def plain_q(c):
                for h, val in enumerate(plain(bx_raw, c, wq)):
                    for r in range(4):
                        q[4 * c + r, h] = (val[r * T:(r + 1) * T] * SCALE_B).astype(BF16)

            stage = [act_copy(0, 0), head_copy(0, 0, 0), head_copy(1, 0, 0)]
            start(*stage[::-1], act_copy(0, 1))
            wait(*stage)
            start(act_copy(0, 2), act_copy(0, 3), act_copy(1, 0), head_copy(2, 0, 0))
            stage = [act_copy(0, 1), act_copy(0, 2)]
            wkv = [w.astype(BF16) for raw in (wk_raw, wv_raw) for w in _split(raw[0])]
            queue(FQ * 2048, jobs_c(0))
            plain_kv(0)
            flush()
            wait(*stage)
            stage = [act_copy(0, 3), act_copy(1, 0), head_copy(2, 0, 0)]
            start(act_copy(1, 1), act_copy(1, 2))
            queue(FQ * 4096, jobs_c(1) + jobs_c(2))
            plain_kv(1)
            plain_kv(2)
            flush()
            wait(*stage)
            stage = [act_copy(1, 1), act_copy(1, 2)]
            wq = [w.astype(BF16) for w in _split(wq_raw[0])]
            queue(FQ * 4096, jobs_c(3) + jobs_x(0))
            plain_kv(3)
            plain_q(0)
            attention(range(4))
            flush()
            wait(*stage)
            stage = [act_copy(1, 3), side_copy(0, 0, 0), side_copy(1, 0, 0)]
            stage += [head_copy(n, 1, 1) for n in range(3)]
            start(*stage)
            lax.fori_loop(0, WO1, lambda word, carry: wo_copy(word).start(), None)
            queue(FQ * (4096 + 2 * sum(range(5, FW + 1)) * tile_time), jobs_x(1) + jobs_x(2))
            plain_q(1)
            attention(range(4, 8))
            plain_q(2)
            attention(range(8, FW))
            flush()
            wait(*stage)
            start(*[wo_copy(word) for word in range(WO1, 16)])
            start(*[side_copy(n, 1, 1) for n in range(2)], *[head_copy(n, 2, 0) for n in range(3)])
            queue(FQ * (2048 + 2 * sum(range(FW + 1, 15)) * tile_time),
                  interleave(jobs_x(3) + interleave(jobs_wob, jobs_wa), jobs_wkv(1) + jobs_wq(1)))
            attention(range(FW, 12))
            plain_q(3)
            attention(range(12, 14))
            flush()
            wait(*[wo_copy(word) for word in range(16)])
            prefetch_ax()
            queue(FQ * 40 * tile_time, jobs_wo)
            attention(range(14, 16), drain=True)
            flush()
        else:
            first_block = 0 if END == 'n' else 2
            queue(SIDE * (3 * q_time + 4 * kv_time + 2 * sum(range(first_block + 1, 13)) * tile_time), side)
            proj_kv(0)
            proj_q(0)
            if E1 == 0:
                proj_kv(1)
            attention(range(first_block, max(E1, first_block)))
            if E1:
                proj_kv(1)
            attention(range(max(E1, first_block), 4))
            proj_q(1)
            attention(range(4, E2))
            proj_kv(2)
            attention(range(E2, 8))
            proj_q(2)
            attention(range(8, E3))
            proj_kv(3)
            attention(range(E3, 12))
            flush()
            more = jobs_wkv(1 - slot)
            queue(q_time * 0.95, more[:NKV])
            proj_q(3)
            flush()
            queue(TAILF * tile_time * 2 * sum(range(13, 17)), interleave(more[NKV:], jobs_wq(1 - slot)))
            attention(list(range(12, 16)) + list(range(first_block)), drain=True)
            flush()
        guard[0] = functools.reduce(jnp.add, [x for x, _ in checks], guard[0])
        guard[1] = functools.reduce(jnp.maximum, [x for _, x in checks], guard[1])

    if CFG.get('only') != '1':
        if True:
            pair_body(0, first=True)
    def it(j, carry):
        if True:
            pair_body(j)
    if CFG.get('only') != 'f': lax.fori_loop(1, NP, it, None)
    for n in range(3):
        head_copy(n, NP - 1, (NP - 1) % 2).wait()
    for n in range(2):
        side_copy(n, NP - 1, NP % 2).wait()

    safe = jnp.logical_and(jnp.abs(guard[0]) < jnp.inf, guard[1] < SAFE_SUM)

    @pl.when(jnp.max(jnp.where(safe, 0.0, 1.0)) > 0.0)
    def _():
        pl.run_scoped(exact_pairs, pltpu.VMEM((3, S, T), BF16), pltpu.VMEM((2, S, T), F32))


def _outputs(ax_hbm, out_hbm, ctx_t, wob_t, waq_t, wakv_t, wo_t, zero_smem,
             ax_raw, sem_ax, ax_t, o_t, kbuf, vbuf, qbuf, acc, obuf, sem_out):

    def ax_copy(c, slot):
        rows = pl.ds(_aligned(c * CO, CO), CO)
        return pltpu.make_async_copy(ax_hbm.at[rows, :], ax_raw.at[slot], sem_ax.at[slot])

    def out_copy(c, slot):
        rows = pl.ds(_aligned(c * CO, CO), CO)
        return pltpu.make_async_copy(obuf.at[slot], out_hbm.at[rows, :], sem_out.at[slot])

    def store_ax(src, i, n, r):
        def block(row, col):
            return ax_raw[src, pl.ds(row * RO + r, 16), pl.ds((2 * col + n) * T, T)].astype(F32)
        outer = [_term(LHS, i, lambda m: block(2 * (m // 2) + x // 2, 2 * (m % 2) + x % 2))
                 for x in range(4)]
        for x, val in enumerate(_terms(LHS, outer.__getitem__) + outer[1:3]):
            ax_t[9 * i + x, n, pl.ds(r, 16), :] = val.astype(BF16)

    ax_jobs = [(i, n, r) for n in range(2) for r in range(0, RO, 16) for i in range(7)]

    for buf in (kbuf, vbuf):
        for t in range(8):
            buf[t, pl.ds(CO, HALO), :] = jnp.zeros((HALO, T), F32)
    ax_copy(0, 0).wait()
    for job in ax_jobs:
        store_ax(0, *job)

    small, medium, large = RO, 4 * RO, 4 * RO
    costs = [small] * 49 + [medium] * 14 + [small] * 49 + [large] * 42 + [small] * 49 + [large] * 7
    starts = [sum(costs[:n]) for n in range(len(costs) + 1)]
    t_q, t_v, t_b, t_o, t_last = (starts[n] for n in (49, 63, 112, 154, 203))

    def chunk_body(c, carry):
        slot = c & 1

        @pl.when(c >= 2)
        def _():
            out_copy(c - 2, slot).wait()

        ax_copy(c, 1 - slot).wait()
        ax_copy(jnp.minimum(c + 2, NO - 1), slot).start()
        tok = _Tokens(zero_smem)

        plan, due, clock = {}, {}, [0]

        def schedule(job, begin, end, release=True):
            first = max([clock[0]] + [n for n in range(len(costs)) if starts[n + 1] <= begin])
            last = min(n for n in range(len(costs)) if starts[n] >= end)
            plan.setdefault(first, []).append((job, last, release))

        def step(a, w):
            n = clock[0]
            clock[0] += 1
            for x, token in enumerate(due.pop(n, [])):
                a[x % len(a)] = _or_first(a[x % len(a)], token)
            a = [x.astype(BF16) if x.dtype == F32 else pltpu.bitcast(x, BF16) for x in a]
            res = [None] * len(w)
            for x in range(len(a)):
                for y in range(len(w)):
                    d = _dot(a[x], w[y](x))
                    res[y] = d if res[y] is None else res[y] + d
            return n, res

        def finish(n, res):
            token = None
            for job, last, release in plan.pop(n, []):
                if release and token is None:
                    token = tok.of(res[0][:8])
                due.setdefault(last, []).append(job(token) if release else job())
            return res

        for buf in (kbuf, vbuf):
            for t in range(8):
                buf[t, pl.ds(0, HALO), :] = buf[t, pl.ds(CO, HALO), :]

        def project2(lhs_t, stride, rhs_t, tile0, write, begin, end):
            m = []

            def recombine(y, r):
                blocks = _combine2([x[y][r:r + 8] for x in m])
                return write(blocks, y, r)

            slabs = [(y, r) for r in range(0, RO, 8) for y in range(2)]
            for x, slab in enumerate(slabs):
                schedule(P(recombine, *slab), begin, begin + (end - begin) * (x + 1) // len(slabs), False)
            for i in range(49):
                n, res = step([_words(lhs_t, (stride * (i // 7) + i % 7, x), 0, RO) for x in range(2)],
                              [P(lambda y, x: _load(rhs_t, (i, tile0 + y), x * T, T), y) for y in range(2)])
                m.append(res)
                finish(n, res)

        def write_rows(buf, blocks, y, r):
            for row in range(4):
                for col in range(4):
                    buf[2 * col + y, pl.ds(HALO + row * RO + r, 8), :] = blocks[row][col]
            return tok.of(*[x for row in blocks for x in row])

        project2(ax_t, 9, wakv_t, 0, P(write_rows, kbuf), t_q, t_v - 300)

        def write_q(m, half, y):
            vals = [val * SCALE_A for val in _combine([x[y] for x in m])]
            for quad, val in enumerate(vals):
                qbuf[4 * (quad % 2) + y, pl.ds((2 * (quad // 2) + half) * RO, RO), :] = val
            return tok.of(*[val[r:r + 8] for val in vals for r in range(0, RO, 8)])

        for half in range(2):
            m = []
            done = t_q + (t_v - t_q) * (half + 1) // 2
            for y in range(4):
                schedule(P(write_q, m, half, y), done, done + 200 + 100 * y, False)
            for i in range(7):
                a = [_words(ax_t, (9 * i + x, n), 0, RO) for x in ((2, 7), (8, 3))[half] for n in range(2)]
                n, res = step(a, [P(lambda y, x: _load(waq_t, (i, y), x * T, T), y) for y in range(4)])
                m.append(res)
                finish(n, res)

        att = {}

        def job_weights(row, r, release):
            base = HALO + row * RO + r
            qs = [_or_first(qbuf[t, pl.ds(row * RO + r, 8), :], release) for t in range(8)]
            logits = []
            for w in range(WIN):
                rows = pl.ds(base - DIL * w, 8)
                x = functools.reduce(jnp.add, [qs[t] * kbuf[t, rows, :] for t in range(8)])
                x = x + pltpu.roll(x, 64, 1)
                x = x + pltpu.roll(x, 32, 1)
                if row == 0 and r < DIL * w:
                    pos = lax.broadcasted_iota(jnp.int32, (8, T), 0) + (c * CO + r)
                    x = jnp.where(pos >= DIL * w, x, MASKED)
                logits.append(x)
            m = functools.reduce(jnp.maximum, logits)
            p = [jnp.exp2(x - m) for x in logits]
            l = functools.reduce(jnp.add, p)
            inv = pl.reciprocal(l, approx=True)
            inv = inv * (2.0 - l * inv)
            att[row, r] = [x * inv for x in p]
            return tok.of(*att[row, r])

        def job_values(row, r, release):
            base = HALO + row * RO + r
            p = [_or_first(x, release) for x in att[row, r]]
            att[row, r] = [
                functools.reduce(jnp.add, [p[w] * vbuf[t, pl.ds(base - DIL * w, 8), :]
                                           for w in range(WIN)])
                for t in range(8)]
            return tok.of(*att[row, r])

        def job_o(n, r, i):
            def block(row, col):
                return _cat([att[row, r][2 * col + n], att[row, r + 8][2 * col + n]], axis=0)
            for x, val in enumerate(_terms2(LHS, i, block)):
                o_t[7 * i + x, n, pl.ds(r, 16), :] = val.astype(BF16)
            return tok.stored(o_t, (7 * i + 6, n), r)

        groups = [(row, r + x) for r in range(0, RO, 16) for row in range(4) for x in (0, 8)]
        w0, w1 = t_v + W0, t_b + W1
        v0, v1 = t_b + V0, t_o - V1
        for g, (row, r) in enumerate(groups):
            begin = w0 + (w1 - w0) * g // len(groups)
            schedule(P(job_weights, row, r), begin, begin + WWIN)
            begin = max(v0 + (v1 - v0) * g // len(groups), begin + WWIN)
            schedule(P(job_values, row, r), begin, begin + VWIN)
            if g % 8 == 7:
                for x, (n, i) in enumerate((n, i) for n in range(2) for i in range(7)):
                    schedule(P(job_o, n, r - 8, i), begin, min(begin + VWIN + OSTEP * (x + 1), t_o), False)
        project2(ax_t, 9, wakv_t, 2, P(write_rows, vbuf), t_b, t_b + VCOMB)

        touched = set()

        def project_b(i):
            m = []

            def accumulate(y, inner):
                val = _combine([x[y] for x in m])[inner]
                token = None
                for outer, sign in OUT[i]:
                    row, col = 2 * (outer // 2) + inner // 2, 2 * (2 * (outer % 2) + inner % 2) + y
                    rows = pl.ds(row * RO, RO)
                    total = val
                    if (outer, inner, y) in touched:
                        total = acc[col, rows, :] + val if sign > 0 else acc[col, rows, :] - val
                    touched.add((outer, inner, y))
                    if any(outer == n for x in range(i + 1, 7) for n, _ in OUT[x]):
                        acc[col, rows, :] = total
                        token = tok.stored(acc, (col,), row * RO)
                    else:
                        obuf[slot, rows, pl.ds(DM + col * T, T)] = total.astype(BF16)
                        if token is None:
                            token = tok.of(*[total[r:r + 8] for r in range(0, RO, 8)])
                return token

            parts = [(y, inner) for y in range(2) for inner in range(4)]
            done = starts[clock[0] + 7]
            if i < 6:
                for x, part in enumerate(parts):
                    schedule(P(accumulate, *part), done, done + AWIN + ASTEP * x, False)
            for n in range(7):
                def quad(kt, x):
                    return (i, 2 * kt + x % 2), (2 * c + x // 2) * RO
                if len(LHS[n]) == 1:
                    a = [_words(ctx_t, *quad(kt, LHS[n][0][0]), RO) for kt in range(8)]
                else:
                    a = [_term(LHS, n, lambda x: _load(ctx_t, *quad(kt, x), RO).astype(F32))
                         for kt in range(8)]
                idx, res = step(a, [P(lambda y, x: _load(wob_t, (7 * i + n, y), x * T, T), y)
                                    for y in range(2)])
                m.append(res)
                finish(idx, res)
            if i == 6:
                for part in parts:
                    accumulate(*part)

        for i in range(6):
            project_b(i)

        def job_ax(i, n, r):
            store_ax(1 - slot, i, n, r)
            return tok.stored(ax_t, (9 * i + 8, n), r)

        for x, job in enumerate(ax_jobs):
            schedule(P(job_ax, *job), t_o, t_o + 100 + (XSPAN - 100) * (x + 1) // len(ax_jobs), False)

        halves = {}

        def write_out(blocks, y, r):
            if r % 16 == 0:
                halves[y] = blocks
            else:
                for row in range(4):
                    for col in range(4):
                        val = _cat([halves[y][row][col], blocks[row][col]], axis=0)
                        obuf[slot, pl.ds(row * RO + r - 8, 16), pl.ds((2 * col + y) * T, T)] = val.astype(BF16)
            return tok.of(*[x for row in blocks for x in row])

        project2(o_t, 7, wo_t, 0, write_out, t_last, starts[-2])
        project_b(6)
        assert not plan and not due, (plan, due)
        out_copy(c, slot).start()
        return carry

    def it(c, carry):
        if True:
            chunk_body(c, carry)
    lax.fori_loop(0, NO, it, None)
    ax_copy(NO - 1, (NO - 1) % 2).wait()
    out_copy(NO - 2, 0).wait()
    out_copy(NO - 1, 1).wait()


def _kernel(ax_hbm, wqkv_hbm, wo_hbm, bx_hbm, c_hbm, wq_hbm, wuk_hbm, wuv_hbm, wob_hbm,
            out_hbm, ctx_t, wob_t, waq_t, wakv_t, wo_t, zero_smem, idle_sem, ax_raw, sem_ax):

    @pl.when(pl.semaphore_read(idle_sem) == 0)
    def _():
        zero_smem[0] = 0

    vmem, dma = pltpu.VMEM, pltpu.SemaphoreType.DMA

    def prefetch_ax():
        for c in range(2):
            pltpu.make_async_copy(ax_hbm.at[pl.ds(c * CO, CO), :], ax_raw.at[c], sem_ax.at[c]).start()

    shared = (ctx_t, wob_t, waq_t, wakv_t, wo_t, zero_smem)
    if CFG.get('only') != '2': pl.run_scoped(
        P(_head_pairs, wqkv_hbm, wo_hbm, bx_hbm, c_hbm, wq_hbm, wuk_hbm, wuv_hbm, wob_hbm, prefetch_ax, *shared),
        vmem((S, DM), BF16),
        vmem((S, DC), BF16),
        vmem((2, DM, T), U32),
        vmem((2, DC, T), U32),
        vmem((2, DC, T), U32),
        vmem((2, 4, 64, DM), BF16),
        vmem((2, 4, 8, 3 * DM), U32),
        vmem((16, NH, DM), U32),
        vmem((7, 4, S // 2, T), BF16),
        vmem((49, S // 4, T), BF16),
        vmem((7, DM // 2, T), BF16),
        vmem((49, T, T), BF16),
        vmem((2, 8, T), F32),
        dma((2 * NC,)), dma((11,)))
    if CFG.get('only') in ('1', 'f'):
        def fin(buf, sem):
            z = zero_smem[0]
            val = ctx_t[z, z, pl.ds(0, 16), :]
            for ref in (wob_t, waq_t, wakv_t, wo_t):
                val = val + ref[z, z, pl.ds(z * 16, 16), :]
            buf[...] = val
            cp = pltpu.make_async_copy(buf, out_hbm.at[pl.ds(0, 16), pl.ds(0, T)], sem)
            cp.start(); cp.wait()
        pl.run_scoped(fin, vmem((16, T), BF16), dma(()))
        return
    pl.run_scoped(
        P(_outputs, ax_hbm, out_hbm, *shared, ax_raw, sem_ax),
        vmem((63, 2, RO, T), BF16),
        vmem((49, 2, RO, T), BF16),
        vmem((8, HALO + CO, T), F32),
        vmem((8, HALO + CO, T), F32),
        vmem((8, CO, T), F32),
        vmem((8, CO, T), F32),
        vmem((2, CO, 2 * DM), BF16),
        dma((2,)))


@jax.jit
def pallas_concat_heads__sliding_local_dilated__compressed_kv_cla__prompt_kernel(
    A_x: jax.Array,
    A_wqkv: jax.Array,
    A_wo: jax.Array,
    B_x: jax.Array,
    B_c_kv: jax.Array,
    B_w_q: jax.Array,
    B_w_uk: jax.Array,
    B_w_uv: jax.Array,
    B_w_o: jax.Array,
):
    vmem = pltpu.VMEM
    out = pl.pallas_call(
        _kernel,
        out_shape=jax.ShapeDtypeStruct((S, 2 * DM), BF16),
        in_specs=[pl.BlockSpec(memory_space=pl.ANY)] * 9,
        out_specs=pl.BlockSpec(memory_space=pl.ANY),
        scratch_shapes=[
            vmem((7, NP, S // 2, T), BF16),
            vmem((49, 2, DM, T), BF16),
            vmem((7, 4, DM // 2, T), BF16),
            vmem((49, 4, 2 * T, T), BF16),
            vmem((49, 2, 2 * T, T), BF16),
            pltpu.SMEM((1,), jnp.int32),
            pltpu.SemaphoreType.REGULAR,
            vmem((2, CO, DM), BF16),
            pltpu.SemaphoreType.DMA((2,)),
        ],
        compiler_params=pltpu.CompilerParams(vmem_limit_bytes=124 * 2**20, disable_bounds_checks=CFG.get('nb', '1') == '1',
            flags={'lp': {'XLA_TPU_FORCE_LP_LLO_SCHEDULER': True}, 'ev': {'XLA_TPU_EVENLY_DISTRIBUTE_CRITICAL_NODES': True}, 'rd': {'XLA_TPU_RESCHEDULE_DMA_DONES': True}, '': None}[CFG.get('fl', '')]),
    )(
        A_x.reshape(S, DM),
        A_wqkv.reshape(4, DM // 4, 3 * DM),
        A_wo.reshape(NH, DM // NH, DM),
        B_x.reshape(S, DM),
        B_c_kv.reshape(S, DC),
        B_w_q,
        B_w_uk,
        B_w_uv,
        B_w_o,
    )
    return out.reshape(1, S, 2 * DM)
```

```python
import functools
import math

import jax
import jax.numpy as jnp
from jax import lax
import jax.experimental.pallas as pl
import jax.experimental.pallas.tpu as pltpu

CFG = {'x': '1'}
PQ = int(CFG.get('pq', 12)); CTX_DELAY = int(CFG.get('cd', 12)); SK = int(CFG.get('sk', 3))
BORD = CFG.get('bord', 'k'); WD = int(CFG.get('wd', 1)); OSK = int(CFG.get('osk', 3)); WSK = int(CFG.get('wsk', 7)); ASK = int(CFG.get('ask', 2))
WQ = float(CFG.get('wq', 0)); WKV = float(CFG.get('wkv', 0.2)); WATT = float(CFG.get('watt', 1)); SIDE = float(CFG.get('side', 0.95)); NKV = int(CFG.get('nkv', 8)); TAILF = float(CFG.get('tailf', 0.9))
LT = CFG.get('lt', ''); LTP = int(CFG.get('ltp', 0)); CTP = int(CFG.get('ctp', -1))
FM = CFG.get('fm', 'prev')
G = int(CFG.get('g', 0)); GL = int(CFG.get('gl', 1))
RP = int(CFG.get('rp', 0))
g_ = lambda k, d: int(CFG.get(k, d))
W0, W1, V0, V1, WWIN, VWIN, OSTEP, VCOMB = g_('w0', 300), g_('w1', 3500), g_('v0', 2500), g_('v1', 700), g_('wwin', 700), g_('vwin', 300), g_('ostep', 60), g_('vcomb', 1500)
AWIN, ASTEP, XSPAN = g_('awin', 256), g_('astep', 150), g_('xspan', 4500)
NFS = g_('nfs', 40); FW = g_('fw', 9); WO1 = g_('wo1', 16)
REL = g_('rel', 1); RQ = g_('rq', 2); RKV = g_('rkv', 12); END = CFG.get('end', 'n'); L7 = g_('l7', 0)
SUBR = g_('sub', 128); FAST = g_('fast', 0)
LAG0 = g_('lag0', 99); LAG1 = g_('lag1', 5); E2 = g_('e2', 8); E3 = g_('e3', 10)
FQ = float(CFG.get('fq', 0.98))
GROUP = g_('grp', 1); DEPTH = g_('dep', 3); UD = g_('ud', 0); E1 = g_('e1', 0)
JW = g_('jw', 16)
WT = g_('wt', 1); VT = g_('vt', 8); VREL = g_('vrel', 1); GO = g_('go', 0); XS0 = g_('xs0', 0); KC = g_('kc', 300); QC = g_('qc', 50)
SH = g_('sh', 0); SR = g_('sr', 16)
WSPAN = int(CFG.get('wspan', 49)); VSPAN = int(CFG.get('vspan', 24))

S = 2048
DM = 1024
DC = 512
NH = 32
NP = NH // 2
T = 128
CH = 4 * T
NC = S // CH
RO = 64
CO = 4 * RO
NO = S // CO
ROWB = lambda inner, outer: 2 * outer + inner
WIN, DIL = 8, 2
HALO = 16

LOG2E = math.log2(math.e)
SCALE_A = (DM // NH) ** -0.5 * LOG2E
SCALE_B = T ** -0.5 * LOG2E
MASKED = -1e9 * LOG2E
SAFE_SUM = 2.0 ** 40

F32, BF16, U32 = jnp.float32, jnp.bfloat16, jnp.uint32
P = functools.partial


def _dot(a, b):
    return jnp.dot(a, b, preferred_element_type=F32)


def _dot_nt(a, b):
    return lax.dot_general(a, b, (((1,), (1,)), ((), ())), preferred_element_type=F32)


def _cat(xs, axis=1):
    return xs[0] if len(xs) == 1 else jnp.concatenate(xs, axis=axis)


def _aligned(x, n):
    return x if isinstance(x, int) else pl.multiple_of(x, n)


def _words(ref, lead, start, n):
    return ref.bitcast(U32)[(*lead, pl.ds(_aligned(start >> 1, 8), n // 2), slice(None))]


def _load(ref, lead, start, n):
    return pltpu.bitcast(_words(ref, lead, start, n), BF16)


def _split(w):
    return (pltpu.bitcast(w << 16, F32), pltpu.bitcast(w & jnp.uint32(0xFFFF0000), F32))


def _fold(op, x):
    return functools.reduce(op, [x[r:r + 8] for r in range(0, x.shape[0], 8)])


def _or_first(w, tok):
    bits = w if w.dtype == U32 else pltpu.bitcast(w, U32)
    bits = bits | tok if bits.shape[0] == 8 else _cat([bits[:8] | tok, bits[8:]], axis=0)
    return bits if w.dtype == U32 else pltpu.bitcast(bits, w.dtype)


LHS = (((0, 1), (3, 1)), ((2, 1), (3, 1)), ((0, 1),), ((3, 1),),
       ((0, 1), (1, 1)), ((2, 1), (0, -1)), ((1, 1), (3, -1)))
RHS = (((0, 1), (3, 1)), ((0, 1),), ((1, 1), (3, -1)), ((2, 1), (0, -1)),
       ((3, 1),), ((0, 1), (1, 1)), ((2, 1), (3, 1)))
OUT = (((0, 1), (3, 1)), ((2, 1), (3, -1)), ((1, 1), (3, 1)), ((0, 1), (2, 1)),
       ((0, -1), (1, 1)), ((3, 1),), ((0, 1),))


def _term(table, i, quad):
    (n, _), *rest = table[i]
    val = quad(n)
    for n, sign in rest:
        val = val + quad(n) if sign > 0 else val - quad(n)
    return val


def _terms(table, quad):
    blocks = [quad(n) for n in range(4)]
    return [_term(table, i, blocks.__getitem__) for i in range(7)]


def _terms2(table, i, block):
    return _terms(table, lambda n: _term(
        table, i, lambda m: block(2 * (m // 2) + n // 2, 2 * (m % 2) + n % 2)))


def _combine(m):
    out = [None] * 4
    for i in range(7):
        for n, sign in OUT[i]:
            if out[n] is None:
                out[n] = m[i]
            else:
                out[n] = out[n] + m[i] if sign > 0 else out[n] - m[i]
    return out


def _combine2(m):
    inner = [_combine(m[7 * i:7 * i + 7]) for i in range(7)]
    out = [[None] * 4 for _ in range(4)]
    for n in range(4):
        for quad, val in enumerate(_combine([x[n] for x in inner])):
            out[2 * (quad // 2) + n // 2][2 * (quad % 2) + n % 2] = val
    return out


class _Tokens:
    def __init__(self, zero_smem):
        self.z = zero_smem[0]
        self.zv = jnp.full((8, T), self.z, jnp.int32).astype(U32)

    def stored(self, ref, lead, start):
        first, *rest = lead
        if FM == 'lead':
            if ref.dtype == BF16:
                return _words(ref, (first + self.z, *rest), start, 16) & self.zv
            return self.of(ref[(first + self.z, *rest, pl.ds(start, 8), slice(None))])
        bit = self.z & 1
        if FM == 'prev':
            if ref.dtype == BF16:
                return _words(ref, (first - bit, *rest), start, 16) & self.zv
            return self.of(ref[(first, *rest, pl.ds(_aligned(start + 8 * bit, 8), 8), slice(None))])

    def of(self, *vals):
        tok = vals[0]
        for x in vals[1:]:
            tok = tok + x
        return pltpu.bitcast(tok, U32) & self.zv


AX_JOBS = [(i, n, r) for n in range(2) for r in range(0, RO, 16) for i in range(7)]


def _job_ax(tok, released, ax_raw, ax_t, src, i, n, r):
    def block(row, col):
        return released(ax_raw[src, pl.ds(row * RO + r, 16), pl.ds((2 * col + n) * T, T)].astype(F32))
    outer = [_term(LHS, i, lambda m: block(2 * (m // 2) + x // 2, 2 * (m % 2) + x % 2))
             for x in range(4)]
    for x, val in enumerate(_terms(LHS, outer.__getitem__) + outer[1:3]):
        ax_t[9 * i + x, n, pl.ds(r, 16), :] = val.astype(BF16)
    return tok.stored(ax_t, (9 * i + 8, n), r)


def _head_pairs(wqkv_hbm, wo_hbm, bx_hbm, c_hbm, wq_hbm, wuk_hbm, wuv_hbm, wob_hbm, ax_copy, ax_raw, ax_t,
                ctx_t, wob_t, waq_t, wakv_t, wo_t, zero_smem,
                bx_raw, c_raw, wq_raw, wk_raw, wv_raw, wob_raw, wqkv_raw, wo_raw,
                bx_t, c_t, wq_t, wkv_t, guard, sem_in, sem_w):
    guard[...] = jnp.zeros(guard.shape, F32)

    def head_copy(n, j, slot):
        src, dst = ((wuk_hbm, wk_raw), (wuv_hbm, wv_raw), (wq_hbm, wq_raw))[n]
        return pltpu.make_async_copy(src.bitcast(U32).at[:, j, :], dst.at[slot], sem_w.at[3 * slot + n])

    def side_copy(n, j, slot):
        if n == 0:
            src = wob_hbm.at[pl.ds(4 * (j >> 1), 4), pl.ds(_aligned((j & 1) * 64, 64), 64), :]
            dst = wob_raw.at[slot]
        else:
            src = wqkv_hbm.bitcast(U32).at[:, pl.ds(_aligned(8 * j, 8), 8), :]
            dst = wqkv_raw.at[slot]
        return pltpu.make_async_copy(src, dst, sem_w.at[6 + 2 * slot + n])

    def wo_copy(word):
        return pltpu.make_async_copy(wo_hbm.bitcast(U32).at[:, word, :], wo_raw.at[word], sem_w.at[10])

    def act_copy(n, c):
        src, dst = ((c_hbm, c_raw), (bx_hbm, bx_raw))[n]
        rows = pl.ds(c * CH, CH)
        return pltpu.make_async_copy(src.at[rows, :], dst.at[rows, :], sem_in.at[2 * c + n])

    def exact_pairs(qkv, ctx):
        def block(i):
            return pl.ds(pl.multiple_of(i * T, T), T)

        def head(h, carry):
            def weight(raw):
                even, odd = _split(raw[0])
                return jnp.where(h == 0, even, odd).astype(BF16)
            wk, wv, wq = weight(wk_raw), weight(wv_raw), weight(wq_raw)

            def project(i, carry):
                qkv[0, block(i), :] = (_dot(bx_raw[block(i), :], wq) * SCALE_B).astype(BF16)
                qkv[1, block(i), :] = _dot(c_raw[block(i), :], wk).astype(BF16)
                qkv[2, block(i), :] = _dot(c_raw[block(i), :], wv).astype(BF16)
            lax.fori_loop(0, S // T, project, None)

            def attend(i, carry):
                def scores(t):
                    row = lax.broadcasted_iota(jnp.int32, (T, T), 0) + i * T
                    col = lax.broadcasted_iota(jnp.int32, (T, T), 1) + t * T
                    return jnp.where(col <= row, _dot_nt(qkv[0, block(i), :], qkv[1, block(t), :]), MASKED)

                m = lax.fori_loop(
                    0, i + 1, lambda t, m: jnp.maximum(m, jnp.max(scores(t), axis=1, keepdims=True)),
                    jnp.full((T, 1), -jnp.inf, F32))

                def accumulate(t, carry):
                    l, o = carry
                    p = jnp.exp2(scores(t) - m)
                    return (l + jnp.sum(p, axis=1, keepdims=True),
                            o + _dot(p.astype(BF16), qkv[2, block(t), :]))
                l, o = lax.fori_loop(0, i + 1, accumulate,
                                     (jnp.zeros((T, 1), F32), jnp.zeros((T, T), F32)))
                ctx[h, block(i), :] = o / l
            lax.fori_loop(0, S // T, attend, None)

        def pair(j, carry):
            for n in range(3):
                head_copy(n, j, 0).start()
            for n in range(3):
                head_copy(n, j, 0).wait()
            lax.fori_loop(0, 2, head, None)

            def store(b, carry):
                for n, val in enumerate(_terms(LHS, lambda m: ctx[m % 2, block(2 * b + m // 2), :])):
                    ctx_t[n, j, block(b), :] = val.astype(BF16)
            lax.fori_loop(0, S // T // 2, store, None)

        lax.fori_loop(0, NP, pair, None)

    def pair_body(j, first=False):
        slot = j & 1
        if not first:
            for n in range(3):
                head_copy(n, j, 1 - slot).wait()
            for n in range(2):
                side_copy(n, j, slot).wait()
            for n in range(3):
                head_copy(n, jnp.minimum(j + 2, NP - 1), slot).start()
            for n in range(2):
                side_copy(n, jnp.minimum(j + 1, NP - 1), 1 - slot).start()
        tok = _Tokens(zero_smem)
        causal = (lax.broadcasted_iota(jnp.int32, (T, T), 1)
                  <= lax.broadcasted_iota(jnp.int32, (T, T), 0))
        jobs, pace = [], dict(period=0, clock=0)

        def background(cycles, recent):
            pace["clock"] += cycles
            token = None
            while jobs and pace["clock"] >= pace["period"]:
                pace["clock"] -= pace["period"]
                pace["release"] = None if recent is None or not REL else tok.of(recent[:8])
                new = jobs.pop(0)()
                pace["release"] = None
                token = new if token is None else token | new
            return token

        def released(x):
            if pace.get("release") is None:
                return x
            bits = x if x.dtype == U32 else pltpu.bitcast(x, U32)
            bits = _cat([bits[r:r + 8] | pace["release"] for r in range(0, bits.shape[0], 8)], axis=0)
            return bits if x.dtype == U32 else pltpu.bitcast(bits, x.dtype)

        same = 0

        def lhs(ref, lead, start, n, cycles, recent):
            w = _words(ref, lead, start, n)
            parts = []
            for r in range(0, n // 2, 8):
                token = background(cycles, None)
                parts.append(w[r:r + 8] if token is None else w[r:r + 8] | token)
            return pltpu.bitcast(_cat(parts, axis=0), BF16)

        def store_terms(dst, first_term, lead, row, terms):
            for i, val in enumerate(terms):
                dst[(first_term + i, *lead, pl.ds(_aligned(row, 16), 16), slice(None))] = val.astype(BF16)
            return tok.stored(dst, (first_term + 6, *lead), row)

        def job_wkv(src, i, r):
            def block(row, col):
                raw = (wk_raw, wv_raw)[col % 2]
                return _split(released(raw[src, pl.ds(_aligned(row * T + r, 16), 16), :]))[col // 2]
            return store_terms(wkv_t, 7 * i, (), r, _terms2(RHS, i, block))

        def job_wq(src, r):
            top, bot = _split(released(wq_raw[src, pl.ds(_aligned(r, 16), 16), :])), _split(released(wq_raw[src, pl.ds(_aligned(DM // 2 + r, 16), 16), :]))
            return store_terms(wq_t, 0, (), r, _terms(RHS, (top + bot).__getitem__))

        def jobs_wkv(src):
            return [P(job_wkv, src, i, r) for r in range(0, T, 16) for i in range(7)]

        def jobs_wq(src):
            return [P(job_wq, src, r) for r in range(0, DM // 2, 16)]

        def job_wob(i, n, r):
            def block(row, col):
                head = 2 * (row % 2) + row // 2
                return released(wob_raw[slot, head, pl.ds(r, 16), pl.ds((2 * col + n) * T, T)].astype(F32))
            return store_terms(wob_t, 7 * i, (n,), j * 64 + r, _terms2(RHS, i, block))

        def job_wo(i, n):
            odd = (j >> 2) & 1

            def block(row, col):
                even_t, odd_t = _split(released(wo_raw[4 * (j & 3) + row, pl.ds(_aligned(16 * (j >> 3), 16), 16),
                                              pl.ds((2 * col + n) * T, T)]))
                return jnp.where(odd == 1, odd_t, even_t)
            return store_terms(wo_t, 7 * i, (n,), odd * T + (j & 3) * NH + (j >> 3) * 16,
                               _terms2(RHS, i, block))

        permuted = {}

        def job_permute(mat):
            lane = lax.broadcasted_iota(jnp.int32, (32, T), 1)
            e, grp, sub = lane >> 5, (lane >> 2) & 7, lane & 3
            x = [released(wqkv_raw[slot, :, :, pl.ds(mat * DM + t * T, T)].reshape(32, T)) for t in range(8)]
            y = [jnp.take_along_axis(x[t], sub * 32 + e * 8 + ((grp - t) & 7), axis=1, mode='promise_in_bounds')
                 for t in range(8)]
            u = [y[-s % 8] for s in range(8)]
            for bit in (1, 2, 4):
                u = [jnp.where((grp & bit) != 0, u[(s - bit) % 8], u[s]) for s in range(8)]
            u = [u[0]] + [jnp.take_along_axis(u[t], e * 32 + ((grp + t) & 7) * 4 + sub, axis=1, mode='promise_in_bounds')
                          for t in range(1, 8)]
            permuted[mat] = u
            return _fold(jnp.bitwise_or, functools.reduce(jnp.bitwise_or, u)) & tok.zv

        def column(mat, row, t):
            return pltpu.bitcast(released(permuted[mat][t][8 * row:8 * row + 8]), BF16).astype(F32)

        def job_waq(half, n):
            terms = _terms(RHS, lambda m: column(0, 2 * (m // 2) + half, 4 * (m % 2) + n))
            return store_terms(waq_t, 0, (n,), half * 2 * T + 16 * j, terms)

        def job_wakv(mat, i, n):
            terms = _terms2(RHS, i, lambda row, col: column(mat, row, 2 * col + n))
            return store_terms(wakv_t, 7 * i, (2 * (mat - 1) + n,), 16 * j, terms)

        jobs_wob = [P(job_wob, i, n, r) for r in range(0, 64, 16) for n in range(2) for i in range(7)]
        jobs_wo = [P(job_wo, i, n) for n in range(2) for i in range(7)]
        idle = [lambda: tok.zv] * g_('pidle', 2)
        jobs_wa = [P(job_permute, 0)] + idle
        jobs_wa += [P(job_waq, half, n) for half in range(2) for n in range(4)]
        for mat in (1, 2):
            jobs_wa += [P(job_permute, mat)] + idle
            jobs_wa += [P(job_wakv, mat, i, n) for n in range(2) for i in range(7)]

        q, k, v, latest = {}, {}, {}, [None]

        def job_x(c, t, r):
            terms = _terms(LHS, lambda m: bx_raw[pl.ds(_aligned(c * CH + (m // 2) * 2 * T + r, 16), 16),
                                                 pl.ds((4 * (m % 2) + t) * T, T)].astype(F32))
            return store_terms(bx_t, 0, (t,), c * 2 * T + r, terms)

        def job_c(c, i, r):
            terms = _terms2(LHS, i, lambda row, col: c_raw[
                pl.ds(_aligned(c * CH + row * T + r, 16), 16), pl.ds(col * T, T)].astype(F32))
            return store_terms(c_t, 7 * i, (), c * T + r, terms)

        def jobs_x(c):
            return [P(job_x, c, t, r) for r in range(0, 2 * T, 16) for t in range(4)]

        def jobs_c(c):
            return [P(job_c, c, i, r) for r in range(0, T, 16) for i in range(7)]

        def proj_q(c):
            m = []
            for i in range(7):
                recent = m[i - RQ] if i >= RQ else latest[0]
                m.append(_dot(_cat([lhs(bx_t, (i, t), c * 2 * T, 2 * T, 4 * WQ, recent) for t in range(4)]),
                              _load(wq_t, (i,), same, DM // 2)))
            latest[0] = m[-2]
            for n, val in enumerate(_combine(m)):
                val = val * SCALE_B
                for r in range(2):
                    q[4 * c + 2 * (n // 2) + r, n % 2] = val[r * T:(r + 1) * T].astype(BF16)

        def proj_kv(c):
            m = []
            for i in range(49):
                recent = m[i - RKV] if i >= RKV else latest[0]
                m.append(_dot(lhs(c_t, (i,), c * T, T, 4 * WKV, recent), _load(wkv_t, (i,), same, T)))
            latest[0] = m[-RKV]
            for r, row in enumerate(_combine2(m)):
                for n, val in enumerate(row):
                    (k, v)[n % 2][4 * c + r, n // 2] = val.astype(BF16)

        scores, ctx, stored, spread, checks = {}, {}, [], {}, []

        partial, ready = {}, []

        def finish_unit(i, h):
            l, o = partial.pop((i, h))
            l = jnp.sum(l, axis=1, keepdims=True)
            r = pl.reciprocal(l, approx=True)
            ctx[i, h] = o * (r * (2.0 - l * r))
            spread[i, h] = _fold(jnp.maximum, jnp.broadcast_to(l + r, (T, T)))
            b = i // 2
            quad = [(2 * b, 0), (2 * b, 1), (2 * b + 1, 0), (2 * b + 1, 1)]
            if all(u in ctx for u in quad):
                terms = _terms(LHS, lambda m: ctx.pop(quad[m]))
                for n, val in enumerate(terms):
                    ctx_t[n, j, pl.ds(b * T, T), :] = val.astype(BF16)
                checks.append((_fold(jnp.add, terms[0] + terms[5] + terms[6]),
                               functools.reduce(jnp.maximum, [spread.pop(u) for u in quad])))
                stored.append([CTX_DELAY, tok.stored(ctx_t, (6, j), b * T) | tok.of(*checks[-1])])
            elif UD:
                stored.append([UD, tok.of(_fold(jnp.add, ctx[i, h]))])

        def weigh(group):
            for x, (i, h, t, p) in enumerate(group):
                l, o = partial.get((i, h), (None, None))
                l = p if l is None else l + p
                if G and x % G == G - 1 and t > 0:
                    p = jnp.where(l < 0, l, p)
                token = background(64 * WATT, p if REL else None)
                if REL and token is not None:
                    stored.append([JW, token])
                    token = None
                if x == 0:
                    for entry in stored:
                        entry[0] -= 1
                    for entry in [e for e in stored if e[0] <= 0]:
                        stored[:] = [e for e in stored if e is not entry]
                        token = entry[1] if token is None else token | entry[1]
                if token is not None:
                    p = _or_first(p, token)
                d = _dot(p.astype(BF16), v[t, h])
                partial[i, h] = (l, d if o is None else o + d)
                if t == i:
                    finish_unit(i, h)

        def attention(blocks, drain=False):
            items = leftover + [(i, h, t) for i in blocks for h in range(2) for t in range(i + 1)]
            leftover.clear()
            while len(items) >= (1 if drain else GROUP):
                group, items = items[:GROUP], items[GROUP:]
                tiles = []
                for i, h, t in group:
                    s = _dot_nt(q[i, h], k[t, h])
                    if t == i:
                        s = jnp.where(causal, s, MASKED)
                    tiles.append((i, h, t, jnp.exp2(s)))
                ready.append(tiles)
                if len(ready) > DEPTH:
                    weigh(ready.pop(0))
            leftover.extend(items)
            while drain and ready:
                weigh(ready.pop(0))

        leftover = []

        def flush():
            while jobs:
                jobs.pop(0)()

        def queue(cycles, more):
            pace["period"], pace["clock"] = cycles / max(len(more), 1), 0
            jobs.extend(more)

        def interleave(x, y):
            order = [((n + 0.5) / len(x), 0, job) for n, job in enumerate(x)]
            order += [((n + 0.5) / max(len(y), 1), 1, job) for n, job in enumerate(y)]
            return [job for _, _, job in sorted(order, key=lambda e: e[:2])]

        def loop(rows, body):
            def step(x, carry):
                body(16 * x)
            lax.fori_loop(0, rows // 16, step, None)

        def start(*copies):
            for cp in copies:
                cp.start()

        def wait(*copies):
            for cp in copies:
                cp.wait()

        late_q = END == 'c' and not first
        side = interleave(jobs_wob, jobs_wo + jobs_wa)
        q_time, kv_time, tile_time = 1792 * WQ, 1568 * WKV, 64 * WATT
        if first:
            def plain(raw, c, weights):
                def operand():
                    rows = []
                    for r in range(c * CH, (c + 1) * CH, 32):
                        part = raw[pl.ds(r, 32), :]
                        token = background(8 * (raw.shape[1] // T), None)
                        if token is not None:
                            part = _cat([_or_first(part[:, :2 * T], _cat([token, token])), part[:, 2 * T:]])
                        rows.append(part)
                    return _cat(rows, axis=0)
                return [_dot(operand(), w) for w in weights]

            def plain_kv(c):
                for n, val in enumerate(plain(c_raw, c, wkv)):
                    for r in range(4):
                        (k, v)[n // 2][4 * c + r, n % 2] = val[r * T:(r + 1) * T].astype(BF16)

            def plain_q(c):
                for h, val in enumerate(plain(bx_raw, c, wq)):
                    for r in range(4):
                        q[4 * c + r, h] = (val[r * T:(r + 1) * T] * SCALE_B).astype(BF16)

            stage = [head_copy(1, 0, 0), head_copy(0, 0, 0), act_copy(0, 0)]
            start(*stage, act_copy(0, 1))
            wait(*stage)
            start(act_copy(0, 2), act_copy(0, 3), act_copy(1, 0), head_copy(2, 0, 0))
            wkv = [w.astype(BF16) for raw in (wk_raw, wv_raw) for w in _split(raw[0])]
            queue(FQ * 2048, jobs_c(0))
            plain_kv(0)
            flush()
            wait(act_copy(0, 1), act_copy(0, 2))
            start(act_copy(1, 1), act_copy(1, 2))
            queue(FQ * 4096, jobs_c(1) + jobs_c(2))
            plain_kv(1)
            plain_kv(2)
            flush()
            wait(act_copy(0, 3))
            queue(FQ * 2048, jobs_c(3))
            plain_kv(3)
            flush()
            wait(act_copy(1, 0), head_copy(2, 0, 0))
            wq = [w.astype(BF16) for w in _split(wq_raw[0])]
            queue(FQ * (2048 + 1280), jobs_wq(0) + jobs_x(0))
            plain_q(0)
            attention(range(4))
            flush()
            wait(act_copy(1, 1), act_copy(1, 2))
            stage = [act_copy(1, 3), side_copy(0, 0, 0), side_copy(1, 0, 0)]
            stage += [head_copy(n, 1, 1) for n in range(3)]
            start(*stage)
            lax.fori_loop(0, WO1, lambda word, carry: wo_copy(word).start(), None)
            queue(FQ * (2048 + 2 * sum(range(5, 9)) * tile_time), jobs_x(2) + jobs_x(1))
            plain_q(1)
            attention(range(4, 8))
            flush()
            proj_q(2)
            attention(range(8, FW))
            wait(*stage)
            start(ax_copy(0, 0), *[wo_copy(word) for word in range(WO1, 16)])
            start(*[head_copy(n, 2, 0) for n in range(3)], *[side_copy(n, 1, 1) for n in range(2)])
            queue(FQ * 2 * sum(range(FW + 1, 15)) * tile_time,
                  jobs_x(3) + interleave(interleave(jobs_wob, jobs_wa), jobs_wkv(1)))
            attention(range(FW, 12))
            proj_q(3)
            attention(range(12, 14))
            flush()
            wait(*[wo_copy(word) for word in range(16)], ax_copy(0, 0))
            start(ax_copy(1, 1))
            queue(0.85 * 2 * (15 + 16) * tile_time,
                  interleave(jobs_wo + jobs_wq(1), [P(_job_ax, tok, released, ax_raw, ax_t, 0, *job) for job in AX_JOBS]))
            attention(range(14, 16), drain=True)
            flush()
        else:
            first_block = 0 if END == 'n' else 2
            queue(SIDE * (3 * q_time + 4 * kv_time + 2 * sum(range(first_block + 1, 13)) * tile_time), side)
            proj_kv(0)
            proj_q(0)
            if E1 == 0:
                proj_kv(1)
            attention(range(first_block, max(E1, first_block)))
            if E1:
                proj_kv(1)
            attention(range(max(E1, first_block), 4))
            proj_q(1)
            attention(range(4, E2))
            proj_kv(2)
            attention(range(E2, 8))
            proj_q(2)
            attention(range(8, E3))
            proj_kv(3)
            attention(range(E3, 12))
            flush()
            more = jobs_wkv(1 - slot)
            queue(q_time * 0.95, more[:NKV])
            proj_q(3)
            flush()
            queue(TAILF * tile_time * 2 * sum(range(13, 17)), interleave(more[NKV:], jobs_wq(1 - slot)))
            attention(list(range(12, 16)) + list(range(first_block)), drain=True)
            flush()
        guard[0] = functools.reduce(jnp.add, [x for x, _ in checks], guard[0])
        guard[1] = functools.reduce(jnp.maximum, [x for _, x in checks], guard[1])

    if CFG.get('only') != '1':
        if True:
            pair_body(0, first=True)
    def it(j, carry):
        if True:
            pair_body(j)
    if CFG.get('only') != 'f': lax.fori_loop(1, NP, it, None)
    for n in range(3):
        head_copy(n, NP - 1, (NP - 1) % 2).wait()
    for n in range(2):
        side_copy(n, NP - 1, NP % 2).wait()

    safe = jnp.logical_and(jnp.abs(guard[0]) < jnp.inf, guard[1] < SAFE_SUM)

    @pl.when(jnp.max(jnp.where(safe, 0.0, 1.0)) > 0.0)
    def _():
        pl.run_scoped(exact_pairs, pltpu.VMEM((3, S, T), BF16), pltpu.VMEM((2, S, T), F32))


def _outputs(ax_copy, out_hbm, ctx_t, wob_t, waq_t, wakv_t, wo_t, zero_smem,
             ax_raw, ax_t, o_t, kbuf, vbuf, qbuf, acc, sums, obuf, sem_out):

    def out_copy(c, slot):
        rows = pl.ds(_aligned(c * CO, CO), CO)
        return pltpu.make_async_copy(obuf.at[slot], out_hbm.at[rows, :], sem_out.at[slot])

    for buf in (kbuf, vbuf):
        for t in range(8):
            buf[t, pl.ds(CO, HALO), :] = jnp.zeros((HALO, T), F32)

    small, medium, large = RO, 4 * RO, 4 * RO
    costs = [small] * 49 + [medium] * 14 + [small] * 49 + [large] * 42 + [small] * 49 + [large] * 7
    starts = [sum(costs[:n]) for n in range(len(costs) + 1)]
    t_q, t_v, t_b, t_o, t_last = (starts[n] for n in (49, 63, 112, 154, 203))

    def chunk_body(c, carry):
        slot = c & 1

        @pl.when(c >= 2)
        def _():
            out_copy(c - 2, slot).wait()

        ax_copy(jnp.minimum(c + 1, NO - 1), 1 - slot).wait()
        ax_copy(jnp.minimum(c + 2, NO - 1), slot).start()
        tok = _Tokens(zero_smem)

        plan, due, clock = {}, {}, [0]

        def schedule(job, begin, end, release=True):
            first = max([clock[0]] + [n for n in range(len(costs)) if starts[n + 1] <= begin])
            last = min(n for n in range(len(costs)) if starts[n] >= end)
            plan.setdefault(first, []).append((job, last, release))

        def step(a, w):
            n = clock[0]
            clock[0] += 1
            for x, token in enumerate(due.pop(n, [])):
                a[x % len(a)] = _or_first(a[x % len(a)], token)
            a = [x.astype(BF16) if x.dtype == F32 else pltpu.bitcast(x, BF16) for x in a]
            res = [None] * len(w)
            for x in range(len(a)):
                for y in range(len(w)):
                    d = _dot(a[x], w[y](x))
                    res[y] = d if res[y] is None else res[y] + d
            return n, res

        def finish(n, res):
            token = None
            for job, last, release in plan.pop(n, []):
                if release and token is None:
                    token = tok.of(res[0][:8])
                due.setdefault(last, []).append(job(token) if release else job())
            return res

        for buf in (kbuf, vbuf):
            for t in range(8):
                buf[t, pl.ds(0, HALO), :] = buf[t, pl.ds(CO, HALO), :]

        def project2(lhs_t, stride, rhs_t, tile0, write, begin, end):
            m = []

            def recombine(y, r):
                blocks = _combine2([x[y][r:r + 8] for x in m])
                return write(blocks, y, r)

            slabs = [(y, r) for r in range(0, RO, 8) for y in range(2)]
            for x, slab in enumerate(slabs):
                schedule(P(recombine, *slab), begin, begin + (end - begin) * (x + 1) // len(slabs), False)
            for i in range(49):
                n, res = step([_words(lhs_t, (stride * (i // 7) + i % 7, x), 0, RO) for x in range(2)],
                              [P(lambda y, x: _load(rhs_t, (i, tile0 + y), x * T, T), y) for y in range(2)])
                m.append(res)
                finish(n, res)

        def write_rows(buf, blocks, y, r):
            for row in range(4):
                for col in range(4):
                    buf[2 * col + y, pl.ds(HALO + row * RO + r, 8), :] = blocks[row][col]
            return tok.of(*[x for row in blocks for x in row])

        project2(ax_t, 9, wakv_t, 0, P(write_rows, kbuf), t_q, t_v - KC)

        def write_q(m, half, y):
            vals = [val * SCALE_A for val in _combine([x[y] for x in m])]
            for quad, val in enumerate(vals):
                qbuf[4 * (quad % 2) + y, pl.ds((2 * (quad // 2) + half) * RO, RO), :] = val
            return tok.of(*[val[r:r + 8] for val in vals for r in range(0, RO, 8)])

        for half in range(2):
            m = []
            done = t_q + (t_v - t_q) * (half + 1) // 2
            for y in range(4):
                schedule(P(write_q, m, half, y), done, done + 200 + QC * y, False)
            for i in range(7):
                a = [_words(ax_t, (9 * i + x, n), 0, RO) for x in ((2, 7), (8, 3))[half] for n in range(2)]
                n, res = step(a, [P(lambda y, x: _load(waq_t, (i, y), x * T, T), y) for y in range(4)])
                m.append(res)
                finish(n, res)

        att = {}

        def job_weights(row, r, release):
            base = HALO + row * RO + r
            qs = [_or_first(qbuf[t, pl.ds(row * RO + r, 8), :], release) for t in range(8)]
            logits = []
            for w in range(WIN):
                rows = pl.ds(base - DIL * w, 8)
                x = functools.reduce(jnp.add, [qs[t] * kbuf[t, rows, :] for t in range(8)])
                x = x + pltpu.roll(x, 64, 1)
                x = x + pltpu.roll(x, 32, 1)
                if row == 0 and r < DIL * w:
                    pos = lax.broadcasted_iota(jnp.int32, (8, T), 0) + (c * CO + r)
                    x = jnp.where(pos >= DIL * w, x, MASKED)
                logits.append(x)
            m = functools.reduce(jnp.maximum, logits)
            p = [jnp.exp2(x - m) for x in logits]
            l = functools.reduce(jnp.add, p)
            inv = pl.reciprocal(l, approx=True)
            inv = inv * (2.0 - l * inv)
            att[row, r] = [x * inv for x in p]
            return tok.of(*att[row, r][:WT])

        def job_values(row, r, release):
            base = HALO + row * RO + r
            p = [_or_first(x, release) if VREL else x for x in att[row, r]]
            att[row, r] = [
                functools.reduce(jnp.add, [p[w] * vbuf[t, pl.ds(base - DIL * w, 8), :]
                                           for w in range(WIN)])
                for t in range(8)]
            return tok.of(*att[row, r][-VT:])

        def job_o(n, r, i):
            def block(row, col):
                return _cat([att[row, r][2 * col + n], att[row, r + 8][2 * col + n]], axis=0)
            for x, val in enumerate(_terms2(LHS, i, block)):
                o_t[7 * i + x, n, pl.ds(r, 16), :] = val.astype(BF16)
            return tok.stored(o_t, (7 * i + 6, n), r)

        groups = [(row, r + x) for r in range(0, RO, 16) for row in ((0, 1, 2, 3), (0, 2, 1, 3))[GO] for x in (0, 8)]
        w0, w1 = t_v + W0, t_b + W1
        v0, v1 = t_b + V0, t_o - V1
        for g, (row, r) in enumerate(groups):
            begin = w0 + (w1 - w0) * g // len(groups)
            schedule(P(job_weights, row, r), begin, begin + WWIN)
            begin = max(v0 + (v1 - v0) * g // len(groups), begin + WWIN)
            schedule(P(job_values, row, r), begin, begin + VWIN)
            if g % 8 == 7:
                for x, (n, i) in enumerate((n, i) for n in range(2) for i in range(7)):
                    schedule(P(job_o, n, r - 8, i), begin, min(begin + VWIN + OSTEP * (x + 1), t_o), False)

        def job_sums(i, kt, r):
            terms = _terms(LHS, lambda x: _load(
                ctx_t, (i, 2 * kt + x % 2), (2 * c + x // 2) * RO + r, SR).astype(F32))
            for n, val in enumerate(terms):
                if len(LHS[n]) > 1:
                    sums[7 * (i % 2) + n, kt, pl.ds(r, SR), :] = val.astype(BF16)
            return tok.stored(sums, (7 * (i % 2) + 6, kt), r + SR - 16)

        def queue_sums(i, begin, end):
            work = [(kt, r) for kt in range(8) for r in range(0, RO, SR)]
            for x, part in enumerate(work):
                schedule(P(job_sums, i, *part), begin, begin + (end - begin) * (x + 1) // len(work), False)

        if SH:
            queue_sums(0, t_v, t_b)
        project2(ax_t, 9, wakv_t, 2, P(write_rows, vbuf), t_b, t_b + VCOMB)

        touched = set()

        def project_b(i):
            m = []

            def accumulate(y, inner):
                val = _combine([x[y] for x in m])[inner]
                token = None
                for outer, sign in OUT[i]:
                    row, col = 2 * (outer // 2) + inner // 2, 2 * (2 * (outer % 2) + inner % 2) + y
                    rows = pl.ds(row * RO, RO)
                    total = val
                    if (outer, inner, y) in touched:
                        total = acc[col, rows, :] + val if sign > 0 else acc[col, rows, :] - val
                    touched.add((outer, inner, y))
                    if any(outer == n for x in range(i + 1, 7) for n, _ in OUT[x]):
                        acc[col, rows, :] = total
                        token = tok.stored(acc, (col,), row * RO)
                    else:
                        obuf[slot, rows, pl.ds(DM + col * T, T)] = total.astype(BF16)
                        if token is None:
                            token = tok.of(*[total[r:r + 8] for r in range(0, RO, 8)])
                return token

            parts = [(y, inner) for y in range(2) for inner in range(4)]
            done = starts[clock[0] + 7]
            if i < 6:
                for x, part in enumerate(parts):
                    schedule(P(accumulate, *part), done, done + AWIN + ASTEP * x, False)
            if SH and i < 6:
                queue_sums(i + 1, starts[clock[0]], t_last if i == 5 else done)
            for n in range(7):
                def quad(kt, x):
                    return (i, 2 * kt + x % 2), (2 * c + x // 2) * RO
                if len(LHS[n]) == 1:
                    a = [_words(ctx_t, *quad(kt, LHS[n][0][0]), RO) for kt in range(8)]
                elif SH:
                    a = [_words(sums, (7 * (i % 2) + n, kt), 0, RO) for kt in range(8)]
                else:
                    a = [_term(LHS, n, lambda x: _load(ctx_t, *quad(kt, x), RO).astype(F32))
                         for kt in range(8)]
                idx, res = step(a, [P(lambda y, x: _load(wob_t, (7 * i + n, y), x * T, T), y)
                                    for y in range(2)])
                m.append(res)
                finish(idx, res)
            if i == 6:
                for part in parts:
                    accumulate(*part)

        for i in range(6):
            project_b(i)

        for x, job in enumerate(AX_JOBS):
            schedule(P(_job_ax, tok, lambda val: val, ax_raw, ax_t, 1 - slot, *job),
                     t_o, t_o + 100 + XS0 + (XSPAN - 100 - XS0) * (x + 1) // len(AX_JOBS), False)

        halves = {}

        def write_out(blocks, y, r):
            if r % 16 == 0:
                halves[y] = blocks
            else:
                for row in range(4):
                    for col in range(4):
                        val = _cat([halves[y][row][col], blocks[row][col]], axis=0)
                        obuf[slot, pl.ds(row * RO + r - 8, 16), pl.ds((2 * col + y) * T, T)] = val.astype(BF16)
            return tok.of(*[x for row in blocks for x in row])

        project2(o_t, 7, wo_t, 0, write_out, t_last, starts[-2])
        project_b(6)
        assert not plan and not due, (plan, due)
        out_copy(c, slot).start()
        return carry

    def it(c, carry):
        if True:
            chunk_body(c, carry)
    lax.fori_loop(0, NO, it, None)
    ax_copy(NO - 1, (NO - 1) % 2).wait()
    out_copy(NO - 2, 0).wait()
    out_copy(NO - 1, 1).wait()


def _kernel(ax_hbm, wqkv_hbm, wo_hbm, bx_hbm, c_hbm, wq_hbm, wuk_hbm, wuv_hbm, wob_hbm,
            out_hbm, ctx_t, wob_t, waq_t, wakv_t, wo_t, zero_smem, idle_sem, ax_raw, ax_t, sem_ax):

    @pl.when(pl.semaphore_read(idle_sem) == 0)
    def _():
        zero_smem[0] = 0

    vmem, dma = pltpu.VMEM, pltpu.SemaphoreType.DMA

    def ax_copy(c, slot):
        rows = pl.ds(_aligned(c * CO, CO), CO)
        return pltpu.make_async_copy(ax_hbm.at[rows, :], ax_raw.at[slot], sem_ax.at[slot])

    shared = (ctx_t, wob_t, waq_t, wakv_t, wo_t, zero_smem)
    if CFG.get('only') != '2': pl.run_scoped(
        P(_head_pairs, wqkv_hbm, wo_hbm, bx_hbm, c_hbm, wq_hbm, wuk_hbm, wuv_hbm, wob_hbm, ax_copy, ax_raw, ax_t, *shared),
        vmem((S, DM), BF16),
        vmem((S, DC), BF16),
        vmem((2, DM, T), U32),
        vmem((2, DC, T), U32),
        vmem((2, DC, T), U32),
        vmem((2, 4, 64, DM), BF16),
        vmem((2, 4, 8, 3 * DM), U32),
        vmem((16, NH, DM), U32),
        vmem((7, 4, S // 2, T), BF16),
        vmem((49, S // 4, T), BF16),
        vmem((7, DM // 2, T), BF16),
        vmem((49, T, T), BF16),
        vmem((2, 8, T), F32),
        dma((2 * NC,)), dma((11,)))
    if CFG.get('only') in ('1', 'f'):
        def fin(buf, sem):
            z = zero_smem[0]
            val = ctx_t[z, z, pl.ds(0, 16), :]
            for ref in (wob_t, waq_t, wakv_t, wo_t):
                val = val + ref[z, z, pl.ds(z * 16, 16), :]
            buf[...] = val
            cp = pltpu.make_async_copy(buf, out_hbm.at[pl.ds(0, 16), pl.ds(0, T)], sem)
            cp.start(); cp.wait()
        pl.run_scoped(fin, vmem((16, T), BF16), dma(()))
        return
    pl.run_scoped(
        P(_outputs, ax_copy, out_hbm, *shared, ax_raw, ax_t),
        vmem((49, 2, RO, T), BF16),
        vmem((8, HALO + CO, T), F32),
        vmem((8, HALO + CO, T), F32),
        vmem((8, CO, T), F32),
        vmem((8, CO, T), F32),
        vmem((14, 8, RO, T), BF16),
        vmem((2, CO, 2 * DM), BF16),
        dma((2,)))


@jax.jit
def pallas_concat_heads__sliding_local_dilated__compressed_kv_cla__prompt_kernel(
    A_x: jax.Array,
    A_wqkv: jax.Array,
    A_wo: jax.Array,
    B_x: jax.Array,
    B_c_kv: jax.Array,
    B_w_q: jax.Array,
    B_w_uk: jax.Array,
    B_w_uv: jax.Array,
    B_w_o: jax.Array,
):
    vmem = pltpu.VMEM
    out = pl.pallas_call(
        _kernel,
        out_shape=jax.ShapeDtypeStruct((S, 2 * DM), BF16),
        in_specs=[pl.BlockSpec(memory_space=pl.ANY)] * 9,
        out_specs=pl.BlockSpec(memory_space=pl.ANY),
        scratch_shapes=[
            vmem((7, NP, S // 2, T), BF16),
            vmem((49, 2, DM, T), BF16),
            vmem((7, 4, DM // 2, T), BF16),
            vmem((49, 4, 2 * T, T), BF16),
            vmem((49, 2, 2 * T, T), BF16),
            pltpu.SMEM((1,), jnp.int32),
            pltpu.SemaphoreType.REGULAR,
            vmem((2, CO, DM), BF16),
            vmem((63, 2, RO, T), BF16),
            pltpu.SemaphoreType.DMA((2,)),
        ],
        compiler_params=pltpu.CompilerParams(vmem_limit_bytes=124 * 2**20, disable_bounds_checks=CFG.get('nb', '1') == '1',
            flags={'lp': {'XLA_TPU_FORCE_LP_LLO_SCHEDULER': True}, 'ev': {'XLA_TPU_EVENLY_DISTRIBUTE_CRITICAL_NODES': True}, 'rd': {'XLA_TPU_RESCHEDULE_DMA_DONES': True}, '': None}[CFG.get('fl', '')]),
    )(
        A_x.reshape(S, DM),
        A_wqkv.reshape(4, DM // 4, 3 * DM),
        A_wo.reshape(NH, DM // NH, DM),
        B_x.reshape(S, DM),
        B_c_kv.reshape(S, DC),
        B_w_q,
        B_w_uk,
        B_w_uv,
        B_w_o,
    )
    return out.reshape(1, S, 2 * DM)
```

```python
import functools
import math

import jax
import jax.numpy as jnp
from jax import lax
import jax.experimental.pallas as pl
import jax.experimental.pallas.tpu as pltpu

S = 2048
DM = 1024
DC = 512
NH = 32
NP = NH // 2
T = 128
CH = 4 * T
RO = 64
CO = 4 * RO
NO = S // CO
WIN, DIL = 8, 2
HALO = 16

LOG2E = math.log2(math.e)
SCALE_A = (DM // NH) ** -0.5 * LOG2E
SCALE_B = T ** -0.5 * LOG2E
MASKED = -1e9 * LOG2E
SAFE_SUM = 2.0 ** 40

DEPTH = 3
JOB_TILES = 16
CTX_TILES = 12

F32, BF16, U32 = jnp.float32, jnp.bfloat16, jnp.uint32
P = functools.partial


def _dot(a, b):
    return jnp.dot(a, b, preferred_element_type=F32)


def _dot_nt(a, b):
    return lax.dot_general(a, b, (((1,), (1,)), ((), ())), preferred_element_type=F32)


def _cat(xs, axis=1):
    return xs[0] if len(xs) == 1 else jnp.concatenate(xs, axis=axis)


def _sum(xs):
    return functools.reduce(jnp.add, xs)


def _fold(op, x):
    return functools.reduce(op, [x[r:r + 8] for r in range(0, x.shape[0], 8)])


def _aligned(x, n):
    return x if isinstance(x, int) else pl.multiple_of(x, n)


def _rows(start, n):
    return pl.ds(_aligned(start, 16), n)


def _words(ref, lead, start, n):
    return ref.bitcast(U32)[(*lead, pl.ds(_aligned(start >> 1, 8), n // 2), slice(None))]


def _load(ref, lead, start, n):
    return pltpu.bitcast(_words(ref, lead, start, n), BF16)


def _split(w):
    return (pltpu.bitcast(w << 16, F32), pltpu.bitcast(w & jnp.uint32(0xFFFF0000), F32))


def _inverse(l):
    r = pl.reciprocal(l, approx=True)
    return r * (2.0 - l * r)


def _interleave(x, y):
    order = [((n + 0.5) / len(z), m, job) for m, z in enumerate((x, y)) for n, job in enumerate(z)]
    return [job for _, _, job in sorted(order, key=lambda e: e[:2])]


def _start(*copies):
    for cp in copies:
        cp.start()


def _wait(*copies):
    for cp in copies:
        cp.wait()


LHS = (((0, 1), (3, 1)), ((2, 1), (3, 1)), ((0, 1),), ((3, 1),),
       ((0, 1), (1, 1)), ((2, 1), (0, -1)), ((1, 1), (3, -1)))
RHS = (((0, 1), (3, 1)), ((0, 1),), ((1, 1), (3, -1)), ((2, 1), (0, -1)),
       ((3, 1),), ((0, 1), (1, 1)), ((2, 1), (3, 1)))
OUT = (((0, 1), (3, 1)), ((2, 1), (3, -1)), ((1, 1), (3, 1)), ((0, 1), (2, 1)),
       ((0, -1), (1, 1)), ((3, 1),), ((0, 1),))


def _term(table, i, quad):
    (n, _), *rest = table[i]
    val = quad(n)
    for n, sign in rest:
        val = val + quad(n) if sign > 0 else val - quad(n)
    return val


def _terms(table, quad):
    blocks = [quad(n) for n in range(4)]
    return [_term(table, i, blocks.__getitem__) for i in range(7)]


def _outer_term(table, i, block):
    return [_term(table, i, lambda m: block(2 * (m // 2) + n // 2, 2 * (m % 2) + n % 2))
            for n in range(4)]


def _terms2(table, i, block):
    return _terms(table, _outer_term(table, i, block).__getitem__)


def _combine(m):
    out = [None] * 4
    for i in range(7):
        for n, sign in OUT[i]:
            if out[n] is None:
                out[n] = m[i]
            else:
                out[n] = out[n] + m[i] if sign > 0 else out[n] - m[i]
    return out


def _combine2(m):
    inner = [_combine(m[7 * i:7 * i + 7]) for i in range(7)]
    out = [[None] * 4 for _ in range(4)]
    for n in range(4):
        for quad, val in enumerate(_combine([x[n] for x in inner])):
            out[2 * (quad // 2) + n // 2][2 * (quad % 2) + n % 2] = val
    return out


class _Tokens:
    def __init__(self, zero_smem):
        self.z = zero_smem[0]
        self.zero = jnp.full((8, T), self.z, jnp.int32).astype(U32)

    def stored(self, ref, lead, start):
        first, *rest = lead
        if ref.dtype == BF16:
            return _words(ref, (first - (self.z & 1), *rest), start, 16) & self.zero
        return self.of(ref[(*lead, pl.ds(_aligned(start + 8 * (self.z & 1), 8), 8), slice(None))])

    def of(self, *vals):
        return pltpu.bitcast(_sum(vals), U32) & self.zero


def _after(token, x, everywhere=False):
    if token is None:
        return x
    bits = x if x.dtype == U32 else pltpu.bitcast(x, U32)
    cut = bits.shape[0] if everywhere else 8
    parts = [bits[r:r + 8] | token for r in range(0, cut, 8)]
    bits = _cat(parts + ([bits[cut:]] if cut < bits.shape[0] else []), axis=0)
    return bits if x.dtype == U32 else pltpu.bitcast(bits, x.dtype)


AX_JOBS = [(i, n, r) for n in range(2) for r in range(0, RO, 16) for i in range(7)]


def _job_ax(tok, released, ax_raw, ax_t, src, i, n, r):
    outer = _outer_term(LHS, i, lambda row, col: released(
        ax_raw[src, pl.ds(row * RO + r, 16), pl.ds((2 * col + n) * T, T)].astype(F32)))
    for x, val in enumerate(_terms(LHS, outer.__getitem__) + outer[1:3]):
        ax_t[9 * i + x, n, pl.ds(r, 16), :] = val.astype(BF16)
    return tok.stored(ax_t, (9 * i + 8, n), r)


def _head_pairs(wqkv_hbm, wo_hbm, bx_hbm, c_hbm, wq_hbm, wuk_hbm, wuv_hbm, wob_hbm,
                ax_copy, ax_raw, ax_t, ctx_t, wob_t, waq_t, wakv_t, wo_t, zero_smem,
                bx_raw, c_raw, wq_raw, wk_raw, wv_raw, wob_raw, wqkv_raw, wo_raw,
                bx_t, c_t, wq_t, wkv_t, guard, sem_in, sem_w):
    def head_copies(j, slot):
        return [pltpu.make_async_copy(src.bitcast(U32).at[:, j, :], dst.at[slot], sem_w.at[3 * slot + n])
                for n, (src, dst) in enumerate(((wuk_hbm, wk_raw), (wuv_hbm, wv_raw), (wq_hbm, wq_raw)))]

    def side_copies(j, slot):
        wob = wob_hbm.at[pl.ds(4 * (j >> 1), 4), pl.ds(_aligned((j & 1) * 64, 64), 64), :]
        wqkv = wqkv_hbm.bitcast(U32).at[:, pl.ds(_aligned(8 * j, 8), 8), :]
        return [pltpu.make_async_copy(wob, wob_raw.at[slot], sem_w.at[6 + 2 * slot]),
                pltpu.make_async_copy(wqkv, wqkv_raw.at[slot], sem_w.at[7 + 2 * slot])]

    def wo_copy(word):
        return pltpu.make_async_copy(wo_hbm.bitcast(U32).at[:, word, :], wo_raw.at[word], sem_w.at[10])

    def c_copy(c):
        rows = pl.ds(c * CH, CH)
        return pltpu.make_async_copy(c_hbm.at[rows, :], c_raw.at[rows, :], sem_in.at[2 * c])

    def x_copy(c):
        rows = pl.ds(c * CH, CH)
        return pltpu.make_async_copy(bx_hbm.at[rows, :], bx_raw.at[rows, :], sem_in.at[2 * c + 1])

    def pair_body(j, first=False):
        slot = j & 1
        if not first:
            _wait(*head_copies(jnp.minimum(j + 1, NP - 1), 1 - slot), *side_copies(j, slot))
            _start(*head_copies(jnp.minimum(j + 2, NP - 1), slot),
                   *side_copies(jnp.minimum(j + 1, NP - 1), 1 - slot))
        tok = _Tokens(zero_smem)
        causal = (lax.broadcasted_iota(jnp.int32, (T, T), 1)
                  <= lax.broadcasted_iota(jnp.int32, (T, T), 0))

        jobs, pace = [], dict(period=0, clock=0, release=None)

        def queue(cycles, more):
            pace.update(period=cycles / len(more), clock=0)
            jobs.extend(more)

        def flush():
            while jobs:
                jobs.pop(0)()

        def background(cycles, recent=None):
            pace["clock"] += cycles
            token = None
            while jobs and pace["clock"] >= pace["period"]:
                pace["clock"] -= pace["period"]
                pace["release"] = None if recent is None else tok.of(recent[:8])
                new = jobs.pop(0)()
                pace["release"] = None
                token = new if token is None else token | new
            return token

        def released(x):
            return _after(pace["release"], x, everywhere=True)

        def store_terms(dst, first_term, lead, row, terms):
            for i, val in enumerate(terms):
                dst[(first_term + i, *lead, _rows(row, 16), slice(None))] = val.astype(BF16)
            return tok.stored(dst, (first_term + 6, *lead), row)

        def job_x(c, t, r):
            terms = _terms(LHS, lambda m: bx_raw[pl.ds(c * CH + (m // 2) * 2 * T + r, 16),
                                                 pl.ds((4 * (m % 2) + t) * T, T)].astype(F32))
            return store_terms(bx_t, 0, (t,), c * 2 * T + r, terms)

        def job_c(c, i, r):
            terms = _terms2(LHS, i, lambda row, col: c_raw[
                pl.ds(c * CH + row * T + r, 16), pl.ds(col * T, T)].astype(F32))
            return store_terms(c_t, 7 * i, (), c * T + r, terms)

        def jobs_x(c):
            return [P(job_x, c, t, r) for r in range(0, 2 * T, 16) for t in range(4)]

        def jobs_c(c):
            return [P(job_c, c, i, r) for r in range(0, T, 16) for i in range(7)]

        def job_wkv(src, i, r):
            def block(row, col):
                raw = (wk_raw, wv_raw)[col % 2]
                return _split(released(raw[src, pl.ds(row * T + r, 16), :]))[col // 2]
            return store_terms(wkv_t, 7 * i, (), r, _terms2(RHS, i, block))

        def job_wq(src, r):
            top, bottom = (_split(released(wq_raw[src, pl.ds(row + r, 16), :])) for row in (0, DM // 2))
            return store_terms(wq_t, 0, (), r, _terms(RHS, (top + bottom).__getitem__))

        def jobs_wkv(src):
            return [P(job_wkv, src, i, r) for r in range(0, T, 16) for i in range(7)]

        def jobs_wq(src):
            return [P(job_wq, src, r) for r in range(0, DM // 2, 16)]

        def job_wob(i, n, r):
            def block(row, col):
                head = 2 * (row % 2) + row // 2
                return released(wob_raw[slot, head, pl.ds(r, 16), pl.ds((2 * col + n) * T, T)].astype(F32))
            return store_terms(wob_t, 7 * i, (n,), j * 64 + r, _terms2(RHS, i, block))

        def job_wo(i, n):
            e, odd, head = j & 3, (j >> 2) & 1, 16 * (j >> 3)

            def block(row, col):
                even_t, odd_t = _split(released(
                    wo_raw[4 * e + row, _rows(head, 16), pl.ds((2 * col + n) * T, T)]))
                return jnp.where(odd == 1, odd_t, even_t)
            return store_terms(wo_t, 7 * i, (n,), odd * T + e * NH + head, _terms2(RHS, i, block))

        permuted = {}

        def job_permute(mat):
            lane = lax.broadcasted_iota(jnp.int32, (32, T), 1)
            e, grp, sub = lane >> 5, (lane >> 2) & 7, lane & 3

            def gather(x, index):
                return jnp.take_along_axis(x, index, axis=1, mode="promise_in_bounds")
            x = [released(wqkv_raw[slot, :, :, pl.ds(mat * DM + t * T, T)].reshape(32, T))
                 for t in range(8)]
            y = [gather(x[t], sub * 32 + e * 8 + ((grp - t) & 7)) for t in range(8)]
            u = [y[-s % 8] for s in range(8)]
            for bit in (1, 2, 4):
                u = [jnp.where((grp & bit) != 0, u[(s - bit) % 8], u[s]) for s in range(8)]
            u = [u[0]] + [gather(u[t], e * 32 + ((grp + t) & 7) * 4 + sub) for t in range(1, 8)]
            permuted[mat] = u
            return _fold(jnp.bitwise_or, functools.reduce(jnp.bitwise_or, u)) & tok.zero

        def column(mat, row, t):
            return pltpu.bitcast(released(permuted[mat][t][8 * row:8 * row + 8]), BF16).astype(F32)

        def job_waq(half, n):
            terms = _terms(RHS, lambda m: column(0, 2 * (m // 2) + half, 4 * (m % 2) + n))
            return store_terms(waq_t, 0, (n,), half * 2 * T + 16 * j, terms)

        def job_wakv(mat, i, n):
            terms = _terms2(RHS, i, lambda row, col: column(mat, row, 2 * col + n))
            return store_terms(wakv_t, 7 * i, (2 * (mat - 1) + n,), 16 * j, terms)

        pause = [lambda: tok.zero] * 2
        jobs_wob = [P(job_wob, i, n, r) for r in range(0, 64, 16) for n in range(2) for i in range(7)]
        jobs_wo = [P(job_wo, i, n) for n in range(2) for i in range(7)]
        jobs_wa = [P(job_permute, 0)] + pause + [P(job_waq, half, n) for half in range(2) for n in range(4)]
        for mat in (1, 2):
            jobs_wa += [P(job_permute, mat)] + pause
            jobs_wa += [P(job_wakv, mat, i, n) for n in range(2) for i in range(7)]

        q, k, v = {}, {}, {}

        def project_q(c):
            m = [_dot(_cat([_load(bx_t, (i, t), c * 2 * T, 2 * T) for t in range(4)]),
                      _load(wq_t, (i,), 0, DM // 2)) for i in range(7)]
            for n, val in enumerate(_combine(m)):
                val = val * SCALE_B
                for r in range(2):
                    q[4 * c + 2 * (n // 2) + r, n % 2] = val[r * T:(r + 1) * T].astype(BF16)

        def project_kv(c):
            m = [_dot(_load(c_t, (i,), c * T, T), _load(wkv_t, (i,), 0, T)) for i in range(49)]
            for r, row in enumerate(_combine2(m)):
                for n, val in enumerate(row):
                    (k, v)[n % 2][4 * c + r, n // 2] = val.astype(BF16)

        def plain(raw, c, weights):
            def operand():
                parts = []
                for r in range(c * CH, (c + 1) * CH, 32):
                    part = raw[pl.ds(r, 32), :]
                    token = background(8 * (raw.shape[1] // T))
                    if token is not None:
                        part = _cat([_after(_cat([token, token]), part[:, :2 * T]), part[:, 2 * T:]])
                    parts.append(part)
                return _cat(parts, axis=0)
            return [_dot(operand(), w) for w in weights]

        def plain_kv(c, weights):
            for n, val in enumerate(plain(c_raw, c, weights)):
                for r in range(4):
                    (k, v)[n // 2][4 * c + r, n % 2] = val[r * T:(r + 1) * T].astype(BF16)

        def plain_q(c, weights):
            for h, val in enumerate(plain(bx_raw, c, weights)):
                for r in range(4):
                    q[4 * c + r, h] = (val[r * T:(r + 1) * T] * SCALE_B).astype(BF16)

        in_flight, partial, ctx, spread, checks, due = [], {}, {}, {}, [], []

        def finish(i, h):
            l, o = partial.pop((i, h))
            l = jnp.sum(l, axis=1, keepdims=True)
            r = _inverse(l)
            ctx[i, h] = o * r
            spread[i, h] = _fold(jnp.maximum, jnp.broadcast_to(l + r, (T, T)))
            b = i // 2
            quad = [(2 * b, 0), (2 * b, 1), (2 * b + 1, 0), (2 * b + 1, 1)]
            if all(u in ctx for u in quad):
                terms = _terms(LHS, lambda m: ctx.pop(quad[m]))
                for n, val in enumerate(terms):
                    ctx_t[n, j, pl.ds(b * T, T), :] = val.astype(BF16)
                checks.append((_fold(jnp.add, terms[0] + terms[5] + terms[6]),
                               functools.reduce(jnp.maximum, [spread.pop(u) for u in quad])))
                due.append([CTX_TILES, tok.stored(ctx_t, (6, j), b * T) | tok.of(*checks[-1])])

        def weigh(i, h, t, p):
            l, o = partial.get((i, h), (None, None))
            l = p if l is None else l + p
            token = background(64, p)
            if token is not None:
                due.append([JOB_TILES, token])
            for entry in due:
                entry[0] -= 1
            now = [token for left, token in due if left <= 0]
            due[:] = [entry for entry in due if entry[0] > 0]
            if now:
                p = _after(functools.reduce(jnp.bitwise_or, now), p)
            d = _dot(p.astype(BF16), v[t, h])
            partial[i, h] = (l, d if o is None else o + d)
            if t == i:
                finish(i, h)

        def attention(lo, hi):
            for i in range(lo, hi):
                for h in range(2):
                    for t in range(i + 1):
                        s = _dot_nt(q[i, h], k[t, h])
                        if t == i:
                            s = jnp.where(causal, s, MASKED)
                        in_flight.append((i, h, t, jnp.exp2(s)))
                        if len(in_flight) > DEPTH:
                            weigh(*in_flight.pop(0))
            while hi == S // T and in_flight:
                weigh(*in_flight.pop(0))

        def cycles(lo, hi):
            return 2 * 64 * sum(range(lo + 1, hi + 1))

        if first:
            wk, wv, wq = head_copies(0, 0)
            _start(wv, wk, c_copy(0), c_copy(1))
            _wait(wv, wk, c_copy(0))
            _start(c_copy(2), c_copy(3), x_copy(0), wq)
            weights = [w.astype(BF16) for raw in (wk_raw, wv_raw) for w in _split(raw[0])]
            queue(0.98 * 2048, jobs_c(0))
            plain_kv(0, weights)
            flush()
            _wait(c_copy(1), c_copy(2))
            _start(x_copy(1), x_copy(2))
            queue(0.98 * 4096, jobs_c(1) + jobs_c(2))
            plain_kv(1, weights)
            plain_kv(2, weights)
            flush()
            _wait(c_copy(3))
            queue(0.98 * 2048, jobs_c(3))
            plain_kv(3, weights)
            flush()
            _wait(x_copy(0), wq)
            weights = [w.astype(BF16) for w in _split(wq_raw[0])]
            queue(0.98 * (2048 + cycles(0, 4)), jobs_wq(0) + jobs_x(0))
            plain_q(0, weights)
            attention(0, 4)
            flush()
            _wait(x_copy(1), x_copy(2))
            stage = [x_copy(3), *side_copies(0, 0), *head_copies(1, 1)]
            _start(*stage)
            lax.fori_loop(0, 16, lambda word, carry: wo_copy(word).start(), None)
            queue(0.98 * (2048 + cycles(4, 8)), jobs_x(2) + jobs_x(1))
            plain_q(1, weights)
            attention(4, 8)
            flush()
            project_q(2)
            attention(8, 9)
            _wait(*stage)
            _start(ax_copy(0, 0), *head_copies(2, 0), *side_copies(1, 1))
            queue(0.98 * cycles(9, 14), jobs_x(3) + _interleave(_interleave(jobs_wob, jobs_wa), jobs_wkv(1)))
            attention(9, 12)
            assert not any(getattr(job, "func", None) is job_x for job in jobs)
            project_q(3)
            attention(12, 14)
            flush()
            _wait(*[wo_copy(word) for word in range(16)], ax_copy(0, 0))
            _start(ax_copy(1, 1))
            queue(0.85 * cycles(14, 16),
                  _interleave(jobs_wo + jobs_wq(1),
                              [P(_job_ax, tok, released, ax_raw, ax_t, 0, *job) for job in AX_JOBS]))
            attention(14, 16)
            flush()
        else:
            queue(0.98 * cycles(0, 12), _interleave(jobs_wob, jobs_wo + jobs_wa))
            project_kv(0)
            project_q(0)
            project_kv(1)
            attention(0, 4)
            project_q(1)
            attention(4, 8)
            project_kv(2)
            project_q(2)
            attention(8, 10)
            project_kv(3)
            attention(10, 12)
            flush()
            project_q(3)
            queue(0.9 * cycles(12, 16), _interleave(jobs_wkv(1 - slot), jobs_wq(1 - slot)))
            attention(12, 16)
            flush()
        guard[0] = _sum([guard[0]] + [x for x, _ in checks])
        guard[1] = functools.reduce(jnp.maximum, [guard[1]] + [x for _, x in checks])

    def exact_pairs(qkv, ctx):
        def block(i):
            return pl.ds(pl.multiple_of(i * T, T), T)

        def head(h, carry):
            def weight(raw):
                even, odd = _split(raw[0])
                return jnp.where(h == 0, even, odd).astype(BF16)
            wk, wv, wq = weight(wk_raw), weight(wv_raw), weight(wq_raw)

            def project(i, carry):
                qkv[0, block(i), :] = (_dot(bx_raw[block(i), :], wq) * SCALE_B).astype(BF16)
                qkv[1, block(i), :] = _dot(c_raw[block(i), :], wk).astype(BF16)
                qkv[2, block(i), :] = _dot(c_raw[block(i), :], wv).astype(BF16)
            lax.fori_loop(0, S // T, project, None)

            def attend(i, carry):
                def scores(t):
                    row = lax.broadcasted_iota(jnp.int32, (T, T), 0) + i * T
                    col = lax.broadcasted_iota(jnp.int32, (T, T), 1) + t * T
                    return jnp.where(col <= row, _dot_nt(qkv[0, block(i), :], qkv[1, block(t), :]), MASKED)

                m = lax.fori_loop(
                    0, i + 1, lambda t, m: jnp.maximum(m, jnp.max(scores(t), axis=1, keepdims=True)),
                    jnp.full((T, 1), -jnp.inf, F32))

                def accumulate(t, carry):
                    l, o = carry
                    p = jnp.exp2(scores(t) - m)
                    return (l + jnp.sum(p, axis=1, keepdims=True),
                            o + _dot(p.astype(BF16), qkv[2, block(t), :]))
                l, o = lax.fori_loop(0, i + 1, accumulate,
                                     (jnp.zeros((T, 1), F32), jnp.zeros((T, T), F32)))
                ctx[h, block(i), :] = o / l
            lax.fori_loop(0, S // T, attend, None)

        def pair(j, carry):
            _start(*head_copies(j, 0))
            _wait(*head_copies(j, 0))
            lax.fori_loop(0, 2, head, None)

            def store(b, carry):
                for n, val in enumerate(_terms(LHS, lambda m: ctx[m % 2, block(2 * b + m // 2), :])):
                    ctx_t[n, j, block(b), :] = val.astype(BF16)
            lax.fori_loop(0, S // T // 2, store, None)

        lax.fori_loop(0, NP, pair, None)

    guard[...] = jnp.zeros(guard.shape, F32)
    pair_body(0, first=True)
    lax.fori_loop(1, NP, lambda j, carry: pair_body(j), None)
    _wait(*head_copies(NP - 1, (NP - 1) % 2), *side_copies(NP - 1, NP % 2))

    safe = jnp.logical_and(jnp.abs(guard[0]) < jnp.inf, guard[1] < SAFE_SUM)

    @pl.when(jnp.max(jnp.where(safe, 0.0, 1.0)) > 0.0)
    def _():
        pl.run_scoped(exact_pairs, pltpu.VMEM((3, S, T), BF16), pltpu.VMEM((2, S, T), F32))


def _outputs(out_hbm, ax_copy, ax_raw, ax_t, ctx_t, wob_t, waq_t, wakv_t, wo_t, zero_smem,
             o_t, kbuf, vbuf, qbuf, acc, obuf, sem_out):
    def out_copy(c, slot):
        rows = pl.ds(_aligned(c * CO, CO), CO)
        return pltpu.make_async_copy(obuf.at[slot], out_hbm.at[rows, :], sem_out.at[slot])

    for buf in (kbuf, vbuf):
        for t in range(8):
            buf[t, pl.ds(CO, HALO), :] = jnp.zeros((HALO, T), F32)

    costs = [RO] * 49 + [4 * RO] * 14 + [RO] * 49 + [4 * RO] * 42 + [RO] * 49 + [4 * RO] * 7
    starts = [sum(costs[:n]) for n in range(len(costs) + 1)]
    t_q, t_v, t_b, t_o, t_last = (starts[n] for n in (49, 63, 112, 154, 203))

    def chunk_body(c, carry):
        slot = c & 1

        @pl.when(c >= 2)
        def _():
            out_copy(c - 2, slot).wait()

        ax_copy(jnp.minimum(c + 1, NO - 1), 1 - slot).wait()
        ax_copy(jnp.minimum(c + 2, NO - 1), slot).start()
        tok = _Tokens(zero_smem)
        plan, due, clock = {}, {}, [0]

        def schedule(job, begin, end, release=False):
            first = max([clock[0]] + [n for n in range(len(costs)) if starts[n + 1] <= begin])
            last = min(n for n in range(len(costs)) if starts[n] >= end)
            plan.setdefault(first, []).append((job, last, release))

        def step(results, a, w):
            n = clock[0]
            clock[0] += 1
            for x, token in enumerate(due.pop(n, [])):
                a[x % len(a)] = _after(token, a[x % len(a)])
            a = [x.astype(BF16) if x.dtype == F32 else pltpu.bitcast(x, BF16) for x in a]
            res = [None] * len(w)
            for x in range(len(a)):
                for y in range(len(w)):
                    d = _dot(a[x], w[y](x))
                    res[y] = d if res[y] is None else res[y] + d
            results.append(res)
            token = None
            for job, last, release in plan.pop(n, []):
                if release and token is None:
                    token = tok.of(res[0][:8])
                due.setdefault(last, []).append(job(token) if release else job())

        def project2(lhs_t, stride, rhs_t, tile0, write, begin, end):
            m = []

            def recombine(y, r):
                blocks = _combine2([x[y][r:r + 8] for x in m])
                write(blocks, y, r)
                return tok.of(*[x for row in blocks for x in row])

            slabs = [(y, r) for r in range(0, RO, 8) for y in range(2)]
            for x, slab in enumerate(slabs):
                schedule(P(recombine, *slab), begin, begin + (end - begin) * (x + 1) // len(slabs))
            for i in range(49):
                step(m, [_words(lhs_t, (stride * (i // 7) + i % 7, x), 0, RO) for x in range(2)],
                     [P(lambda y, x: _load(rhs_t, (i, tile0 + y), x * T, T), y) for y in range(2)])

        for buf in (kbuf, vbuf):
            for t in range(8):
                buf[t, pl.ds(0, HALO), :] = buf[t, pl.ds(CO, HALO), :]

        def write_rows(buf, blocks, y, r):
            for row in range(4):
                for col in range(4):
                    buf[2 * col + y, pl.ds(HALO + row * RO + r, 8), :] = blocks[row][col]

        def write_q(m, half, y):
            vals = [val * SCALE_A for val in _combine([x[y] for x in m])]
            for quad, val in enumerate(vals):
                qbuf[4 * (quad % 2) + y, pl.ds((2 * (quad // 2) + half) * RO, RO), :] = val
            return tok.of(*[val[r:r + 8] for val in vals for r in range(0, RO, 8)])

        project2(ax_t, 9, wakv_t, 0, P(write_rows, kbuf), t_q, t_v - 300)
        for half in range(2):
            m = []
            done = t_q + (t_v - t_q) * (half + 1) // 2
            for y in range(4):
                schedule(P(write_q, m, half, y), done, done + 200 + 50 * y)
            for i in range(7):
                a = [_words(ax_t, (9 * i + x, n), 0, RO) for x in ((2, 7), (8, 3))[half] for n in range(2)]
                step(m, a, [P(lambda y, x: _load(waq_t, (i, y), x * T, T), y) for y in range(4)])

        att = {}

        def job_weights(row, r, release):
            base = HALO + row * RO + r
            qs = [_after(release, qbuf[t, pl.ds(row * RO + r, 8), :]) for t in range(8)]
            logits = []
            for w in range(WIN):
                x = _sum([qs[t] * kbuf[t, pl.ds(base - DIL * w, 8), :] for t in range(8)])
                x = x + pltpu.roll(x, 64, 1)
                x = x + pltpu.roll(x, 32, 1)
                if row == 0 and r < DIL * w:
                    pos = lax.broadcasted_iota(jnp.int32, (8, T), 0) + (c * CO + r)
                    x = jnp.where(pos >= DIL * w, x, MASKED)
                logits.append(x)
            m = functools.reduce(jnp.maximum, logits)
            p = [jnp.exp2(x - m) for x in logits]
            inv = _inverse(_sum(p))
            att[row, r] = [x * inv for x in p]
            return tok.of(att[row, r][0])

        def job_values(row, r, release):
            base = HALO + row * RO + r
            p = [_after(release, x) for x in att[row, r]]
            att[row, r] = [_sum([p[w] * vbuf[t, pl.ds(base - DIL * w, 8), :] for w in range(WIN)])
                           for t in range(8)]
            return tok.of(*att[row, r])

        def job_o(n, r, i):
            def block(row, col):
                return _cat([att[row, r][2 * col + n], att[row, r + 8][2 * col + n]], axis=0)
            for x, val in enumerate(_terms2(LHS, i, block)):
                o_t[7 * i + x, n, pl.ds(r, 16), :] = val.astype(BF16)
            return tok.stored(o_t, (7 * i + 6, n), r)

        groups = [(row, r + x) for r in range(0, RO, 16) for row in range(4) for x in (0, 8)]
        w0, w1, v0, v1 = t_v + 300, t_b + 3500, t_b + 2500, t_o - 700
        for g, (row, r) in enumerate(groups):
            begin = w0 + (w1 - w0) * g // len(groups)
            schedule(P(job_weights, row, r), begin, begin + 700, release=True)
            begin = max(v0 + (v1 - v0) * g // len(groups), begin + 700)
            schedule(P(job_values, row, r), begin, begin + 300, release=True)
            if g % 8 == 7:
                for x, (n, i) in enumerate((n, i) for n in range(2) for i in range(7)):
                    schedule(P(job_o, n, r - 8, i), begin, min(begin + 300 + 60 * (x + 1), t_o))
        project2(ax_t, 9, wakv_t, 2, P(write_rows, vbuf), t_b, t_b + 1500)

        touched = {}

        def project_b(i):
            m = []

            def accumulate(y, inner):
                val = _combine([x[y] for x in m])[inner]
                token = None
                for outer, sign in OUT[i]:
                    row, col = 2 * (outer // 2) + inner // 2, 2 * (2 * (outer % 2) + inner % 2) + y
                    rows = pl.ds(row * RO, RO)
                    total = val
                    if (outer, inner, y) in touched:
                        total = acc[col, rows, :] + val if sign > 0 else acc[col, rows, :] - val
                    touched[outer, inner, y] = True
                    if any(outer == n for x in range(i + 1, 7) for n, _ in OUT[x]):
                        acc[col, rows, :] = total
                        token = tok.stored(acc, (col,), row * RO)
                    else:
                        obuf[slot, rows, pl.ds(DM + col * T, T)] = total.astype(BF16)
                        if token is None:
                            token = tok.of(_fold(jnp.add, total))
                return token

            parts = [(y, inner) for y in range(2) for inner in range(4)]
            done = starts[clock[0] + 7]
            if i < 6:
                for x, part in enumerate(parts):
                    schedule(P(accumulate, *part), done, done + 256 + 150 * x)
            for n in range(7):
                def quad(kt, x):
                    return (i, 2 * kt + x % 2), (2 * c + x // 2) * RO
                if len(LHS[n]) == 1:
                    a = [_words(ctx_t, *quad(kt, LHS[n][0][0]), RO) for kt in range(8)]
                else:
                    a = [_term(LHS, n, lambda x: _load(ctx_t, *quad(kt, x), RO).astype(F32))
                         for kt in range(8)]
                step(m, a, [P(lambda y, x: _load(wob_t, (7 * i + n, y), x * T, T), y) for y in range(2)])
            if i == 6:
                for part in parts:
                    accumulate(*part)

        for i in range(6):
            project_b(i)

        for x, job in enumerate(AX_JOBS):
            schedule(P(_job_ax, tok, lambda val: val, ax_raw, ax_t, 1 - slot, *job),
                     t_o, t_o + 100 + 4400 * (x + 1) // len(AX_JOBS))
        upper = {}

        def write_out(blocks, y, r):
            if r % 16 == 0:
                upper[y] = blocks
                return
            for row in range(4):
                for col in range(4):
                    val = _cat([upper[y][row][col], blocks[row][col]], axis=0)
                    obuf[slot, pl.ds(row * RO + r - 8, 16), pl.ds((2 * col + y) * T, T)] = val.astype(BF16)

        project2(o_t, 7, wo_t, 0, write_out, t_last, starts[-2])
        project_b(6)
        assert not plan and not due
        out_copy(c, slot).start()

    lax.fori_loop(0, NO, chunk_body, None)
    ax_copy(NO - 1, (NO - 1) % 2).wait()
    out_copy(NO - 2, 0).wait()
    out_copy(NO - 1, 1).wait()


def _kernel(ax_hbm, wqkv_hbm, wo_hbm, bx_hbm, c_hbm, wq_hbm, wuk_hbm, wuv_hbm, wob_hbm, out_hbm,
            ax_raw, ax_t, ctx_t, wob_t, waq_t, wakv_t, wo_t, zero_smem, idle_sem, sem_ax):
    vmem, dma = pltpu.VMEM, pltpu.SemaphoreType.DMA

    @pl.when(pl.semaphore_read(idle_sem) == 0)
    def _():
        zero_smem[0] = 0

    def ax_copy(c, slot):
        rows = pl.ds(_aligned(c * CO, CO), CO)
        return pltpu.make_async_copy(ax_hbm.at[rows, :], ax_raw.at[slot], sem_ax.at[slot])

    shared = (ax_copy, ax_raw, ax_t, ctx_t, wob_t, waq_t, wakv_t, wo_t, zero_smem)
    pl.run_scoped(
        P(_head_pairs, wqkv_hbm, wo_hbm, bx_hbm, c_hbm, wq_hbm, wuk_hbm, wuv_hbm, wob_hbm, *shared),
        vmem((S, DM), BF16),
        vmem((S, DC), BF16),
        vmem((2, DM, T), U32),
        vmem((2, DC, T), U32),
        vmem((2, DC, T), U32),
        vmem((2, 4, 64, DM), BF16),
        vmem((2, 4, 8, 3 * DM), U32),
        vmem((16, NH, DM), U32),
        vmem((7, 4, S // 2, T), BF16),
        vmem((49, S // 4, T), BF16),
        vmem((7, DM // 2, T), BF16),
        vmem((49, T, T), BF16),
        vmem((2, 8, T), F32),
        dma((2 * S // CH,)), dma((11,)))
    pl.run_scoped(
        P(_outputs, out_hbm, *shared),
        vmem((49, 2, RO, T), BF16),
        vmem((8, HALO + CO, T), F32),
        vmem((8, HALO + CO, T), F32),
        vmem((8, CO, T), F32),
        vmem((8, CO, T), F32),
        vmem((2, CO, 2 * DM), BF16),
        dma((2,)))


@jax.jit
def pallas_concat_heads__sliding_local_dilated__compressed_kv_cla__prompt_kernel(
    A_x: jax.Array,
    A_wqkv: jax.Array,
    A_wo: jax.Array,
    B_x: jax.Array,
    B_c_kv: jax.Array,
    B_w_q: jax.Array,
    B_w_uk: jax.Array,
    B_w_uv: jax.Array,
    B_w_o: jax.Array,
):
    vmem = pltpu.VMEM
    out = pl.pallas_call(
        _kernel,
        out_shape=jax.ShapeDtypeStruct((S, 2 * DM), BF16),
        in_specs=[pl.BlockSpec(memory_space=pl.ANY)] * 9,
        out_specs=pl.BlockSpec(memory_space=pl.ANY),
        scratch_shapes=[
            vmem((2, CO, DM), BF16),
            vmem((63, 2, RO, T), BF16),
            vmem((7, NP, S // 2, T), BF16),
            vmem((49, 2, DM, T), BF16),
            vmem((7, 4, DM // 2, T), BF16),
            vmem((49, 4, 2 * T, T), BF16),
            vmem((49, 2, 2 * T, T), BF16),
            pltpu.SMEM((1,), jnp.int32),
            pltpu.SemaphoreType.REGULAR,
            pltpu.SemaphoreType.DMA((2,)),
        ],
        compiler_params=pltpu.CompilerParams(
            vmem_limit_bytes=124 * 2**20, disable_bounds_checks=True),
    )(
        A_x.reshape(S, DM),
        A_wqkv.reshape(4, DM // 4, 3 * DM),
        A_wo.reshape(NH, DM // NH, DM),
        B_x.reshape(S, DM),
        B_c_kv.reshape(S, DC),
        B_w_q,
        B_w_uk,
        B_w_uv,
        B_w_o,
    )
    return out.reshape(1, S, 2 * DM)
```

```python
import functools
import math

import jax
import jax.numpy as jnp
from jax import lax
import jax.experimental.pallas as pl
import jax.experimental.pallas.tpu as pltpu

S = 2048
DM = 1024
DC = 512
NH = 32
NP = NH // 2
T = 128
CH = 4 * T
RO = 64
CO = 4 * RO
NO = S // CO
WIN, DIL = 8, 2
HALO = 16

LOG2E = math.log2(math.e)
SCALE_A = (DM // NH) ** -0.5 * LOG2E
SCALE_B = T ** -0.5 * LOG2E
MASKED = -1e9 * LOG2E
SAFE_SUM = 2.0 ** 40

DEPTH = 3
JOB_TILES = 16, 10
CTX_TILES = 12, 20

F32, BF16, U32 = jnp.float32, jnp.bfloat16, jnp.uint32
P = functools.partial


def _dot(a, b):
    return jnp.dot(a, b, preferred_element_type=F32)


def _dot_nt(a, b):
    return lax.dot_general(a, b, (((1,), (1,)), ((), ())), preferred_element_type=F32)


def _cat(xs, axis=1):
    return xs[0] if len(xs) == 1 else jnp.concatenate(xs, axis=axis)


def _sum(xs):
    return functools.reduce(jnp.add, xs)


def _fold(op, x):
    return functools.reduce(op, [x[r:r + 8] for r in range(0, x.shape[0], 8)])


def _aligned(x, n):
    return x if isinstance(x, int) else pl.multiple_of(x, n)


def _rows(start, n):
    return pl.ds(_aligned(start, 16), n)


def _words(ref, lead, start, n):
    return ref.bitcast(U32)[(*lead, pl.ds(_aligned(start >> 1, 8), n // 2), slice(None))]


def _load(ref, lead, start, n):
    return pltpu.bitcast(_words(ref, lead, start, n), BF16)


def _split(w):
    return (pltpu.bitcast(w << 16, F32), pltpu.bitcast(w & jnp.uint32(0xFFFF0000), F32))


def _inverse(l):
    r = pl.reciprocal(l, approx=True)
    return r * (2.0 - l * r)


def _interleave(x, y):
    order = [((n + 0.5) / len(z), m, job) for m, z in enumerate((x, y)) for n, job in enumerate(z)]
    return [job for _, _, job in sorted(order, key=lambda e: e[:2])]


def _start(*copies):
    for cp in copies:
        cp.start()


def _wait(*copies):
    for cp in copies:
        cp.wait()


LHS = (((0, 1), (3, 1)), ((2, 1), (3, 1)), ((0, 1),), ((3, 1),),
       ((0, 1), (1, 1)), ((2, 1), (0, -1)), ((1, 1), (3, -1)))
RHS = (((0, 1), (3, 1)), ((0, 1),), ((1, 1), (3, -1)), ((2, 1), (0, -1)),
       ((3, 1),), ((0, 1), (1, 1)), ((2, 1), (3, 1)))
OUT = (((0, 1), (3, 1)), ((2, 1), (3, -1)), ((1, 1), (3, 1)), ((0, 1), (2, 1)),
       ((0, -1), (1, 1)), ((3, 1),), ((0, 1),))


def _term(table, i, quad):
    (n, _), *rest = table[i]
    val = quad(n)
    for n, sign in rest:
        val = val + quad(n) if sign > 0 else val - quad(n)
    return val


def _terms(table, quad):
    blocks = [quad(n) for n in range(4)]
    return [_term(table, i, blocks.__getitem__) for i in range(7)]


def _outer_term(table, i, block):
    return [_term(table, i, lambda m: block(2 * (m // 2) + n // 2, 2 * (m % 2) + n % 2))
            for n in range(4)]


def _terms2(table, i, block):
    return _terms(table, _outer_term(table, i, block).__getitem__)


def _combine(m):
    out = [None] * 4
    for i in range(7):
        for n, sign in OUT[i]:
            if out[n] is None:
                out[n] = m[i]
            else:
                out[n] = out[n] + m[i] if sign > 0 else out[n] - m[i]
    return out


def _combine2(m):
    inner = [_combine(m[7 * i:7 * i + 7]) for i in range(7)]
    out = [[None] * 4 for _ in range(4)]
    for n in range(4):
        for quad, val in enumerate(_combine([x[n] for x in inner])):
            out[2 * (quad // 2) + n // 2][2 * (quad % 2) + n % 2] = val
    return out


class _Tokens:
    def __init__(self, zero_smem):
        self.z = zero_smem[0]
        self.zero = jnp.full((8, T), self.z, jnp.int32).astype(U32)

    def stored(self, ref, lead, start):
        first, *rest = lead
        if ref.dtype == BF16:
            return _words(ref, (first - (self.z & 1), *rest), start, 16) & self.zero
        return self.of(ref[(*lead, pl.ds(_aligned(start + 8 * (self.z & 1), 8), 8), slice(None))])

    def of(self, *vals):
        return pltpu.bitcast(_sum(vals), U32) & self.zero


def _after(token, x, everywhere=False):
    if token is None:
        return x
    bits = x if x.dtype == U32 else pltpu.bitcast(x, U32)
    cut = bits.shape[0] if everywhere else 8
    parts = [bits[r:r + 8] | token for r in range(0, cut, 8)]
    bits = _cat(parts + ([bits[cut:]] if cut < bits.shape[0] else []), axis=0)
    return bits if x.dtype == U32 else pltpu.bitcast(bits, x.dtype)


AX_JOBS = [(i, n, r) for n in range(2) for r in range(0, RO, 16) for i in range(7)]


def _job_ax(tok, released, ax_raw, ax_t, src, i, n, r):
    outer = _outer_term(LHS, i, lambda row, col: released(
        ax_raw[src, pl.ds(row * RO + r, 16), pl.ds((2 * col + n) * T, T)].astype(F32)))
    for x, val in enumerate(_terms(LHS, outer.__getitem__) + outer[1:3]):
        ax_t[9 * i + x, n, pl.ds(r, 16), :] = val.astype(BF16)
    return tok.stored(ax_t, (9 * i + 8, n), r)


def _head_pairs(wqkv_hbm, wo_hbm, bx_hbm, c_hbm, wq_hbm, wuk_hbm, wuv_hbm, wob_hbm,
                ax_copy, ax_raw, ax_t, ctx_t, wob_t, waq_t, wakv_t, wo_t, zero_smem,
                bx_raw, c_raw, wq_raw, wk_raw, wv_raw, wob_raw, wqkv_raw, wo_raw,
                bx_t, c_t, wq_t, wkv_t, guard, sem_in, sem_w):
    def head_copies(j, slot):
        return [pltpu.make_async_copy(src.bitcast(U32).at[:, j, :], dst.at[slot], sem_w.at[3 * slot + n])
                for n, (src, dst) in enumerate(((wuk_hbm, wk_raw), (wuv_hbm, wv_raw), (wq_hbm, wq_raw)))]

    def side_copies(j, slot):
        wob = wob_hbm.at[pl.ds(4 * (j >> 1), 4), pl.ds(_aligned((j & 1) * 64, 64), 64), :]
        wqkv = wqkv_hbm.bitcast(U32).at[:, pl.ds(_aligned(8 * j, 8), 8), :]
        return [pltpu.make_async_copy(wob, wob_raw.at[slot], sem_w.at[6 + 2 * slot]),
                pltpu.make_async_copy(wqkv, wqkv_raw.at[slot], sem_w.at[7 + 2 * slot])]

    def wo_copy(word):
        return pltpu.make_async_copy(wo_hbm.bitcast(U32).at[:, word, :], wo_raw.at[word], sem_w.at[10])

    def c_copy(c):
        rows = pl.ds(c * CH, CH)
        return pltpu.make_async_copy(c_hbm.at[rows, :], c_raw.at[rows, :], sem_in.at[2 * c])

    def x_copy(c):
        rows = pl.ds(c * CH, CH)
        return pltpu.make_async_copy(bx_hbm.at[rows, :], bx_raw.at[rows, :], sem_in.at[2 * c + 1])

    def pair_body(j, first=False):
        slot = j & 1
        tok = _Tokens(zero_smem)
        causal = (lax.broadcasted_iota(jnp.int32, (T, T), 1)
                  <= lax.broadcasted_iota(jnp.int32, (T, T), 0))

        jobs, pace = [], dict(period=0, clock=0, release=None)

        def queue(cycles, more):
            pace.update(period=cycles / len(more), clock=0)
            jobs.extend(more)

        def flush():
            while jobs:
                jobs.pop(0)()

        def background(cycles, recent=None):
            pace["clock"] += cycles
            token = None
            while jobs and pace["clock"] >= pace["period"]:
                pace["clock"] -= pace["period"]
                pace["release"] = None if recent is None else tok.of(recent[:8])
                new = jobs.pop(0)()
                pace["release"] = None
                token = new if token is None else token | new
            return token

        def released(x):
            return _after(pace["release"], x, everywhere=True)

        def store_terms(dst, first_term, lead, row, terms):
            for i, val in enumerate(terms):
                dst[(first_term + i, *lead, _rows(row, 16), slice(None))] = val.astype(BF16)
            return tok.stored(dst, (first_term + 6, *lead), row)

        def job_x(c, t, r):
            terms = _terms(LHS, lambda m: bx_raw[pl.ds(c * CH + (m // 2) * 2 * T + r, 16),
                                                 pl.ds((4 * (m % 2) + t) * T, T)].astype(F32))
            return store_terms(bx_t, 0, (t,), c * 2 * T + r, terms)

        def job_c(c, i, r):
            terms = _terms2(LHS, i, lambda row, col: c_raw[
                pl.ds(c * CH + row * T + r, 16), pl.ds(col * T, T)].astype(F32))
            return store_terms(c_t, 7 * i, (), c * T + r, terms)

        def jobs_x(c):
            return [P(job_x, c, t, r) for r in range(0, 2 * T, 16) for t in range(4)]

        def jobs_c(c):
            return [P(job_c, c, i, r) for r in range(0, T, 16) for i in range(7)]

        def job_wkv(src, i, r):
            def block(row, col):
                raw = (wk_raw, wv_raw)[col % 2]
                return _split(released(raw[src, pl.ds(row * T + r, 16), :]))[col // 2]
            return store_terms(wkv_t, 7 * i, (), r, _terms2(RHS, i, block))

        def job_wq(src, r):
            top, bottom = (_split(released(wq_raw[src, pl.ds(row + r, 16), :])) for row in (0, DM // 2))
            return store_terms(wq_t, 0, (), r, _terms(RHS, (top + bottom).__getitem__))

        def jobs_wkv(src):
            return [P(job_wkv, src, i, r) for r in range(0, T, 16) for i in range(7)]

        def jobs_wq(src):
            return [P(job_wq, src, r) for r in range(0, DM // 2, 16)]

        def job_wob(i, n, r):
            def block(row, col):
                head = 2 * (row % 2) + row // 2
                return released(wob_raw[slot, head, pl.ds(r, 16), pl.ds((2 * col + n) * T, T)].astype(F32))
            return store_terms(wob_t, 7 * i, (n,), j * 64 + r, _terms2(RHS, i, block))

        def job_wo(i, n):
            e, odd, head = j & 3, (j >> 2) & 1, 16 * (j >> 3)

            def block(row, col):
                even_t, odd_t = _split(released(
                    wo_raw[4 * e + row, _rows(head, 16), pl.ds((2 * col + n) * T, T)]))
                return jnp.where(odd == 1, odd_t, even_t)
            return store_terms(wo_t, 7 * i, (n,), odd * T + e * NH + head, _terms2(RHS, i, block))

        permuted = {}

        def job_permute(mat):
            lane = lax.broadcasted_iota(jnp.int32, (32, T), 1)
            e, grp, sub = lane >> 5, (lane >> 2) & 7, lane & 3

            def gather(x, index):
                return jnp.take_along_axis(x, index, axis=1, mode="promise_in_bounds")
            x = [released(wqkv_raw[slot, :, :, pl.ds(mat * DM + t * T, T)].reshape(32, T))
                 for t in range(8)]
            y = [gather(x[t], sub * 32 + e * 8 + ((grp - t) & 7)) for t in range(8)]
            u = [y[-s % 8] for s in range(8)]
            for bit in (1, 2, 4):
                u = [jnp.where((grp & bit) != 0, u[(s - bit) % 8], u[s]) for s in range(8)]
            u = [u[0]] + [gather(u[t], e * 32 + ((grp + t) & 7) * 4 + sub) for t in range(1, 8)]
            permuted[mat] = u
            return _fold(jnp.bitwise_or, functools.reduce(jnp.bitwise_or, u)) & tok.zero

        def column(mat, row, t):
            return pltpu.bitcast(released(permuted[mat][t][8 * row:8 * row + 8]), BF16).astype(F32)

        def job_waq(half, n):
            terms = _terms(RHS, lambda m: column(0, 2 * (m // 2) + half, 4 * (m % 2) + n))
            return store_terms(waq_t, 0, (n,), half * 2 * T + 16 * j, terms)

        def job_wakv(mat, i, n):
            terms = _terms2(RHS, i, lambda row, col: column(mat, row, 2 * col + n))
            return store_terms(wakv_t, 7 * i, (2 * (mat - 1) + n,), 16 * j, terms)

        pause = [lambda: tok.zero] * 2
        jobs_wob = [P(job_wob, i, n, r) for r in range(0, 64, 16) for n in range(2) for i in range(7)]
        jobs_wo = [P(job_wo, i, n) for n in range(2) for i in range(7)]
        jobs_wa = [P(job_permute, 0)] + pause + [P(job_waq, half, n) for half in range(2) for n in range(4)]
        for mat in (1, 2):
            jobs_wa += [P(job_permute, mat)] + pause
            jobs_wa += [P(job_wakv, mat, i, n) for n in range(2) for i in range(7)]

        q, k, v = {}, {}, {}

        def project_q(c):
            m = [_dot(_cat([_load(bx_t, (i, t), c * 2 * T, 2 * T) for t in range(4)]),
                      _load(wq_t, (i,), 0, DM // 2)) for i in range(7)]
            for n, val in enumerate(_combine(m)):
                val = val * SCALE_B
                for r in range(2):
                    q[4 * c + 2 * (n // 2) + r, n % 2] = val[r * T:(r + 1) * T].astype(BF16)

        def project_kv(c):
            m = [_dot(_load(c_t, (i,), c * T, T), _load(wkv_t, (i,), 0, T)) for i in range(49)]
            for r, row in enumerate(_combine2(m)):
                for n, val in enumerate(row):
                    (k, v)[n % 2][4 * c + r, n // 2] = val.astype(BF16)

        def plain(raw, c, weights):
            def operand():
                parts = []
                for r in range(c * CH, (c + 1) * CH, 32):
                    part = raw[pl.ds(r, 32), :]
                    token = background(8 * (raw.shape[1] // T))
                    if token is not None:
                        part = _cat([_after(_cat([token, token]), part[:, :2 * T]), part[:, 2 * T:]])
                    parts.append(part)
                return _cat(parts, axis=0)
            return [_dot(operand(), w) for w in weights]

        def plain_kv(c, weights):
            for n, val in enumerate(plain(c_raw, c, weights)):
                for r in range(4):
                    (k, v)[n // 2][4 * c + r, n % 2] = val[r * T:(r + 1) * T].astype(BF16)

        def plain_q(c, weights):
            for h, val in enumerate(plain(bx_raw, c, weights)):
                for r in range(4):
                    q[4 * c + r, h] = (val[r * T:(r + 1) * T] * SCALE_B).astype(BF16)

        in_flight, partial, ctx, spread, checks, due = [], {}, {}, {}, [], []

        def finish(i, h):
            l, o = partial.pop((i, h))
            l = jnp.sum(l, axis=1, keepdims=True)
            r = _inverse(l)
            ctx[i, h] = o * r
            spread[i, h] = _fold(jnp.maximum, jnp.broadcast_to(l + r, (T, T)))
            b = i // 2
            quad = [(2 * b, 0), (2 * b, 1), (2 * b + 1, 0), (2 * b + 1, 1)]
            if all(u in ctx for u in quad):
                terms = _terms(LHS, lambda m: ctx.pop(quad[m]))
                for n, val in enumerate(terms):
                    ctx_t[n, j, pl.ds(b * T, T), :] = val.astype(BF16)
                checks.append((_fold(jnp.add, terms[0] + terms[5] + terms[6]),
                               functools.reduce(jnp.maximum, [spread.pop(u) for u in quad])))
                due.append([CTX_TILES[first], tok.stored(ctx_t, (6, j), b * T) | tok.of(*checks[-1])])

        def weigh(i, h, t, p):
            l, o = partial.get((i, h), (None, None))
            l = p if l is None else l + p
            token = background(64, p)
            if token is not None:
                due.append([JOB_TILES[first], token])
            for entry in due:
                entry[0] -= 1
            now = [token for left, token in due if left <= 0]
            due[:] = [entry for entry in due if entry[0] > 0]
            if now:
                p = _after(functools.reduce(jnp.bitwise_or, now), p)
            d = _dot(p.astype(BF16), v[t, h])
            partial[i, h] = (l, d if o is None else o + d)
            if t == i:
                finish(i, h)

        def attention(lo, hi):
            for i in range(lo, hi):
                for h in range(2):
                    for t in range(i + 1):
                        s = _dot_nt(q[i, h], k[t, h])
                        if t == i:
                            s = jnp.where(causal, s, MASKED)
                        in_flight.append((i, h, t, jnp.exp2(s)))
                        if len(in_flight) > DEPTH:
                            weigh(*in_flight.pop(0))
            while hi == S // T and in_flight:
                weigh(*in_flight.pop(0))

        def cycles(lo, hi):
            return 2 * 64 * sum(range(lo + 1, hi + 1))

        if first:
            wk, wv, wq = head_copies(0, 0)
            _start(wv, wk, c_copy(0), c_copy(1))
            _wait(wv, wk, c_copy(0))
            _start(c_copy(2), c_copy(3), x_copy(0), wq)
            weights = [w.astype(BF16) for raw in (wk_raw, wv_raw) for w in _split(raw[0])]
            queue(0.98 * 2048, jobs_c(0))
            plain_kv(0, weights)
            flush()
            _wait(c_copy(1), c_copy(2))
            _start(x_copy(1), x_copy(2))
            queue(0.98 * 4096, jobs_c(1) + jobs_c(2))
            plain_kv(1, weights)
            plain_kv(2, weights)
            flush()
            _wait(c_copy(3))
            queue(0.98 * 2048, jobs_c(3))
            plain_kv(3, weights)
            flush()
            _wait(x_copy(0), wq)
            weights = [w.astype(BF16) for w in _split(wq_raw[0])]
            queue(0.85 * (2048 + cycles(0, 4)), jobs_wq(0) + jobs_x(0))
            plain_q(0, weights)
            attention(0, 4)
            flush()
            _wait(x_copy(1), x_copy(2))
            stage = [x_copy(3), *side_copies(0, 0), *head_copies(1, 1)]
            _start(*stage)
            lax.fori_loop(0, 16, lambda word, carry: wo_copy(word).start(), None)
            queue(0.98 * (2048 + cycles(4, 8)), jobs_x(2) + jobs_x(1))
            plain_q(1, weights)
            attention(4, 8)
            flush()
            project_q(2)
            attention(8, 9)
            _wait(*stage)
            _start(ax_copy(0, 0), *head_copies(2, 0), *side_copies(1, 1))
            queue(0.92 * cycles(9, 14), jobs_x(3) + _interleave(_interleave(jobs_wob, jobs_wa), jobs_wkv(1)))
            attention(9, 12)
            assert not any(getattr(job, "func", None) is job_x for job in jobs)
            project_q(3)
            attention(12, 14)
            flush()
            _wait(*[wo_copy(word) for word in range(16)], ax_copy(0, 0))
            _start(ax_copy(1, 1))
            queue(0.92 * cycles(14, 16),
                  _interleave(jobs_wo + jobs_wq(1),
                              [P(_job_ax, tok, released, ax_raw, ax_t, 0, *job) for job in AX_JOBS]))
            attention(14, 16)
            flush()
        else:
            queue(0.98 * cycles(0, 12), _interleave(jobs_wob, jobs_wo + jobs_wa))
            project_kv(0)
            project_q(0)
            project_kv(1)
            attention(0, 4)
            project_q(1)
            attention(4, 8)
            project_kv(2)
            project_q(2)
            attention(8, 10)
            project_kv(3)
            attention(10, 12)
            flush()
            project_q(3)
            queue(0.9 * cycles(12, 16), _interleave(jobs_wkv(1 - slot), jobs_wq(1 - slot)))
            attention(12, 16)
            flush()
        guard[0] = _sum([guard[0]] + [x for x, _ in checks])
        guard[1] = functools.reduce(jnp.maximum, [guard[1]] + [x for _, x in checks])

        def ahead(n):
            return j + n if first else jnp.minimum(j + n, NP - 1)
        _wait(*head_copies(ahead(2), slot), *side_copies(ahead(1), 1 - slot))

        @pl.when(j < NP - 1)
        def _():
            _start(*head_copies(ahead(3), 1 - slot), *side_copies(ahead(2), slot))

    def exact_pairs(qkv, ctx):
        def block(i):
            return pl.ds(pl.multiple_of(i * T, T), T)

        def head(h, carry):
            def weight(raw):
                even, odd = _split(raw[0])
                return jnp.where(h == 0, even, odd).astype(BF16)
            wk, wv, wq = weight(wk_raw), weight(wv_raw), weight(wq_raw)

            def project(i, carry):
                qkv[0, block(i), :] = (_dot(bx_raw[block(i), :], wq) * SCALE_B).astype(BF16)
                qkv[1, block(i), :] = _dot(c_raw[block(i), :], wk).astype(BF16)
                qkv[2, block(i), :] = _dot(c_raw[block(i), :], wv).astype(BF16)
            lax.fori_loop(0, S // T, project, None)

            def attend(i, carry):
                def scores(t):
                    row = lax.broadcasted_iota(jnp.int32, (T, T), 0) + i * T
                    col = lax.broadcasted_iota(jnp.int32, (T, T), 1) + t * T
                    return jnp.where(col <= row, _dot_nt(qkv[0, block(i), :], qkv[1, block(t), :]), MASKED)

                m = lax.fori_loop(
                    0, i + 1, lambda t, m: jnp.maximum(m, jnp.max(scores(t), axis=1, keepdims=True)),
                    jnp.full((T, 1), -jnp.inf, F32))

                def accumulate(t, carry):
                    l, o = carry
                    p = jnp.exp2(scores(t) - m)
                    return (l + jnp.sum(p, axis=1, keepdims=True),
                            o + _dot(p.astype(BF16), qkv[2, block(t), :]))
                l, o = lax.fori_loop(0, i + 1, accumulate,
                                     (jnp.zeros((T, 1), F32), jnp.zeros((T, T), F32)))
                ctx[h, block(i), :] = o / l
            lax.fori_loop(0, S // T, attend, None)

        def pair(j, carry):
            _start(*head_copies(j, 0))
            _wait(*head_copies(j, 0))
            lax.fori_loop(0, 2, head, None)

            def store(b, carry):
                for n, val in enumerate(_terms(LHS, lambda m: ctx[m % 2, block(2 * b + m // 2), :])):
                    ctx_t[n, j, block(b), :] = val.astype(BF16)
            lax.fori_loop(0, S // T // 2, store, None)

        lax.fori_loop(0, NP, pair, None)

    guard[...] = jnp.zeros(guard.shape, F32)
    pair_body(0, first=True)
    lax.fori_loop(1, NP, lambda j, carry: pair_body(j), None)

    safe = jnp.logical_and(jnp.abs(guard[0]) < jnp.inf, guard[1] < SAFE_SUM)

    @pl.when(jnp.max(jnp.where(safe, 0.0, 1.0)) > 0.0)
    def _():
        pl.run_scoped(exact_pairs, pltpu.VMEM((3, S, T), BF16), pltpu.VMEM((2, S, T), F32))


def _outputs(out_hbm, ax_copy, ax_raw, ax_t, ctx_t, wob_t, waq_t, wakv_t, wo_t, zero_smem,
             o_t, kbuf, vbuf, qbuf, acc, obuf, sem_out):
    def out_copy(c, slot):
        rows = pl.ds(_aligned(c * CO, CO), CO)
        return pltpu.make_async_copy(obuf.at[slot], out_hbm.at[rows, :], sem_out.at[slot])

    for buf in (kbuf, vbuf):
        for t in range(8):
            buf[t, pl.ds(CO, HALO), :] = jnp.zeros((HALO, T), F32)

    costs = [RO] * 49 + [4 * RO] * 14 + [RO] * 49 + [4 * RO] * 42 + [RO] * 49 + [4 * RO] * 7
    starts = [sum(costs[:n]) for n in range(len(costs) + 1)]
    t_q, t_v, t_b, t_o, t_last = (starts[n] for n in (49, 63, 112, 154, 203))

    def chunk_body(c, carry):
        slot = c & 1
        tok = _Tokens(zero_smem)
        plan, due, clock = {}, {}, [0]

        def schedule(job, begin, end, release=False):
            first = max([clock[0]] + [n for n in range(len(costs)) if starts[n + 1] <= begin])
            last = min(n for n in range(len(costs)) if starts[n] >= end)
            plan.setdefault(first, []).append((job, last, release))

        def step(results, a, w):
            n = clock[0]
            clock[0] += 1
            for x, token in enumerate(due.pop(n, [])):
                a[x % len(a)] = _after(token, a[x % len(a)])
            a = [x.astype(BF16) if x.dtype == F32 else pltpu.bitcast(x, BF16) for x in a]
            res = [None] * len(w)
            for x in range(len(a)):
                for y in range(len(w)):
                    d = _dot(a[x], w[y](x))
                    res[y] = d if res[y] is None else res[y] + d
            results.append(res)
            token = None
            for job, last, release in plan.pop(n, []):
                if release and token is None:
                    token = tok.of(res[0][:8])
                due.setdefault(last, []).append(job(token) if release else job())

        def project2(lhs_t, stride, rhs_t, tile0, write, begin, end):
            m = []

            def recombine(y, r):
                blocks = _combine2([x[y][r:r + 8] for x in m])
                write(blocks, y, r)
                return tok.of(*[x for row in blocks for x in row])

            slabs = [(y, r) for r in range(0, RO, 8) for y in range(2)]
            for x, slab in enumerate(slabs):
                schedule(P(recombine, *slab), begin, begin + (end - begin) * (x + 1) // len(slabs))
            for i in range(49):
                step(m, [_words(lhs_t, (stride * (i // 7) + i % 7, x), 0, RO) for x in range(2)],
                     [P(lambda y, x: _load(rhs_t, (i, tile0 + y), x * T, T), y) for y in range(2)])

        for buf in (kbuf, vbuf):
            for t in range(8):
                buf[t, pl.ds(0, HALO), :] = buf[t, pl.ds(CO, HALO), :]

        def write_rows(buf, blocks, y, r):
            for row in range(4):
                for col in range(4):
                    buf[2 * col + y, pl.ds(HALO + row * RO + r, 8), :] = blocks[row][col]

        def write_q(m, half, y):
            vals = [val * SCALE_A for val in _combine([x[y] for x in m])]
            for quad, val in enumerate(vals):
                qbuf[4 * (quad % 2) + y, pl.ds((2 * (quad // 2) + half) * RO, RO), :] = val
            return tok.of(*[val[r:r + 8] for val in vals for r in range(0, RO, 8)])

        project2(ax_t, 9, wakv_t, 0, P(write_rows, kbuf), t_q, t_v - 1000)
        for half in range(2):
            m = []
            done = t_q + (t_v - t_q) * (half + 1) // 2
            for y in range(4):
                schedule(P(write_q, m, half, y), done, done + 200 + 200 * y)
            for i in range(7):
                a = [_words(ax_t, (9 * i + x, n), 0, RO) for x in ((2, 7), (8, 3))[half] for n in range(2)]
                step(m, a, [P(lambda y, x: _load(waq_t, (i, y), x * T, T), y) for y in range(4)])

        att = {}

        def job_weights(row, r, release):
            base = HALO + row * RO + r
            qs = [_after(release, qbuf[t, pl.ds(row * RO + r, 8), :]) for t in range(8)]
            logits = []
            for w in range(WIN):
                x = _sum([qs[t] * kbuf[t, pl.ds(base - DIL * w, 8), :] for t in range(8)])
                x = x + pltpu.roll(x, 64, 1)
                x = x + pltpu.roll(x, 32, 1)
                if row == 0 and r < DIL * w:
                    pos = lax.broadcasted_iota(jnp.int32, (8, T), 0) + (c * CO + r)
                    x = jnp.where(pos >= DIL * w, x, MASKED)
                logits.append(x)
            m = functools.reduce(jnp.maximum, logits)
            p = [jnp.exp2(x - m) for x in logits]
            inv = _inverse(_sum(p))
            att[row, r] = [x * inv for x in p]
            return tok.of(att[row, r][0])

        def job_values(row, r, release):
            base = HALO + row * RO + r
            p = [_after(release, x) for x in att[row, r]]
            att[row, r] = [_sum([p[w] * vbuf[t, pl.ds(base - DIL * w, 8), :] for w in range(WIN)])
                           for t in range(8)]
            return tok.of(*att[row, r])

        def job_o(n, r, i):
            def block(row, col):
                return _cat([att[row, r][2 * col + n], att[row, r + 8][2 * col + n]], axis=0)
            for x, val in enumerate(_terms2(LHS, i, block)):
                o_t[7 * i + x, n, pl.ds(r, 16), :] = val.astype(BF16)
            return tok.stored(o_t, (7 * i + 6, n), r)

        groups = [(row, r + x) for r in range(0, RO, 16) for row in range(4) for x in (0, 8)]
        w0, w1, v0, v1 = t_v + 300, t_b + 3500, t_b + 2500, t_o - 700
        for g, (row, r) in enumerate(groups):
            begin = w0 + (w1 - w0) * g // len(groups)
            schedule(P(job_weights, row, r), begin, begin + 700, release=True)
            begin = max(v0 + (v1 - v0) * g // len(groups), begin + 700)
            schedule(P(job_values, row, r), begin, begin + 300, release=True)
            if g % 8 == 7:
                for x, (n, i) in enumerate((n, i) for n in range(2) for i in range(7)):
                    schedule(P(job_o, n, r - 8, i), begin, min(begin + 500 + 60 * (x + 1), t_o))
        project2(ax_t, 9, wakv_t, 2, P(write_rows, vbuf), t_b, t_b + 1500)

        touched = {}

        def project_b(i):
            m = []

            def accumulate(y, inner):
                val = _combine([x[y] for x in m])[inner]
                token = None
                for outer, sign in OUT[i]:
                    row, col = 2 * (outer // 2) + inner // 2, 2 * (2 * (outer % 2) + inner % 2) + y
                    rows = pl.ds(row * RO, RO)
                    total = val
                    if (outer, inner, y) in touched:
                        total = acc[col, rows, :] + val if sign > 0 else acc[col, rows, :] - val
                    touched[outer, inner, y] = True
                    if any(outer == n for x in range(i + 1, 7) for n, _ in OUT[x]):
                        acc[col, rows, :] = total
                        token = tok.stored(acc, (col,), row * RO)
                    else:
                        obuf[slot, rows, pl.ds(DM + col * T, T)] = total.astype(BF16)
                        if token is None:
                            token = tok.of(_fold(jnp.add, total))
                return token

            parts = [(y, inner) for y in range(2) for inner in range(4)]
            done = starts[clock[0] + 7]
            if i < 6:
                for x, part in enumerate(parts):
                    schedule(P(accumulate, *part), done, done + 256 + 150 * x)
            for n in range(7):
                def quad(kt, x):
                    return (i, 2 * kt + x % 2), (2 * c + x // 2) * RO
                if len(LHS[n]) == 1:
                    a = [_words(ctx_t, *quad(kt, LHS[n][0][0]), RO) for kt in range(8)]
                else:
                    a = [_term(LHS, n, lambda x: _load(ctx_t, *quad(kt, x), RO).astype(F32))
                         for kt in range(8)]
                step(m, a, [P(lambda y, x: _load(wob_t, (7 * i + n, y), x * T, T), y) for y in range(2)])
            if i == 6:
                for part in parts:
                    accumulate(*part)

        for i in range(6):
            project_b(i)

        for x, job in enumerate(AX_JOBS):
            schedule(P(_job_ax, tok, lambda val: val, ax_raw, ax_t, 1 - slot, *job),
                     t_o, t_o + 100 + 3600 * (x + 1) // len(AX_JOBS))
        upper = {}

        def write_out(blocks, y, r):
            if r % 16 == 0:
                upper[y] = blocks
                return
            for row in range(4):
                for col in range(4):
                    val = _cat([upper[y][row][col], blocks[row][col]], axis=0)
                    obuf[slot, pl.ds(row * RO + r - 8, 16), pl.ds((2 * col + y) * T, T)] = val.astype(BF16)

        project2(o_t, 7, wo_t, 0, write_out, t_last, starts[-2])
        project_b(6)
        assert not plan and not due
        out_copy(c, slot).start()
        ax_copy(jnp.minimum(c + 2, NO - 1), slot).wait()

        @pl.when(c < NO - 1)
        def _():
            ax_copy(jnp.minimum(c + 3, NO - 1), 1 - slot).start()

        @pl.when(c >= 1)
        def _():
            out_copy(c - 1, 1 - slot).wait()

    ax_copy(1, 1).wait()
    ax_copy(2, 0).start()
    lax.fori_loop(0, NO, chunk_body, None)
    out_copy(NO - 1, (NO - 1) % 2).wait()


def _kernel(ax_hbm, wqkv_hbm, wo_hbm, bx_hbm, c_hbm, wq_hbm, wuk_hbm, wuv_hbm, wob_hbm, out_hbm,
            ax_raw, ax_t, ctx_t, wob_t, waq_t, wakv_t, wo_t, zero_smem, sem_ax):
    vmem, dma = pltpu.VMEM, pltpu.SemaphoreType.DMA

    def clear(i, carry):
        zero_smem[0] = i >> 1
    lax.fori_loop(0, 2, clear, None)

    def ax_copy(c, slot):
        rows = pl.ds(_aligned(c * CO, CO), CO)
        return pltpu.make_async_copy(ax_hbm.at[rows, :], ax_raw.at[slot], sem_ax.at[slot])

    shared = (ax_copy, ax_raw, ax_t, ctx_t, wob_t, waq_t, wakv_t, wo_t, zero_smem)
    pl.run_scoped(
        P(_head_pairs, wqkv_hbm, wo_hbm, bx_hbm, c_hbm, wq_hbm, wuk_hbm, wuv_hbm, wob_hbm, *shared),
        vmem((S, DM), BF16),
        vmem((S, DC), BF16),
        vmem((2, DM, T), U32),
        vmem((2, DC, T), U32),
        vmem((2, DC, T), U32),
        vmem((2, 4, 64, DM), BF16),
        vmem((2, 4, 8, 3 * DM), U32),
        vmem((16, NH, DM), U32),
        vmem((7, 4, S // 2, T), BF16),
        vmem((49, S // 4, T), BF16),
        vmem((7, DM // 2, T), BF16),
        vmem((49, T, T), BF16),
        vmem((2, 8, T), F32),
        dma((2 * S // CH,)), dma((11,)))
    pl.run_scoped(
        P(_outputs, out_hbm, *shared),
        vmem((49, 2, RO, T), BF16),
        vmem((8, HALO + CO, T), F32),
        vmem((8, HALO + CO, T), F32),
        vmem((8, CO, T), F32),
        vmem((8, CO, T), F32),
        vmem((2, CO, 2 * DM), BF16),
        dma((2,)))


@jax.jit
def pallas_concat_heads__sliding_local_dilated__compressed_kv_cla__prompt_kernel(
    A_x: jax.Array,
    A_wqkv: jax.Array,
    A_wo: jax.Array,
    B_x: jax.Array,
    B_c_kv: jax.Array,
    B_w_q: jax.Array,
    B_w_uk: jax.Array,
    B_w_uv: jax.Array,
    B_w_o: jax.Array,
):
    vmem = pltpu.VMEM
    out = pl.pallas_call(
        _kernel,
        out_shape=jax.ShapeDtypeStruct((S, 2 * DM), BF16),
        in_specs=[pl.BlockSpec(memory_space=pl.ANY)] * 9,
        out_specs=pl.BlockSpec(memory_space=pl.ANY),
        scratch_shapes=[
            vmem((2, CO, DM), BF16),
            vmem((63, 2, RO, T), BF16),
            vmem((7, NP, S // 2, T), BF16),
            vmem((49, 2, DM, T), BF16),
            vmem((7, 4, DM // 2, T), BF16),
            vmem((49, 4, 2 * T, T), BF16),
            vmem((49, 2, 2 * T, T), BF16),
            pltpu.SMEM((1,), jnp.int32),
            pltpu.SemaphoreType.DMA((2,)),
        ],
        compiler_params=pltpu.CompilerParams(
            vmem_limit_bytes=124 * 2**20, disable_bounds_checks=True),
    )(
        A_x.reshape(S, DM),
        A_wqkv.reshape(4, DM // 4, 3 * DM),
        A_wo.reshape(NH, DM // NH, DM),
        B_x.reshape(S, DM),
        B_c_kv.reshape(S, DC),
        B_w_q,
        B_w_uk,
        B_w_uv,
        B_w_o,
    )
    return out.reshape(1, S, 2 * DM)
```

```python
import functools
import math

import jax
import jax.numpy as jnp
from jax import lax
import jax.experimental.pallas as pl
import jax.experimental.pallas.tpu as pltpu

S = 2048
DM = 1024
DC = 512
NH = 32
NP = NH // 2
T = 128
CH = 4 * T
RO = 64
CO = 4 * RO
NO = S // CO
WIN, DIL = 8, 2
HALO = 16

LOG2E = math.log2(math.e)
SCALE_A = (DM // NH) ** -0.5 * LOG2E
SCALE_B = T ** -0.5 * LOG2E
MASKED = -1e9 * LOG2E
SAFE_SUM = 2.0 ** 40

DEPTH = 3
JOB_TILES = 16
CTX_TILES = 12, 20

F32, BF16, U32 = jnp.float32, jnp.bfloat16, jnp.uint32
P = functools.partial


def _dot(a, b):
    return jnp.dot(a, b, preferred_element_type=F32)


def _dot_nt(a, b):
    return lax.dot_general(a, b, (((1,), (1,)), ((), ())), preferred_element_type=F32)


def _cat(xs, axis=1):
    return xs[0] if len(xs) == 1 else jnp.concatenate(xs, axis=axis)


def _sum(xs):
    return functools.reduce(jnp.add, xs)


def _fold(op, x):
    return functools.reduce(op, [x[r:r + 8] for r in range(0, x.shape[0], 8)])


def _aligned(x, n):
    return x if isinstance(x, int) else pl.multiple_of(x, n)


def _rows(start, n):
    return pl.ds(_aligned(start, 16), n)


def _words(ref, lead, start, n):
    return ref.bitcast(U32)[(*lead, pl.ds(_aligned(start >> 1, 8), n // 2), slice(None))]


def _load(ref, lead, start, n):
    return pltpu.bitcast(_words(ref, lead, start, n), BF16)


def _split(w):
    return (pltpu.bitcast(w << 16, F32), pltpu.bitcast(w & jnp.uint32(0xFFFF0000), F32))


def _inverse(l):
    r = pl.reciprocal(l, approx=True)
    return r * (2.0 - l * r)


def _interleave(x, y):
    order = [((n + 0.5) / len(z), m, job) for m, z in enumerate((x, y)) for n, job in enumerate(z)]
    return [job for _, _, job in sorted(order, key=lambda e: e[:2])]


def _start(*copies):
    for cp in copies:
        cp.start()


def _wait(*copies):
    for cp in copies:
        cp.wait()


LHS = (((0, 1), (3, 1)), ((2, 1), (3, 1)), ((0, 1),), ((3, 1),),
       ((0, 1), (1, 1)), ((2, 1), (0, -1)), ((1, 1), (3, -1)))
RHS = (((0, 1), (3, 1)), ((0, 1),), ((1, 1), (3, -1)), ((2, 1), (0, -1)),
       ((3, 1),), ((0, 1), (1, 1)), ((2, 1), (3, 1)))
OUT = (((0, 1), (3, 1)), ((2, 1), (3, -1)), ((1, 1), (3, 1)), ((0, 1), (2, 1)),
       ((0, -1), (1, 1)), ((3, 1),), ((0, 1),))


def _term(table, i, quad):
    (n, _), *rest = table[i]
    val = quad(n)
    for n, sign in rest:
        val = val + quad(n) if sign > 0 else val - quad(n)
    return val


def _terms(table, quad):
    blocks = [quad(n) for n in range(4)]
    return [_term(table, i, blocks.__getitem__) for i in range(7)]


def _outer_term(table, i, block):
    return [_term(table, i, lambda m: block(2 * (m // 2) + n // 2, 2 * (m % 2) + n % 2))
            for n in range(4)]


def _terms2(table, i, block):
    return _terms(table, _outer_term(table, i, block).__getitem__)


def _combine(m):
    out = [None] * 4
    for i in range(7):
        for n, sign in OUT[i]:
            if out[n] is None:
                out[n] = m[i]
            else:
                out[n] = out[n] + m[i] if sign > 0 else out[n] - m[i]
    return out


def _combine2(m):
    inner = [_combine(m[7 * i:7 * i + 7]) for i in range(7)]
    out = [[None] * 4 for _ in range(4)]
    for n in range(4):
        for quad, val in enumerate(_combine([x[n] for x in inner])):
            out[2 * (quad // 2) + n // 2][2 * (quad % 2) + n % 2] = val
    return out


class _Tokens:
    def __init__(self, zero_smem):
        self.z = zero_smem[0]
        self.zero = jnp.full((8, T), self.z, jnp.int32).astype(U32)

    def stored(self, ref, lead, start):
        first, *rest = lead
        if ref.dtype == BF16:
            return _words(ref, (first - (self.z & 1), *rest), start, 16) & self.zero
        return self.of(ref[(*lead, pl.ds(_aligned(start + 8 * (self.z & 1), 8), 8), slice(None))])

    def of(self, *vals):
        return pltpu.bitcast(_sum(vals), U32) & self.zero


def _after(token, x, everywhere=False):
    if token is None:
        return x
    bits = x if x.dtype == U32 else pltpu.bitcast(x, U32)
    cut = bits.shape[0] if everywhere else 8
    parts = [bits[r:r + 8] | token for r in range(0, cut, 8)]
    bits = _cat(parts + ([bits[cut:]] if cut < bits.shape[0] else []), axis=0)
    return bits if x.dtype == U32 else pltpu.bitcast(bits, x.dtype)


AX_JOBS = [(i, n, r) for n in range(2) for r in range(0, RO, 16) for i in range(7)]


def _job_ax(tok, released, ax_raw, ax_t, src, i, n, r):
    outer = _outer_term(LHS, i, lambda row, col: released(
        ax_raw[src, pl.ds(row * RO + r, 16), pl.ds((2 * col + n) * T, T)].astype(F32)))
    for x, val in enumerate(_terms(LHS, outer.__getitem__) + outer[1:3]):
        ax_t[9 * i + x, n, pl.ds(r, 16), :] = val.astype(BF16)
    return tok.stored(ax_t, (9 * i + 8, n), r)


def _head_pairs(wqkv_hbm, wo_hbm, bx_hbm, c_hbm, wq_hbm, wuk_hbm, wuv_hbm, wob_hbm,
                ax_copy, ax_raw, ax_t, ctx_t, wob_t, waq_t, wakv_t, wo_t, zero_smem,
                bx_raw, c_raw, wq_raw, wk_raw, wv_raw, wob_raw, wqkv_raw, wo_raw,
                bx_t, c_t, wq_t, wkv_t, guard, sem_in, sem_w):
    def head_copies(j, slot):
        return [pltpu.make_async_copy(src.bitcast(U32).at[:, j, :], dst.at[slot], sem_w.at[3 * slot + n])
                for n, (src, dst) in enumerate(((wuk_hbm, wk_raw), (wuv_hbm, wv_raw), (wq_hbm, wq_raw)))]

    def side_copies(j, slot):
        wob = wob_hbm.at[pl.ds(4 * (j >> 1), 4), pl.ds(_aligned((j & 1) * 64, 64), 64), :]
        wqkv = wqkv_hbm.bitcast(U32).at[:, pl.ds(_aligned(8 * j, 8), 8), :]
        return [pltpu.make_async_copy(wob, wob_raw.at[slot], sem_w.at[6 + 2 * slot]),
                pltpu.make_async_copy(wqkv, wqkv_raw.at[slot], sem_w.at[7 + 2 * slot])]

    def wo_copy(word):
        return pltpu.make_async_copy(wo_hbm.bitcast(U32).at[:, word, :], wo_raw.at[word], sem_w.at[10])

    def c_copy(c):
        rows = pl.ds(c * CH, CH)
        return pltpu.make_async_copy(c_hbm.at[rows, :], c_raw.at[rows, :], sem_in.at[2 * c])

    def x_copy(c):
        rows = pl.ds(c * CH, CH)
        return pltpu.make_async_copy(bx_hbm.at[rows, :], bx_raw.at[rows, :], sem_in.at[2 * c + 1])

    def pair_body(j, first=False):
        slot = j & 1
        tok = _Tokens(zero_smem)
        causal = (lax.broadcasted_iota(jnp.int32, (T, T), 1)
                  <= lax.broadcasted_iota(jnp.int32, (T, T), 0))

        jobs, pace = [], dict(period=0, clock=0, release=None)

        def queue(cycles, more):
            pace.update(period=cycles / len(more), clock=0)
            jobs.extend(more)

        def flush():
            while jobs:
                jobs.pop(0)()

        def background(cycles, recent=None):
            pace["clock"] += cycles
            token = None
            while jobs and pace["clock"] >= pace["period"]:
                pace["clock"] -= pace["period"]
                pace["release"] = None if recent is None else tok.of(recent[:8])
                new = jobs.pop(0)()
                pace["release"] = None
                token = new if token is None else token | new
            return token

        def released(x):
            return _after(pace["release"], x, everywhere=True)

        def store_terms(dst, first_term, lead, row, terms):
            for i, val in enumerate(terms):
                dst[(first_term + i, *lead, _rows(row, 16), slice(None))] = val.astype(BF16)
            return tok.stored(dst, (first_term + 6, *lead), row)

        def job_x(c, t, r):
            terms = _terms(LHS, lambda m: bx_raw[pl.ds(c * CH + (m // 2) * 2 * T + r, 16),
                                                 pl.ds((4 * (m % 2) + t) * T, T)].astype(F32))
            return store_terms(bx_t, 0, (t,), c * 2 * T + r, terms)

        def job_c(c, i, r):
            terms = _terms2(LHS, i, lambda row, col: c_raw[
                pl.ds(c * CH + row * T + r, 16), pl.ds(col * T, T)].astype(F32))
            return store_terms(c_t, 7 * i, (), c * T + r, terms)

        def jobs_x(c):
            return [P(job_x, c, t, r) for r in range(0, 2 * T, 16) for t in range(4)]

        def jobs_c(c):
            return [P(job_c, c, i, r) for r in range(0, T, 16) for i in range(7)]

        def job_wkv(src, i, r):
            def block(row, col):
                raw = (wk_raw, wv_raw)[col % 2]
                return _split(released(raw[src, pl.ds(row * T + r, 16), :]))[col // 2]
            return store_terms(wkv_t, 7 * i, (), r, _terms2(RHS, i, block))

        def job_wq(src, r):
            top, bottom = (_split(released(wq_raw[src, pl.ds(row + r, 16), :])) for row in (0, DM // 2))
            return store_terms(wq_t, 0, (), r, _terms(RHS, (top + bottom).__getitem__))

        def jobs_wkv(src):
            return [P(job_wkv, src, i, r) for r in range(0, T, 16) for i in range(7)]

        def jobs_wq(src):
            return [P(job_wq, src, r) for r in range(0, DM // 2, 16)]

        def job_wob(i, n, r):
            def block(row, col):
                head = 2 * (row % 2) + row // 2
                return released(wob_raw[slot, head, pl.ds(r, 16), pl.ds((2 * col + n) * T, T)].astype(F32))
            return store_terms(wob_t, 7 * i, (n,), j * 64 + r, _terms2(RHS, i, block))

        def job_wo(i, n):
            e, odd, head = j & 3, (j >> 2) & 1, 16 * (j >> 3)

            def block(row, col):
                even_t, odd_t = _split(released(
                    wo_raw[4 * e + row, _rows(head, 16), pl.ds((2 * col + n) * T, T)]))
                return jnp.where(odd == 1, odd_t, even_t)
            return store_terms(wo_t, 7 * i, (n,), odd * T + e * NH + head, _terms2(RHS, i, block))

        permuted = {}

        def job_permute(mat):
            lane = lax.broadcasted_iota(jnp.int32, (32, T), 1)
            e, grp, sub = lane >> 5, (lane >> 2) & 7, lane & 3

            def gather(x, index):
                return jnp.take_along_axis(x, index, axis=1, mode="promise_in_bounds")
            x = [released(wqkv_raw[slot, :, :, pl.ds(mat * DM + t * T, T)].reshape(32, T))
                 for t in range(8)]
            y = [gather(x[t], sub * 32 + e * 8 + ((grp - t) & 7)) for t in range(8)]
            u = [y[-s % 8] for s in range(8)]
            for bit in (1, 2, 4):
                u = [jnp.where((grp & bit) != 0, u[(s - bit) % 8], u[s]) for s in range(8)]
            u = [u[0]] + [gather(u[t], e * 32 + ((grp + t) & 7) * 4 + sub) for t in range(1, 8)]
            permuted[mat] = u
            return _fold(jnp.bitwise_or, functools.reduce(jnp.bitwise_or, u)) & tok.zero

        def column(mat, row, t):
            return pltpu.bitcast(released(permuted[mat][t][8 * row:8 * row + 8]), BF16).astype(F32)

        def job_waq(half, n):
            terms = _terms(RHS, lambda m: column(0, 2 * (m // 2) + half, 4 * (m % 2) + n))
            return store_terms(waq_t, 0, (n,), half * 2 * T + 16 * j, terms)

        def job_wakv(mat, i, n):
            terms = _terms2(RHS, i, lambda row, col: column(mat, row, 2 * col + n))
            return store_terms(wakv_t, 7 * i, (2 * (mat - 1) + n,), 16 * j, terms)

        pause = [lambda: tok.zero] * 2
        jobs_wob = [P(job_wob, i, n, r) for r in range(0, 64, 16) for n in range(2) for i in range(7)]
        jobs_wo = [P(job_wo, i, n) for n in range(2) for i in range(7)]
        jobs_wa = [P(job_permute, 0)] + pause + [P(job_waq, half, n) for half in range(2) for n in range(4)]
        for mat in (1, 2):
            jobs_wa += [P(job_permute, mat)] + pause
            jobs_wa += [P(job_wakv, mat, i, n) for n in range(2) for i in range(7)]

        q, k, v = {}, {}, {}

        def project_q(c):
            m = [_dot(_cat([_load(bx_t, (i, t), c * 2 * T, 2 * T) for t in range(4)]),
                      _load(wq_t, (i,), 0, DM // 2)) for i in range(7)]
            for n, val in enumerate(_combine(m)):
                val = val * SCALE_B
                for r in range(2):
                    q[4 * c + 2 * (n // 2) + r, n % 2] = val[r * T:(r + 1) * T].astype(BF16)

        def project_kv(c):
            m = [_dot(_load(c_t, (i,), c * T, T), _load(wkv_t, (i,), 0, T)) for i in range(49)]
            for r, row in enumerate(_combine2(m)):
                for n, val in enumerate(row):
                    (k, v)[n % 2][4 * c + r, n // 2] = val.astype(BF16)

        def plain(raw, c, weights):
            def operand():
                parts = []
                for r in range(c * CH, (c + 1) * CH, 32):
                    part = raw[pl.ds(r, 32), :]
                    token = background(8 * (raw.shape[1] // T))
                    if token is not None:
                        part = _cat([_after(_cat([token, token]), part[:, :2 * T]), part[:, 2 * T:]])
                    parts.append(part)
                return _cat(parts, axis=0)
            return [_dot(operand(), w) for w in weights]

        def plain_kv(c, weights):
            for n, val in enumerate(plain(c_raw, c, weights)):
                for r in range(4):
                    (k, v)[n // 2][4 * c + r, n % 2] = val[r * T:(r + 1) * T].astype(BF16)

        def plain_q(c, weights):
            for h, val in enumerate(plain(bx_raw, c, weights)):
                for r in range(4):
                    q[4 * c + r, h] = (val[r * T:(r + 1) * T] * SCALE_B).astype(BF16)

        in_flight, partial, ctx, spread, checks, due = [], {}, {}, {}, [], []

        def finish(i, h):
            l, o = partial.pop((i, h))
            l = jnp.sum(l, axis=1, keepdims=True)
            r = _inverse(l)
            ctx[i, h] = o * r
            spread[i, h] = _fold(jnp.maximum, jnp.broadcast_to(l + r, (T, T)))
            b = i // 2
            quad = [(2 * b, 0), (2 * b, 1), (2 * b + 1, 0), (2 * b + 1, 1)]
            if all(u in ctx for u in quad):
                terms = _terms(LHS, lambda m: ctx.pop(quad[m]))
                for n, val in enumerate(terms):
                    ctx_t[n, j, pl.ds(b * T, T), :] = val.astype(BF16)
                checks.append((_fold(jnp.add, terms[0] + terms[5] + terms[6]),
                               functools.reduce(jnp.maximum, [spread.pop(u) for u in quad])))
                due.append([CTX_TILES[first], tok.stored(ctx_t, (6, j), b * T) | tok.of(*checks[-1])])

        def weigh(i, h, t, p):
            l, o = partial.get((i, h), (None, None))
            l = p if l is None else l + p
            token = background(64, p)
            if token is not None:
                due.append([JOB_TILES, token])
            for entry in due:
                entry[0] -= 1
            now = [token for left, token in due if left <= 0]
            due[:] = [entry for entry in due if entry[0] > 0]
            if now:
                p = _after(functools.reduce(jnp.bitwise_or, now), p)
            d = _dot(p.astype(BF16), v[t, h])
            partial[i, h] = (l, d if o is None else o + d)
            if t == i:
                finish(i, h)

        def attention(lo, hi):
            for i in range(lo, hi):
                for h in range(2):
                    for t in range(i + 1):
                        s = _dot_nt(q[i, h], k[t, h])
                        if t == i:
                            s = jnp.where(causal, s, MASKED)
                        in_flight.append((i, h, t, jnp.exp2(s)))
                        if len(in_flight) > DEPTH:
                            weigh(*in_flight.pop(0))
            while hi == S // T and in_flight:
                weigh(*in_flight.pop(0))

        def cycles(lo, hi):
            return 2 * 64 * sum(range(lo + 1, hi + 1))

        if first:
            wk, wv, wq = head_copies(0, 0)
            _start(wv, wk, c_copy(0), c_copy(1))
            _wait(wv, wk, c_copy(0))
            _start(c_copy(2), c_copy(3), x_copy(0), wq)
            weights = [w.astype(BF16) for raw in (wk_raw, wv_raw) for w in _split(raw[0])]
            queue(0.98 * 2048, jobs_c(0))
            plain_kv(0, weights)
            flush()
            _wait(c_copy(1), c_copy(2))
            _start(x_copy(1), x_copy(2))
            queue(0.98 * 4096, jobs_c(1) + jobs_c(2))
            plain_kv(1, weights)
            plain_kv(2, weights)
            flush()
            _wait(c_copy(3))
            queue(0.98 * 2048, jobs_c(3))
            plain_kv(3, weights)
            flush()
            _wait(x_copy(0), wq)
            weights = [w.astype(BF16) for w in _split(wq_raw[0])]
            queue(0.92 * (2048 + cycles(0, 4)), jobs_wq(0) + jobs_x(0))
            plain_q(0, weights)
            attention(0, 4)
            flush()
            _wait(x_copy(1), x_copy(2))
            stage = [x_copy(3), *side_copies(0, 0), *head_copies(1, 1)]
            _start(*stage)
            lax.fori_loop(0, 16, lambda word, carry: wo_copy(word).start(), None)
            queue(0.98 * (2048 + cycles(4, 8)), jobs_x(2) + jobs_x(1))
            plain_q(1, weights)
            attention(4, 8)
            flush()
            project_q(2)
            attention(8, 9)
            _wait(*stage)
            _start(ax_copy(0, 0), *head_copies(2, 0), *side_copies(1, 1))
            queue(0.92 * cycles(9, 14), jobs_x(3) + _interleave(_interleave(jobs_wob, jobs_wa), jobs_wkv(1)))
            attention(9, 12)
            assert not any(getattr(job, "func", None) is job_x for job in jobs)
            project_q(3)
            attention(12, 14)
            flush()
            _wait(*[wo_copy(word) for word in range(16)], ax_copy(0, 0))
            _start(ax_copy(1, 1))
            queue(0.92 * cycles(14, 16),
                  _interleave(jobs_wo + jobs_wq(1),
                              [P(_job_ax, tok, released, ax_raw, ax_t, 0, *job) for job in AX_JOBS]))
            attention(14, 16)
            flush()
        else:
            queue(0.98 * cycles(0, 12), _interleave(jobs_wob, jobs_wo + jobs_wa))
            project_kv(0)
            project_q(0)
            project_kv(1)
            attention(0, 4)
            project_q(1)
            attention(4, 8)
            project_kv(2)
            project_q(2)
            attention(8, 10)
            project_kv(3)
            attention(10, 12)
            flush()
            project_q(3)
            queue(0.7 * cycles(12, 16), _interleave(jobs_wkv(1 - slot), jobs_wq(1 - slot)))
            attention(12, 16)
            flush()
        guard[0] = _sum([guard[0]] + [x for x, _ in checks])
        guard[1] = functools.reduce(jnp.maximum, [guard[1]] + [x for _, x in checks])

        def ahead(n):
            return j + n if first else jnp.minimum(j + n, NP - 1)
        _wait(*head_copies(ahead(2), slot), *side_copies(ahead(1), 1 - slot))

        @pl.when(j < NP - 1)
        def _():
            _start(*head_copies(ahead(3), 1 - slot), *side_copies(ahead(2), slot))

    def exact_pairs(qkv, ctx):
        def block(i):
            return pl.ds(pl.multiple_of(i * T, T), T)

        def head(h, carry):
            def weight(raw):
                even, odd = _split(raw[0])
                return jnp.where(h == 0, even, odd).astype(BF16)
            wk, wv, wq = weight(wk_raw), weight(wv_raw), weight(wq_raw)

            def project(i, carry):
                qkv[0, block(i), :] = (_dot(bx_raw[block(i), :], wq) * SCALE_B).astype(BF16)
                qkv[1, block(i), :] = _dot(c_raw[block(i), :], wk).astype(BF16)
                qkv[2, block(i), :] = _dot(c_raw[block(i), :], wv).astype(BF16)
            lax.fori_loop(0, S // T, project, None)

            def attend(i, carry):
                def scores(t):
                    row = lax.broadcasted_iota(jnp.int32, (T, T), 0) + i * T
                    col = lax.broadcasted_iota(jnp.int32, (T, T), 1) + t * T
                    return jnp.where(col <= row, _dot_nt(qkv[0, block(i), :], qkv[1, block(t), :]), MASKED)

                m = lax.fori_loop(
                    0, i + 1, lambda t, m: jnp.maximum(m, jnp.max(scores(t), axis=1, keepdims=True)),
                    jnp.full((T, 1), -jnp.inf, F32))

                def accumulate(t, carry):
                    l, o = carry
                    p = jnp.exp2(scores(t) - m)
                    return (l + jnp.sum(p, axis=1, keepdims=True),
                            o + _dot(p.astype(BF16), qkv[2, block(t), :]))
                l, o = lax.fori_loop(0, i + 1, accumulate,
                                     (jnp.zeros((T, 1), F32), jnp.zeros((T, T), F32)))
                ctx[h, block(i), :] = o / l
            lax.fori_loop(0, S // T, attend, None)

        def pair(j, carry):
            _start(*head_copies(j, 0))
            _wait(*head_copies(j, 0))
            lax.fori_loop(0, 2, head, None)

            def store(b, carry):
                for n, val in enumerate(_terms(LHS, lambda m: ctx[m % 2, block(2 * b + m // 2), :])):
                    ctx_t[n, j, block(b), :] = val.astype(BF16)
            lax.fori_loop(0, S // T // 2, store, None)

        lax.fori_loop(0, NP, pair, None)

    guard[...] = jnp.zeros(guard.shape, F32)
    pair_body(0, first=True)
    lax.fori_loop(1, NP, lambda j, carry: pair_body(j), None)

    safe = jnp.logical_and(jnp.abs(guard[0]) < jnp.inf, guard[1] < SAFE_SUM)

    @pl.when(jnp.max(jnp.where(safe, 0.0, 1.0)) > 0.0)
    def _():
        pl.run_scoped(exact_pairs, pltpu.VMEM((3, S, T), BF16), pltpu.VMEM((2, S, T), F32))


def _outputs(out_hbm, ax_copy, ax_raw, ax_t, ctx_t, wob_t, waq_t, wakv_t, wo_t, zero_smem,
             o_t, kbuf, vbuf, qbuf, acc, obuf, sem_out):
    def out_copy(c, slot):
        rows = pl.ds(_aligned(c * CO, CO), CO)
        return pltpu.make_async_copy(obuf.at[slot], out_hbm.at[rows, :], sem_out.at[slot])

    for buf in (kbuf, vbuf):
        for t in range(8):
            buf[t, pl.ds(CO, HALO), :] = jnp.zeros((HALO, T), F32)

    costs = [RO] * 49 + [4 * RO] * 14 + [RO] * 49 + [4 * RO] * 42 + [RO] * 49 + [4 * RO] * 7
    starts = [sum(costs[:n]) for n in range(len(costs) + 1)]
    t_q, t_v, t_b, t_o, t_last = (starts[n] for n in (49, 63, 112, 154, 203))

    def chunk_body(c, carry):
        slot = c & 1
        tok = _Tokens(zero_smem)
        plan, due, clock = {}, {}, [0]

        def schedule(job, begin, end, release=False):
            first = max([clock[0]] + [n for n in range(len(costs)) if starts[n + 1] <= begin])
            last = min(n for n in range(len(costs)) if starts[n] >= end)
            plan.setdefault(first, []).append((job, last, release))

        def step(results, a, w):
            n = clock[0]
            clock[0] += 1
            for x, token in enumerate(due.pop(n, [])):
                a[x % len(a)] = _after(token, a[x % len(a)])
            a = [x.astype(BF16) if x.dtype == F32 else pltpu.bitcast(x, BF16) for x in a]
            res = [None] * len(w)
            for x in range(len(a)):
                for y in range(len(w)):
                    d = _dot(a[x], w[y](x))
                    res[y] = d if res[y] is None else res[y] + d
            results.append(res)
            token = None
            for job, last, release in plan.pop(n, []):
                if release and token is None:
                    token = tok.of(res[0][:8])
                due.setdefault(last, []).append(job(token) if release else job())

        def project2(lhs_t, stride, rhs_t, tile0, write, begin, end):
            m = []

            def recombine(y, r):
                blocks = _combine2([x[y][r:r + 8] for x in m])
                write(blocks, y, r)
                return tok.of(*[x for row in blocks for x in row])

            slabs = [(y, r) for r in range(0, RO, 8) for y in range(2)]
            for x, slab in enumerate(slabs):
                schedule(P(recombine, *slab), begin, begin + (end - begin) * (x + 1) // len(slabs))
            for i in range(49):
                step(m, [_words(lhs_t, (stride * (i // 7) + i % 7, x), 0, RO) for x in range(2)],
                     [P(lambda y, x: _load(rhs_t, (i, tile0 + y), x * T, T), y) for y in range(2)])

        for buf in (kbuf, vbuf):
            for t in range(8):
                buf[t, pl.ds(0, HALO), :] = buf[t, pl.ds(CO, HALO), :]

        def write_rows(buf, blocks, y, r):
            for row in range(4):
                for col in range(4):
                    buf[2 * col + y, pl.ds(HALO + row * RO + r, 8), :] = blocks[row][col]

        def write_q(m, half, y):
            vals = [val * SCALE_A for val in _combine([x[y] for x in m])]
            for quad, val in enumerate(vals):
                qbuf[4 * (quad % 2) + y, pl.ds((2 * (quad // 2) + half) * RO, RO), :] = val
            return tok.of(*[val[r:r + 8] for val in vals for r in range(0, RO, 8)])

        project2(ax_t, 9, wakv_t, 0, P(write_rows, kbuf), t_q, t_v - 1000)
        for half in range(2):
            m = []
            done = t_q + (t_v - t_q) * (half + 1) // 2
            for y in range(4):
                schedule(P(write_q, m, half, y), done, done + 200 + 200 * y)
            for i in range(7):
                a = [_words(ax_t, (9 * i + x, n), 0, RO) for x in ((2, 7), (8, 3))[half] for n in range(2)]
                step(m, a, [P(lambda y, x: _load(waq_t, (i, y), x * T, T), y) for y in range(4)])

        att = {}

        def job_weights(row, r, release):
            base = HALO + row * RO + r
            qs = [_after(release, qbuf[t, pl.ds(row * RO + r, 8), :]) for t in range(8)]
            logits = []
            for w in range(WIN):
                x = _sum([qs[t] * kbuf[t, pl.ds(base - DIL * w, 8), :] for t in range(8)])
                x = x + pltpu.roll(x, 64, 1)
                x = x + pltpu.roll(x, 32, 1)
                if row == 0 and r < DIL * w:
                    pos = lax.broadcasted_iota(jnp.int32, (8, T), 0) + (c * CO + r)
                    x = jnp.where(pos >= DIL * w, x, MASKED)
                logits.append(x)
            m = functools.reduce(jnp.maximum, logits)
            p = [jnp.exp2(x - m) for x in logits]
            inv = _inverse(_sum(p))
            att[row, r] = [x * inv for x in p]
            return tok.of(att[row, r][0])

        def job_values(row, r, release):
            base = HALO + row * RO + r
            p = [_after(release, x) for x in att[row, r]]
            att[row, r] = [_sum([p[w] * vbuf[t, pl.ds(base - DIL * w, 8), :] for w in range(WIN)])
                           for t in range(8)]
            return tok.of(*att[row, r])

        def job_o(n, r, i):
            def block(row, col):
                return _cat([att[row, r][2 * col + n], att[row, r + 8][2 * col + n]], axis=0)
            for x, val in enumerate(_terms2(LHS, i, block)):
                o_t[7 * i + x, n, pl.ds(r, 16), :] = val.astype(BF16)
            return tok.stored(o_t, (7 * i + 6, n), r)

        groups = [(row, r + x) for r in range(0, RO, 16) for row in (0, 2, 1, 3) for x in (0, 8)]
        w0, w1, v0, v1 = t_v + 300, t_b + 3500, t_b + 2500, t_o - 700
        for g, (row, r) in enumerate(groups):
            begin = w0 + (w1 - w0) * g // len(groups)
            schedule(P(job_weights, row, r), begin, begin + 700, release=True)
            begin = max(v0 + (v1 - v0) * g // len(groups), begin + 700)
            schedule(P(job_values, row, r), begin, begin + 300, release=True)
            if g % 8 == 7:
                for x, (n, i) in enumerate((n, i) for n in range(2) for i in range(7)):
                    schedule(P(job_o, n, r - 8, i), begin, min(begin + 500 + 60 * (x + 1), t_o))
        project2(ax_t, 9, wakv_t, 2, P(write_rows, vbuf), t_b, t_b + 1500)

        touched = {}

        def project_b(i):
            m = []

            def accumulate(y, inner):
                val = _combine([x[y] for x in m])[inner]
                token = None
                for outer, sign in OUT[i]:
                    row, col = 2 * (outer // 2) + inner // 2, 2 * (2 * (outer % 2) + inner % 2) + y
                    rows = pl.ds(row * RO, RO)
                    total = val
                    if (outer, inner, y) in touched:
                        total = acc[col, rows, :] + val if sign > 0 else acc[col, rows, :] - val
                    touched[outer, inner, y] = True
                    if any(outer == n for x in range(i + 1, 7) for n, _ in OUT[x]):
                        acc[col, rows, :] = total
                        token = tok.stored(acc, (col,), row * RO)
                    else:
                        obuf[slot, rows, pl.ds(DM + col * T, T)] = total.astype(BF16)
                        if token is None:
                            token = tok.of(_fold(jnp.add, total))
                return token

            parts = [(y, inner) for y in range(2) for inner in range(4)]
            done = starts[clock[0] + 7]
            if i < 6:
                for x, part in enumerate(parts):
                    schedule(P(accumulate, *part), done, done + 256 + 150 * x)
            for n in range(7):
                def quad(kt, x):
                    return (i, 2 * kt + x % 2), (2 * c + x // 2) * RO
                if len(LHS[n]) == 1:
                    a = [_words(ctx_t, *quad(kt, LHS[n][0][0]), RO) for kt in range(8)]
                else:
                    a = [_term(LHS, n, lambda x: _load(ctx_t, *quad(kt, x), RO).astype(F32))
                         for kt in range(8)]
                step(m, a, [P(lambda y, x: _load(wob_t, (7 * i + n, y), x * T, T), y) for y in range(2)])
            if i == 6:
                for part in parts:
                    accumulate(*part)

        for i in range(6):
            project_b(i)

        for x, job in enumerate(AX_JOBS):
            schedule(P(_job_ax, tok, lambda val: val, ax_raw, ax_t, 1 - slot, *job),
                     t_o, t_o + 100 + 3000 * (x + 1) // len(AX_JOBS))
        upper = {}

        def write_out(blocks, y, r):
            if r % 16 == 0:
                upper[y] = blocks
                return
            for row in range(4):
                for col in range(4):
                    val = _cat([upper[y][row][col], blocks[row][col]], axis=0)
                    obuf[slot, pl.ds(row * RO + r - 8, 16), pl.ds((2 * col + y) * T, T)] = val.astype(BF16)

        project2(o_t, 7, wo_t, 0, write_out, t_last, starts[-2])
        project_b(6)
        assert not plan and not due
        out_copy(c, slot).start()
        ax_copy(jnp.minimum(c + 2, NO - 1), slot).wait()

        @pl.when(c < NO - 1)
        def _():
            ax_copy(jnp.minimum(c + 3, NO - 1), 1 - slot).start()

        @pl.when(c >= 1)
        def _():
            out_copy(c - 1, 1 - slot).wait()

    ax_copy(1, 1).wait()
    ax_copy(2, 0).start()
    lax.fori_loop(0, NO, chunk_body, None)
    out_copy(NO - 1, (NO - 1) % 2).wait()


def _kernel(ax_hbm, wqkv_hbm, wo_hbm, bx_hbm, c_hbm, wq_hbm, wuk_hbm, wuv_hbm, wob_hbm, out_hbm,
            ax_raw, ax_t, ctx_t, wob_t, waq_t, wakv_t, wo_t, zero_smem, sem_ax):
    vmem, dma = pltpu.VMEM, pltpu.SemaphoreType.DMA

    def clear(i, carry):
        zero_smem[0] = i >> 1
    lax.fori_loop(0, 2, clear, None)

    def ax_copy(c, slot):
        rows = pl.ds(_aligned(c * CO, CO), CO)
        return pltpu.make_async_copy(ax_hbm.at[rows, :], ax_raw.at[slot], sem_ax.at[slot])

    shared = (ax_copy, ax_raw, ax_t, ctx_t, wob_t, waq_t, wakv_t, wo_t, zero_smem)
    pl.run_scoped(
        P(_head_pairs, wqkv_hbm, wo_hbm, bx_hbm, c_hbm, wq_hbm, wuk_hbm, wuv_hbm, wob_hbm, *shared),
        vmem((S, DM), BF16),
        vmem((S, DC), BF16),
        vmem((2, DM, T), U32),
        vmem((2, DC, T), U32),
        vmem((2, DC, T), U32),
        vmem((2, 4, 64, DM), BF16),
        vmem((2, 4, 8, 3 * DM), U32),
        vmem((16, NH, DM), U32),
        vmem((7, 4, S // 2, T), BF16),
        vmem((49, S // 4, T), BF16),
        vmem((7, DM // 2, T), BF16),
        vmem((49, T, T), BF16),
        vmem((2, 8, T), F32),
        dma((2 * S // CH,)), dma((11,)))
    pl.run_scoped(
        P(_outputs, out_hbm, *shared),
        vmem((49, 2, RO, T), BF16),
        vmem((8, HALO + CO, T), F32),
        vmem((8, HALO + CO, T), F32),
        vmem((8, CO, T), F32),
        vmem((8, CO, T), F32),
        vmem((2, CO, 2 * DM), BF16),
        dma((2,)))


@jax.jit
def pallas_concat_heads__sliding_local_dilated__compressed_kv_cla__prompt_kernel(
    A_x: jax.Array,
    A_wqkv: jax.Array,
    A_wo: jax.Array,
    B_x: jax.Array,
    B_c_kv: jax.Array,
    B_w_q: jax.Array,
    B_w_uk: jax.Array,
    B_w_uv: jax.Array,
    B_w_o: jax.Array,
):
    vmem = pltpu.VMEM
    out = pl.pallas_call(
        _kernel,
        out_shape=jax.ShapeDtypeStruct((S, 2 * DM), BF16),
        in_specs=[pl.BlockSpec(memory_space=pl.ANY)] * 9,
        out_specs=pl.BlockSpec(memory_space=pl.ANY),
        scratch_shapes=[
            vmem((2, CO, DM), BF16),
            vmem((63, 2, RO, T), BF16),
            vmem((7, NP, S // 2, T), BF16),
            vmem((49, 2, DM, T), BF16),
            vmem((7, 4, DM // 2, T), BF16),
            vmem((49, 4, 2 * T, T), BF16),
            vmem((49, 2, 2 * T, T), BF16),
            pltpu.SMEM((1,), jnp.int32),
            pltpu.SemaphoreType.DMA((2,)),
        ],
        compiler_params=pltpu.CompilerParams(
            vmem_limit_bytes=124 * 2**20, disable_bounds_checks=True),
    )(
        A_x.reshape(S, DM),
        A_wqkv.reshape(4, DM // 4, 3 * DM),
        A_wo.reshape(NH, DM // NH, DM),
        B_x.reshape(S, DM),
        B_c_kv.reshape(S, DC),
        B_w_q,
        B_w_uk,
        B_w_uv,
        B_w_o,
    )
    return out.reshape(1, S, 2 * DM)
```

```python
import functools
import math

import jax
import jax.numpy as jnp
from jax import lax
import jax.experimental.pallas as pl
import jax.experimental.pallas.tpu as pltpu

S = 2048
DM = 1024
DC = 512
NH = 32
NP = NH // 2
T = 128
CH = 4 * T
RO = 64
CO = 4 * RO
NO = S // CO
WIN, DIL = 8, 2
HALO = 16

LOG2E = math.log2(math.e)
SCALE_A = (DM // NH) ** -0.5 * LOG2E
SCALE_B = T ** -0.5 * LOG2E
MASKED = -1e9 * LOG2E
SAFE_SUM = 2.0 ** 40

DEPTH = 3
JOB_CYCLES = 1024, 256
CTX_CYCLES = 768, 1536

NX0, NX3 = 49, 84
F32, BF16, U32 = jnp.float32, jnp.bfloat16, jnp.uint32
P = functools.partial


def _dot(a, b):
    return jnp.dot(a, b, preferred_element_type=F32)


def _dot_nt(a, b):
    return lax.dot_general(a, b, (((1,), (1,)), ((), ())), preferred_element_type=F32)


def _cat(xs, axis=1):
    return xs[0] if len(xs) == 1 else jnp.concatenate(xs, axis=axis)


def _sum(xs):
    return functools.reduce(jnp.add, xs)


def _fold(op, x):
    return functools.reduce(op, [x[r:r + 8] for r in range(0, x.shape[0], 8)])


def _aligned(x, n):
    return x if isinstance(x, int) else pl.multiple_of(x, n)


def _rows(start, n):
    return pl.ds(_aligned(start, 16), n)


def _words(ref, lead, start, n):
    return ref.bitcast(U32)[(*lead, pl.ds(_aligned(start >> 1, 8), n // 2), slice(None))]


def _load(ref, lead, start, n):
    return pltpu.bitcast(_words(ref, lead, start, n), BF16)


def _split(w):
    return (pltpu.bitcast(w << 16, F32), pltpu.bitcast(w & jnp.uint32(0xFFFF0000), F32))


def _inverse(l):
    r = pl.reciprocal(l, approx=True)
    return r * (2.0 - l * r)


def _interleave(x, y):
    order = [((n + 0.5) / len(z), m, job) for m, z in enumerate((x, y)) for n, job in enumerate(z)]
    return [job for _, _, job in sorted(order, key=lambda e: e[:2])]


def _start(*copies):
    for cp in copies:
        cp.start()


def _wait(*copies):
    for cp in copies:
        cp.wait()


LHS = (((0, 1), (3, 1)), ((2, 1), (3, 1)), ((0, 1),), ((3, 1),),
       ((0, 1), (1, 1)), ((2, 1), (0, -1)), ((1, 1), (3, -1)))
RHS = (((0, 1), (3, 1)), ((0, 1),), ((1, 1), (3, -1)), ((2, 1), (0, -1)),
       ((3, 1),), ((0, 1), (1, 1)), ((2, 1), (3, 1)))
OUT = (((0, 1), (3, 1)), ((2, 1), (3, -1)), ((1, 1), (3, 1)), ((0, 1), (2, 1)),
       ((0, -1), (1, 1)), ((3, 1),), ((0, 1),))


def _term(table, i, quad):
    (n, _), *rest = table[i]
    val = quad(n)
    for n, sign in rest:
        val = val + quad(n) if sign > 0 else val - quad(n)
    return val


def _terms(table, quad):
    blocks = [quad(n) for n in range(4)]
    return [_term(table, i, blocks.__getitem__) for i in range(7)]


def _terms2(table, i, block):
    return _terms(table, lambda n: _term(
        table, i, lambda m: block(2 * (m // 2) + n // 2, 2 * (m % 2) + n % 2)))


def _combine(m):
    out = [None] * 4
    for i in range(7):
        for n, sign in OUT[i]:
            if out[n] is None:
                out[n] = m[i]
            else:
                out[n] = out[n] + m[i] if sign > 0 else out[n] - m[i]
    return out


def _combine2(m):
    inner = [_combine(m[7 * i:7 * i + 7]) for i in range(7)]
    out = [[None] * 4 for _ in range(4)]
    for n in range(4):
        for quad, val in enumerate(_combine([x[n] for x in inner])):
            out[2 * (quad // 2) + n // 2][2 * (quad % 2) + n % 2] = val
    return out


class _Tokens:
    def __init__(self, zero_smem):
        self.z = zero_smem[0]
        self.zero = jnp.full((8, T), self.z, jnp.int32).astype(U32)

    def stored(self, ref, lead, start):
        first, *rest = lead
        if ref.dtype == BF16:
            return _words(ref, (first - (self.z & 1), *rest), start, 16) & self.zero
        return self.of(ref[(*lead, pl.ds(_aligned(start + 8 * (self.z & 1), 8), 8), slice(None))])

    def of(self, *vals):
        return pltpu.bitcast(_sum(vals), U32) & self.zero


def _after(token, x, everywhere=False):
    if token is None:
        return x
    bits = x if x.dtype == U32 else pltpu.bitcast(x, U32)
    cut = bits.shape[0] if everywhere else 8
    parts = [bits[r:r + 8] | token for r in range(0, cut, 8)]
    bits = _cat(parts + ([bits[cut:]] if cut < bits.shape[0] else []), axis=0)
    return bits if x.dtype == U32 else pltpu.bitcast(bits, x.dtype)


AX_JOBS = [(i, n, r) for n in range(2) for r in range(0, RO, 16) for i in range(7)]


def _job_ax(tok, released, ax_raw, ax_t, src, i, n, r):
    terms = _terms2(LHS, i, lambda row, col: released(
        ax_raw[src, pl.ds(row * RO + r, 16), pl.ds((2 * col + n) * T, T)].astype(F32)))
    for x, val in enumerate(terms):
        ax_t[7 * i + x, n, pl.ds(r, 16), :] = val.astype(BF16)
    return tok.stored(ax_t, (7 * i + 6, n), r)


def _head_pairs(wqkv_hbm, wo_hbm, bx_hbm, c_hbm, wq_hbm, wuk_hbm, wuv_hbm, wob_hbm,
                ax_copy, ax_raw, ax_t, ctx_t, wob_t, wa_t, wo_t, zero_smem,
                bx_raw, c_raw, wq_raw, wk_raw, wv_raw, wob_raw, wqkv_raw, wo_raw,
                bx_t, c_t, wq_turned, wq_t, wkv_t, guard, sem_in, sem_w):
    def head_copies(j, slot):
        return [pltpu.make_async_copy(src.bitcast(U32).at[:, j, :], dst.at[slot], sem_w.at[3 * slot + n])
                for n, (src, dst) in enumerate(((wuk_hbm, wk_raw), (wuv_hbm, wv_raw), (wq_hbm, wq_raw)))]

    def side_copies(j, slot):
        wob = wob_hbm.at[pl.ds(4 * (j >> 1), 4), pl.ds(_aligned((j & 1) * 64, 64), 64), :]
        wqkv = wqkv_hbm.bitcast(U32).at[:, pl.ds(_aligned(8 * j, 8), 8), :]
        return [pltpu.make_async_copy(wob, wob_raw.at[slot], sem_w.at[6 + 2 * slot]),
                pltpu.make_async_copy(wqkv, wqkv_raw.at[slot], sem_w.at[7 + 2 * slot])]

    def wo_copy(word):
        return pltpu.make_async_copy(wo_hbm.bitcast(U32).at[:, word, :], wo_raw.at[word], sem_w.at[10])

    def c_copy(c):
        rows = pl.ds(c * CH, CH)
        return pltpu.make_async_copy(c_hbm.at[rows, :], c_raw.at[rows, :], sem_in.at[2 * c])

    def x_copy(c):
        rows = pl.ds(c * CH, CH)
        return pltpu.make_async_copy(bx_hbm.at[rows, :], bx_raw.at[rows, :], sem_in.at[2 * c + 1])

    def pair_body(j, first=False):
        slot = j & 1
        tok = _Tokens(zero_smem)
        causal = (lax.broadcasted_iota(jnp.int32, (T, T), 1)
                  <= lax.broadcasted_iota(jnp.int32, (T, T), 0))

        jobs, due, pace = [], [], dict(period=0, clock=0, release=None)

        def queue(cycles, more):
            pace.update(period=cycles / len(more), clock=0)
            jobs.extend(more)

        def flush():
            while jobs:
                jobs.pop(0)()

        def background(cycles, recent=None):
            pace["clock"] += cycles
            token = None
            while jobs and pace["clock"] >= pace["period"]:
                pace["clock"] -= pace["period"]
                pace["release"] = None if recent is None else tok.of(recent[:8])
                new = jobs.pop(0)()
                pace["release"] = None
                token = new if token is None else token | new
            if token is not None:
                due.append([JOB_CYCLES[recent is None], token])
            for entry in due:
                entry[0] -= cycles
            now = [token for left, token in due if left <= 0]
            due[:] = [entry for entry in due if entry[0] > 0]
            return functools.reduce(jnp.bitwise_or, now) if now else None

        def released(x):
            return _after(pace["release"], x, everywhere=True)

        def store_terms(dst, first_term, lead, row, terms):
            for i, val in enumerate(terms):
                dst[(first_term + i, *lead, _rows(row, 16), slice(None))] = val.astype(BF16)
            return tok.stored(dst, (first_term + 6, *lead), row)

        def job_x(c, i, n, r):
            terms = _terms2(RHS, i, lambda row, col: bx_raw[
                pl.ds(c * CH + (col ^ 2) * T + r, 16), pl.ds((2 * row + n) * T, T)].astype(F32))
            return store_terms(bx_t, 7 * i, (n,), c * T + r, terms)

        def job_c(c, i, r):
            terms = _terms2(LHS, i, lambda row, col: c_raw[
                pl.ds(c * CH + row * T + r, 16), pl.ds(col * T, T)].astype(F32))
            return store_terms(c_t, 7 * i, (), c * T + r, terms)

        def jobs_x(c):
            return [P(job_x, c, i, n, r) for r in range(0, T, 16) for n in range(2) for i in range(7)]

        def jobs_c(c):
            return [P(job_c, c, i, r) for r in range(0, T, 16) for i in range(7)]

        def job_wkv(src, i, r):
            def block(row, col):
                raw = (wk_raw, wv_raw)[col % 2]
                return _split(released(raw[src, pl.ds(row * T + r, 16), :]))[col // 2]
            return store_terms(wkv_t, 7 * i, (), r, _terms2(RHS, i, block))

        def job_turn(src, n):
            words = released(wq_raw[src, pl.ds(n * T, T), :])
            wq_turned[n] = pltpu.bitcast(pltpu.bitcast(words, F32).T, U32)
            return tok.stored(wq_turned, (n,), T - 16)

        def job_wq(i, n, r):
            def block(row, col):
                return _split(released(wq_turned[2 * col + n, pl.ds((row % 2) * RO + r, 16), :]))[row // 2]
            return store_terms(wq_t, 7 * i, (n,), r, _terms2(LHS, i, block))

        def jobs_wkv(src):
            return [P(job_wkv, src, i, r) for r in range(0, T, 16) for i in range(7)]

        def jobs_wq(src):
            return ([P(job_turn, src, n) for n in range(DM // T)],
                    [P(job_wq, i, n, r) for n in range(2) for r in range(0, RO, 16) for i in range(7)])

        def job_wob(i, n, r):
            def block(row, col):
                head = 2 * (row % 2) + row // 2
                return released(wob_raw[slot, head, pl.ds(r, 16), pl.ds((2 * col + n) * T, T)].astype(F32))
            return store_terms(wob_t, 7 * i, (n,), j * 64 + r, _terms2(RHS, i, block))

        def job_wo(i, n):
            e, odd, head = j & 3, (j >> 2) & 1, 16 * (j >> 3)

            def block(row, col):
                even_t, odd_t = _split(released(
                    wo_raw[4 * e + row, _rows(head, 16), pl.ds((2 * col + n) * T, T)]))
                return jnp.where(odd == 1, odd_t, even_t)
            return store_terms(wo_t, 7 * i, (n,), odd * T + e * NH + head, _terms2(RHS, i, block))

        permuted = {}

        def job_permute(mat):
            lane = lax.broadcasted_iota(jnp.int32, (32, T), 1)
            e, grp, sub = lane >> 5, (lane >> 2) & 7, lane & 3

            def gather(x, index):
                return jnp.take_along_axis(x, index, axis=1, mode="promise_in_bounds")
            x = [released(wqkv_raw[slot, :, :, pl.ds(mat * DM + t * T, T)].reshape(32, T))
                 for t in range(8)]
            y = [gather(x[t], sub * 32 + e * 8 + ((grp - t) & 7)) for t in range(8)]
            u = [y[-s % 8] for s in range(8)]
            for bit in (1, 2, 4):
                u = [jnp.where((grp & bit) != 0, u[(s - bit) % 8], u[s]) for s in range(8)]
            u = [u[0]] + [gather(u[t], e * 32 + ((grp + t) & 7) * 4 + sub) for t in range(1, 8)]
            permuted[mat] = u
            return _fold(jnp.bitwise_or, functools.reduce(jnp.bitwise_or, u)) & tok.zero

        def column(mat, row, t):
            return pltpu.bitcast(released(permuted[mat][t][8 * row:8 * row + 8]), BF16).astype(F32)

        def job_wa(mat, i, n):
            terms = _terms2(RHS, i, lambda row, col: column(mat, row, 2 * col + n))
            return store_terms(wa_t, 7 * i, (2 * mat + n,), 16 * j, terms)

        pause = [P(lambda: tok.zero)] * 2
        jobs_wob = [P(job_wob, i, n, r) for r in range(0, 64, 16) for n in range(2) for i in range(7)]
        jobs_wo = [P(job_wo, i, n) for n in range(2) for i in range(7)]
        jobs_wa = []
        for mat in range(3):
            jobs_wa += [P(job_permute, mat)] + pause
            jobs_wa += [P(job_wa, mat, i, n) for n in range(2) for i in range(7)]

        q, k, v = {}, {}, {}

        def project_q(c):
            def product(i, n):
                left = _after(background(16) if first else None, _words(wq_t, (i, n), 0, RO))
                return _dot_nt(pltpu.bitcast(left, BF16), _load(bx_t, (i, n), c * T, T))
            m = [product(i, 0) + product(i, 1) for i in range(49)]
            blocks = _combine2(m)
            for h in range(2):
                for col in range(4):
                    val = _cat([blocks[2 * h][col], blocks[2 * h + 1][col]], axis=0) * SCALE_B
                    q[4 * c + (col ^ 2), h] = val.T.astype(BF16)

        def project_kv(c):
            m = [_dot(_load(c_t, (i,), c * T, T), _load(wkv_t, (i,), 0, T)) for i in range(49)]
            for r, row in enumerate(_combine2(m)):
                for n, val in enumerate(row):
                    (k, v)[n % 2][4 * c + r, n // 2] = val.astype(BF16)

        def plain(raw, c, weights):
            def operand():
                parts = []
                for r in range(c * CH, (c + 1) * CH, 32):
                    part = raw[pl.ds(r, 32), :]
                    token = background(8 * (raw.shape[1] // T))
                    if token is not None:
                        part = _cat([_after(_cat([token, token]), part[:, :2 * T]), part[:, 2 * T:]])
                    parts.append(part)
                return _cat(parts, axis=0)
            return [_dot(operand(), w) for w in weights]

        def plain_kv(c, weights):
            for n, val in enumerate(plain(c_raw, c, weights)):
                for r in range(4):
                    (k, v)[n // 2][4 * c + r, n % 2] = val[r * T:(r + 1) * T].astype(BF16)

        def plain_q(c, weights):
            for h, val in enumerate(plain(bx_raw, c, weights)):
                for r in range(4):
                    q[4 * c + r, h] = (val[r * T:(r + 1) * T] * SCALE_B).astype(BF16)

        in_flight, partial, ctx, spread, checks = [], {}, {}, {}, []

        def finish(i, h):
            l, o = partial.pop((i, h))
            l = jnp.sum(l, axis=1, keepdims=True)
            r = _inverse(l)
            ctx[i, h] = o * r
            spread[i, h] = _fold(jnp.maximum, jnp.broadcast_to(l + r, (T, T)))
            b = i // 2
            quad = [(2 * b, 0), (2 * b, 1), (2 * b + 1, 0), (2 * b + 1, 1)]
            if all(u in ctx for u in quad):
                terms = _terms(LHS, lambda m: ctx.pop(quad[m]))
                for n, val in enumerate(terms):
                    ctx_t[n, j, pl.ds(b * T, T), :] = val.astype(BF16)
                checks.append((_fold(jnp.add, terms[0] + terms[5] + terms[6]),
                               functools.reduce(jnp.maximum, [spread.pop(u) for u in quad])))
                due.append([CTX_CYCLES[first], tok.stored(ctx_t, (6, j), b * T) | tok.of(*checks[-1])])

        def weigh(i, h, t, p):
            l, o = partial.get((i, h), (None, None))
            l = p if l is None else l + p
            d = _dot(_after(background(64, p), p).astype(BF16), v[t, h])
            partial[i, h] = (l, d if o is None else o + d)
            if t == i:
                finish(i, h)

        def attention(lo, hi):
            for i in range(lo, hi):
                for h in range(2):
                    for t in range(i + 1):
                        s = _dot_nt(q[i, h], k[t, h])
                        if t == i:
                            s = jnp.where(causal, s, MASKED)
                        in_flight.append((i, h, t, jnp.exp2(s)))
                        if len(in_flight) > DEPTH:
                            weigh(*in_flight.pop(0))
            while hi == S // T and in_flight:
                weigh(*in_flight.pop(0))

        def cycles(lo, hi):
            return 2 * 64 * sum(range(lo + 1, hi + 1))

        if first:
            wk, wv, wq = head_copies(0, 0)
            _start(wv, wk, c_copy(0), c_copy(1))
            _wait(wv, wk, c_copy(0))
            _start(c_copy(2), c_copy(3), wq, x_copy(0))
            weights = [w.astype(BF16) for raw in (wk_raw, wv_raw) for w in _split(raw[0])]
            queue(0.98 * 2048, jobs_c(0))
            plain_kv(0, weights)
            flush()
            _wait(c_copy(1), c_copy(2))
            _start(x_copy(1), x_copy(2))
            queue(0.98 * 4096, jobs_c(1) + jobs_c(2))
            plain_kv(1, weights)
            plain_kv(2, weights)
            flush()
            _wait(c_copy(3), wq)
            turn, terms = jobs_wq(0)
            queue(0.98 * 2048, _interleave(turn, jobs_c(3)))
            plain_kv(3, weights)
            flush()
            _wait(x_copy(0))
            weights = [w.astype(BF16) for w in _split(wq_raw[0])]
            queue(0.95 * (2048 + cycles(0, 4)), jobs_x(0)[:96])
            plain_q(0, weights)
            attention(0, 4)
            flush()
            _wait(x_copy(1), x_copy(2))
            stage = [*side_copies(0, 0), *head_copies(1, 1)]
            _start(x_copy(3), *stage)
            lax.fori_loop(0, 16, lambda word, carry: wo_copy(word).start(), None)
            queue(0.98 * (2048 + cycles(4, 8)), jobs_x(2) + terms + jobs_x(0)[96:] + jobs_x(1)[:14])
            plain_q(1, weights)
            attention(4, 8)
            flush()
            _wait(x_copy(3))
            queue(0.98 * (1568 + cycles(8, 9)), jobs_x(3)[:98])
            project_q(2)
            attention(8, 9)
            flush()
            _wait(*stage)
            _start(ax_copy(0, 0), *head_copies(2, 0), *side_copies(1, 1))
            turn, terms = jobs_wq(1)
            queue(0.92 * (1568 + cycles(9, 14)), jobs_x(3)[98:] + _interleave(
                _interleave(jobs_wob, jobs_wa), _interleave(jobs_x(1)[14:], _interleave(turn, jobs_wkv(1)))))
            attention(9, 12)
            assert not any(job.func is job_x and job.args[0] == 3 for job in jobs)
            project_q(3)
            attention(12, 14)
            flush()
            _wait(*[wo_copy(word) for word in range(16)], ax_copy(0, 0))
            _start(ax_copy(1, 1))
            queue(0.92 * cycles(14, 16), _interleave(
                jobs_wo + terms, [P(_job_ax, tok, released, ax_raw, ax_t, 0, *job) for job in AX_JOBS]))
            attention(14, 16)
            flush()
        else:
            queue(0.98 * cycles(0, 12), _interleave(jobs_wob, jobs_wo + jobs_wa))
            project_kv(0)
            project_q(0)
            project_kv(1)
            done = 0
            for row, project, c in ((3, project_q, 1), (6, project_q, 2), (7, project_kv, 2),
                                    (10, project_q, 3), (11, project_kv, 3)):
                attention(done, row)
                project(c)
                done = row
            attention(done, 12)
            flush()
            turn, terms = jobs_wq(1 - slot)
            queue(0.9 * cycles(12, 16), _interleave(jobs_wkv(1 - slot), turn + pause + terms))
            attention(12, 16)
            flush()
        guard[0] = _sum([guard[0]] + [x for x, _ in checks])
        guard[1] = functools.reduce(jnp.maximum, [guard[1]] + [x for _, x in checks])

        def ahead(n):
            return j + n if first else jnp.minimum(j + n, NP - 1)
        _wait(*head_copies(ahead(2), slot), *side_copies(ahead(1), 1 - slot))

        @pl.when(j < NP - 1)
        def _():
            _start(*head_copies(ahead(3), 1 - slot), *side_copies(ahead(2), slot))

    def exact_pairs(ctx):
        def block(i):
            return pl.ds(pl.multiple_of(i * T, T), T)

        def qkv(n, h, i):
            return c_t.at[(2 * n + h) * 4 + (i >> 2), block(i & 3), :]

        def project(x, carry):
            h, i = x & 1, x >> 1
            for n, (rows, w, scale) in enumerate(
                    ((bx_raw, wq_raw, SCALE_B), (c_raw, wk_raw, 1.0), (c_raw, wv_raw, 1.0))):
                def add(t, val):
                    even, odd = _split(w[0, block(t), :])
                    return val + _dot(rows[block(i), block(t)], jnp.where(h == 0, even, odd).astype(BF16))
                val = lax.fori_loop(0, w.shape[1] // T, add, jnp.zeros((T, T), F32))
                qkv(n, h, i)[...] = (val * scale).astype(BF16)

        def attend(b, x, carry):
            quad, part = x >> 3, pl.ds(pl.multiple_of((x & 7) * 16, 16), 16)
            h, i = quad & 1, 2 * b + (quad >> 1)

            def scores(t):
                row = lax.broadcasted_iota(jnp.int32, (16, T), 0) + (i * T + (x & 7) * 16)
                col = lax.broadcasted_iota(jnp.int32, (16, T), 1) + t * T
                return jnp.where(col <= row, _dot_nt(qkv(0, h, i)[part, :], qkv(1, h, t)[...]), MASKED)

            m = lax.fori_loop(
                0, i + 1, lambda t, m: jnp.maximum(m, jnp.max(scores(t), axis=1, keepdims=True)),
                jnp.full((16, 1), -jnp.inf, F32))

            def accumulate(t, carry):
                l, o = carry
                p = jnp.exp2(scores(t) - m)
                return (l + jnp.sum(p, axis=1, keepdims=True),
                        o + _dot(p.astype(BF16), qkv(2, h, t)[...]))
            l, o = lax.fori_loop(0, i + 1, accumulate,
                                 (jnp.zeros((16, 1), F32), jnp.zeros((16, T), F32)))
            ctx[quad, part, :] = o / l

        def pair(j, carry):
            _start(*head_copies(j, 0))
            _wait(*head_copies(j, 0))
            lax.fori_loop(0, 2 * S // T, project, None)

            def rows(b, carry):
                lax.fori_loop(0, 32, P(attend, b), None)
                for n, val in enumerate(_terms(LHS, lambda m: ctx[m])):
                    ctx_t[n, j, block(b), :] = val.astype(BF16)
            lax.fori_loop(0, S // T // 2, rows, None)

        lax.fori_loop(0, NP, pair, None)

    guard[...] = jnp.zeros(guard.shape, F32)
    pair_body(0, first=True)
    lax.fori_loop(1, NP, lambda j, carry: pair_body(j), None)

    safe = jnp.logical_and(jnp.abs(guard[0]) < jnp.inf, guard[1] < SAFE_SUM)

    @pl.when(jnp.max(jnp.where(safe, 0.0, 1.0)) > 0.0)
    def _():
        pl.run_scoped(exact_pairs, pltpu.VMEM((4, T, T), F32))


def _outputs(out_hbm, ax_copy, ax_raw, ax_t, ctx_t, wob_t, wa_t, wo_t, zero_smem,
             o_t, kbuf, vbuf, qbuf, acc, obuf, sem_out):
    def out_copy(c, slot):
        rows = pl.ds(_aligned(c * CO, CO), CO)
        return pltpu.make_async_copy(obuf.at[slot], out_hbm.at[rows, :], sem_out.at[slot])

    for buf in (kbuf, vbuf):
        for t in range(8):
            buf[t, pl.ds(CO, HALO), :] = jnp.zeros((HALO, T), F32)

    costs = [RO] * (3 * 49) + [4 * RO] * 42 + [RO] * 49 + [4 * RO] * 7
    starts = [sum(costs[:n]) for n in range(len(costs) + 1)]
    t_q, t_v, t_b, t_o, t_last = (starts[n] for n in (49, 98, 147, 189, 238))

    def chunk_body(c, carry):
        slot = c & 1
        tok = _Tokens(zero_smem)
        plan, due, clock = {}, {}, [0]

        def schedule(job, begin, end, release=False):
            first = max([clock[0]] + [n for n in range(len(costs)) if starts[n + 1] <= begin])
            last = min(n for n in range(len(costs)) if starts[n] >= end)
            plan.setdefault(first, []).append((job, last, release))

        def step(results, a, w):
            n = clock[0]
            clock[0] += 1
            for x, token in enumerate(due.pop(n, [])):
                a[x % len(a)] = _after(token, a[x % len(a)])
            a = [x.astype(BF16) if x.dtype == F32 else pltpu.bitcast(x, BF16) for x in a]
            res = [None] * len(w)
            for x in range(len(a)):
                for y in range(len(w)):
                    d = _dot(a[x], w[y](x))
                    res[y] = d if res[y] is None else res[y] + d
            results.append(res)
            token = None
            for job, last, release in plan.pop(n, []):
                if release and token is None:
                    token = tok.of(res[0][:8])
                due.setdefault(last, []).append(job(token) if release else job())

        def project(lhs_t, rhs_t, tile0, write, begin, end):
            m = []

            def recombine(y, r):
                blocks = _combine2([x[y][r:r + 8] for x in m])
                write(blocks, y, r)
                return tok.of(*[x for row in blocks for x in row])

            slabs = [(y, r) for r in range(0, RO, 8) for y in range(2)]
            for x, slab in enumerate(slabs):
                schedule(P(recombine, *slab), begin, begin + (end - begin) * (x + 1) // len(slabs))
            for i in range(49):
                step(m, [_words(lhs_t, (i, x), 0, RO) for x in range(2)],
                     [P(lambda y, x: _load(rhs_t, (i, tile0 + y), x * T, T), y) for y in range(2)])

        for buf in (kbuf, vbuf):
            for t in range(8):
                buf[t, pl.ds(0, HALO), :] = buf[t, pl.ds(CO, HALO), :]

        def write_rows(buf, blocks, y, r):
            for row in range(4):
                for col in range(4):
                    buf[2 * col + y, pl.ds(HALO + row * RO + r, 8), :] = blocks[row][col]

        def write_q(blocks, y, r):
            for row in range(4):
                for col in range(4):
                    qbuf[2 * col + y, pl.ds(row * RO + r, 8), :] = blocks[row][col] * SCALE_A

        project(ax_t, wa_t, 2, P(write_rows, kbuf), t_q, t_q + 2800)
        project(ax_t, wa_t, 0, write_q, t_v, t_v + 2500)

        att = {}

        def job_weights(row, r, release):
            base = HALO + row * RO + r
            qs = [_after(release, qbuf[t, pl.ds(row * RO + r, 8), :]) for t in range(8)]
            logits = []
            for w in range(WIN):
                x = _sum([qs[t] * kbuf[t, pl.ds(base - DIL * w, 8), :] for t in range(8)])
                x = x + pltpu.roll(x, 64, 1)
                x = x + pltpu.roll(x, 32, 1)
                if row == 0 and r < DIL * w:
                    pos = lax.broadcasted_iota(jnp.int32, (8, T), 0) + (c * CO + r)
                    x = jnp.where(pos >= DIL * w, x, MASKED)
                logits.append(x)
            m = functools.reduce(jnp.maximum, logits)
            p = [jnp.exp2(x - m) for x in logits]
            inv = _inverse(_sum(p))
            att[row, r] = [x * inv for x in p]
            return tok.of(att[row, r][0])

        def job_values(row, r, release):
            base = HALO + row * RO + r
            p = [_after(release, x) for x in att[row, r]]
            att[row, r] = [_sum([p[w] * vbuf[t, pl.ds(base - DIL * w, 8), :] for w in range(WIN)])
                           for t in range(8)]
            return tok.of(*att[row, r])

        def job_o(n, r, i):
            def block(row, col):
                return _cat([att[row, r][2 * col + n], att[row, r + 8][2 * col + n]], axis=0)
            for x, val in enumerate(_terms2(LHS, i, block)):
                o_t[7 * i + x, n, pl.ds(r, 16), :] = val.astype(BF16)
            return tok.stored(o_t, (7 * i + 6, n), r)

        groups = [(row, r + x) for r in range(0, RO, 16) for row in (0, 2, 1, 3) for x in (0, 8)]
        w0, w1, v0, v1 = t_v + 300, t_b + 3500, t_b + 2500, t_o - 700
        for g, (row, r) in enumerate(groups):
            begin = w0 + (w1 - w0) * g // len(groups)
            schedule(P(job_weights, row, r), begin, begin + 700, release=True)
            begin = max(v0 + (v1 - v0) * g // len(groups), begin + 700)
            schedule(P(job_values, row, r), begin, begin + 300, release=True)
            if g % 8 == 7:
                for x, (n, i) in enumerate((n, i) for n in range(2) for i in range(7)):
                    schedule(P(job_o, n, r - 8, i), begin, min(begin + 500 + 60 * (x + 1), t_o))
        project(ax_t, wa_t, 4, P(write_rows, vbuf), t_b, t_b + 1500)

        touched = {}

        def project_b(i):
            m = []

            def accumulate(y, inner):
                val = _combine([x[y] for x in m])[inner]
                token = None
                for outer, sign in OUT[i]:
                    row, col = 2 * (outer // 2) + inner // 2, 2 * (2 * (outer % 2) + inner % 2) + y
                    rows = pl.ds(row * RO, RO)
                    total = val
                    if (outer, inner, y) in touched:
                        total = acc[col, rows, :] + val if sign > 0 else acc[col, rows, :] - val
                    touched[outer, inner, y] = True
                    if any(outer == n for x in range(i + 1, 7) for n, _ in OUT[x]):
                        acc[col, rows, :] = total
                        token = tok.stored(acc, (col,), row * RO)
                    else:
                        obuf[slot, rows, pl.ds(DM + col * T, T)] = total.astype(BF16)
                        if token is None:
                            token = tok.of(_fold(jnp.add, total))
                return token

            parts = [(y, inner) for y in range(2) for inner in range(4)]
            done = starts[clock[0] + 7]
            if i < 6:
                for x, part in enumerate(parts):
                    schedule(P(accumulate, *part), done, done + 256 + 150 * x)
            for n in range(7):
                def quad(kt, x):
                    return (i, 2 * kt + x % 2), (2 * c + x // 2) * RO
                if len(LHS[n]) == 1:
                    a = [_words(ctx_t, *quad(kt, LHS[n][0][0]), RO) for kt in range(8)]
                else:
                    a = [_term(LHS, n, lambda x: _load(ctx_t, *quad(kt, x), RO).astype(F32))
                         for kt in range(8)]
                step(m, a, [P(lambda y, x: _load(wob_t, (7 * i + n, y), x * T, T), y) for y in range(2)])
            if i == 6:
                for part in parts:
                    accumulate(*part)

        for i in range(6):
            project_b(i)

        for x, job in enumerate(AX_JOBS):
            schedule(P(_job_ax, tok, lambda val: val, ax_raw, ax_t, 1 - slot, *job),
                     t_o, t_o + 100 + 3600 * (x + 1) // len(AX_JOBS))
        upper = {}

        def write_out(blocks, y, r):
            if r % 16 == 0:
                upper[y] = blocks
                return
            for row in range(4):
                for col in range(4):
                    val = _cat([upper[y][row][col], blocks[row][col]], axis=0)
                    obuf[slot, pl.ds(row * RO + r - 8, 16), pl.ds((2 * col + y) * T, T)] = val.astype(BF16)

        project(o_t, wo_t, 0, write_out, t_last, starts[-2])
        project_b(6)
        assert not plan and not due
        out_copy(c, slot).start()
        ax_copy(jnp.minimum(c + 2, NO - 1), slot).wait()

        @pl.when(c < NO - 1)
        def _():
            ax_copy(jnp.minimum(c + 3, NO - 1), 1 - slot).start()

        @pl.when(c >= 1)
        def _():
            out_copy(c - 1, 1 - slot).wait()

    ax_copy(1, 1).wait()
    ax_copy(2, 0).start()
    lax.fori_loop(0, NO, chunk_body, None)
    out_copy(NO - 1, (NO - 1) % 2).wait()


def _kernel(ax_hbm, wqkv_hbm, wo_hbm, bx_hbm, c_hbm, wq_hbm, wuk_hbm, wuv_hbm, wob_hbm, out_hbm,
            ax_raw, ax_t, ctx_t, wob_t, wa_t, wo_t, zero_smem, sem_ax):
    vmem, dma = pltpu.VMEM, pltpu.SemaphoreType.DMA

    def clear(i, carry):
        zero_smem[0] = i >> 1
    lax.fori_loop(0, 2, clear, None)

    def ax_copy(c, slot):
        rows = pl.ds(_aligned(c * CO, CO), CO)
        return pltpu.make_async_copy(ax_hbm.at[rows, :], ax_raw.at[slot], sem_ax.at[slot])

    shared = (ax_copy, ax_raw, ax_t, ctx_t, wob_t, wa_t, wo_t, zero_smem)
    pl.run_scoped(
        P(_head_pairs, wqkv_hbm, wo_hbm, bx_hbm, c_hbm, wq_hbm, wuk_hbm, wuv_hbm, wob_hbm, *shared),
        vmem((S, DM), BF16),
        vmem((S, DC), BF16),
        vmem((2, DM, T), U32),
        vmem((2, DC, T), U32),
        vmem((2, DC, T), U32),
        vmem((2, 4, 64, DM), BF16),
        vmem((2, 4, 8, 3 * DM), U32),
        vmem((16, NH, DM), U32),
        vmem((49, 2, S // 4, T), BF16),
        vmem((49, S // 4, T), BF16),
        vmem((DM // T, T, T), U32),
        vmem((49, 2, RO, T), BF16),
        vmem((49, T, T), BF16),
        vmem((2, 8, T), F32),
        dma((2 * S // CH,)), dma((11,)))
    pl.run_scoped(
        P(_outputs, out_hbm, *shared),
        vmem((49, 2, RO, T), BF16),
        vmem((8, HALO + CO, T), F32),
        vmem((8, HALO + CO, T), F32),
        vmem((8, CO, T), F32),
        vmem((8, CO, T), F32),
        vmem((2, CO, 2 * DM), BF16),
        dma((2,)))


@jax.jit
def pallas_concat_heads__sliding_local_dilated__compressed_kv_cla__prompt_kernel(
    A_x: jax.Array,
    A_wqkv: jax.Array,
    A_wo: jax.Array,
    B_x: jax.Array,
    B_c_kv: jax.Array,
    B_w_q: jax.Array,
    B_w_uk: jax.Array,
    B_w_uv: jax.Array,
    B_w_o: jax.Array,
):
    vmem = pltpu.VMEM
    out = pl.pallas_call(
        _kernel,
        out_shape=jax.ShapeDtypeStruct((S, 2 * DM), BF16),
        in_specs=[pl.BlockSpec(memory_space=pl.ANY)] * 9,
        out_specs=pl.BlockSpec(memory_space=pl.ANY),
        scratch_shapes=[
            vmem((2, CO, DM), BF16),
            vmem((49, 2, RO, T), BF16),
            vmem((7, NP, S // 2, T), BF16),
            vmem((49, 2, DM, T), BF16),
            vmem((49, 6, 2 * T, T), BF16),
            vmem((49, 2, 2 * T, T), BF16),
            pltpu.SMEM((1,), jnp.int32),
            pltpu.SemaphoreType.DMA((2,)),
        ],
        compiler_params=pltpu.CompilerParams(
            vmem_limit_bytes=127 * 2**20, disable_bounds_checks=True),
    )(
        A_x.reshape(S, DM),
        A_wqkv.reshape(4, DM // 4, 3 * DM),
        A_wo.reshape(NH, DM // NH, DM),
        B_x.reshape(S, DM),
        B_c_kv.reshape(S, DC),
        B_w_q,
        B_w_uk,
        B_w_uv,
        B_w_o,
    )
    return out.reshape(1, S, 2 * DM)
```

```python
import functools
import math

import jax
import jax.numpy as jnp
from jax import lax
import jax.experimental.pallas as pl
import jax.experimental.pallas.tpu as pltpu

S = 2048
DM = 1024
DC = 512
NH = 32
NP = NH // 2
T = 128
CH = 4 * T
RO = 64
CO = 4 * RO
NO = S // CO
WIN, DIL = 8, 2
HALO = 16

LOG2E = math.log2(math.e)
SCALE_A = (DM // NH) ** -0.5 * LOG2E
SCALE_B = T ** -0.5 * LOG2E
MASKED = -1e9 * LOG2E
SAFE_SUM = 2.0 ** 40

DEPTH = 3
JOB_CYCLES = 1024, 256
CTX_CYCLES = 768, 1536

NX0, NX3 = 49, 84
TICK = RO // 2
EARLY_B = 4
F32, BF16, U32 = jnp.float32, jnp.bfloat16, jnp.uint32
P = functools.partial


def _dot(a, b):
    return jnp.dot(a, b, preferred_element_type=F32)


def _dot_nt(a, b):
    return lax.dot_general(a, b, (((1,), (1,)), ((), ())), preferred_element_type=F32)


def _cat(xs, axis=1):
    return xs[0] if len(xs) == 1 else jnp.concatenate(xs, axis=axis)


def _sum(xs):
    return functools.reduce(jnp.add, xs)


def _fold(op, x):
    return functools.reduce(op, [x[r:r + 8] for r in range(0, x.shape[0], 8)])


def _aligned(x, n):
    return x if isinstance(x, int) else pl.multiple_of(x, n)


def _rows(start, n):
    return pl.ds(_aligned(start, 16), n)


def _words(ref, lead, start, n):
    return ref.bitcast(U32)[(*lead, pl.ds(_aligned(start >> 1, 8), n // 2), slice(None))]


def _load(ref, lead, start, n):
    return pltpu.bitcast(_words(ref, lead, start, n), BF16)


def _split(w):
    return (pltpu.bitcast(w << 16, F32), pltpu.bitcast(w & jnp.uint32(0xFFFF0000), F32))


def _inverse(l):
    r = pl.reciprocal(l, approx=True)
    return r * (2.0 - l * r)


def _interleave(x, y):
    order = [((n + 0.5) / len(z), m, job) for m, z in enumerate((x, y)) for n, job in enumerate(z)]
    return [job for _, _, job in sorted(order, key=lambda e: e[:2])]


def _start(*copies):
    for cp in copies:
        cp.start()


def _wait(*copies):
    for cp in copies:
        cp.wait()


LHS = (((0, 1), (3, 1)), ((2, 1), (3, 1)), ((0, 1),), ((3, 1),),
       ((0, 1), (1, 1)), ((2, 1), (0, -1)), ((1, 1), (3, -1)))
RHS = (((0, 1), (3, 1)), ((0, 1),), ((1, 1), (3, -1)), ((2, 1), (0, -1)),
       ((3, 1),), ((0, 1), (1, 1)), ((2, 1), (3, 1)))
OUT = (((0, 1), (3, 1)), ((2, 1), (3, -1)), ((1, 1), (3, 1)), ((0, 1), (2, 1)),
       ((0, -1), (1, 1)), ((3, 1),), ((0, 1),))
SUMS = tuple(tuple((i, sign) for i in range(7) for m, sign in OUT[i] if m == n) for n in range(4))
FINAL = tuple(tuple(n for n in range(4) if SUMS[n][-1][0] == i) for i in range(7))


def _term(table, i, quad):
    (n, _), *rest = table[i]
    val = quad(n)
    for n, sign in rest:
        val = val + quad(n) if sign > 0 else val - quad(n)
    return val


def _terms(table, quad):
    blocks = [quad(n) for n in range(4)]
    return [_term(table, i, blocks.__getitem__) for i in range(7)]


def _block(outer, inner):
    return 2 * (outer // 2) + inner // 2, 2 * (outer % 2) + inner % 2


def _terms2(table, i, block):
    return _terms(table, lambda n: _term(table, i, lambda m: block(*_block(m, n))))


def _combine(m):
    return [_term(SUMS, n, m.__getitem__) for n in range(4)]


def _combine2(m):
    inner = [_combine(m[i:i + 7]) for i in range(0, 49, 7)]
    return {_block(outer, n): val for n in range(4)
            for outer, val in enumerate(_combine([x[n] for x in inner]))}


class _Tokens:
    def __init__(self, zero_smem):
        self.z = zero_smem[0]
        self.zero = jnp.full((8, T), self.z, jnp.int32).astype(U32)

    def stored(self, ref, lead, start):
        first, *rest = lead
        if ref.dtype == BF16:
            return _words(ref, (first - (self.z & 1), *rest), start, 16) & self.zero
        return self.of(ref[(*lead, pl.ds(_aligned(start + 8 * (self.z & 1), 8), 8), slice(None))])

    def of(self, *vals):
        return pltpu.bitcast(_sum(vals), U32) & self.zero


def _after(token, x, everywhere=False):
    if token is None:
        return x
    bits = x if x.dtype == U32 else pltpu.bitcast(x, U32)
    cut = bits.shape[0] if everywhere else 8
    parts = [bits[r:r + 8] | token for r in range(0, cut, 8)]
    bits = _cat(parts + ([bits[cut:]] if cut < bits.shape[0] else []), axis=0)
    return bits if x.dtype == U32 else pltpu.bitcast(bits, x.dtype)


AX_JOBS = [(i, n, r) for n in range(2) for r in range(0, RO, 16) for i in range(7)]


def _job_ax(tok, released, ax_raw, ax_t, src, i, n, r):
    terms = _terms2(LHS, i, lambda row, col: released(
        ax_raw[src, pl.ds(row * RO + r, 16), pl.ds((2 * col + n) * T, T)].astype(F32)))
    for x, val in enumerate(terms):
        ax_t[7 * i + x, n, pl.ds(r, 16), :] = val.astype(BF16)
    return tok.stored(ax_t, (7 * i + 6, n), r)


def _head_pairs(wqkv_hbm, wo_hbm, bx_hbm, c_hbm, wq_hbm, wuk_hbm, wuv_hbm, wob_hbm,
                ax_copy, ax_raw, ax_t, ctx_t, wob_t, wa_t, wo_t, zero_smem,
                bx_raw, c_raw, wq_raw, wk_raw, wv_raw, wob_raw, wqkv_raw, wo_raw,
                bx_t, c_t, wq_turned, wq_t, wkv_t, guard, sem_in, sem_w):
    def head_copies(j, slot):
        return [pltpu.make_async_copy(src.bitcast(U32).at[:, j, :], dst.at[slot], sem_w.at[3 * slot + n])
                for n, (src, dst) in enumerate(((wuk_hbm, wk_raw), (wuv_hbm, wv_raw), (wq_hbm, wq_raw)))]

    def side_copies(j, slot):
        wob = wob_hbm.at[pl.ds(4 * (j >> 1), 4), pl.ds(_aligned((j & 1) * 64, 64), 64), :]
        wqkv = wqkv_hbm.bitcast(U32).at[:, pl.ds(_aligned(8 * j, 8), 8), :]
        return [pltpu.make_async_copy(wob, wob_raw.at[slot], sem_w.at[6 + 2 * slot]),
                pltpu.make_async_copy(wqkv, wqkv_raw.at[slot], sem_w.at[7 + 2 * slot])]

    def wo_copy(word):
        return pltpu.make_async_copy(wo_hbm.bitcast(U32).at[:, word, :], wo_raw.at[word], sem_w.at[10])

    def c_copy(c):
        rows = pl.ds(c * CH, CH)
        return pltpu.make_async_copy(c_hbm.at[rows, :], c_raw.at[rows, :], sem_in.at[2 * c])

    def x_copy(c):
        rows = pl.ds(c * CH, CH)
        return pltpu.make_async_copy(bx_hbm.at[rows, :], bx_raw.at[rows, :], sem_in.at[2 * c + 1])

    def pair_body(j, first=False):
        slot = j & 1
        tok = _Tokens(zero_smem)
        causal = (lax.broadcasted_iota(jnp.int32, (T, T), 1)
                  <= lax.broadcasted_iota(jnp.int32, (T, T), 0))

        jobs, due, pace = [], [], dict(period=0, clock=0, release=None)

        def queue(cycles, more):
            pace.update(period=cycles / len(more), clock=0)
            jobs.extend(more)

        def flush():
            while jobs:
                jobs.pop(0)()

        def background(cycles, recent=None):
            pace["clock"] += cycles
            token = None
            while jobs and pace["clock"] >= pace["period"]:
                pace["clock"] -= pace["period"]
                pace["release"] = None if recent is None else tok.of(recent[:8])
                new = jobs.pop(0)()
                pace["release"] = None
                token = new if token is None else token | new
            if token is not None:
                due.append([JOB_CYCLES[recent is None], token])
            for entry in due:
                entry[0] -= cycles
            now = [token for left, token in due if left <= 0]
            due[:] = [entry for entry in due if entry[0] > 0]
            return functools.reduce(jnp.bitwise_or, now) if now else None

        def released(x):
            return _after(pace["release"], x, everywhere=True)

        def store_terms(dst, first_term, lead, row, terms):
            for i, val in enumerate(terms):
                dst[(first_term + i, *lead, _rows(row, 16), slice(None))] = val.astype(BF16)
            return tok.stored(dst, (first_term + 6, *lead), row)

        def job_x(c, i, n, r):
            terms = _terms2(RHS, i, lambda row, col: bx_raw[
                pl.ds(c * CH + (col ^ 2) * T + r, 16), pl.ds((2 * row + n) * T, T)].astype(F32))
            return store_terms(bx_t, 7 * i, (n,), c * T + r, terms)

        def job_c(c, i, r):
            terms = _terms2(LHS, i, lambda row, col: c_raw[
                pl.ds(c * CH + row * T + r, 16), pl.ds(col * T, T)].astype(F32))
            return store_terms(c_t, 7 * i, (), c * T + r, terms)

        def jobs_x(c):
            return [P(job_x, c, i, n, r) for r in range(0, T, 16) for n in range(2) for i in range(7)]

        def jobs_c(c):
            return [P(job_c, c, i, r) for r in range(0, T, 16) for i in range(7)]

        def job_wkv(src, i, r):
            def block(row, col):
                raw = (wk_raw, wv_raw)[col % 2]
                return _split(released(raw[src, pl.ds(row * T + r, 16), :]))[col // 2]
            return store_terms(wkv_t, 7 * i, (), r, _terms2(RHS, i, block))

        def job_turn(src, n):
            words = released(wq_raw[src, pl.ds(n * T, T), :])
            wq_turned[n] = pltpu.bitcast(pltpu.bitcast(words, F32).T, U32)
            return tok.stored(wq_turned, (n,), T - 16)

        def job_wq(i, n, r):
            def block(row, col):
                return _split(released(wq_turned[2 * col + n, pl.ds((row % 2) * RO + r, 16), :]))[row // 2]
            return store_terms(wq_t, 7 * i, (n,), r, _terms2(LHS, i, block))

        def jobs_wkv(src):
            return [P(job_wkv, src, i, r) for r in range(0, T, 16) for i in range(7)]

        def jobs_wq(src):
            return ([P(job_turn, src, n) for n in range(DM // T)],
                    [P(job_wq, i, n, r) for n in range(2) for r in range(0, RO, 16) for i in range(7)])

        def job_wob(i, n, r):
            def block(row, col):
                head = 2 * (row % 2) + row // 2
                return released(wob_raw[slot, head, pl.ds(r, 16), pl.ds((2 * col + n) * T, T)].astype(F32))
            return store_terms(wob_t, 7 * i, (n,), j * 64 + r, _terms2(RHS, i, block))

        def job_wo(i, n):
            e, odd, head = j & 3, (j >> 2) & 1, 16 * (j >> 3)

            def block(row, col):
                even_t, odd_t = _split(released(
                    wo_raw[4 * e + row, _rows(head, 16), pl.ds((2 * col + n) * T, T)]))
                return jnp.where(odd == 1, odd_t, even_t)
            return store_terms(wo_t, 7 * i, (n,), odd * T + e * NH + head, _terms2(RHS, i, block))

        permuted = {}

        def job_permute(mat):
            lane = lax.broadcasted_iota(jnp.int32, (32, T), 1)
            e, grp, sub = lane >> 5, (lane >> 2) & 7, lane & 3

            def gather(x, index):
                return jnp.take_along_axis(x, index, axis=1, mode="promise_in_bounds")
            x = [released(wqkv_raw[slot, :, :, pl.ds(mat * DM + t * T, T)].reshape(32, T))
                 for t in range(8)]
            y = [gather(x[t], sub * 32 + e * 8 + ((grp - t) & 7)) for t in range(8)]
            u = [y[-s % 8] for s in range(8)]
            for bit in (1, 2, 4):
                u = [jnp.where((grp & bit) != 0, u[(s - bit) % 8], u[s]) for s in range(8)]
            u = [u[0]] + [gather(u[t], e * 32 + ((grp + t) & 7) * 4 + sub) for t in range(1, 8)]
            permuted[mat] = u
            return _fold(jnp.bitwise_or, functools.reduce(jnp.bitwise_or, u)) & tok.zero

        def column(mat, row, t):
            return pltpu.bitcast(released(permuted[mat][t][8 * row:8 * row + 8]), BF16).astype(F32)

        def job_wa(mat, i, n):
            terms = _terms2(RHS, i, lambda row, col: column(mat, row, 2 * col + n))
            return store_terms(wa_t, 7 * i, (2 * mat + n,), 16 * j, terms)

        pause = [P(lambda: tok.zero)] * 2
        jobs_wob = [P(job_wob, i, n, r) for r in range(0, 64, 16) for n in range(2) for i in range(7)]
        jobs_wo = [P(job_wo, i, n) for n in range(2) for i in range(7)]
        jobs_wa = []
        for mat in range(3):
            jobs_wa += [P(job_permute, mat)] + pause
            jobs_wa += [P(job_wa, mat, i, n) for n in range(2) for i in range(7)]

        q, k, v = {}, {}, {}

        def project_q(c):
            def product(i, n):
                left = _after(background(16) if first else None, _words(wq_t, (i, n), 0, RO))
                return _dot_nt(pltpu.bitcast(left, BF16), _load(bx_t, (i, n), c * T, T))
            blocks = _combine2([product(i, 0) + product(i, 1) for i in range(49)])
            for h in range(2):
                for col in range(4):
                    val = _cat([blocks[2 * h, col], blocks[2 * h + 1, col]], axis=0) * SCALE_B
                    q[4 * c + (col ^ 2), h] = val.T.astype(BF16)

        def project_kv(c):
            m = [_dot(_load(c_t, (i,), c * T, T), _load(wkv_t, (i,), 0, T)) for i in range(49)]
            for (row, col), val in sorted(_combine2(m).items()):
                (k, v)[col % 2][4 * c + row, col // 2] = val.astype(BF16)

        def plain(raw, c, weights):
            def operand():
                parts = []
                for r in range(c * CH, (c + 1) * CH, 32):
                    part = raw[pl.ds(r, 32), :]
                    token = background(8 * (raw.shape[1] // T))
                    if token is not None:
                        part = _cat([_after(_cat([token, token]), part[:, :2 * T]), part[:, 2 * T:]])
                    parts.append(part)
                return _cat(parts, axis=0)
            return [_dot(operand(), w) for w in weights]

        def plain_kv(c, weights):
            for n, val in enumerate(plain(c_raw, c, weights)):
                for r in range(4):
                    (k, v)[n // 2][4 * c + r, n % 2] = val[r * T:(r + 1) * T].astype(BF16)

        def plain_q(c, weights):
            for h, val in enumerate(plain(bx_raw, c, weights)):
                for r in range(4):
                    q[4 * c + r, h] = (val[r * T:(r + 1) * T] * SCALE_B).astype(BF16)

        in_flight, partial, ctx, spread, checks = [], {}, {}, {}, []

        def finish(i, h):
            l, o = partial.pop((i, h))
            l = jnp.sum(l, axis=1, keepdims=True)
            r = _inverse(l)
            ctx[i, h] = o * r
            spread[i, h] = _fold(jnp.maximum, jnp.broadcast_to(l + r, (T, T)))
            b = i // 2
            quad = [(2 * b, 0), (2 * b, 1), (2 * b + 1, 0), (2 * b + 1, 1)]
            if all(u in ctx for u in quad):
                terms = _terms(LHS, lambda m: ctx.pop(quad[m]))
                for n, val in enumerate(terms):
                    ctx_t[n, j, pl.ds(b * T, T), :] = val.astype(BF16)
                checks.append((_fold(jnp.add, terms[0] + terms[5] + terms[6]),
                               functools.reduce(jnp.maximum, [spread.pop(u) for u in quad])))
                due.append([CTX_CYCLES[first], tok.stored(ctx_t, (6, j), b * T) | tok.of(*checks[-1])])

        def weigh(i, h, t, p):
            l, o = partial.get((i, h), (None, None))
            l = p if l is None else l + p
            d = _dot(_after(background(64, p), p).astype(BF16), v[t, h])
            partial[i, h] = (l, d if o is None else o + d)
            if t == i:
                finish(i, h)

        def attention(lo, hi):
            for i in range(lo, hi):
                for h in range(2):
                    for t in range(i + 1):
                        s = _dot_nt(q[i, h], k[t, h])
                        if t == i:
                            s = jnp.where(causal, s, MASKED)
                        in_flight.append((i, h, t, jnp.exp2(s)))
                        if len(in_flight) > DEPTH:
                            weigh(*in_flight.pop(0))
            while hi == S // T and in_flight:
                weigh(*in_flight.pop(0))

        def cycles(lo, hi):
            return 2 * 64 * sum(range(lo + 1, hi + 1))

        if first:
            wk, wv, wq = head_copies(0, 0)
            _start(wv, wk, c_copy(0), c_copy(1))
            _wait(wv, wk, c_copy(0))
            _start(c_copy(2), c_copy(3), wq, x_copy(0))
            weights = [w.astype(BF16) for raw in (wk_raw, wv_raw) for w in _split(raw[0])]
            queue(0.98 * 2048, jobs_c(0))
            plain_kv(0, weights)
            flush()
            _wait(c_copy(1), c_copy(2))
            _start(x_copy(1), x_copy(2))
            queue(0.98 * 4096, jobs_c(1) + jobs_c(2))
            plain_kv(1, weights)
            plain_kv(2, weights)
            flush()
            _wait(c_copy(3), wq)
            turn, terms = jobs_wq(0)
            queue(0.98 * 2048, _interleave(turn, jobs_c(3)))
            plain_kv(3, weights)
            flush()
            _wait(x_copy(0))
            weights = [w.astype(BF16) for w in _split(wq_raw[0])]
            queue(0.95 * (2048 + cycles(0, 4)), jobs_x(0)[:96])
            plain_q(0, weights)
            attention(0, 4)
            flush()
            _wait(x_copy(1), x_copy(2))
            stage = [*side_copies(0, 0), *head_copies(1, 1)]
            _start(x_copy(3), *stage)
            lax.fori_loop(0, 16, lambda word, carry: wo_copy(word).start(), None)
            queue(0.98 * (2048 + cycles(4, 8)), jobs_x(2) + terms + jobs_x(0)[96:] + jobs_x(1)[:14])
            plain_q(1, weights)
            attention(4, 8)
            flush()
            _wait(x_copy(3))
            queue(0.98 * (1568 + cycles(8, 9)), jobs_x(3)[:98])
            project_q(2)
            attention(8, 9)
            flush()
            _wait(*stage)
            _start(ax_copy(0, 0), *head_copies(2, 0), *side_copies(1, 1))
            turn, terms = jobs_wq(1)
            queue(0.92 * (1568 + cycles(9, 14)), jobs_x(3)[98:] + _interleave(
                _interleave(jobs_wob, jobs_wa), _interleave(jobs_x(1)[14:], _interleave(turn, jobs_wkv(1)))))
            attention(9, 12)
            assert not any(job.func is job_x and job.args[0] == 3 for job in jobs)
            project_q(3)
            attention(12, 14)
            flush()
            _wait(*[wo_copy(word) for word in range(16)], ax_copy(0, 0))
            _start(ax_copy(1, 1))
            queue(0.92 * cycles(14, 16), _interleave(
                jobs_wo + terms, [P(_job_ax, tok, released, ax_raw, ax_t, 0, *job) for job in AX_JOBS]))
            attention(14, 16)
            flush()
        else:
            queue(0.98 * cycles(0, 12), _interleave(jobs_wob, jobs_wo + jobs_wa))
            project_kv(0)
            project_q(0)
            project_kv(1)
            done = 0
            for row, project, c in ((3, project_q, 1), (6, project_q, 2), (7, project_kv, 2),
                                    (10, project_q, 3), (11, project_kv, 3)):
                attention(done, row)
                project(c)
                done = row
            attention(done, 12)
            flush()
            turn, terms = jobs_wq(1 - slot)
            queue(0.9 * cycles(12, 16), _interleave(jobs_wkv(1 - slot), turn + pause + terms))
            attention(12, 16)
            flush()
        guard[0] = _sum([guard[0]] + [x for x, _ in checks])
        guard[1] = functools.reduce(jnp.maximum, [guard[1]] + [x for _, x in checks])

        def ahead(n):
            return j + n if first else jnp.minimum(j + n, NP - 1)
        _wait(*head_copies(ahead(2), slot), *side_copies(ahead(1), 1 - slot))

        @pl.when(j < NP - 1)
        def _():
            _start(*head_copies(ahead(3), 1 - slot), *side_copies(ahead(2), slot))

    def exact_pairs(ctx):
        def block(i):
            return pl.ds(pl.multiple_of(i * T, T), T)

        def qkv(n, h, i):
            return c_t.at[(2 * n + h) * 4 + (i >> 2), block(i & 3), :]

        def project(x, carry):
            h, i = x & 1, x >> 1
            for n, (rows, w, scale) in enumerate(
                    ((bx_raw, wq_raw, SCALE_B), (c_raw, wk_raw, 1.0), (c_raw, wv_raw, 1.0))):
                def add(t, val):
                    even, odd = _split(w[0, block(t), :])
                    return val + _dot(rows[block(i), block(t)], jnp.where(h == 0, even, odd).astype(BF16))
                val = lax.fori_loop(0, w.shape[1] // T, add, jnp.zeros((T, T), F32))
                qkv(n, h, i)[...] = (val * scale).astype(BF16)

        def attend(b, x, carry):
            quad, part = x >> 3, pl.ds(pl.multiple_of((x & 7) * 16, 16), 16)
            h, i = quad & 1, 2 * b + (quad >> 1)

            def scores(t):
                row = lax.broadcasted_iota(jnp.int32, (16, T), 0) + (i * T + (x & 7) * 16)
                col = lax.broadcasted_iota(jnp.int32, (16, T), 1) + t * T
                return jnp.where(col <= row, _dot_nt(qkv(0, h, i)[part, :], qkv(1, h, t)[...]), MASKED)

            m = lax.fori_loop(
                0, i + 1, lambda t, m: jnp.maximum(m, jnp.max(scores(t), axis=1, keepdims=True)),
                jnp.full((16, 1), -jnp.inf, F32))

            def accumulate(t, carry):
                l, o = carry
                p = jnp.exp2(scores(t) - m)
                return (l + jnp.sum(p, axis=1, keepdims=True),
                        o + _dot(p.astype(BF16), qkv(2, h, t)[...]))
            l, o = lax.fori_loop(0, i + 1, accumulate,
                                 (jnp.zeros((16, 1), F32), jnp.zeros((16, T), F32)))
            ctx[quad, part, :] = o / l

        def pair(j, carry):
            _start(*head_copies(j, 0))
            _wait(*head_copies(j, 0))
            lax.fori_loop(0, 2 * S // T, project, None)

            def rows(b, carry):
                lax.fori_loop(0, 32, P(attend, b), None)
                for n, val in enumerate(_terms(LHS, lambda m: ctx[m])):
                    ctx_t[n, j, block(b), :] = val.astype(BF16)
            lax.fori_loop(0, S // T // 2, rows, None)

        lax.fori_loop(0, NP, pair, None)

    guard[...] = jnp.zeros(guard.shape, F32)
    pair_body(0, first=True)
    lax.fori_loop(1, NP, lambda j, carry: pair_body(j), None)

    safe = jnp.logical_and(jnp.abs(guard[0]) < jnp.inf, guard[1] < SAFE_SUM)

    @pl.when(jnp.max(jnp.where(safe, 0.0, 1.0)) > 0.0)
    def _():
        pl.run_scoped(exact_pairs, pltpu.VMEM((4, T, T), F32))


def _outputs(out_hbm, ax_copy, ax_raw, ax_t, ctx_t, wob_t, wa_t, wo_t, zero_smem,
             o_t, kbuf, vbuf, qbuf, acc, obuf, sem_out):
    def out_copy(c, slot):
        rows = pl.ds(_aligned(c * CO, CO), CO)
        return pltpu.make_async_copy(obuf.at[slot], out_hbm.at[rows, :], sem_out.at[slot])

    for buf in (kbuf, vbuf):
        for t in range(8):
            buf[t, pl.ds(CO, HALO), :] = jnp.zeros((HALO, T), F32)

    t_q, t_v, t_b = (49 * RO * n for n in (1, 2, 3))
    t_o = t_b + (42 + EARLY_B) * 4 * RO

    def chunk_body(c, carry):
        slot = c & 1
        tok = _Tokens(zero_smem)
        plan, due, clock = {}, {}, [0]

        def schedule(job, begin, end, release=False):
            plan.setdefault(max(clock[0], begin // TICK), []).append((job, -(-end // TICK), release))

        def step(results, a, w):
            res = [None] * len(w)
            for x, left in enumerate(a):
                n = clock[0]
                clock[0] += 1
                if n in due:
                    left = _after(functools.reduce(jnp.bitwise_or, due.pop(n)), left)
                left = left.astype(BF16) if left.dtype == F32 else pltpu.bitcast(left, BF16)
                for y in range(len(w)):
                    d = _dot(left, w[y](x))
                    res[y] = d if res[y] is None else res[y] + d
                token = None
                for job, last, release in plan.pop(n, []):
                    if release and token is None:
                        token = tok.of(d[:8])
                    due.setdefault(max(last, n + 1), []).append(job(token) if release else job())
            results.append(res)

        def project(lhs_t, rhs_t, tile0, write, span):
            inner = {}

            def combine(i, y, m):
                inner[i, y] = _combine([x[y] for x in m])
                return tok.of(*[x[r + 8:r + 16] for x in inner[i, y] for r in range(0, RO, 16)])

            def finish(outer, y, r):
                vals = [_term(SUMS, outer, lambda i: inner[i, y][n][r:r + 16]) for n in range(4)]
                for n, val in enumerate(vals):
                    row, col = _block(outer, n)
                    write(row * RO + r, 2 * col + y, val)
                return tok.of(*[x[8:] for x in vals])

            for i in range(7):
                m = []
                done = clock[0] * TICK + 7 * RO
                for y in range(2):
                    schedule(P(combine, i, y, m), done, done + 200 + 100 * y)
                for outer in FINAL[i]:
                    slabs = [(y, r) for r in range(0, RO, 16) for y in range(2)]
                    for x, slab in enumerate(slabs):
                        window = (span if i == 6 else 7 * RO) * (x + 1) // len(slabs)
                        schedule(P(finish, outer, *slab), done, done + 300 + window)
                for n in range(7 * i, 7 * i + 7):
                    step(m, [_words(lhs_t, (n, x), 0, RO) for x in range(2)],
                         [P(lambda y, x: _load(rhs_t, (n, tile0 + y), x * T, T), y) for y in range(2)])

        for buf in (kbuf, vbuf):
            for t in range(8):
                buf[t, pl.ds(0, HALO), :] = buf[t, pl.ds(CO, HALO), :]

        def write_rows(buf, row, t, val):
            buf[t, pl.ds(HALO + row, 16), :] = val

        def write_q(row, t, val):
            qbuf[t, pl.ds(row, 16), :] = val * SCALE_A

        project(ax_t, wa_t, 2, P(write_rows, kbuf), 2800)
        project(ax_t, wa_t, 0, write_q, 1000)

        att = {}

        def job_weights(row, r, release):
            base = HALO + row * RO + r
            qs = [_after(release, qbuf[t, pl.ds(row * RO + r, 8), :]) for t in range(8)]
            logits = []
            for w in range(WIN):
                x = _sum([qs[t] * kbuf[t, pl.ds(base - DIL * w, 8), :] for t in range(8)])
                x = x + pltpu.roll(x, 64, 1)
                x = x + pltpu.roll(x, 32, 1)
                if row == 0 and r < DIL * w:
                    pos = lax.broadcasted_iota(jnp.int32, (8, T), 0) + (c * CO + r)
                    x = jnp.where(pos >= DIL * w, x, MASKED)
                logits.append(x)
            m = functools.reduce(jnp.maximum, logits)
            p = [jnp.exp2(x - m) for x in logits]
            inv = _inverse(_sum(p))
            att[row, r] = [x * inv for x in p]
            return tok.of(att[row, r][0])

        def job_values(row, r, release):
            base = HALO + row * RO + r
            p = [_after(release, x) for x in att[row, r]]
            att[row, r] = [_sum([p[w] * vbuf[t, pl.ds(base - DIL * w, 8), :] for w in range(WIN)])
                           for t in range(8)]
            return tok.of(att[row, r][-1])

        def job_o(n, r, i):
            def block(row, col):
                return _cat([att[row, r][2 * col + n], att[row, r + 8][2 * col + n]], axis=0)
            for x, val in enumerate(_terms2(LHS, i, block)):
                o_t[7 * i + x, n, pl.ds(r, 16), :] = val.astype(BF16)
            return tok.stored(o_t, (7 * i + 6, n), r)

        groups = [(row, r + x) for r in range(0, RO, 16) for row in (2, 0, 3, 1) for x in (0, 8)]
        w0, w1, v0, v1 = t_v + 1300, t_b + 4500, t_b + 3500, t_o - 700
        for g, (row, r) in enumerate(groups):
            begin = w0 + (w1 - w0) * g // len(groups)
            schedule(P(job_weights, row, r), begin, begin + 500, release=True)
            begin = max(v0 + (v1 - v0) * g // len(groups), begin + 700)
            schedule(P(job_values, row, r), begin, begin + 500, release=True)
            if g % 8 == 7:
                for x, (n, i) in enumerate((n, i) for n in range(2) for i in range(7)):
                    schedule(P(job_o, n, r - 8, i), begin, min(begin + 500 + 60 * (x + 1), t_o))
        project(ax_t, wa_t, 4, P(write_rows, vbuf), 1000)

        touched = {}

        def project_b(i):
            m = []

            def accumulate(y, inner):
                val = _combine([x[y] for x in m])[inner]
                token = None
                for outer, sign in OUT[i]:
                    row, col = _block(outer, inner)
                    rows, col = pl.ds(row * RO, RO), 2 * col + y
                    total = val
                    if (outer, inner, y) in touched:
                        total = acc[col, rows, :] + val if sign > 0 else acc[col, rows, :] - val
                    touched[outer, inner, y] = True
                    if outer not in FINAL[i]:
                        acc[col, rows, :] = total
                        token = tok.stored(acc, (col,), row * RO)
                    else:
                        obuf[slot, rows, pl.ds(DM + col * T, T)] = total.astype(BF16)
                        if token is None:
                            token = tok.of(_fold(jnp.add, total))
                return token

            parts = [(y, inner) for y in range(2) for inner in range(4)]
            done = clock[0] * TICK + 7 * 4 * RO
            if i < 6:
                for x, part in enumerate(parts):
                    schedule(P(accumulate, *part), done, done + 256 + 200 * x)
            for n in range(7):
                if i == 6 and n == EARLY_B:
                    yield

                def quad(kt, x):
                    return (i, 2 * kt + x % 2), (2 * c + x // 2) * RO
                if len(LHS[n]) == 1:
                    a = [_words(ctx_t, *quad(kt, LHS[n][0][0]), RO) for kt in range(8)]
                else:
                    a = [_term(LHS, n, lambda x: _load(ctx_t, (i + tok.z * n, 2 * kt + x % 2), quad(kt, x)[1], RO).astype(F32))
                         for kt in range(8)]
                step(m, a, [P(lambda y, x: _load(wob_t, (7 * i + n, y), x * T, T), y) for y in range(2)])
            if i == 6:
                for part in parts:
                    accumulate(*part)

        for i in range(6):
            list(project_b(i))
        last_b = project_b(6)
        next(last_b)

        for x, job in enumerate(AX_JOBS):
            schedule(P(_job_ax, tok, lambda val: val, ax_raw, ax_t, 1 - slot, *job),
                     t_o, t_o + 100 + 3000 * (x + 1) // len(AX_JOBS))

        def write_out(row, t, val):
            obuf[slot, pl.ds(row, 16), pl.ds(t * T, T)] = val.astype(BF16)

        project(o_t, wo_t, 0, write_out, 300)
        list(last_b)
        assert not plan and not due
        out_copy(c, slot).start()
        ax_copy(jnp.minimum(c + 2, NO - 1), slot).wait()

        @pl.when(c < NO - 1)
        def _():
            ax_copy(jnp.minimum(c + 3, NO - 1), 1 - slot).start()

        @pl.when(c >= 1)
        def _():
            out_copy(c - 1, 1 - slot).wait()

    ax_copy(1, 1).wait()
    ax_copy(2, 0).start()
    lax.fori_loop(0, NO, chunk_body, None)
    out_copy(NO - 1, (NO - 1) % 2).wait()


def _kernel(ax_hbm, wqkv_hbm, wo_hbm, bx_hbm, c_hbm, wq_hbm, wuk_hbm, wuv_hbm, wob_hbm, out_hbm,
            ax_raw, ax_t, ctx_t, wob_t, wa_t, wo_t, zero_smem, sem_ax):
    vmem, dma = pltpu.VMEM, pltpu.SemaphoreType.DMA

    def clear(i, carry):
        zero_smem[0] = i >> 1
    lax.fori_loop(0, 2, clear, None)

    def ax_copy(c, slot):
        rows = pl.ds(_aligned(c * CO, CO), CO)
        return pltpu.make_async_copy(ax_hbm.at[rows, :], ax_raw.at[slot], sem_ax.at[slot])

    shared = (ax_copy, ax_raw, ax_t, ctx_t, wob_t, wa_t, wo_t, zero_smem)
    pl.run_scoped(
        P(_head_pairs, wqkv_hbm, wo_hbm, bx_hbm, c_hbm, wq_hbm, wuk_hbm, wuv_hbm, wob_hbm, *shared),
        vmem((S, DM), BF16),
        vmem((S, DC), BF16),
        vmem((2, DM, T), U32),
        vmem((2, DC, T), U32),
        vmem((2, DC, T), U32),
        vmem((2, 4, 64, DM), BF16),
        vmem((2, 4, 8, 3 * DM), U32),
        vmem((16, NH, DM), U32),
        vmem((49, 2, S // 4, T), BF16),
        vmem((49, S // 4, T), BF16),
        vmem((DM // T, T, T), U32),
        vmem((49, 2, RO, T), BF16),
        vmem((49, T, T), BF16),
        vmem((2, 8, T), F32),
        dma((2 * S // CH,)), dma((11,)))
    pl.run_scoped(
        P(_outputs, out_hbm, *shared),
        vmem((49, 2, RO, T), BF16),
        vmem((8, HALO + CO, T), F32),
        vmem((8, HALO + CO, T), F32),
        vmem((8, CO, T), F32),
        vmem((8, CO, T), F32),
        vmem((2, CO, 2 * DM), BF16),
        dma((2,)))


@jax.jit
def pallas_concat_heads__sliding_local_dilated__compressed_kv_cla__prompt_kernel(
    A_x: jax.Array,
    A_wqkv: jax.Array,
    A_wo: jax.Array,
    B_x: jax.Array,
    B_c_kv: jax.Array,
    B_w_q: jax.Array,
    B_w_uk: jax.Array,
    B_w_uv: jax.Array,
    B_w_o: jax.Array,
):
    vmem = pltpu.VMEM
    out = pl.pallas_call(
        _kernel,
        out_shape=jax.ShapeDtypeStruct((S, 2 * DM), BF16),
        in_specs=[pl.BlockSpec(memory_space=pl.ANY)] * 9,
        out_specs=pl.BlockSpec(memory_space=pl.ANY),
        scratch_shapes=[
            vmem((2, CO, DM), BF16),
            vmem((49, 2, RO, T), BF16),
            vmem((7, NP, S // 2, T), BF16),
            vmem((49, 2, DM, T), BF16),
            vmem((49, 6, 2 * T, T), BF16),
            vmem((49, 2, 2 * T, T), BF16),
            pltpu.SMEM((1,), jnp.int32),
            pltpu.SemaphoreType.DMA((2,)),
        ],
        compiler_params=pltpu.CompilerParams(
            vmem_limit_bytes=127 * 2**20, disable_bounds_checks=True),
    )(
        A_x.reshape(S, DM),
        A_wqkv.reshape(4, DM // 4, 3 * DM),
        A_wo.reshape(NH, DM // NH, DM),
        B_x.reshape(S, DM),
        B_c_kv.reshape(S, DC),
        B_w_q,
        B_w_uk,
        B_w_uv,
        B_w_o,
    )
    return out.reshape(1, S, 2 * DM)
```

```python
import functools
import math

import jax
import jax.numpy as jnp
from jax import lax
import jax.experimental.pallas as pl
import jax.experimental.pallas.tpu as pltpu

S = 2048
DM = 1024
DC = 512
NH = 32
NP = NH // 2
T = 128
CH = 4 * T
RO = 64
CO = 4 * RO
NO = S // CO
WIN, DIL = 8, 2
HALO = 16

LOG2E = math.log2(math.e)
SCALE_A = (DM // NH) ** -0.5 * LOG2E
SCALE_B = T ** -0.5 * LOG2E
MASKED = -1e9 * LOG2E
SAFE_SUM = 2.0 ** 40

DEPTH = 3
JOB_CYCLES = 1024, 256
CTX_CYCLES = 1024, 1536

NX0, NX3 = 49, 84
TICK = RO // 2
EARLY_B = 4
F32, BF16, U32 = jnp.float32, jnp.bfloat16, jnp.uint32
P = functools.partial


def _dot(a, b):
    return jnp.dot(a, b, preferred_element_type=F32)


def _dot_nt(a, b):
    return lax.dot_general(a, b, (((1,), (1,)), ((), ())), preferred_element_type=F32)


def _cat(xs, axis=1):
    return xs[0] if len(xs) == 1 else jnp.concatenate(xs, axis=axis)


def _sum(xs):
    return functools.reduce(jnp.add, xs)


def _fold(op, x):
    return functools.reduce(op, [x[r:r + 8] for r in range(0, x.shape[0], 8)])


def _aligned(x, n):
    return x if isinstance(x, int) else pl.multiple_of(x, n)


def _rows(start, n):
    return pl.ds(_aligned(start, 16), n)


def _words(ref, lead, start, n):
    return ref.bitcast(U32)[(*lead, pl.ds(_aligned(start >> 1, 8), n // 2), slice(None))]


def _load(ref, lead, start, n):
    return pltpu.bitcast(_words(ref, lead, start, n), BF16)


def _split(w):
    return (pltpu.bitcast(w << 16, F32), pltpu.bitcast(w & jnp.uint32(0xFFFF0000), F32))


def _inverse(l):
    r = pl.reciprocal(l, approx=True)
    return r * (2.0 - l * r)


def _interleave(x, y):
    order = [((n + 0.5) / len(z), m, job) for m, z in enumerate((x, y)) for n, job in enumerate(z)]
    return [job for _, _, job in sorted(order, key=lambda e: e[:2])]


def _start(*copies):
    for cp in copies:
        cp.start()


def _wait(*copies):
    for cp in copies:
        cp.wait()


LHS = (((0, 1), (3, 1)), ((2, 1), (3, 1)), ((0, 1),), ((3, 1),),
       ((0, 1), (1, 1)), ((2, 1), (0, -1)), ((1, 1), (3, -1)))
RHS = (((0, 1), (3, 1)), ((0, 1),), ((1, 1), (3, -1)), ((2, 1), (0, -1)),
       ((3, 1),), ((0, 1), (1, 1)), ((2, 1), (3, 1)))
OUT = (((0, 1), (3, 1)), ((2, 1), (3, -1)), ((1, 1), (3, 1)), ((0, 1), (2, 1)),
       ((0, -1), (1, 1)), ((3, 1),), ((0, 1),))
SUMS = tuple(tuple((i, sign) for i in range(7) for m, sign in OUT[i] if m == n) for n in range(4))
FINAL = tuple(tuple(n for n in range(4) if SUMS[n][-1][0] == i) for i in range(7))


def _term(table, i, quad):
    (n, _), *rest = table[i]
    val = quad(n)
    for n, sign in rest:
        val = val + quad(n) if sign > 0 else val - quad(n)
    return val


def _terms(table, quad):
    blocks = [quad(n) for n in range(4)]
    return [_term(table, i, blocks.__getitem__) for i in range(7)]


def _block(outer, inner):
    return 2 * (outer // 2) + inner // 2, 2 * (outer % 2) + inner % 2


def _terms2(table, i, block):
    return _terms(table, lambda n: _term(table, i, lambda m: block(*_block(m, n))))


def _combine(m):
    return [_term(SUMS, n, m.__getitem__) for n in range(4)]


def _combine2(m):
    inner = [_combine(m[i:i + 7]) for i in range(0, 49, 7)]
    return {_block(outer, n): val for n in range(4)
            for outer, val in enumerate(_combine([x[n] for x in inner]))}


class _Tokens:
    def __init__(self, zero_smem):
        self.z = zero_smem[0]
        self.zero = jnp.full((8, T), self.z, jnp.int32).astype(U32)

    def stored(self, ref, lead, start):
        first, *rest = lead
        if ref.dtype == BF16:
            return _words(ref, (first - (self.z & 1), *rest), start, 16) & self.zero
        return self.of(ref[(*lead, pl.ds(_aligned(start + 8 * (self.z & 1), 8), 8), slice(None))])

    def of(self, *vals):
        return pltpu.bitcast(_sum(vals), U32) & self.zero


def _after(token, x, everywhere=False):
    if token is None:
        return x
    bits = x if x.dtype == U32 else pltpu.bitcast(x, U32)
    cut = bits.shape[0] if everywhere else 8
    parts = [bits[r:r + 8] | token for r in range(0, cut, 8)]
    bits = _cat(parts + ([bits[cut:]] if cut < bits.shape[0] else []), axis=0)
    return bits if x.dtype == U32 else pltpu.bitcast(bits, x.dtype)


AX_JOBS = [(i, n, r) for n in range(2) for r in range(0, RO, 16) for i in range(7)]


def _job_ax(tok, released, ax_raw, ax_t, src, i, n, r):
    terms = _terms2(LHS, i, lambda row, col: released(
        ax_raw[src, pl.ds(row * RO + r, 16), pl.ds((2 * col + n) * T, T)].astype(F32)))
    for x, val in enumerate(terms):
        ax_t[7 * i + x, n, pl.ds(r, 16), :] = val.astype(BF16)
    return tok.stored(ax_t, (7 * i + 6, n), r)


def _head_pairs(wqkv_hbm, wo_hbm, bx_hbm, c_hbm, wq_hbm, wuk_hbm, wuv_hbm, wob_hbm,
                ax_copy, ax_raw, ax_t, ctx_t, wob_t, wa_t, wo_t, zero_smem,
                bx_raw, c_raw, wq_raw, wk_raw, wv_raw, wob_raw, wqkv_raw, wo_raw,
                bx_t, c_t, wq_turned, wq_t, wkv_t, guard, sem_in, sem_w):
    def head_copies(j, slot):
        return [pltpu.make_async_copy(src.bitcast(U32).at[:, j, :], dst.at[slot], sem_w.at[3 * slot + n])
                for n, (src, dst) in enumerate(((wuk_hbm, wk_raw), (wuv_hbm, wv_raw), (wq_hbm, wq_raw)))]

    def side_copies(j, slot):
        wob = wob_hbm.at[pl.ds(4 * (j >> 1), 4), pl.ds(_aligned((j & 1) * 64, 64), 64), :]
        wqkv = wqkv_hbm.bitcast(U32).at[:, pl.ds(_aligned(8 * j, 8), 8), :]
        return [pltpu.make_async_copy(wob, wob_raw.at[slot], sem_w.at[6 + 2 * slot]),
                pltpu.make_async_copy(wqkv, wqkv_raw.at[slot], sem_w.at[7 + 2 * slot])]

    def wo_copy(word):
        return pltpu.make_async_copy(wo_hbm.bitcast(U32).at[:, word, :], wo_raw.at[word], sem_w.at[10])

    def c_copy(c):
        rows = pl.ds(c * CH, CH)
        return pltpu.make_async_copy(c_hbm.at[rows, :], c_raw.at[rows, :], sem_in.at[2 * c])

    def x_copy(c):
        rows = pl.ds(c * CH, CH)
        return pltpu.make_async_copy(bx_hbm.at[rows, :], bx_raw.at[rows, :], sem_in.at[2 * c + 1])

    def pair_body(j, first=False):
        slot = j & 1
        tok = _Tokens(zero_smem)
        causal = (lax.broadcasted_iota(jnp.int32, (T, T), 1)
                  <= lax.broadcasted_iota(jnp.int32, (T, T), 0))

        jobs, due, pace = [], [], dict(release=None, recent=None)

        def queue(cycles, more, q=1.0, kv=1.0, attention=1.0):
            pace.update(period=cycles / len(more), clock=0, q=q, kv=kv, attention=attention)
            jobs.extend(more)

        def flush():
            while jobs:
                jobs.pop(0)()

        def background(cycles, share=1.0, recent=None):
            pace["clock"] += cycles * share
            token = None
            while jobs and pace["clock"] >= pace["period"]:
                pace["clock"] -= pace["period"]
                pace["release"] = None if recent is None else tok.of(recent[:8])
                new = jobs.pop(0)()
                pace["release"] = None
                token = new if token is None else token | new
            if token is not None:
                due.append([JOB_CYCLES[recent is None], token])
            for entry in due:
                entry[0] -= cycles
            now = [token for left, token in due if left <= 0]
            due[:] = [entry for entry in due if entry[0] > 0]
            return functools.reduce(jnp.bitwise_or, now) if now else None

        def released(x):
            return _after(pace["release"], x, everywhere=True)

        def store_terms(dst, first_term, lead, row, terms):
            for i, val in enumerate(terms):
                dst[(first_term + i, *lead, _rows(row, 16), slice(None))] = val.astype(BF16)
            return tok.stored(dst, (first_term + 6, *lead), row)

        def job_x(c, i, n, r):
            terms = _terms2(RHS, i, lambda row, col: bx_raw[
                pl.ds(c * CH + (col ^ 2) * T + r, 16), pl.ds((2 * row + n) * T, T)].astype(F32))
            return store_terms(bx_t, 7 * i, (n,), c * T + r, terms)

        def job_c(c, i, r):
            terms = _terms2(LHS, i, lambda row, col: c_raw[
                pl.ds(c * CH + row * T + r, 16), pl.ds(col * T, T)].astype(F32))
            return store_terms(c_t, 7 * i, (), c * T + r, terms)

        def jobs_x(c):
            return [P(job_x, c, i, n, r) for r in range(0, T, 16) for n in range(2) for i in range(7)]

        def jobs_c(c):
            return [P(job_c, c, i, r) for r in range(0, T, 16) for i in range(7)]

        def job_wkv(src, i, r):
            def block(row, col):
                raw = (wk_raw, wv_raw)[col % 2]
                return _split(released(raw[src, pl.ds(row * T + r, 16), :]))[col // 2]
            return store_terms(wkv_t, 7 * i, (), r, _terms2(RHS, i, block))

        def job_turn(src, n):
            words = released(wq_raw[src, pl.ds(n * T, T), :])
            wq_turned[n] = pltpu.bitcast(pltpu.bitcast(words, F32).T, U32)
            return tok.stored(wq_turned, (n,), T - 16)

        def job_wq(i, n, r):
            def block(row, col):
                return _split(released(wq_turned[2 * col + n, pl.ds((row % 2) * RO + r, 16), :]))[row // 2]
            return store_terms(wq_t, 7 * i, (n,), r, _terms2(LHS, i, block))

        def jobs_wkv(src):
            return [P(job_wkv, src, i, r) for r in range(0, T, 16) for i in range(7)]

        def jobs_wq(src):
            return ([P(job_turn, src, n) for n in range(DM // T)],
                    [P(job_wq, i, n, r) for n in range(2) for r in range(0, RO, 16) for i in range(7)])

        def job_wob(i, n, r):
            def block(row, col):
                head = 2 * (row % 2) + row // 2
                return released(wob_raw[slot, head, pl.ds(r, 16), pl.ds((2 * col + n) * T, T)].astype(F32))
            return store_terms(wob_t, 7 * i, (n,), j * 64 + r, _terms2(RHS, i, block))

        def job_wo(i, n):
            e, odd, head = j & 3, (j >> 2) & 1, 16 * (j >> 3)

            def block(row, col):
                even_t, odd_t = _split(released(
                    wo_raw[4 * e + row, _rows(head, 16), pl.ds((2 * col + n) * T, T)]))
                return jnp.where(odd == 1, odd_t, even_t)
            return store_terms(wo_t, 7 * i, (n,), odd * T + e * NH + head, _terms2(RHS, i, block))

        permuted = {}

        def job_permute(mat):
            lane = lax.broadcasted_iota(jnp.int32, (32, T), 1)
            e, grp, sub = lane >> 5, (lane >> 2) & 7, lane & 3

            def gather(x, index):
                return jnp.take_along_axis(x, index, axis=1, mode="promise_in_bounds")
            x = [released(wqkv_raw[slot, :, :, pl.ds(mat * DM + t * T, T)].reshape(32, T))
                 for t in range(8)]
            y = [gather(x[t], sub * 32 + e * 8 + ((grp - t) & 7)) for t in range(8)]
            u = [y[-s % 8] for s in range(8)]
            for bit in (1, 2, 4):
                u = [jnp.where((grp & bit) != 0, u[(s - bit) % 8], u[s]) for s in range(8)]
            u = [u[0]] + [gather(u[t], e * 32 + ((grp + t) & 7) * 4 + sub) for t in range(1, 8)]
            permuted[mat] = u
            return _fold(jnp.bitwise_or, functools.reduce(jnp.bitwise_or, u)) & tok.zero

        def column(mat, row, t):
            return pltpu.bitcast(released(permuted[mat][t][8 * row:8 * row + 8]), BF16).astype(F32)

        def job_wa(mat, i, n):
            terms = _terms2(RHS, i, lambda row, col: column(mat, row, 2 * col + n))
            return store_terms(wa_t, 7 * i, (2 * mat + n,), 16 * j, terms)

        pause = [P(lambda: tok.zero)] * 2
        jobs_wob = [P(job_wob, i, n, r) for r in range(0, 64, 16) for n in range(2) for i in range(7)]
        jobs_wo = [P(job_wo, i, n) for n in range(2) for i in range(7)]
        jobs_wa = []
        for mat in range(3):
            jobs_wa += [P(job_permute, mat)] + pause
            jobs_wa += [P(job_wa, mat, i, n) for n in range(2) for i in range(7)]

        q, k, v = {}, {}, {}

        def product(dot, share, left, right):
            token = background(left.shape[0] // 2, share, pace["recent"])
            pace["recent"] = dot(pltpu.bitcast(_after(token, left), BF16), right)
            return pace["recent"]

        def project_q(c):
            blocks = _combine2([_sum([
                product(_dot_nt, pace["q"], _words(wq_t, (i, n), 0, RO), _load(bx_t, (i, n), c * T, T))
                for n in range(2)]) for i in range(49)])
            for h in range(2):
                for col in range(4):
                    val = _cat([blocks[2 * h, col], blocks[2 * h + 1, col]], axis=0) * SCALE_B
                    q[4 * c + (col ^ 2), h] = val.T.astype(BF16)

        def project_kv(c):
            m = [product(_dot, pace["kv"], _words(c_t, (i,), c * T, T), _load(wkv_t, (i,), 0, T))
                 for i in range(49)]
            for (row, col), val in sorted(_combine2(m).items()):
                (k, v)[col % 2][4 * c + row, col // 2] = val.astype(BF16)

        def plain(raw, c, weights):
            def operand():
                parts = []
                for r in range(c * CH, (c + 1) * CH, 32):
                    part = raw[pl.ds(r, 32), :]
                    token = background(8 * (raw.shape[1] // T))
                    if token is not None:
                        part = _cat([_after(_cat([token, token]), part[:, :2 * T]), part[:, 2 * T:]])
                    parts.append(part)
                return _cat(parts, axis=0)
            return [_dot(operand(), w) for w in weights]

        def plain_kv(c, weights):
            for n, val in enumerate(plain(c_raw, c, weights)):
                for r in range(4):
                    (k, v)[n // 2][4 * c + r, n % 2] = val[r * T:(r + 1) * T].astype(BF16)

        def plain_q(c, weights):
            for h, val in enumerate(plain(bx_raw, c, weights)):
                for r in range(4):
                    q[4 * c + r, h] = (val[r * T:(r + 1) * T] * SCALE_B).astype(BF16)

        in_flight, partial, ctx, spread, checks = [], {}, {}, {}, []

        def finish(i, h):
            l, o = partial.pop((i, h))
            l = jnp.sum(l, axis=1, keepdims=True)
            r = _inverse(l)
            ctx[i, h] = o * r
            spread[i, h] = _fold(jnp.maximum, jnp.broadcast_to(l + r, (T, T)))
            b = i // 2
            quad = [(2 * b, 0), (2 * b, 1), (2 * b + 1, 0), (2 * b + 1, 1)]
            if all(u in ctx for u in quad):
                terms = _terms(LHS, lambda m: ctx.pop(quad[m]))
                for n, val in enumerate(terms):
                    ctx_t[n, j, pl.ds(b * T, T), :] = val.astype(BF16)
                checks.append((_fold(jnp.add, terms[0] + terms[5] + terms[6]),
                               functools.reduce(jnp.maximum, [spread.pop(u) for u in quad])))
                due.append([CTX_CYCLES[first], tok.stored(ctx_t, (6, j), b * T) | tok.of(*checks[-1])])

        def weigh(i, h, t, p):
            l, o = partial.get((i, h), (None, None))
            l = p if l is None else l + p
            d = _dot(_after(background(64, pace["attention"], p), p).astype(BF16), v[t, h])
            partial[i, h] = (l, d if o is None else o + d)
            if t == i:
                finish(i, h)

        def attention(lo, hi):
            for i in range(lo, hi):
                for h in range(2):
                    for t in range(i + 1):
                        s = _dot_nt(q[i, h], k[t, h])
                        if t == i:
                            s = jnp.where(causal, s, MASKED)
                        in_flight.append((i, h, t, jnp.exp2(s)))
                        if len(in_flight) > DEPTH:
                            weigh(*in_flight.pop(0))
            while hi == S // T and in_flight:
                weigh(*in_flight.pop(0))

        def cycles(lo, hi):
            return 2 * 64 * sum(range(lo + 1, hi + 1))

        if first:
            wk, wv, wq = head_copies(0, 0)
            _start(wv, wk, c_copy(0), c_copy(1))
            _wait(wv, wk, c_copy(0))
            _start(c_copy(2), c_copy(3), wq, x_copy(0))
            weights = [w.astype(BF16) for raw in (wk_raw, wv_raw) for w in _split(raw[0])]
            queue(0.98 * 2048, jobs_c(0))
            plain_kv(0, weights)
            flush()
            _wait(c_copy(1), c_copy(2))
            _start(x_copy(1), x_copy(2))
            queue(0.98 * 4096, jobs_c(1) + jobs_c(2))
            plain_kv(1, weights)
            plain_kv(2, weights)
            flush()
            _wait(c_copy(3), wq)
            turn, terms = jobs_wq(0)
            queue(0.98 * 2048, _interleave(turn, jobs_c(3)))
            plain_kv(3, weights)
            flush()
            _wait(x_copy(0))
            weights = [w.astype(BF16) for w in _split(wq_raw[0])]
            queue(0.95 * (2048 + cycles(0, 4)), jobs_x(0)[:96])
            plain_q(0, weights)
            attention(0, 4)
            flush()
            _wait(x_copy(1), x_copy(2))
            stage = [*side_copies(0, 0), *head_copies(1, 1)]
            _start(x_copy(3), *stage)
            lax.fori_loop(0, 16, lambda word, carry: wo_copy(word).start(), None)
            queue(0.98 * (2048 + cycles(4, 8)), jobs_x(2) + terms + jobs_x(0)[96:] + jobs_x(1)[:14])
            plain_q(1, weights)
            attention(4, 8)
            flush()
            _wait(x_copy(3))
            queue(0.98 * (1568 + cycles(8, 9)), jobs_x(3)[:98])
            project_q(2)
            attention(8, 9)
            flush()
            _wait(*stage)
            _start(ax_copy(0, 0), *head_copies(2, 0), *side_copies(1, 1))
            turn, terms = jobs_wq(1)
            queue(0.92 * (1568 + cycles(9, 14)), jobs_x(3)[98:] + _interleave(
                _interleave(jobs_wob, jobs_wa), _interleave(jobs_x(1)[14:], _interleave(turn, jobs_wkv(1)))))
            attention(9, 12)
            assert not any(job.func is job_x and job.args[0] == 3 for job in jobs)
            project_q(3)
            attention(12, 14)
            flush()
            _wait(*[wo_copy(word) for word in range(16)], ax_copy(0, 0))
            _start(ax_copy(1, 1))
            queue(0.92 * cycles(14, 16), _interleave(
                jobs_wo + terms, [P(_job_ax, tok, released, ax_raw, ax_t, 0, *job) for job in AX_JOBS]))
            attention(14, 16)
            flush()
        else:
            queue(0.98 * 4 * 1568 * (0.5 + 0.3), _interleave(jobs_wob, jobs_wo + jobs_wa),
                  q=0.5, kv=0.3, attention=0)
            project_kv(0)
            project_q(0)
            project_kv(1)
            attention(0, 3)
            project_q(1)
            attention(3, 7)
            project_kv(2)
            project_q(2)
            attention(7, 9)
            project_q(3)
            attention(9, 11)
            project_kv(3)
            attention(11, 12)
            flush()
            turn, terms = jobs_wq(1 - slot)
            queue(0.9 * cycles(12, 16), _interleave(jobs_wkv(1 - slot), turn + pause + terms))
            attention(12, 16)
            flush()
        guard[0] = _sum([guard[0]] + [x for x, _ in checks])
        guard[1] = functools.reduce(jnp.maximum, [guard[1]] + [x for _, x in checks])

        def ahead(n):
            return j + n if first else jnp.minimum(j + n, NP - 1)
        _wait(*head_copies(ahead(2), slot), *side_copies(ahead(1), 1 - slot))

        @pl.when(j < NP - 1)
        def _():
            _start(*head_copies(ahead(3), 1 - slot), *side_copies(ahead(2), slot))

    def exact_pairs(ctx):
        def block(i):
            return pl.ds(pl.multiple_of(i * T, T), T)

        def qkv(n, h, i):
            return c_t.at[(2 * n + h) * 4 + (i >> 2), block(i & 3), :]

        def project(x, carry):
            h, i = x & 1, x >> 1
            for n, (rows, w, scale) in enumerate(
                    ((bx_raw, wq_raw, SCALE_B), (c_raw, wk_raw, 1.0), (c_raw, wv_raw, 1.0))):
                def add(t, val):
                    even, odd = _split(w[0, block(t), :])
                    return val + _dot(rows[block(i), block(t)], jnp.where(h == 0, even, odd).astype(BF16))
                val = lax.fori_loop(0, w.shape[1] // T, add, jnp.zeros((T, T), F32))
                qkv(n, h, i)[...] = (val * scale).astype(BF16)

        def attend(b, x, carry):
            quad, part = x >> 3, pl.ds(pl.multiple_of((x & 7) * 16, 16), 16)
            h, i = quad & 1, 2 * b + (quad >> 1)

            def scores(t):
                row = lax.broadcasted_iota(jnp.int32, (16, T), 0) + (i * T + (x & 7) * 16)
                col = lax.broadcasted_iota(jnp.int32, (16, T), 1) + t * T
                return jnp.where(col <= row, _dot_nt(qkv(0, h, i)[part, :], qkv(1, h, t)[...]), MASKED)

            m = lax.fori_loop(
                0, i + 1, lambda t, m: jnp.maximum(m, jnp.max(scores(t), axis=1, keepdims=True)),
                jnp.full((16, 1), -jnp.inf, F32))

            def accumulate(t, carry):
                l, o = carry
                p = jnp.exp2(scores(t) - m)
                return (l + jnp.sum(p, axis=1, keepdims=True),
                        o + _dot(p.astype(BF16), qkv(2, h, t)[...]))
            l, o = lax.fori_loop(0, i + 1, accumulate,
                                 (jnp.zeros((16, 1), F32), jnp.zeros((16, T), F32)))
            ctx[quad, part, :] = o / l

        def pair(j, carry):
            _start(*head_copies(j, 0))
            _wait(*head_copies(j, 0))
            lax.fori_loop(0, 2 * S // T, project, None)

            def rows(b, carry):
                lax.fori_loop(0, 32, P(attend, b), None)
                for n, val in enumerate(_terms(LHS, lambda m: ctx[m])):
                    ctx_t[n, j, block(b), :] = val.astype(BF16)
            lax.fori_loop(0, S // T // 2, rows, None)

        lax.fori_loop(0, NP, pair, None)

    guard[...] = jnp.zeros(guard.shape, F32)
    pair_body(0, first=True)
    lax.fori_loop(1, NP, lambda j, carry: pair_body(j), None)

    safe = jnp.logical_and(jnp.abs(guard[0]) < jnp.inf, guard[1] < SAFE_SUM)

    @pl.when(jnp.max(jnp.where(safe, 0.0, 1.0)) > 0.0)
    def _():
        pl.run_scoped(exact_pairs, pltpu.VMEM((4, T, T), F32))


def _outputs(out_hbm, ax_copy, ax_raw, ax_t, ctx_t, wob_t, wa_t, wo_t, zero_smem,
             o_t, kbuf, vbuf, qbuf, acc, obuf, sem_out):
    def out_copy(c, slot):
        rows = pl.ds(_aligned(c * CO, CO), CO)
        return pltpu.make_async_copy(obuf.at[slot], out_hbm.at[rows, :], sem_out.at[slot])

    for buf in (kbuf, vbuf):
        for t in range(8):
            buf[t, pl.ds(CO, HALO), :] = jnp.zeros((HALO, T), F32)

    t_q = 2 * 49 * RO
    t_v = t_q + 21 * 4 * RO + 49 * RO
    t_o = t_v + (21 + EARLY_B) * 4 * RO

    def chunk_body(c, carry):
        slot = c & 1
        tok = _Tokens(zero_smem)
        plan, due, clock = {}, {}, [0]

        def schedule(job, begin, end, release=False):
            plan.setdefault(max(clock[0], begin // TICK), []).append((job, -(-end // TICK), release))

        def step(results, a, w):
            res = [None] * len(w)
            for x, left in enumerate(a):
                n = clock[0]
                clock[0] += 1
                if n in due:
                    left = _after(functools.reduce(jnp.bitwise_or, due.pop(n)), left)
                left = left.astype(BF16) if left.dtype == F32 else pltpu.bitcast(left, BF16)
                for y in range(len(w)):
                    d = _dot(left, w[y](x))
                    res[y] = d if res[y] is None else res[y] + d
                token = None
                for job, last, release in plan.pop(n, []):
                    if release and token is None:
                        token = tok.of(d[:8])
                    due.setdefault(max(last, n + 1), []).append(job(token) if release else job())
            results.append(res)

        def project(lhs_t, rhs_t, tile0, write):
            inner = {}

            def combine(i, y, m):
                inner[i, y] = _combine([x[y] for x in m])
                return tok.of(*[x[r + 8:r + 16] for x in inner[i, y] for r in range(0, RO, 16)])

            def finish(outer, y, r):
                vals = [_term(SUMS, outer, lambda i: inner[i, y][n][r:r + 16]) for n in range(4)]
                for n, val in enumerate(vals):
                    row, col = _block(outer, n)
                    write(row * RO + r, 2 * col + y, val)
                return tok.of(*[x[8:] for x in vals])

            for i in range(7):
                m = []
                done = clock[0] * TICK + 7 * RO
                for y in range(2):
                    schedule(P(combine, i, y, m), done, done + 400 + 100 * y)
                for outer in FINAL[i]:
                    slabs = [(y, r) for r in range(0, RO, 16) for y in range(2)]
                    for x, slab in enumerate(slabs):
                        schedule(P(finish, outer, *slab), done, done + 400 + 40 * (x + 1))
                for n in range(7 * i, 7 * i + 7):
                    step(m, [_words(lhs_t, (n, x), 0, RO) for x in range(2)],
                         [P(lambda y, x: _load(rhs_t, (n, tile0 + y), x * T, T), y) for y in range(2)])

        for buf in (kbuf, vbuf):
            for t in range(8):
                buf[t, pl.ds(0, HALO), :] = buf[t, pl.ds(CO, HALO), :]

        def write_rows(buf, row, t, val):
            buf[t, pl.ds(HALO + row, 16), :] = val

        def write_q(row, t, val):
            qbuf[t, pl.ds(row, 16), :] = val * SCALE_A

        project(ax_t, wa_t, 2, P(write_rows, kbuf))
        project(ax_t, wa_t, 0, write_q)

        att = {}

        def job_weights(row, r, release):
            base = HALO + row * RO + r
            qs = [_after(release, qbuf[t, pl.ds(row * RO + r, 8), :]) for t in range(8)]
            logits = []
            for w in range(WIN):
                x = _sum([qs[t] * kbuf[t, pl.ds(base - DIL * w, 8), :] for t in range(8)])
                x = x + pltpu.roll(x, 64, 1)
                x = x + pltpu.roll(x, 32, 1)
                if row == 0 and r < DIL * w:
                    pos = lax.broadcasted_iota(jnp.int32, (8, T), 0) + (c * CO + r)
                    x = jnp.where(pos >= DIL * w, x, MASKED)
                logits.append(x)
            m = functools.reduce(jnp.maximum, logits)
            p = [jnp.exp2(x - m) for x in logits]
            inv = _inverse(_sum(p))
            att[row, r] = [x * inv for x in p]
            return tok.of(att[row, r][0])

        def job_values(row, r, release):
            base = HALO + row * RO + r
            p = [_after(release, x) for x in att[row, r]]
            att[row, r] = [_sum([p[w] * vbuf[t, pl.ds(base - DIL * w, 8), :] for w in range(WIN)])
                           for t in range(8)]
            return tok.of(att[row, r][-1])

        def job_o(n, r, i):
            def block(row, col):
                return _cat([att[row, r][2 * col + n], att[row, r + 8][2 * col + n]], axis=0)
            for x, val in enumerate(_terms2(LHS, i, block)):
                o_t[7 * i + x, n, pl.ds(r, 16), :] = val.astype(BF16)
            return tok.stored(o_t, (7 * i + 6, n), r)

        groups = [(row, r + x) for r in range(0, RO, 16) for row in (2, 0, 3, 1) for x in (0, 8)]
        w0, w1, v0, v1 = t_q + 1000, t_v - 1400, t_v + 400, t_o - 700
        for g, (row, r) in enumerate(groups):
            begin = w0 + (w1 - w0) * g // len(groups)
            schedule(P(job_weights, row, r), begin, begin + 500, release=True)
            begin = v0 + (v1 - v0) * g // len(groups)
            schedule(P(job_values, row, r), begin, begin + 600, release=True)
            if g % 8 == 7:
                for x, (n, i) in enumerate((n, i) for n in range(2) for i in range(7)):
                    schedule(P(job_o, n, r - 8, i), begin, min(begin + 400 + 60 * (x + 1), t_o))

        touched = {}

        def project_b(i):
            m = []

            def accumulate(y, inner):
                val = _combine([x[y] for x in m])[inner]
                token = None
                for outer, sign in OUT[i]:
                    row, col = _block(outer, inner)
                    rows, col = pl.ds(row * RO, RO), 2 * col + y
                    total = val
                    if (outer, inner, y) in touched:
                        total = acc[col, rows, :] + val if sign > 0 else acc[col, rows, :] - val
                    touched[outer, inner, y] = True
                    if outer not in FINAL[i]:
                        acc[col, rows, :] = total
                        token = tok.stored(acc, (col,), row * RO)
                    else:
                        obuf[slot, rows, pl.ds(DM + col * T, T)] = total.astype(BF16)
                        if token is None:
                            token = tok.of(_fold(jnp.add, total))
                return token

            parts = [(y, inner) for y in range(2) for inner in range(4)]
            done = clock[0] * TICK + 7 * 4 * RO
            if i < 6:
                for x, part in enumerate(parts):
                    schedule(P(accumulate, *part), done, done + 256 + 200 * x)
            for n in range(7):
                if i == 6 and n == EARLY_B:
                    yield

                def quad(kt, x):
                    return (i, 2 * kt + x % 2), (2 * c + x // 2) * RO
                if len(LHS[n]) == 1:
                    a = [_words(ctx_t, *quad(kt, LHS[n][0][0]), RO) for kt in range(8)]
                else:
                    a = [_term(LHS, n, lambda x: _load(ctx_t, (i + tok.z * n, 2 * kt + x % 2), quad(kt, x)[1], RO).astype(F32))
                         for kt in range(8)]
                step(m, a, [P(lambda y, x: _load(wob_t, (7 * i + n, y), x * T, T), y) for y in range(2)])
            if i == 6:
                for part in parts:
                    accumulate(*part)

        for i in range(6):
            if i == 3:
                project(ax_t, wa_t, 4, P(write_rows, vbuf))
            list(project_b(i))
        last_b = project_b(6)
        next(last_b)

        for x, job in enumerate(AX_JOBS):
            schedule(P(_job_ax, tok, lambda val: val, ax_raw, ax_t, 1 - slot, *job),
                     t_o, t_o + 100 + 3000 * (x + 1) // len(AX_JOBS))

        def write_out(row, t, val):
            obuf[slot, pl.ds(row, 16), pl.ds(t * T, T)] = val.astype(BF16)

        project(o_t, wo_t, 0, write_out)
        list(last_b)
        assert not plan and not due
        out_copy(c, slot).start()
        ax_copy(jnp.minimum(c + 2, NO - 1), slot).wait()

        @pl.when(c < NO - 1)
        def _():
            ax_copy(jnp.minimum(c + 3, NO - 1), 1 - slot).start()

        @pl.when(c >= 1)
        def _():
            out_copy(c - 1, 1 - slot).wait()

    ax_copy(1, 1).wait()
    ax_copy(2, 0).start()
    lax.fori_loop(0, NO, chunk_body, None)
    out_copy(NO - 1, (NO - 1) % 2).wait()


def _kernel(ax_hbm, wqkv_hbm, wo_hbm, bx_hbm, c_hbm, wq_hbm, wuk_hbm, wuv_hbm, wob_hbm, out_hbm,
            ax_raw, ax_t, ctx_t, wob_t, wa_t, wo_t, zero_smem, sem_ax):
    vmem, dma = pltpu.VMEM, pltpu.SemaphoreType.DMA

    def clear(i, carry):
        zero_smem[0] = i >> 1
    lax.fori_loop(0, 2, clear, None)

    def ax_copy(c, slot):
        rows = pl.ds(_aligned(c * CO, CO), CO)
        return pltpu.make_async_copy(ax_hbm.at[rows, :], ax_raw.at[slot], sem_ax.at[slot])

    shared = (ax_copy, ax_raw, ax_t, ctx_t, wob_t, wa_t, wo_t, zero_smem)
    pl.run_scoped(
        P(_head_pairs, wqkv_hbm, wo_hbm, bx_hbm, c_hbm, wq_hbm, wuk_hbm, wuv_hbm, wob_hbm, *shared),
        vmem((S, DM), BF16),
        vmem((S, DC), BF16),
        vmem((2, DM, T), U32),
        vmem((2, DC, T), U32),
        vmem((2, DC, T), U32),
        vmem((2, 4, 64, DM), BF16),
        vmem((2, 4, 8, 3 * DM), U32),
        vmem((16, NH, DM), U32),
        vmem((49, 2, S // 4, T), BF16),
        vmem((49, S // 4, T), BF16),
        vmem((DM // T, T, T), U32),
        vmem((49, 2, RO, T), BF16),
        vmem((49, T, T), BF16),
        vmem((2, 8, T), F32),
        dma((2 * S // CH,)), dma((11,)))
    pl.run_scoped(
        P(_outputs, out_hbm, *shared),
        vmem((49, 2, RO, T), BF16),
        vmem((8, HALO + CO, T), F32),
        vmem((8, HALO + CO, T), F32),
        vmem((8, CO, T), F32),
        vmem((8, CO, T), F32),
        vmem((2, CO, 2 * DM), BF16),
        dma((2,)))


@jax.jit
def pallas_concat_heads__sliding_local_dilated__compressed_kv_cla__prompt_kernel(
    A_x: jax.Array,
    A_wqkv: jax.Array,
    A_wo: jax.Array,
    B_x: jax.Array,
    B_c_kv: jax.Array,
    B_w_q: jax.Array,
    B_w_uk: jax.Array,
    B_w_uv: jax.Array,
    B_w_o: jax.Array,
):
    vmem = pltpu.VMEM
    out = pl.pallas_call(
        _kernel,
        out_shape=jax.ShapeDtypeStruct((S, 2 * DM), BF16),
        in_specs=[pl.BlockSpec(memory_space=pl.ANY)] * 9,
        out_specs=pl.BlockSpec(memory_space=pl.ANY),
        scratch_shapes=[
            vmem((2, CO, DM), BF16),
            vmem((49, 2, RO, T), BF16),
            vmem((7, NP, S // 2, T), BF16),
            vmem((49, 2, DM, T), BF16),
            vmem((49, 6, 2 * T, T), BF16),
            vmem((49, 2, 2 * T, T), BF16),
            pltpu.SMEM((1,), jnp.int32),
            pltpu.SemaphoreType.DMA((2,)),
        ],
        compiler_params=pltpu.CompilerParams(
            vmem_limit_bytes=127 * 2**20, disable_bounds_checks=True),
    )(
        A_x.reshape(S, DM),
        A_wqkv.reshape(4, DM // 4, 3 * DM),
        A_wo.reshape(NH, DM // NH, DM),
        B_x.reshape(S, DM),
        B_c_kv.reshape(S, DC),
        B_w_q,
        B_w_uk,
        B_w_uv,
        B_w_o,
    )
    return out.reshape(1, S, 2 * DM)
```

```python
import functools
import math

import jax
import jax.numpy as jnp
from jax import lax
import jax.experimental.pallas as pl
import jax.experimental.pallas.tpu as pltpu

S = 2048
DM = 1024
DC = 512
NH = 32
NP = NH // 2
T = 128
CH = 4 * T
RO = 64
CO = 4 * RO
NO = S // CO
WIN, DIL = 8, 2
HALO = 16

LOG2E = math.log2(math.e)
SCALE_A = (DM // NH) ** -0.5 * LOG2E
SCALE_B = T ** -0.5 * LOG2E
MASKED = -1e9 * LOG2E
SAFE_SUM = 2.0 ** 40

DEPTH = 3
JOB_CYCLES = 1024, 896
CTX_CYCLES = 1024, 768

NX0, NX3 = 49, 84
TICK = RO // 2
EARLY_B = 4
F32, BF16, U32 = jnp.float32, jnp.bfloat16, jnp.uint32
P = functools.partial


def _dot(a, b):
    return jnp.dot(a, b, preferred_element_type=F32)


def _dot_nt(a, b):
    return lax.dot_general(a, b, (((1,), (1,)), ((), ())), preferred_element_type=F32)


def _cat(xs, axis=1):
    return xs[0] if len(xs) == 1 else jnp.concatenate(xs, axis=axis)


def _sum(xs):
    return functools.reduce(jnp.add, xs)


def _fold(op, x):
    return functools.reduce(op, [x[r:r + 8] for r in range(0, x.shape[0], 8)])


def _aligned(x, n):
    return x if isinstance(x, int) else pl.multiple_of(x, n)


def _rows(start, n):
    return pl.ds(_aligned(start, 16), n)


def _words(ref, lead, start, n):
    return ref.bitcast(U32)[(*lead, pl.ds(_aligned(start >> 1, 8), n // 2), slice(None))]


def _load(ref, lead, start, n):
    return pltpu.bitcast(_words(ref, lead, start, n), BF16)


def _split(w):
    return (pltpu.bitcast(w << 16, F32), pltpu.bitcast(w & jnp.uint32(0xFFFF0000), F32))


def _inverse(l):
    r = pl.reciprocal(l, approx=True)
    return r * (2.0 - l * r)


def _interleave(x, y):
    order = [((n + 0.5) / len(z), m, job) for m, z in enumerate((x, y)) for n, job in enumerate(z)]
    return [job for _, _, job in sorted(order, key=lambda e: e[:2])]


def _start(*copies):
    for cp in copies:
        cp.start()


def _wait(*copies):
    for cp in copies:
        cp.wait()


LHS = (((0, 1), (3, 1)), ((2, 1), (3, 1)), ((0, 1),), ((3, 1),),
       ((0, 1), (1, 1)), ((2, 1), (0, -1)), ((1, 1), (3, -1)))
RHS = (((0, 1), (3, 1)), ((0, 1),), ((1, 1), (3, -1)), ((2, 1), (0, -1)),
       ((3, 1),), ((0, 1), (1, 1)), ((2, 1), (3, 1)))
OUT = (((0, 1), (3, 1)), ((2, 1), (3, -1)), ((1, 1), (3, 1)), ((0, 1), (2, 1)),
       ((0, -1), (1, 1)), ((3, 1),), ((0, 1),))
SUMS = tuple(tuple((i, sign) for i in range(7) for m, sign in OUT[i] if m == n) for n in range(4))
FINAL = tuple(tuple(n for n in range(4) if SUMS[n][-1][0] == i) for i in range(7))


def _term(table, i, quad):
    (n, _), *rest = table[i]
    val = quad(n)
    for n, sign in rest:
        val = val + quad(n) if sign > 0 else val - quad(n)
    return val


def _terms(table, quad):
    blocks = [quad(n) for n in range(4)]
    return [_term(table, i, blocks.__getitem__) for i in range(7)]


def _block(outer, inner):
    return 2 * (outer // 2) + inner // 2, 2 * (outer % 2) + inner % 2


def _terms2(table, i, block):
    return _terms(table, lambda n: _term(table, i, lambda m: block(*_block(m, n))))


def _combine(m):
    return [_term(SUMS, n, m.__getitem__) for n in range(4)]


def _combine2(m):
    inner = [_combine(m[i:i + 7]) for i in range(0, 49, 7)]
    return {_block(outer, n): val for n in range(4)
            for outer, val in enumerate(_combine([x[n] for x in inner]))}


class _Tokens:
    def __init__(self, zero_smem):
        self.z = zero_smem[0]
        self.zero = jnp.full((8, T), self.z, jnp.int32).astype(U32)

    def stored(self, ref, lead, start):
        first, *rest = lead
        if ref.dtype == BF16:
            return _words(ref, (first - (self.z & 1), *rest), start, 16) & self.zero
        return self.of(ref[(*lead, pl.ds(_aligned(start + 8 * (self.z & 1), 8), 8), slice(None))])

    def of(self, *vals):
        return pltpu.bitcast(_sum(vals), U32) & self.zero


def _after(token, x, everywhere=False):
    if token is None:
        return x
    bits = x if x.dtype == U32 else pltpu.bitcast(x, U32)
    cut = bits.shape[0] if everywhere else 8
    parts = [bits[r:r + 8] | token for r in range(0, cut, 8)]
    bits = _cat(parts + ([bits[cut:]] if cut < bits.shape[0] else []), axis=0)
    return bits if x.dtype == U32 else pltpu.bitcast(bits, x.dtype)


AX_JOBS = [(i, n, r) for n in range(2) for r in range(0, RO, 16) for i in range(7)]


def _job_ax(tok, released, ax_raw, ax_t, src, i, n, r):
    terms = _terms2(LHS, i, lambda row, col: released(
        ax_raw[src, pl.ds(row * RO + r, 16), pl.ds((2 * col + n) * T, T)].astype(F32)))
    for x, val in enumerate(terms):
        ax_t[7 * i + x, n, pl.ds(r, 16), :] = val.astype(BF16)
    return tok.stored(ax_t, (7 * i + 6, n), r)


def _head_pairs(wqkv_hbm, wo_hbm, bx_hbm, c_hbm, wq_hbm, wuk_hbm, wuv_hbm, wob_hbm,
                ax_copy, ax_raw, ax_t, ctx_t, wob_t, wa_t, wo_t, zero_smem,
                bx_raw, c_raw, wq_raw, wk_raw, wv_raw, wob_raw, wqkv_raw, wo_raw,
                bx_t, c_t, wq_turned, wq_t, wkv_t, guard, sem_in, sem_w):
    def head_copies(j, slot):
        return [pltpu.make_async_copy(src.bitcast(U32).at[:, j, :], dst.at[slot], sem_w.at[3 * slot + n])
                for n, (src, dst) in enumerate(((wuk_hbm, wk_raw), (wuv_hbm, wv_raw), (wq_hbm, wq_raw)))]

    def side_copies(j, slot):
        wob = wob_hbm.at[pl.ds(4 * (j >> 1), 4), pl.ds(_aligned((j & 1) * 64, 64), 64), :]
        wqkv = wqkv_hbm.bitcast(U32).at[:, pl.ds(_aligned(8 * j, 8), 8), :]
        return [pltpu.make_async_copy(wob, wob_raw.at[slot], sem_w.at[6 + 2 * slot]),
                pltpu.make_async_copy(wqkv, wqkv_raw.at[slot], sem_w.at[7 + 2 * slot])]

    def wo_copy(word):
        return pltpu.make_async_copy(wo_hbm.bitcast(U32).at[:, word, :], wo_raw.at[word], sem_w.at[10])

    def c_copy(c):
        rows = pl.ds(c * CH, CH)
        return pltpu.make_async_copy(c_hbm.at[rows, :], c_raw.at[rows, :], sem_in.at[2 * c])

    def x_copy(c):
        rows = pl.ds(c * CH, CH)
        return pltpu.make_async_copy(bx_hbm.at[rows, :], bx_raw.at[rows, :], sem_in.at[2 * c + 1])

    def pair_body(j, first=False):
        slot = j & 1
        tok = _Tokens(zero_smem)
        causal = (lax.broadcasted_iota(jnp.int32, (T, T), 1)
                  <= lax.broadcasted_iota(jnp.int32, (T, T), 0))

        jobs, due, pace = [], [], dict(release=None, recent=None)

        def queue(cycles, more, q=1.0, kv=1.0, attention=1.0):
            pace.update(period=cycles / len(more), clock=0, q=q, kv=kv, attention=attention)
            jobs.extend(more)

        def flush():
            while jobs:
                jobs.pop(0)()

        def background(cycles, share, delay, recent=None):
            pace["clock"] += cycles * share
            token = None
            while jobs and pace["clock"] >= pace["period"]:
                pace["clock"] -= pace["period"]
                pace["release"] = None if recent is None else tok.of(recent[:8])
                new = jobs.pop(0)()
                pace["release"] = None
                token = new if token is None else token | new
            if token is not None:
                due.append([delay, token])
            for entry in due:
                entry[0] -= cycles
            now = [token for left, token in due if left <= 0]
            due[:] = [entry for entry in due if entry[0] > 0]
            return functools.reduce(jnp.bitwise_or, now) if now else None

        def released(x):
            return _after(pace["release"], x, everywhere=True)

        def store_terms(dst, first_term, lead, row, terms):
            for i, val in enumerate(terms):
                dst[(first_term + i, *lead, _rows(row, 16), slice(None))] = val.astype(BF16)
            return tok.stored(dst, (first_term + 6, *lead), row)

        def job_x(c, i, n, r):
            terms = _terms2(RHS, i, lambda row, col: bx_raw[
                pl.ds(c * CH + (col ^ 2) * T + r, 16), pl.ds((2 * row + n) * T, T)].astype(F32))
            return store_terms(bx_t, 7 * i, (n,), c * T + r, terms)

        def job_c(c, i, r):
            terms = _terms2(LHS, i, lambda row, col: c_raw[
                pl.ds(c * CH + row * T + r, 16), pl.ds(col * T, T)].astype(F32))
            return store_terms(c_t, 7 * i, (), c * T + r, terms)

        def jobs_x(c):
            return [P(job_x, c, i, n, r) for r in range(0, T, 16) for n in range(2) for i in range(7)]

        def jobs_c(c):
            return [P(job_c, c, i, r) for r in range(0, T, 16) for i in range(7)]

        def job_wkv(src, i, r):
            def block(row, col):
                raw = (wk_raw, wv_raw)[col % 2]
                return _split(released(raw[src, pl.ds(row * T + r, 16), :]))[col // 2]
            return store_terms(wkv_t, 7 * i, (), r, _terms2(RHS, i, block))

        def job_turn(src, n):
            words = released(wq_raw[src, pl.ds(n * T, T), :])
            wq_turned[n] = pltpu.bitcast(pltpu.bitcast(words, F32).T, U32)
            return tok.stored(wq_turned, (n,), T - 16)

        def job_wq(i, n, r):
            def block(row, col):
                return _split(released(wq_turned[2 * col + n, pl.ds((row % 2) * RO + r, 16), :]))[row // 2]
            return store_terms(wq_t, 7 * i, (n,), r, _terms2(LHS, i, block))

        def jobs_wkv(src):
            return [P(job_wkv, src, i, r) for r in range(0, T, 16) for i in range(7)]

        def jobs_wq(src):
            return ([P(job_turn, src, n) for n in range(DM // T)],
                    [P(job_wq, i, n, r) for n in range(2) for r in range(0, RO, 16) for i in range(7)])

        def job_wob(i, n, r):
            def block(row, col):
                head = 2 * (row % 2) + row // 2
                return released(wob_raw[slot, head, pl.ds(r, 16), pl.ds((2 * col + n) * T, T)].astype(F32))
            return store_terms(wob_t, 7 * i, (n,), j * 64 + r, _terms2(RHS, i, block))

        def job_wo(i, n):
            e, odd, head = j & 3, (j >> 2) & 1, 16 * (j >> 3)

            def block(row, col):
                even_t, odd_t = _split(released(
                    wo_raw[4 * e + row, _rows(head, 16), pl.ds((2 * col + n) * T, T)]))
                return jnp.where(odd == 1, odd_t, even_t)
            return store_terms(wo_t, 7 * i, (n,), odd * T + e * NH + head, _terms2(RHS, i, block))

        permuted = {}

        def job_permute(mat):
            lane = lax.broadcasted_iota(jnp.int32, (32, T), 1)
            e, grp, sub = lane >> 5, (lane >> 2) & 7, lane & 3

            def gather(x, index):
                return jnp.take_along_axis(x, index, axis=1, mode="promise_in_bounds")
            x = [released(wqkv_raw[slot, :, :, pl.ds(mat * DM + t * T, T)].reshape(32, T))
                 for t in range(8)]
            y = [gather(x[t], sub * 32 + e * 8 + ((grp - t) & 7)) for t in range(8)]
            u = [y[-s % 8] for s in range(8)]
            for bit in (1, 2, 4):
                u = [jnp.where((grp & bit) != 0, u[(s - bit) % 8], u[s]) for s in range(8)]
            u = [u[0]] + [gather(u[t], e * 32 + ((grp + t) & 7) * 4 + sub) for t in range(1, 8)]
            permuted[mat] = u
            return _fold(jnp.bitwise_or, functools.reduce(jnp.bitwise_or, u)) & tok.zero

        def column(mat, row, t):
            return pltpu.bitcast(released(permuted[mat][t][8 * row:8 * row + 8]), BF16).astype(F32)

        def job_wa(mat, i, n):
            terms = _terms2(RHS, i, lambda row, col: column(mat, row, 2 * col + n))
            return store_terms(wa_t, 7 * i, (2 * mat + n,), 16 * j, terms)

        pause = [P(lambda: tok.zero)] * 2
        jobs_wob = [P(job_wob, i, n, r) for r in range(0, 64, 16) for n in range(2) for i in range(7)]
        jobs_wo = [P(job_wo, i, n) for n in range(2) for i in range(7)]
        jobs_wa = []
        for mat in range(3):
            jobs_wa += [P(job_permute, mat)] + pause
            jobs_wa += [P(job_wa, mat, i, n) for n in range(2) for i in range(7)]

        q, k, v = {}, {}, {}

        def product(dot, share, left, right):
            token = background(left.shape[0] // 2, share, JOB_CYCLES[first], pace["recent"])
            pace["recent"] = dot(pltpu.bitcast(_after(token, left), BF16), right)
            return pace["recent"]

        def project_q(c):
            blocks = _combine2([_sum([
                product(_dot_nt, pace["q"], _words(wq_t, (i, n), 0, RO), _load(bx_t, (i, n), c * T, T))
                for n in range(2)]) for i in range(49)])
            for h in range(2):
                for col in range(4):
                    val = _cat([blocks[2 * h, col], blocks[2 * h + 1, col]], axis=0) * SCALE_B
                    q[4 * c + (col ^ 2), h] = val.T.astype(BF16)

        def project_kv(c):
            m = [product(_dot, pace["kv"], _words(c_t, (i,), c * T, T), _load(wkv_t, (i,), 0, T))
                 for i in range(49)]
            for (row, col), val in sorted(_combine2(m).items()):
                (k, v)[col % 2][4 * c + row, col // 2] = val.astype(BF16)

        def plain(raw, c, weights):
            def part(r, col):
                left = raw[pl.ds(c * CH + r, 32), pl.ds(col, 4 * T)]
                token = background(32, 1.0, 128)
                if token is None:
                    return left
                return _cat([_after(_cat([token, token]), left[:, :2 * T]), left[:, 2 * T:]])
            return [_dot(_cat([_cat([part(r, col) for r in range(0, CH, 32)], axis=0)
                               for col in range(0, raw.shape[1], 4 * T)]), w) for w in weights]

        def plain_kv(c, weights):
            for n, val in enumerate(plain(c_raw, c, weights)):
                for r in range(4):
                    (k, v)[n // 2][4 * c + r, n % 2] = val[r * T:(r + 1) * T].astype(BF16)

        def plain_q(c, weights):
            for h, val in enumerate(plain(bx_raw, c, weights)):
                for r in range(4):
                    q[4 * c + r, h] = (val[r * T:(r + 1) * T] * SCALE_B).astype(BF16)

        in_flight, partial, ctx, spread, checks = [], {}, {}, {}, []

        def finish(i, h):
            l, o = partial.pop((i, h))
            l = jnp.sum(l, axis=1, keepdims=True)
            r = _inverse(l)
            ctx[i, h] = o * r
            spread[i, h] = _fold(jnp.maximum, jnp.broadcast_to(l + r, (T, T)))
            b = i // 2
            quad = [(2 * b, 0), (2 * b, 1), (2 * b + 1, 0), (2 * b + 1, 1)]
            if all(u in ctx for u in quad):
                terms = _terms(LHS, lambda m: ctx.pop(quad[m]))
                for n, val in enumerate(terms):
                    ctx_t[n, j, pl.ds(b * T, T), :] = val.astype(BF16)
                checks.append((_fold(jnp.add, terms[0] + terms[5] + terms[6]),
                               functools.reduce(jnp.maximum, [spread.pop(u) for u in quad])))
                due.append([CTX_CYCLES[first], tok.stored(ctx_t, (6, j), b * T) | tok.of(*checks[-1])])

        def weigh(i, h, t, p):
            l, o = partial.get((i, h), (None, None))
            l = p if l is None else l + p
            d = _dot(_after(background(64, pace["attention"], JOB_CYCLES[first], p), p).astype(BF16), v[t, h])
            partial[i, h] = (l, d if o is None else o + d)
            if t == i:
                finish(i, h)

        def attention(lo, hi):
            for i in range(lo, hi):
                for h in range(2):
                    for t in range(i + 1):
                        s = _dot_nt(q[i, h], k[t, h])
                        if t == i:
                            s = jnp.where(causal, s, MASKED)
                        in_flight.append((i, h, t, jnp.exp2(s)))
                        if len(in_flight) > DEPTH:
                            weigh(*in_flight.pop(0))
            while hi == S // T and in_flight:
                weigh(*in_flight.pop(0))

        def cycles(lo, hi):
            return 2 * 64 * sum(range(lo + 1, hi + 1))

        if first:
            wk, wv, wq = head_copies(0, 0)
            _start(wv, wk, c_copy(0), c_copy(1))
            _wait(wv, wk, c_copy(0))
            _start(c_copy(2), c_copy(3), wq, x_copy(0))
            weights = [w.astype(BF16) for raw in (wk_raw, wv_raw) for w in _split(raw[0])]
            queue(0.98 * 2048, jobs_c(0)[:49])
            plain_kv(0, weights)
            flush()
            _wait(c_copy(1), c_copy(2))
            _start(x_copy(1), x_copy(2))
            queue(0.92 * 4096, jobs_c(0)[49:] + jobs_c(1) + jobs_c(2))
            plain_kv(1, weights)
            plain_kv(2, weights)
            flush()
            _wait(c_copy(3), wq)
            turn, terms = jobs_wq(0)
            queue(0.9 * 2048, _interleave(turn, jobs_c(3)))
            plain_kv(3, weights)
            flush()
            _wait(x_copy(0))
            weights = [w.astype(BF16) for w in _split(wq_raw[0])]
            queue(0.85 * (2048 + 0.2 * cycles(0, 4)), jobs_x(0)[:96], attention=0.2)
            plain_q(0, weights)
            attention(0, 4)
            flush()
            _wait(x_copy(1), x_copy(2))
            stage = [*side_copies(0, 0), *head_copies(1, 1)]
            _start(x_copy(3), *stage)
            lax.fori_loop(0, 16, lambda word, carry: wo_copy(word).start(), None)
            queue(0.98 * (2048 + 0.5 * cycles(4, 7)),
                  jobs_x(2) + terms + jobs_x(0)[96:] + jobs_x(1)[:14], attention=0.5)
            plain_q(1, weights)
            attention(4, 7)
            flush()
            _wait(x_copy(3))
            queue(0.85 * (1568 + cycles(7, 10)), jobs_x(3))
            project_q(2)
            attention(7, 10)
            flush()
            _wait(*stage)
            _start(ax_copy(0, 0), *head_copies(2, 0), *side_copies(1, 1))
            turn, terms = jobs_wq(1)
            queue(0.88 * (1568 + cycles(10, 14)), _interleave(
                _interleave(jobs_wob, jobs_wa), _interleave(jobs_x(1)[14:], _interleave(turn, jobs_wkv(1)))))
            attention(10, 12)
            project_q(3)
            attention(12, 14)
            flush()
            _wait(*[wo_copy(word) for word in range(16)], ax_copy(0, 0))
            _start(ax_copy(1, 1))
            queue(0.92 * cycles(14, 16), _interleave(
                jobs_wo + terms, [P(_job_ax, tok, released, ax_raw, ax_t, 0, *job) for job in AX_JOBS]))
            attention(14, 16)
            flush()
        else:
            queue(0.98 * 4 * 1568 * (0.5 + 0.3), _interleave(jobs_wob, jobs_wo + jobs_wa),
                  q=0.5, kv=0.3, attention=0)
            project_kv(0)
            project_q(0)
            project_kv(1)
            attention(0, 3)
            project_q(1)
            attention(3, 7)
            project_kv(2)
            project_q(2)
            attention(7, 9)
            project_q(3)
            attention(9, 11)
            project_kv(3)
            attention(11, 12)
            flush()
            turn, terms = jobs_wq(1 - slot)
            queue(0.9 * cycles(12, 16), _interleave(jobs_wkv(1 - slot), turn + pause + terms))
            attention(12, 16)
            flush()
        guard[0] = _sum([guard[0]] + [x for x, _ in checks])
        guard[1] = functools.reduce(jnp.maximum, [guard[1]] + [x for _, x in checks])

        def ahead(n):
            return j + n if first else jnp.minimum(j + n, NP - 1)
        _wait(*head_copies(ahead(2), slot), *side_copies(ahead(1), 1 - slot))

        @pl.when(j < NP - 1)
        def _():
            _start(*head_copies(ahead(3), 1 - slot), *side_copies(ahead(2), slot))

    def exact_pairs(ctx):
        def block(i):
            return pl.ds(pl.multiple_of(i * T, T), T)

        def qkv(n, h, i):
            return c_t.at[(2 * n + h) * 4 + (i >> 2), block(i & 3), :]

        def project(x, carry):
            h, i = x & 1, x >> 1
            for n, (rows, w, scale) in enumerate(
                    ((bx_raw, wq_raw, SCALE_B), (c_raw, wk_raw, 1.0), (c_raw, wv_raw, 1.0))):
                def add(t, val):
                    even, odd = _split(w[0, block(t), :])
                    return val + _dot(rows[block(i), block(t)], jnp.where(h == 0, even, odd).astype(BF16))
                val = lax.fori_loop(0, w.shape[1] // T, add, jnp.zeros((T, T), F32))
                qkv(n, h, i)[...] = (val * scale).astype(BF16)

        def attend(b, x, carry):
            quad, part = x >> 3, pl.ds(pl.multiple_of((x & 7) * 16, 16), 16)
            h, i = quad & 1, 2 * b + (quad >> 1)

            def scores(t):
                row = lax.broadcasted_iota(jnp.int32, (16, T), 0) + (i * T + (x & 7) * 16)
                col = lax.broadcasted_iota(jnp.int32, (16, T), 1) + t * T
                return jnp.where(col <= row, _dot_nt(qkv(0, h, i)[part, :], qkv(1, h, t)[...]), MASKED)

            m = lax.fori_loop(
                0, i + 1, lambda t, m: jnp.maximum(m, jnp.max(scores(t), axis=1, keepdims=True)),
                jnp.full((16, 1), -jnp.inf, F32))

            def accumulate(t, carry):
                l, o = carry
                p = jnp.exp2(scores(t) - m)
                return (l + jnp.sum(p, axis=1, keepdims=True),
                        o + _dot(p.astype(BF16), qkv(2, h, t)[...]))
            l, o = lax.fori_loop(0, i + 1, accumulate,
                                 (jnp.zeros((16, 1), F32), jnp.zeros((16, T), F32)))
            ctx[quad, part, :] = o / l

        def pair(j, carry):
            _start(*head_copies(j, 0))
            _wait(*head_copies(j, 0))
            lax.fori_loop(0, 2 * S // T, project, None)

            def rows(b, carry):
                lax.fori_loop(0, 32, P(attend, b), None)
                for n, val in enumerate(_terms(LHS, lambda m: ctx[m])):
                    ctx_t[n, j, block(b), :] = val.astype(BF16)
            lax.fori_loop(0, S // T // 2, rows, None)

        lax.fori_loop(0, NP, pair, None)

    guard[...] = jnp.zeros(guard.shape, F32)
    pair_body(0, first=True)
    lax.fori_loop(1, NP, lambda j, carry: pair_body(j), None)

    safe = jnp.logical_and(jnp.abs(guard[0]) < jnp.inf, guard[1] < SAFE_SUM)

    @pl.when(jnp.max(jnp.where(safe, 0.0, 1.0)) > 0.0)
    def _():
        pl.run_scoped(exact_pairs, pltpu.VMEM((4, T, T), F32))


def _outputs(out_hbm, ax_copy, ax_raw, ax_t, ctx_t, wob_t, wa_t, wo_t, zero_smem,
             o_t, kbuf, vbuf, qbuf, acc, obuf, sem_out):
    def out_copy(c, slot):
        rows = pl.ds(_aligned(c * CO, CO), CO)
        return pltpu.make_async_copy(obuf.at[slot], out_hbm.at[rows, :], sem_out.at[slot])

    for buf in (kbuf, vbuf):
        for t in range(8):
            buf[t, pl.ds(CO, HALO), :] = jnp.zeros((HALO, T), F32)

    t_q = 2 * 49 * RO
    t_v = t_q + 21 * 4 * RO + 49 * RO
    t_o = t_v + (21 + EARLY_B) * 4 * RO

    def chunk_body(c, carry):
        slot = c & 1
        tok = _Tokens(zero_smem)
        plan, due, clock = {}, {}, [0]

        def schedule(job, begin, end, release=False):
            plan.setdefault(max(clock[0], begin // TICK), []).append((job, -(-end // TICK), release))

        def step(results, a, w):
            res = [None] * len(w)
            for x, left in enumerate(a):
                n = clock[0]
                clock[0] += 1
                if n in due:
                    left = _after(functools.reduce(jnp.bitwise_or, due.pop(n)), left)
                left = left.astype(BF16) if left.dtype == F32 else pltpu.bitcast(left, BF16)
                for y in range(len(w)):
                    d = _dot(left, w[y](x))
                    res[y] = d if res[y] is None else res[y] + d
                token = None
                for job, last, release in plan.pop(n, []):
                    if release and token is None:
                        token = tok.of(d[:8])
                    due.setdefault(max(last, n + 1), []).append(job(token) if release else job())
            results.append(res)

        def project(lhs_t, rhs_t, tile0, write):
            inner = {}

            def combine(i, y, m):
                inner[i, y] = _combine([x[y] for x in m])
                return tok.of(*[x[r + 8:r + 16] for x in inner[i, y] for r in range(0, RO, 16)])

            def finish(outer, y, r):
                vals = [_term(SUMS, outer, lambda i: inner[i, y][n][r:r + 16]) for n in range(4)]
                for n, val in enumerate(vals):
                    row, col = _block(outer, n)
                    write(row * RO + r, 2 * col + y, val)
                return tok.of(*[x[8:] for x in vals])

            for i in range(7):
                m = []
                done = clock[0] * TICK + 7 * RO
                for y in range(2):
                    schedule(P(combine, i, y, m), done, done + 400 + 100 * y)
                for outer in FINAL[i]:
                    slabs = [(y, r) for r in range(0, RO, 16) for y in range(2)]
                    for x, slab in enumerate(slabs):
                        schedule(P(finish, outer, *slab), done, done + 400 + 40 * (x + 1))
                for n in range(7 * i, 7 * i + 7):
                    step(m, [_words(lhs_t, (n, x), 0, RO) for x in range(2)],
                         [P(lambda y, x: _load(rhs_t, (n, tile0 + y), x * T, T), y) for y in range(2)])

        for buf in (kbuf, vbuf):
            for t in range(8):
                buf[t, pl.ds(0, HALO), :] = buf[t, pl.ds(CO, HALO), :]

        def write_rows(buf, row, t, val):
            buf[t, pl.ds(HALO + row, 16), :] = val

        def write_q(row, t, val):
            qbuf[t, pl.ds(row, 16), :] = val * SCALE_A

        project(ax_t, wa_t, 2, P(write_rows, kbuf))
        project(ax_t, wa_t, 0, write_q)

        att = {}

        def job_weights(row, r, release):
            base = HALO + row * RO + r
            qs = [_after(release, qbuf[t, pl.ds(row * RO + r, 8), :]) for t in range(8)]
            logits = []
            for w in range(WIN):
                x = _sum([qs[t] * kbuf[t, pl.ds(base - DIL * w, 8), :] for t in range(8)])
                x = x + pltpu.roll(x, 64, 1)
                x = x + pltpu.roll(x, 32, 1)
                if row == 0 and r < DIL * w:
                    pos = lax.broadcasted_iota(jnp.int32, (8, T), 0) + (c * CO + r)
                    x = jnp.where(pos >= DIL * w, x, MASKED)
                logits.append(x)
            m = functools.reduce(jnp.maximum, logits)
            p = [jnp.exp2(x - m) for x in logits]
            inv = _inverse(_sum(p))
            att[row, r] = [x * inv for x in p]
            return tok.of(att[row, r][0])

        def job_values(row, r, release):
            base = HALO + row * RO + r
            p = [_after(release, x) for x in att[row, r]]
            att[row, r] = [_sum([p[w] * vbuf[t, pl.ds(base - DIL * w, 8), :] for w in range(WIN)])
                           for t in range(8)]
            return tok.of(att[row, r][-1])

        def job_o(n, r, i):
            def block(row, col):
                return _cat([att[row, r][2 * col + n], att[row, r + 8][2 * col + n]], axis=0)
            for x, val in enumerate(_terms2(LHS, i, block)):
                o_t[7 * i + x, n, pl.ds(r, 16), :] = val.astype(BF16)
            return tok.stored(o_t, (7 * i + 6, n), r)

        groups = [(row, r + x) for r in range(0, RO, 16) for row in (2, 0, 3, 1) for x in (0, 8)]
        w0, w1, v0, v1 = t_q + 1000, t_v - 1400, t_v + 400, t_o - 700
        for g, (row, r) in enumerate(groups):
            begin = w0 + (w1 - w0) * g // len(groups)
            schedule(P(job_weights, row, r), begin, begin + 500, release=True)
            begin = v0 + (v1 - v0) * g // len(groups)
            schedule(P(job_values, row, r), begin, begin + 600, release=True)
            if g % 8 == 7:
                for x, (n, i) in enumerate((n, i) for n in range(2) for i in range(7)):
                    schedule(P(job_o, n, r - 8, i), begin, min(begin + 400 + 60 * (x + 1), t_o))

        touched = {}

        def project_b(i):
            m = []

            def accumulate(y, inner):
                val = _combine([x[y] for x in m])[inner]
                token = None
                for outer, sign in OUT[i]:
                    row, col = _block(outer, inner)
                    rows, col = pl.ds(row * RO, RO), 2 * col + y
                    total = val
                    if (outer, inner, y) in touched:
                        total = acc[col, rows, :] + val if sign > 0 else acc[col, rows, :] - val
                    touched[outer, inner, y] = True
                    if outer not in FINAL[i]:
                        acc[col, rows, :] = total
                        token = tok.stored(acc, (col,), row * RO)
                    else:
                        obuf[slot, rows, pl.ds(DM + col * T, T)] = total.astype(BF16)
                        if token is None:
                            token = tok.of(_fold(jnp.add, total))
                return token

            parts = [(y, inner) for y in range(2) for inner in range(4)]
            done = clock[0] * TICK + 7 * 4 * RO
            if i < 6:
                for x, part in enumerate(parts):
                    schedule(P(accumulate, *part), done, done + 256 + 200 * x)
            for n in range(7):
                if i == 6 and n == EARLY_B:
                    yield

                def quad(kt, x):
                    return (i, 2 * kt + x % 2), (2 * c + x // 2) * RO
                if len(LHS[n]) == 1:
                    a = [_words(ctx_t, *quad(kt, LHS[n][0][0]), RO) for kt in range(8)]
                else:
                    a = [_term(LHS, n, lambda x: _load(ctx_t, (i + tok.z * n, 2 * kt + x % 2), quad(kt, x)[1], RO).astype(F32))
                         for kt in range(8)]
                step(m, a, [P(lambda y, x: _load(wob_t, (7 * i + n, y), x * T, T), y) for y in range(2)])
            if i == 6:
                for part in parts:
                    accumulate(*part)

        for i in range(6):
            if i == 3:
                project(ax_t, wa_t, 4, P(write_rows, vbuf))
            list(project_b(i))
        last_b = project_b(6)
        next(last_b)

        for x, job in enumerate(AX_JOBS):
            schedule(P(_job_ax, tok, lambda val: val, ax_raw, ax_t, 1 - slot, *job),
                     t_o, t_o + 100 + 3000 * (x + 1) // len(AX_JOBS))

        def write_out(row, t, val):
            obuf[slot, pl.ds(row, 16), pl.ds(t * T, T)] = val.astype(BF16)

        project(o_t, wo_t, 0, write_out)
        list(last_b)
        assert not plan and not due
        out_copy(c, slot).start()
        ax_copy(jnp.minimum(c + 2, NO - 1), slot).wait()

        @pl.when(c < NO - 1)
        def _():
            ax_copy(jnp.minimum(c + 3, NO - 1), 1 - slot).start()

        @pl.when(c >= 1)
        def _():
            out_copy(c - 1, 1 - slot).wait()

    ax_copy(1, 1).wait()
    ax_copy(2, 0).start()
    lax.fori_loop(0, NO, chunk_body, None)
    out_copy(NO - 1, (NO - 1) % 2).wait()


def _kernel(ax_hbm, wqkv_hbm, wo_hbm, bx_hbm, c_hbm, wq_hbm, wuk_hbm, wuv_hbm, wob_hbm, out_hbm,
            ax_raw, ax_t, ctx_t, wob_t, wa_t, wo_t, zero_smem, sem_ax):
    vmem, dma = pltpu.VMEM, pltpu.SemaphoreType.DMA

    def clear(i, carry):
        zero_smem[0] = i >> 1
    lax.fori_loop(0, 2, clear, None)

    def ax_copy(c, slot):
        rows = pl.ds(_aligned(c * CO, CO), CO)
        return pltpu.make_async_copy(ax_hbm.at[rows, :], ax_raw.at[slot], sem_ax.at[slot])

    shared = (ax_copy, ax_raw, ax_t, ctx_t, wob_t, wa_t, wo_t, zero_smem)
    pl.run_scoped(
        P(_head_pairs, wqkv_hbm, wo_hbm, bx_hbm, c_hbm, wq_hbm, wuk_hbm, wuv_hbm, wob_hbm, *shared),
        vmem((S, DM), BF16),
        vmem((S, DC), BF16),
        vmem((2, DM, T), U32),
        vmem((2, DC, T), U32),
        vmem((2, DC, T), U32),
        vmem((2, 4, 64, DM), BF16),
        vmem((2, 4, 8, 3 * DM), U32),
        vmem((16, NH, DM), U32),
        vmem((49, 2, S // 4, T), BF16),
        vmem((49, S // 4, T), BF16),
        vmem((DM // T, T, T), U32),
        vmem((49, 2, RO, T), BF16),
        vmem((49, T, T), BF16),
        vmem((2, 8, T), F32),
        dma((2 * S // CH,)), dma((11,)))
    pl.run_scoped(
        P(_outputs, out_hbm, *shared),
        vmem((49, 2, RO, T), BF16),
        vmem((8, HALO + CO, T), F32),
        vmem((8, HALO + CO, T), F32),
        vmem((8, CO, T), F32),
        vmem((8, CO, T), F32),
        vmem((2, CO, 2 * DM), BF16),
        dma((2,)))


@jax.jit
def pallas_concat_heads__sliding_local_dilated__compressed_kv_cla__prompt_kernel(
    A_x: jax.Array,
    A_wqkv: jax.Array,
    A_wo: jax.Array,
    B_x: jax.Array,
    B_c_kv: jax.Array,
    B_w_q: jax.Array,
    B_w_uk: jax.Array,
    B_w_uv: jax.Array,
    B_w_o: jax.Array,
):
    vmem = pltpu.VMEM
    out = pl.pallas_call(
        _kernel,
        out_shape=jax.ShapeDtypeStruct((S, 2 * DM), BF16),
        in_specs=[pl.BlockSpec(memory_space=pl.ANY)] * 9,
        out_specs=pl.BlockSpec(memory_space=pl.ANY),
        scratch_shapes=[
            vmem((2, CO, DM), BF16),
            vmem((49, 2, RO, T), BF16),
            vmem((7, NP, S // 2, T), BF16),
            vmem((49, 2, DM, T), BF16),
            vmem((49, 6, 2 * T, T), BF16),
            vmem((49, 2, 2 * T, T), BF16),
            pltpu.SMEM((1,), jnp.int32),
            pltpu.SemaphoreType.DMA((2,)),
        ],
        compiler_params=pltpu.CompilerParams(
            vmem_limit_bytes=127 * 2**20, disable_bounds_checks=True),
    )(
        A_x.reshape(S, DM),
        A_wqkv.reshape(4, DM // 4, 3 * DM),
        A_wo.reshape(NH, DM // NH, DM),
        B_x.reshape(S, DM),
        B_c_kv.reshape(S, DC),
        B_w_q,
        B_w_uk,
        B_w_uv,
        B_w_o,
    )
    return out.reshape(1, S, 2 * DM)
```

```python
import functools
import math

import jax
import jax.numpy as jnp
from jax import lax
import jax.experimental.pallas as pl
import jax.experimental.pallas.tpu as pltpu

S = 2048
DM = 1024
DC = 512
NH = 32
NP = NH // 2
T = 128
CH = 4 * T
RO = 64
CO = 4 * RO
NO = S // CO
WIN, DIL = 8, 2
HALO = 16

LOG2E = math.log2(math.e)
SCALE_A = (DM // NH) ** -0.5 * LOG2E
SCALE_B = T ** -0.5 * LOG2E
MASKED = -1e9 * LOG2E
SAFE_SUM = 2.0 ** 40

DEPTH = 3
JOB_CYCLES = 896
CTX_CYCLES = 1024, 768

NX0, NX3 = 49, 84
TICK = RO // 2
EARLY_B = 4
F32, BF16, U32 = jnp.float32, jnp.bfloat16, jnp.uint32
P = functools.partial


def _dot(a, b):
    return jnp.dot(a, b, preferred_element_type=F32)


def _dot_nt(a, b):
    return lax.dot_general(a, b, (((1,), (1,)), ((), ())), preferred_element_type=F32)


def _cat(xs, axis=1):
    return xs[0] if len(xs) == 1 else jnp.concatenate(xs, axis=axis)


def _sum(xs):
    return functools.reduce(jnp.add, xs)


def _fold(op, x):
    return functools.reduce(op, [x[r:r + 8] for r in range(0, x.shape[0], 8)])


def _aligned(x, n):
    return x if isinstance(x, int) else pl.multiple_of(x, n)


def _rows(start, n):
    return pl.ds(_aligned(start, 16), n)


def _words(ref, lead, start, n):
    return ref.bitcast(U32)[(*lead, pl.ds(_aligned(start >> 1, 8), n // 2), slice(None))]


def _load(ref, lead, start, n):
    return pltpu.bitcast(_words(ref, lead, start, n), BF16)


def _split(w):
    return (pltpu.bitcast(w << 16, F32), pltpu.bitcast(w & jnp.uint32(0xFFFF0000), F32))


def _inverse(l):
    r = pl.reciprocal(l, approx=True)
    return r * (2.0 - l * r)


def _interleave(x, y):
    order = [((n + 0.5) / len(z), m, job) for m, z in enumerate((x, y)) for n, job in enumerate(z)]
    return [job for _, _, job in sorted(order, key=lambda e: e[:2])]


def _start(*copies):
    for cp in copies:
        cp.start()


def _wait(*copies):
    for cp in copies:
        cp.wait()


LHS = (((0, 1), (3, 1)), ((2, 1), (3, 1)), ((0, 1),), ((3, 1),),
       ((0, 1), (1, 1)), ((2, 1), (0, -1)), ((1, 1), (3, -1)))
RHS = (((0, 1), (3, 1)), ((0, 1),), ((1, 1), (3, -1)), ((2, 1), (0, -1)),
       ((3, 1),), ((0, 1), (1, 1)), ((2, 1), (3, 1)))
OUT = (((0, 1), (3, 1)), ((2, 1), (3, -1)), ((1, 1), (3, 1)), ((0, 1), (2, 1)),
       ((0, -1), (1, 1)), ((3, 1),), ((0, 1),))
SUMS = tuple(tuple((i, sign) for i in range(7) for m, sign in OUT[i] if m == n) for n in range(4))
FINAL = tuple(tuple(n for n in range(4) if SUMS[n][-1][0] == i) for i in range(7))


def _term(table, i, quad):
    (n, _), *rest = table[i]
    val = quad(n)
    for n, sign in rest:
        val = val + quad(n) if sign > 0 else val - quad(n)
    return val


def _terms(table, quad):
    blocks = [quad(n) for n in range(4)]
    return [_term(table, i, blocks.__getitem__) for i in range(7)]


def _block(outer, inner):
    return 2 * (outer // 2) + inner // 2, 2 * (outer % 2) + inner % 2


def _terms2(table, i, block):
    return _terms(table, lambda n: _term(table, i, lambda m: block(*_block(m, n))))


def _combine(m):
    return [_term(SUMS, n, m.__getitem__) for n in range(4)]


def _combine_outer(inner):
    return {_block(outer, n): val for n in range(4)
            for outer, val in enumerate(_combine([x[n] for x in inner]))}


class _Tokens:
    def __init__(self, zero_smem):
        self.z = zero_smem[0]
        self.zero = jnp.full((8, T), self.z, jnp.int32).astype(U32)

    def stored(self, ref, lead, start):
        first, *rest = lead
        if ref.dtype == BF16:
            return _words(ref, (first - (self.z & 1), *rest), start, 16) & self.zero
        return self.of(ref[(*lead, pl.ds(_aligned(start + 8 * (self.z & 1), 8), 8), slice(None))])

    def of(self, *vals):
        return pltpu.bitcast(_sum(vals), U32) & self.zero


def _after(token, x, everywhere=False):
    if token is None:
        return x
    bits = x if x.dtype == U32 else pltpu.bitcast(x, U32)
    cut = bits.shape[0] if everywhere else 8
    parts = [bits[r:r + 8] | token for r in range(0, cut, 8)]
    bits = _cat(parts + ([bits[cut:]] if cut < bits.shape[0] else []), axis=0)
    return bits if x.dtype == U32 else pltpu.bitcast(bits, x.dtype)


AX_JOBS = [(i, n, r) for n in range(2) for r in range(0, RO, 16) for i in range(7)]


def _job_ax(tok, released, ax_raw, ax_t, src, i, n, r):
    terms = _terms2(LHS, i, lambda row, col: released(
        ax_raw[src, pl.ds(row * RO + r, 16), pl.ds((2 * col + n) * T, T)].astype(F32)))
    for x, val in enumerate(terms):
        ax_t[7 * i + x, n, pl.ds(r, 16), :] = val.astype(BF16)
    return tok.stored(ax_t, (7 * i + 6, n), r)


def _head_pairs(wqkv_hbm, wo_hbm, bx_hbm, c_hbm, wq_hbm, wuk_hbm, wuv_hbm, wob_hbm,
                ax_copy, ax_raw, ax_t, ctx_t, wob_t, wa_t, wo_t, zero_smem,
                bx_raw, c_raw, wq_raw, wk_raw, wv_raw, wob_raw, wqkv_raw, wo_raw,
                bx_t, c_t, wq_turned, wq_t, wkv_t, guard, sem_in, sem_w):
    def head_copies(j, slot):
        return [pltpu.make_async_copy(src.bitcast(U32).at[:, j, :], dst.at[slot], sem_w.at[3 * slot + n])
                for n, (src, dst) in enumerate(((wuk_hbm, wk_raw), (wuv_hbm, wv_raw), (wq_hbm, wq_raw)))]

    def side_copies(j, slot):
        wob = wob_hbm.at[pl.ds(4 * (j >> 1), 4), pl.ds(_aligned((j & 1) * 64, 64), 64), :]
        wqkv = wqkv_hbm.bitcast(U32).at[:, pl.ds(_aligned(8 * j, 8), 8), :]
        return [pltpu.make_async_copy(wob, wob_raw.at[slot], sem_w.at[6 + 2 * slot]),
                pltpu.make_async_copy(wqkv, wqkv_raw.at[slot], sem_w.at[7 + 2 * slot])]

    def wo_copy(word):
        return pltpu.make_async_copy(wo_hbm.bitcast(U32).at[:, word, :], wo_raw.at[word], sem_w.at[10])

    def c_copy(c):
        rows = pl.ds(c * CH, CH)
        return pltpu.make_async_copy(c_hbm.at[rows, :], c_raw.at[rows, :], sem_in.at[2 * c])

    def x_copy(c):
        rows = pl.ds(c * CH, CH)
        return pltpu.make_async_copy(bx_hbm.at[rows, :], bx_raw.at[rows, :], sem_in.at[2 * c + 1])

    def pair_body(j, first=False):
        slot = j & 1
        tok = _Tokens(zero_smem)
        causal = (lax.broadcasted_iota(jnp.int32, (T, T), 1)
                  <= lax.broadcasted_iota(jnp.int32, (T, T), 0))

        jobs, due, pace = [], [], dict(release=None, recent=None)

        def queue(cycles, more, q=1.0, kv=1.0, attention=1.0):
            pace.update(period=cycles / len(more), clock=0, q=q, kv=kv, attention=attention)
            jobs.extend(more)

        def flush():
            while jobs:
                jobs.pop(0)()

        def background(cycles, share, delay, recent=None):
            pace["clock"] += cycles * share
            token = None
            while jobs and pace["clock"] >= pace["period"]:
                pace["clock"] -= pace["period"]
                pace["release"] = None if recent is None else tok.of(recent[:8])
                new = jobs.pop(0)()
                pace["release"] = None
                token = new if token is None else token | new
            if token is not None:
                due.append([delay, token])
            for entry in due:
                entry[0] -= cycles
            now = [token for left, token in due if left <= 0]
            due[:] = [entry for entry in due if entry[0] > 0]
            return functools.reduce(jnp.bitwise_or, now) if now else None

        def released(x):
            return _after(pace["release"], x, everywhere=True)

        def store_terms(dst, first_term, lead, row, terms):
            for i, val in enumerate(terms):
                dst[(first_term + i, *lead, _rows(row, 16), slice(None))] = val.astype(BF16)
            return tok.stored(dst, (first_term + 6, *lead), row)

        def job_x(c, i, n, r):
            terms = _terms2(RHS, i, lambda row, col: bx_raw[
                pl.ds(c * CH + (col ^ 2) * T + r, 16), pl.ds((2 * row + n) * T, T)].astype(F32))
            return store_terms(bx_t, 7 * i, (n,), c * T + r, terms)

        def job_c(c, i, r):
            terms = _terms2(LHS, i, lambda row, col: c_raw[
                pl.ds(c * CH + row * T + r, 16), pl.ds(col * T, T)].astype(F32))
            return store_terms(c_t, 7 * i, (), c * T + r, terms)

        def jobs_x(c):
            return [P(job_x, c, i, n, r) for r in range(0, T, 16) for n in range(2) for i in range(7)]

        def jobs_c(c):
            return [P(job_c, c, i, r) for r in range(0, T, 16) for i in range(7)]

        def job_wkv(src, i, r):
            def block(row, col):
                raw = (wk_raw, wv_raw)[col % 2]
                return _split(released(raw[src, pl.ds(row * T + r, 16), :]))[col // 2]
            return store_terms(wkv_t, 7 * i, (), r, _terms2(RHS, i, block))

        def job_turn(src, n):
            words = released(wq_raw[src, pl.ds(n * T, T), :])
            wq_turned[n] = pltpu.bitcast(pltpu.bitcast(words, F32).T, U32)
            return tok.stored(wq_turned, (n,), T - 16)

        def job_wq(i, n, r):
            def block(row, col):
                return _split(released(wq_turned[2 * col + n, pl.ds((row % 2) * RO + r, 16), :]))[row // 2]
            return store_terms(wq_t, 7 * i, (n,), r, _terms2(LHS, i, block))

        def jobs_wkv(src):
            return [P(job_wkv, src, i, r) for r in range(0, T, 16) for i in range(7)]

        def jobs_wq(src):
            return ([P(job_turn, src, n) for n in range(DM // T)],
                    [P(job_wq, i, n, r) for n in range(2) for r in range(0, RO, 16) for i in range(7)])

        def job_wob(i, n, r):
            def block(row, col):
                head = 2 * (row % 2) + row // 2
                return released(wob_raw[slot, head, pl.ds(r, 16), pl.ds((2 * col + n) * T, T)].astype(F32))
            return store_terms(wob_t, 7 * i, (n,), j * 64 + r, _terms2(RHS, i, block))

        def job_wo(i, n):
            e, odd, head = j & 3, (j >> 2) & 1, 16 * (j >> 3)

            def block(row, col):
                even_t, odd_t = _split(released(
                    wo_raw[4 * e + row, _rows(head, 16), pl.ds((2 * col + n) * T, T)]))
                return jnp.where(odd == 1, odd_t, even_t)
            return store_terms(wo_t, 7 * i, (n,), odd * T + e * NH + head, _terms2(RHS, i, block))

        permuted = {}

        def job_permute(mat):
            lane = lax.broadcasted_iota(jnp.int32, (32, T), 1)
            e, grp, sub = lane >> 5, (lane >> 2) & 7, lane & 3

            def gather(x, index):
                return jnp.take_along_axis(x, index, axis=1, mode="promise_in_bounds")
            x = [released(wqkv_raw[slot, :, :, pl.ds(mat * DM + t * T, T)].reshape(32, T))
                 for t in range(8)]
            y = [gather(x[t], sub * 32 + e * 8 + ((grp - t) & 7)) for t in range(8)]
            u = [y[-s % 8] for s in range(8)]
            for bit in (1, 2, 4):
                u = [jnp.where((grp & bit) != 0, u[(s - bit) % 8], u[s]) for s in range(8)]
            u = [u[0]] + [gather(u[t], e * 32 + ((grp + t) & 7) * 4 + sub) for t in range(1, 8)]
            permuted[mat] = u
            return _fold(jnp.bitwise_or, functools.reduce(jnp.bitwise_or, u)) & tok.zero

        def column(mat, row, t):
            return pltpu.bitcast(released(permuted[mat][t][8 * row:8 * row + 8]), BF16).astype(F32)

        def job_wa(mat, i, n):
            terms = _terms2(RHS, i, lambda row, col: column(mat, row, 2 * col + n))
            return store_terms(wa_t, 7 * i, (2 * mat + n,), 16 * j, terms)

        pause = [P(lambda: tok.zero)] * 2
        jobs_wob = [P(job_wob, i, n, r) for r in range(0, 64, 16) for n in range(2) for i in range(7)]
        jobs_wo = [P(job_wo, i, n) for n in range(2) for i in range(7)]
        jobs_wa = []
        for mat in range(3):
            jobs_wa += [P(job_permute, mat)] + pause
            jobs_wa += [P(job_wa, mat, i, n) for n in range(2) for i in range(7)]

        q, k, v = {}, {}, {}

        def product(dot, share, left, right):
            token = background(left.shape[0] // 2, share, JOB_CYCLES, pace["recent"])
            pace["recent"] = dot(pltpu.bitcast(_after(token, left), BF16), right)
            return pace["recent"]

        def project_q(c):
            inner = []
            for first_product in range(0, 49, 7):
                inner.append(_combine([_sum([
                    product(_dot_nt, pace["q"], _words(wq_t, (i, n), 0, RO), _load(bx_t, (i, n), c * T, T))
                    for n in range(2)]) for i in range(first_product, first_product + 7)]))
                if len(inner) <= 4:
                    due.append([400, tok.of(*[x[RO - 8:] for x in inner[-1]])])
            blocks = _combine_outer(inner)
            for h in range(2):
                for col in range(4):
                    val = _cat([blocks[2 * h, col], blocks[2 * h + 1, col]], axis=0) * SCALE_B
                    q[4 * c + (col ^ 2), h] = val.T.astype(BF16)

        def project_kv(c):
            m = [product(_dot, pace["kv"], _words(c_t, (i,), c * T, T), _load(wkv_t, (i,), 0, T))
                 for i in range(49)]
            for (row, col), val in sorted(_combine_outer([_combine(m[i:i + 7]) for i in range(0, 49, 7)]).items()):
                (k, v)[col % 2][4 * c + row, col // 2] = val.astype(BF16)

        def plain(raw, c, weights):
            def part(r, col):
                left = raw[pl.ds(c * CH + r, 32), pl.ds(col, 4 * T)]
                token = background(32, 1.0, 128)
                if token is None:
                    return left
                return _cat([_after(_cat([token, token]), left[:, :2 * T]), left[:, 2 * T:]])
            return [_dot(_cat([_cat([part(r, col) for r in range(0, CH, 32)], axis=0)
                               for col in range(0, raw.shape[1], 4 * T)]), w) for w in weights]

        def plain_kv(c, weights):
            for n, val in enumerate(plain(c_raw, c, weights)):
                for r in range(4):
                    (k, v)[n // 2][4 * c + r, n % 2] = val[r * T:(r + 1) * T].astype(BF16)

        def plain_q(c, weights):
            for h, val in enumerate(plain(bx_raw, c, weights)):
                for r in range(4):
                    q[4 * c + r, h] = (val[r * T:(r + 1) * T] * SCALE_B).astype(BF16)

        in_flight, partial, ctx, spread, checks = [], {}, {}, {}, []

        def finish(i, h):
            l, o = partial.pop((i, h))
            l = jnp.sum(l, axis=1, keepdims=True)
            r = _inverse(l)
            ctx[i, h] = o * r
            spread[i, h] = _fold(jnp.maximum, jnp.broadcast_to(l + r, (T, T)))
            b = i // 2
            quad = [(2 * b, 0), (2 * b, 1), (2 * b + 1, 0), (2 * b + 1, 1)]
            if all(u in ctx for u in quad):
                terms = _terms(LHS, lambda m: ctx.pop(quad[m]))
                for n, val in enumerate(terms):
                    ctx_t[n, j, pl.ds(b * T, T), :] = val.astype(BF16)
                checks.append((_fold(jnp.add, terms[0] + terms[5] + terms[6]),
                               functools.reduce(jnp.maximum, [spread.pop(u) for u in quad])))
                due.append([CTX_CYCLES[first], tok.stored(ctx_t, (6, j), b * T) | tok.of(*checks[-1])])

        def weigh(i, h, t, p):
            l, o = partial.get((i, h), (None, None))
            l = p if l is None else l + p
            d = _dot(_after(background(64, pace["attention"], JOB_CYCLES, p), p).astype(BF16), v[t, h])
            partial[i, h] = (l, d if o is None else o + d)
            if t == i:
                finish(i, h)

        def attention(lo, hi):
            for i in range(lo, hi):
                for h in range(2):
                    for t in range(i + 1):
                        s = _dot_nt(q[i, h], k[t, h])
                        if t == i:
                            s = jnp.where(causal, s, MASKED)
                        in_flight.append((i, h, t, jnp.exp2(s)))
                        ahead = (i, h) == (S // T - 1, 1) and 8 <= t < 13 and not first
                        if len(in_flight) > DEPTH and not ahead:
                            weigh(*in_flight.pop(0))
            while hi == S // T and in_flight:
                weigh(*in_flight.pop(0))

        def cycles(lo, hi):
            return 2 * 64 * sum(range(lo + 1, hi + 1))

        if first:
            wk, wv, wq = head_copies(0, 0)
            _start(wv, wk, c_copy(0), c_copy(1))
            _wait(wv, wk, c_copy(0))
            _start(c_copy(2), c_copy(3), wq, x_copy(0))
            weights = [w.astype(BF16) for raw in (wk_raw, wv_raw) for w in _split(raw[0])]
            queue(0.98 * 2048, jobs_c(0)[:49])
            plain_kv(0, weights)
            flush()
            _wait(c_copy(1), c_copy(2))
            _start(x_copy(1), x_copy(2))
            queue(0.92 * 4096, jobs_c(0)[49:] + jobs_c(1) + jobs_c(2))
            plain_kv(1, weights)
            plain_kv(2, weights)
            flush()
            _wait(c_copy(3), wq)
            turn, terms = jobs_wq(0)
            queue(0.9 * 2048, _interleave(turn, jobs_c(3)))
            plain_kv(3, weights)
            flush()
            _wait(x_copy(0))
            weights = [w.astype(BF16) for w in _split(wq_raw[0])]
            queue(0.9 * (2048 + 0.2 * cycles(0, 4)), jobs_x(0)[:96], attention=0.2)
            plain_q(0, weights)
            attention(0, 4)
            flush()
            _wait(x_copy(1), x_copy(2))
            stage = [*side_copies(0, 0), *head_copies(1, 1)]
            _start(x_copy(3), *stage)
            lax.fori_loop(0, 16, lambda word, carry: wo_copy(word).start(), None)
            queue(0.98 * (2048 + 0.5 * cycles(4, 7)),
                  jobs_x(2) + terms + jobs_x(0)[96:] + jobs_x(1)[:14], attention=0.5)
            plain_q(1, weights)
            attention(4, 7)
            flush()
            _wait(x_copy(3))
            queue(0.85 * (1568 + cycles(7, 10)), jobs_x(3))
            project_q(2)
            attention(7, 10)
            flush()
            _wait(*stage)
            _start(ax_copy(0, 0), *head_copies(2, 0), *side_copies(1, 1))
            turn, terms = jobs_wq(1)
            queue(0.88 * (1568 + cycles(10, 14)), _interleave(
                _interleave(jobs_wob, jobs_wa), _interleave(jobs_x(1)[14:], _interleave(turn, jobs_wkv(1)))))
            attention(10, 11)
            project_q(3)
            attention(11, 14)
            flush()
            _wait(*[wo_copy(word) for word in range(16)], ax_copy(0, 0))
            _start(ax_copy(1, 1))
            queue(0.92 * cycles(14, 16), _interleave(
                jobs_wo + terms, [P(_job_ax, tok, released, ax_raw, ax_t, 0, *job) for job in AX_JOBS]))
            attention(14, 16)
            flush()
        else:
            queue(0.98 * 4 * 1568 * (0.5 + 0.3), _interleave(jobs_wob, jobs_wo + jobs_wa),
                  q=0.5, kv=0.3, attention=0)
            project_kv(0)
            project_q(0)
            project_kv(1)
            attention(0, 3)
            project_q(1)
            attention(3, 7)
            project_q(2)
            project_kv(2)
            attention(7, 10)
            project_q(3)
            project_kv(3)
            attention(10, 12)
            flush()
            turn, terms = jobs_wq(1 - slot)
            queue(0.95 * cycles(12, 16), _interleave(jobs_wkv(1 - slot), turn + pause + terms))
            attention(12, 16)
            flush()
        guard[0] = _sum([guard[0]] + [x for x, _ in checks])
        guard[1] = functools.reduce(jnp.maximum, [guard[1]] + [x for _, x in checks])

        def ahead(n):
            return j + n if first else jnp.minimum(j + n, NP - 1)
        _wait(*head_copies(ahead(2), slot), *side_copies(ahead(1), 1 - slot))

        @pl.when(j < NP - 1)
        def _():
            _start(*head_copies(ahead(3), 1 - slot), *side_copies(ahead(2), slot))

    def exact_pairs(ctx):
        def block(i):
            return pl.ds(pl.multiple_of(i * T, T), T)

        def qkv(n, h, i):
            return c_t.at[(2 * n + h) * 4 + (i >> 2), block(i & 3), :]

        def project(x, carry):
            h, i = x & 1, x >> 1
            for n, (rows, w, scale) in enumerate(
                    ((bx_raw, wq_raw, SCALE_B), (c_raw, wk_raw, 1.0), (c_raw, wv_raw, 1.0))):
                def add(t, val):
                    even, odd = _split(w[0, block(t), :])
                    return val + _dot(rows[block(i), block(t)], jnp.where(h == 0, even, odd).astype(BF16))
                val = lax.fori_loop(0, w.shape[1] // T, add, jnp.zeros((T, T), F32))
                qkv(n, h, i)[...] = (val * scale).astype(BF16)

        def attend(b, x, carry):
            quad, part = x >> 3, pl.ds(pl.multiple_of((x & 7) * 16, 16), 16)
            h, i = quad & 1, 2 * b + (quad >> 1)

            def scores(t):
                row = lax.broadcasted_iota(jnp.int32, (16, T), 0) + (i * T + (x & 7) * 16)
                col = lax.broadcasted_iota(jnp.int32, (16, T), 1) + t * T
                return jnp.where(col <= row, _dot_nt(qkv(0, h, i)[part, :], qkv(1, h, t)[...]), MASKED)

            m = lax.fori_loop(
                0, i + 1, lambda t, m: jnp.maximum(m, jnp.max(scores(t), axis=1, keepdims=True)),
                jnp.full((16, 1), -jnp.inf, F32))

            def accumulate(t, carry):
                l, o = carry
                p = jnp.exp2(scores(t) - m)
                return (l + jnp.sum(p, axis=1, keepdims=True),
                        o + _dot(p.astype(BF16), qkv(2, h, t)[...]))
            l, o = lax.fori_loop(0, i + 1, accumulate,
                                 (jnp.zeros((16, 1), F32), jnp.zeros((16, T), F32)))
            ctx[quad, part, :] = o / l

        def pair(j, carry):
            _start(*head_copies(j, 0))
            _wait(*head_copies(j, 0))
            lax.fori_loop(0, 2 * S // T, project, None)

            def rows(b, carry):
                lax.fori_loop(0, 32, P(attend, b), None)
                for n, val in enumerate(_terms(LHS, lambda m: ctx[m])):
                    ctx_t[n, j, block(b), :] = val.astype(BF16)
            lax.fori_loop(0, S // T // 2, rows, None)

        lax.fori_loop(0, NP, pair, None)

    guard[...] = jnp.zeros(guard.shape, F32)
    pair_body(0, first=True)
    lax.fori_loop(1, NP, lambda j, carry: pair_body(j), None)

    safe = jnp.logical_and(jnp.abs(guard[0]) < jnp.inf, guard[1] < SAFE_SUM)

    @pl.when(jnp.max(jnp.where(safe, 0.0, 1.0)) > 0.0)
    def _():
        pl.run_scoped(exact_pairs, pltpu.VMEM((4, T, T), F32))


def _outputs(out_hbm, ax_copy, ax_raw, ax_t, ctx_t, wob_t, wa_t, wo_t, zero_smem,
             o_t, kbuf, vbuf, qbuf, acc, obuf, sem_out):
    def out_copy(c, slot):
        rows = pl.ds(_aligned(c * CO, CO), CO)
        return pltpu.make_async_copy(obuf.at[slot], out_hbm.at[rows, :], sem_out.at[slot])

    for buf in (kbuf, vbuf):
        for t in range(8):
            buf[t, pl.ds(CO, HALO), :] = jnp.zeros((HALO, T), F32)

    t_q = 2 * 49 * RO
    t_v = t_q + 21 * 4 * RO + 49 * RO
    t_o = t_v + (21 + EARLY_B) * 4 * RO

    def chunk_body(c, carry):
        slot = c & 1
        tok = _Tokens(zero_smem)
        plan, due, clock = {}, {}, [0]

        def schedule(job, begin, end, release=False):
            plan.setdefault(max(clock[0], begin // TICK), []).append((job, -(-end // TICK), release))

        def step(results, a, w):
            res = [None] * len(w)
            for x, left in enumerate(a):
                n = clock[0]
                clock[0] += 1
                if n in due:
                    left = _after(functools.reduce(jnp.bitwise_or, due.pop(n)), left)
                left = left.astype(BF16) if left.dtype == F32 else pltpu.bitcast(left, BF16)
                for y in range(len(w)):
                    d = _dot(left, w[y](x))
                    res[y] = d if res[y] is None else res[y] + d
                token = None
                for job, last, release in plan.pop(n, []):
                    if release and token is None:
                        token = tok.of(d[:8])
                    due.setdefault(max(last, n + 1), []).append(job(token) if release else job())
            results.append(res)

        def project(lhs_t, rhs_t, tile0, write):
            inner = {}

            def combine(i, y, m):
                inner[i, y] = _combine([x[y] for x in m])
                return tok.of(*[x[r + 8:r + 16] for x in inner[i, y] for r in range(0, RO, 16)])

            def finish(outer, y, r):
                vals = [_term(SUMS, outer, lambda i: inner[i, y][n][r:r + 16]) for n in range(4)]
                for n, val in enumerate(vals):
                    row, col = _block(outer, n)
                    write(row * RO + r, 2 * col + y, val)
                return tok.of(*[x[8:] for x in vals])

            for i in range(7):
                m = []
                done = clock[0] * TICK + 7 * RO
                for y in range(2):
                    schedule(P(combine, i, y, m), done, done + 400)
                for outer in FINAL[i]:
                    slabs = [(y, r) for r in range(0, RO, 16) for y in range(2)]
                    for x, slab in enumerate(slabs):
                        schedule(P(finish, outer, *slab), done, done + 300 + 40 * (x + 1))
                for n in range(7 * i, 7 * i + 7):
                    step(m, [_words(lhs_t, (n, x), 0, RO) for x in range(2)],
                         [P(lambda y, x: _load(rhs_t, (n, tile0 + y), x * T, T), y) for y in range(2)])

        for buf in (kbuf, vbuf):
            for t in range(8):
                buf[t, pl.ds(0, HALO), :] = buf[t, pl.ds(CO, HALO), :]

        def write_rows(buf, row, t, val):
            buf[t, pl.ds(HALO + row, 16), :] = val

        def write_q(row, t, val):
            qbuf[t, pl.ds(row, 16), :] = val * SCALE_A

        project(ax_t, wa_t, 2, P(write_rows, kbuf))
        project(ax_t, wa_t, 0, write_q)

        att = {}

        def job_weights(row, r, release):
            base = HALO + row * RO + r
            qs = [_after(release, qbuf[t, pl.ds(row * RO + r, 8), :]) for t in range(8)]
            logits = []
            for w in range(WIN):
                x = _sum([qs[t] * kbuf[t, pl.ds(base - DIL * w, 8), :] for t in range(8)])
                x = x + pltpu.roll(x, 64, 1)
                x = x + pltpu.roll(x, 32, 1)
                if row == 0 and r < DIL * w:
                    pos = lax.broadcasted_iota(jnp.int32, (8, T), 0) + (c * CO + r)
                    x = jnp.where(pos >= DIL * w, x, MASKED)
                logits.append(x)
            m = functools.reduce(jnp.maximum, logits)
            p = [jnp.exp2(x - m) for x in logits]
            inv = _inverse(_sum(p))
            att[row, r] = [x * inv for x in p]
            return tok.of(att[row, r][0])

        def job_values(row, r, release):
            base = HALO + row * RO + r
            p = [_after(release, x) for x in att[row, r]]
            att[row, r] = [_sum([p[w] * vbuf[t, pl.ds(base - DIL * w, 8), :] for w in range(WIN)])
                           for t in range(8)]
            return tok.of(att[row, r][-1])

        def job_o(n, r, i):
            def block(row, col):
                return _cat([att[row, r][2 * col + n], att[row, r + 8][2 * col + n]], axis=0)
            for x, val in enumerate(_terms2(LHS, i, block)):
                o_t[7 * i + x, n, pl.ds(r, 16), :] = val.astype(BF16)
            return tok.stored(o_t, (7 * i + 6, n), r)

        groups = [(row, r + x) for r in range(0, RO, 16) for row in (2, 0, 3, 1) for x in (0, 8)]
        w0, w1, v0, v1 = t_q + 1000, t_v - 1400, t_v + 400, t_o - 700
        for g, (row, r) in enumerate(groups):
            begin = w0 + (w1 - w0) * g // len(groups)
            schedule(P(job_weights, row, r), begin, begin + 500, release=True)
            begin = v0 + (v1 - v0) * g // len(groups)
            schedule(P(job_values, row, r), begin, begin + 600, release=True)
            if g % 8 == 7:
                for x, (n, i) in enumerate((n, i) for n in range(2) for i in range(7)):
                    schedule(P(job_o, n, r - 8, i), begin, min(begin + 400 + 60 * (x + 1), t_o))

        touched = {}

        def project_b(i):
            m = []

            def accumulate(y, inner):
                val = _combine([x[y] for x in m])[inner]
                token = None
                for outer, sign in OUT[i]:
                    row, col = _block(outer, inner)
                    rows, col = pl.ds(row * RO, RO), 2 * col + y
                    total = val
                    if (outer, inner, y) in touched:
                        total = acc[col, rows, :] + val if sign > 0 else acc[col, rows, :] - val
                    touched[outer, inner, y] = True
                    if outer not in FINAL[i]:
                        acc[col, rows, :] = total
                        token = tok.stored(acc, (col,), row * RO)
                    else:
                        obuf[slot, rows, pl.ds(DM + col * T, T)] = total.astype(BF16)
                        if token is None:
                            token = tok.of(_fold(jnp.add, total))
                return token

            parts = [(y, inner) for y in range(2) for inner in range(4)]
            done = clock[0] * TICK + 7 * 4 * RO
            if i < 6:
                for x, part in enumerate(parts):
                    schedule(P(accumulate, *part), done, done + 256 + 200 * x)
            for n in range(7):
                if i == 6 and n == EARLY_B:
                    yield

                def quad(kt, x):
                    return (i, 2 * kt + x % 2), (2 * c + x // 2) * RO
                if len(LHS[n]) == 1:
                    a = [_words(ctx_t, *quad(kt, LHS[n][0][0]), RO) for kt in range(8)]
                else:
                    a = [_term(LHS, n, lambda x: _load(ctx_t, (i + tok.z * n, 2 * kt + x % 2), quad(kt, x)[1], RO).astype(F32))
                         for kt in range(8)]
                step(m, a, [P(lambda y, x: _load(wob_t, (7 * i + n, y), x * T, T), y) for y in range(2)])
            if i == 6:
                for part in parts:
                    accumulate(*part)

        for i in range(6):
            if i == 3:
                project(ax_t, wa_t, 4, P(write_rows, vbuf))
            list(project_b(i))
        last_b = project_b(6)
        next(last_b)

        for x, job in enumerate(AX_JOBS):
            schedule(P(_job_ax, tok, lambda val: val, ax_raw, ax_t, 1 - slot, *job),
                     t_o, t_o + 100 + 3000 * (x + 1) // len(AX_JOBS))

        def write_out(row, t, val):
            obuf[slot, pl.ds(row, 16), pl.ds(t * T, T)] = val.astype(BF16)

        project(o_t, wo_t, 0, write_out)
        list(last_b)
        assert not plan and not due
        out_copy(c, slot).start()
        ax_copy(jnp.minimum(c + 2, NO - 1), slot).wait()

        @pl.when(c < NO - 1)
        def _():
            ax_copy(jnp.minimum(c + 3, NO - 1), 1 - slot).start()

        @pl.when(c >= 1)
        def _():
            out_copy(c - 1, 1 - slot).wait()

    ax_copy(1, 1).wait()
    ax_copy(2, 0).start()
    lax.fori_loop(0, NO, chunk_body, None)
    out_copy(NO - 1, (NO - 1) % 2).wait()


def _kernel(ax_hbm, wqkv_hbm, wo_hbm, bx_hbm, c_hbm, wq_hbm, wuk_hbm, wuv_hbm, wob_hbm, out_hbm,
            ax_raw, ax_t, ctx_t, wob_t, wa_t, wo_t, zero_smem, sem_ax):
    vmem, dma = pltpu.VMEM, pltpu.SemaphoreType.DMA

    def clear(i, carry):
        zero_smem[0] = i >> 1
    lax.fori_loop(0, 2, clear, None)

    def ax_copy(c, slot):
        rows = pl.ds(_aligned(c * CO, CO), CO)
        return pltpu.make_async_copy(ax_hbm.at[rows, :], ax_raw.at[slot], sem_ax.at[slot])

    shared = (ax_copy, ax_raw, ax_t, ctx_t, wob_t, wa_t, wo_t, zero_smem)
    pl.run_scoped(
        P(_head_pairs, wqkv_hbm, wo_hbm, bx_hbm, c_hbm, wq_hbm, wuk_hbm, wuv_hbm, wob_hbm, *shared),
        vmem((S, DM), BF16),
        vmem((S, DC), BF16),
        vmem((2, DM, T), U32),
        vmem((2, DC, T), U32),
        vmem((2, DC, T), U32),
        vmem((2, 4, 64, DM), BF16),
        vmem((2, 4, 8, 3 * DM), U32),
        vmem((16, NH, DM), U32),
        vmem((49, 2, S // 4, T), BF16),
        vmem((49, S // 4, T), BF16),
        vmem((DM // T, T, T), U32),
        vmem((49, 2, RO, T), BF16),
        vmem((49, T, T), BF16),
        vmem((2, 8, T), F32),
        dma((2 * S // CH,)), dma((11,)))
    pl.run_scoped(
        P(_outputs, out_hbm, *shared),
        vmem((49, 2, RO, T), BF16),
        vmem((8, HALO + CO, T), F32),
        vmem((8, HALO + CO, T), F32),
        vmem((8, CO, T), F32),
        vmem((8, CO, T), F32),
        vmem((2, CO, 2 * DM), BF16),
        dma((2,)))


@jax.jit
def pallas_concat_heads__sliding_local_dilated__compressed_kv_cla__prompt_kernel(
    A_x: jax.Array,
    A_wqkv: jax.Array,
    A_wo: jax.Array,
    B_x: jax.Array,
    B_c_kv: jax.Array,
    B_w_q: jax.Array,
    B_w_uk: jax.Array,
    B_w_uv: jax.Array,
    B_w_o: jax.Array,
):
    vmem = pltpu.VMEM
    out = pl.pallas_call(
        _kernel,
        out_shape=jax.ShapeDtypeStruct((S, 2 * DM), BF16),
        in_specs=[pl.BlockSpec(memory_space=pl.ANY)] * 9,
        out_specs=pl.BlockSpec(memory_space=pl.ANY),
        scratch_shapes=[
            vmem((2, CO, DM), BF16),
            vmem((49, 2, RO, T), BF16),
            vmem((7, NP, S // 2, T), BF16),
            vmem((49, 2, DM, T), BF16),
            vmem((49, 6, 2 * T, T), BF16),
            vmem((49, 2, 2 * T, T), BF16),
            pltpu.SMEM((1,), jnp.int32),
            pltpu.SemaphoreType.DMA((2,)),
        ],
        compiler_params=pltpu.CompilerParams(
            vmem_limit_bytes=127 * 2**20, disable_bounds_checks=True),
    )(
        A_x.reshape(S, DM),
        A_wqkv.reshape(4, DM // 4, 3 * DM),
        A_wo.reshape(NH, DM // NH, DM),
        B_x.reshape(S, DM),
        B_c_kv.reshape(S, DC),
        B_w_q,
        B_w_uk,
        B_w_uv,
        B_w_o,
    )
    return out.reshape(1, S, 2 * DM)
```

```python
import functools
import math

import jax
import jax.numpy as jnp
from jax import lax
import jax.experimental.pallas as pl
import jax.experimental.pallas.tpu as pltpu

S = 2048
DM = 1024
DC = 512
NH = 32
NP = NH // 2
T = 128
CH = 4 * T
RO = 64
CO = 4 * RO
NO = S // CO
WIN, DIL = 8, 2
HALO = 16

LOG2E = math.log2(math.e)
SCALE_A = (DM // NH) ** -0.5 * LOG2E
SCALE_B = T ** -0.5 * LOG2E
MASKED = -1e9 * LOG2E
SAFE_SUM = 2.0 ** 40

DEPTH = 3
JOB_CYCLES = 896
CTX_CYCLES = 1024, 768

NX0, NX3 = 49, 84
TICK = RO // 2
EARLY_B = 4
F32, BF16, U32 = jnp.float32, jnp.bfloat16, jnp.uint32
P = functools.partial


def _dot(a, b):
    return jnp.dot(a, b, preferred_element_type=F32)


def _dot_nt(a, b):
    return lax.dot_general(a, b, (((1,), (1,)), ((), ())), preferred_element_type=F32)


def _cat(xs, axis=1):
    return xs[0] if len(xs) == 1 else jnp.concatenate(xs, axis=axis)


def _sum(xs):
    return functools.reduce(jnp.add, xs)


def _fold(op, x):
    return functools.reduce(op, [x[r:r + 8] for r in range(0, x.shape[0], 8)])


def _aligned(x, n):
    return x if isinstance(x, int) else pl.multiple_of(x, n)


def _rows(start, n):
    return pl.ds(_aligned(start, 16), n)


def _words(ref, lead, start, n):
    return ref.bitcast(U32)[(*lead, pl.ds(_aligned(start >> 1, 8), n // 2), slice(None))]


def _load(ref, lead, start, n):
    return pltpu.bitcast(_words(ref, lead, start, n), BF16)


def _split(w):
    return (pltpu.bitcast(w << 16, F32), pltpu.bitcast(w & jnp.uint32(0xFFFF0000), F32))


def _inverse(l):
    r = pl.reciprocal(l, approx=True)
    return r * (2.0 - l * r)


def _interleave(x, y):
    order = [((n + 0.5) / len(z), m, job) for m, z in enumerate((x, y)) for n, job in enumerate(z)]
    return [job for _, _, job in sorted(order, key=lambda e: e[:2])]


def _start(*copies):
    for cp in copies:
        cp.start()


def _wait(*copies):
    for cp in copies:
        cp.wait()


LHS = (((0, 1), (3, 1)), ((2, 1), (3, 1)), ((0, 1),), ((3, 1),),
       ((0, 1), (1, 1)), ((2, 1), (0, -1)), ((1, 1), (3, -1)))
RHS = (((0, 1), (3, 1)), ((0, 1),), ((1, 1), (3, -1)), ((2, 1), (0, -1)),
       ((3, 1),), ((0, 1), (1, 1)), ((2, 1), (3, 1)))
OUT = (((0, 1), (3, 1)), ((2, 1), (3, -1)), ((1, 1), (3, 1)), ((0, 1), (2, 1)),
       ((0, -1), (1, 1)), ((3, 1),), ((0, 1),))
SUMS = tuple(tuple((i, sign) for i in range(7) for m, sign in OUT[i] if m == n) for n in range(4))
FINAL = tuple(tuple(n for n in range(4) if SUMS[n][-1][0] == i) for i in range(7))


def _term(table, i, quad):
    (n, _), *rest = table[i]
    val = quad(n)
    for n, sign in rest:
        val = val + quad(n) if sign > 0 else val - quad(n)
    return val


def _terms(table, quad):
    blocks = [quad(n) for n in range(4)]
    return [_term(table, i, blocks.__getitem__) for i in range(7)]


def _block(outer, inner):
    return 2 * (outer // 2) + inner // 2, 2 * (outer % 2) + inner % 2


def _terms2(table, i, block):
    return _terms(table, lambda n: _term(table, i, lambda m: block(*_block(m, n))))


def _combine(m):
    return [_term(SUMS, n, m.__getitem__) for n in range(4)]


def _combine_outer(inner):
    return {_block(outer, n): val for n in range(4)
            for outer, val in enumerate(_combine([x[n] for x in inner]))}


class _Tokens:
    def __init__(self, zero_smem):
        self.z = zero_smem[0]
        self.zero = jnp.full((8, T), self.z, jnp.int32).astype(U32)

    def stored(self, ref, lead, start):
        first, *rest = lead
        if ref.dtype == BF16:
            return _words(ref, (first - (self.z & 1), *rest), start, 16) & self.zero
        return self.of(ref[(*lead, pl.ds(_aligned(start + 8 * (self.z & 1), 8), 8), slice(None))])

    def of(self, *vals):
        return pltpu.bitcast(_sum(vals), U32) & self.zero


def _after(token, x, everywhere=False):
    if token is None:
        return x
    bits = x if x.dtype == U32 else pltpu.bitcast(x, U32)
    cut = bits.shape[0] if everywhere else 8
    parts = [bits[r:r + 8] | token for r in range(0, cut, 8)]
    bits = _cat(parts + ([bits[cut:]] if cut < bits.shape[0] else []), axis=0)
    return bits if x.dtype == U32 else pltpu.bitcast(bits, x.dtype)


AX_JOBS = [(i, n, r) for n in range(2) for r in range(0, RO, 16) for i in range(7)]


def _job_ax(tok, released, ax_raw, ax_t, src, i, n, r):
    terms = _terms2(LHS, i, lambda row, col: released(
        ax_raw[src, pl.ds(row * RO + r, 16), pl.ds((2 * col + n) * T, T)].astype(F32)))
    for x, val in enumerate(terms):
        ax_t[7 * i + x, n, pl.ds(r, 16), :] = val.astype(BF16)
    return tok.stored(ax_t, (7 * i + 6, n), r)


def _head_pairs(wqkv_hbm, wo_hbm, bx_hbm, c_hbm, wq_hbm, wuk_hbm, wuv_hbm, wob_hbm,
                ax_copy, ax_raw, ax_t, ctx_t, wob_t, wa_t, wo_t, zero_smem,
                bx_raw, c_raw, wq_raw, wk_raw, wv_raw, wob_raw, wqkv_raw, wo_raw,
                bx_t, c_t, wq_turned, wq_t, wkv_t, guard, sem_in, sem_w):
    def head_copies(j, slot):
        return [pltpu.make_async_copy(src.bitcast(U32).at[:, j, :], dst.at[slot], sem_w.at[3 * slot + n])
                for n, (src, dst) in enumerate(((wuk_hbm, wk_raw), (wuv_hbm, wv_raw), (wq_hbm, wq_raw)))]

    def side_copies(j, slot):
        wob = wob_hbm.at[pl.ds(4 * (j >> 1), 4), pl.ds(_aligned((j & 1) * 64, 64), 64), :]
        wqkv = wqkv_hbm.bitcast(U32).at[:, pl.ds(_aligned(8 * j, 8), 8), :]
        return [pltpu.make_async_copy(wob, wob_raw.at[slot], sem_w.at[6 + 2 * slot]),
                pltpu.make_async_copy(wqkv, wqkv_raw.at[slot], sem_w.at[7 + 2 * slot])]

    def wo_copy(word):
        return pltpu.make_async_copy(wo_hbm.bitcast(U32).at[:, word, :], wo_raw.at[word], sem_w.at[10])

    def c_copy(c):
        rows = pl.ds(c * CH, CH)
        return pltpu.make_async_copy(c_hbm.at[rows, :], c_raw.at[rows, :], sem_in.at[2 * c])

    def x_copy(c):
        rows = pl.ds(c * CH, CH)
        return pltpu.make_async_copy(bx_hbm.at[rows, :], bx_raw.at[rows, :], sem_in.at[2 * c + 1])

    def pair_body(j, first=False):
        slot = j & 1
        tok = _Tokens(zero_smem)
        causal = (lax.broadcasted_iota(jnp.int32, (T, T), 1)
                  <= lax.broadcasted_iota(jnp.int32, (T, T), 0))

        jobs, due, pace = [], [], dict(release=None, recent=None)

        def queue(cycles, more, q=1.0, kv=1.0, attention=1.0):
            pace.update(period=cycles / len(more), clock=0, q=q, kv=kv, attention=attention)
            jobs.extend(more)

        def flush():
            while jobs:
                jobs.pop(0)()

        def background(cycles, share, delay, recent=None):
            pace["clock"] += cycles * share
            token = None
            while jobs and pace["clock"] >= pace["period"]:
                pace["clock"] -= pace["period"]
                pace["release"] = None if recent is None else tok.of(recent[:8])
                new = jobs.pop(0)()
                pace["release"] = None
                token = new if token is None else token | new
            if token is not None:
                due.append([delay, token])
            for entry in due:
                entry[0] -= cycles
            now = [token for left, token in due if left <= 0]
            due[:] = [entry for entry in due if entry[0] > 0]
            return functools.reduce(jnp.bitwise_or, now) if now else None

        def released(x):
            return _after(pace["release"], x, everywhere=True)

        def store_terms(dst, first_term, lead, row, terms):
            for i, val in enumerate(terms):
                dst[(first_term + i, *lead, _rows(row, 16), slice(None))] = val.astype(BF16)
            return tok.stored(dst, (first_term + 6, *lead), row)

        def job_x(c, i, n, r):
            terms = _terms2(RHS, i, lambda row, col: bx_raw[
                pl.ds(c * CH + (col ^ 2) * T + r, 16), pl.ds((2 * row + n) * T, T)].astype(F32))
            return store_terms(bx_t, 7 * i, (n,), c * T + r, terms)

        def job_c(c, i, r):
            terms = _terms2(LHS, i, lambda row, col: c_raw[
                pl.ds(c * CH + row * T + r, 16), pl.ds(col * T, T)].astype(F32))
            return store_terms(c_t, 7 * i, (), c * T + r, terms)

        def jobs_x(c):
            return [P(job_x, c, i, n, r) for r in range(0, T, 16) for n in range(2) for i in range(7)]

        def jobs_c(c):
            return [P(job_c, c, i, r) for r in range(0, T, 16) for i in range(7)]

        def job_wkv(src, i, r):
            def block(row, col):
                raw = (wk_raw, wv_raw)[col % 2]
                return _split(released(raw[src, pl.ds(row * T + r, 16), :]))[col // 2]
            return store_terms(wkv_t, 7 * i, (), r, _terms2(RHS, i, block))

        def job_turn(src, n):
            words = released(wq_raw[src, pl.ds(n * T, T), :])
            wq_turned[n] = pltpu.bitcast(pltpu.bitcast(words, F32).T, U32)
            return tok.stored(wq_turned, (n,), T - 16)

        def job_wq(i, n, r):
            def block(row, col):
                return _split(released(wq_turned[2 * col + n, pl.ds((row % 2) * RO + r, 16), :]))[row // 2]
            return store_terms(wq_t, 7 * i, (n,), r, _terms2(LHS, i, block))

        def jobs_wkv(src):
            return [P(job_wkv, src, i, r) for r in range(0, T, 16) for i in range(7)]

        def jobs_wq(src):
            return ([P(job_turn, src, n) for n in range(DM // T)],
                    [P(job_wq, i, n, r) for n in range(2) for r in range(0, RO, 16) for i in range(7)])

        def job_wob(i, n, r):
            def block(row, col):
                head = 2 * (row % 2) + row // 2
                return released(wob_raw[slot, head, pl.ds(r, 16), pl.ds((2 * col + n) * T, T)].astype(F32))
            return store_terms(wob_t, 7 * i, (n,), j * 64 + r, _terms2(RHS, i, block))

        def job_wo(i, n):
            e, odd, head = j & 3, (j >> 2) & 1, 16 * (j >> 3)

            def block(row, col):
                even_t, odd_t = _split(released(
                    wo_raw[4 * e + row, _rows(head, 16), pl.ds((2 * col + n) * T, T)]))
                return jnp.where(odd == 1, odd_t, even_t)
            return store_terms(wo_t, 7 * i, (n,), odd * T + e * NH + head, _terms2(RHS, i, block))

        permuted = {}

        def job_permute(mat):
            lane = lax.broadcasted_iota(jnp.int32, (32, T), 1)
            e, grp, sub = lane >> 5, (lane >> 2) & 7, lane & 3

            def gather(x, index):
                return jnp.take_along_axis(x, index, axis=1, mode="promise_in_bounds")
            x = [released(wqkv_raw[slot, :, :, pl.ds(mat * DM + t * T, T)].reshape(32, T))
                 for t in range(8)]
            y = [gather(x[t], sub * 32 + e * 8 + ((grp - t) & 7)) for t in range(8)]
            u = [y[-s % 8] for s in range(8)]
            for bit in (1, 2, 4):
                u = [jnp.where((grp & bit) != 0, u[(s - bit) % 8], u[s]) for s in range(8)]
            u = [u[0]] + [gather(u[t], e * 32 + ((grp + t) & 7) * 4 + sub) for t in range(1, 8)]
            permuted[mat] = u
            return _fold(jnp.bitwise_or, functools.reduce(jnp.bitwise_or, u)) & tok.zero

        def column(mat, row, t):
            return pltpu.bitcast(released(permuted[mat][t][8 * row:8 * row + 8]), BF16).astype(F32)

        def job_wa(mat, i, n):
            terms = _terms2(RHS, i, lambda row, col: column(mat, row, 2 * col + n))
            return store_terms(wa_t, 7 * i, (2 * mat + n,), 16 * j, terms)

        pause = [P(lambda: tok.zero)] * 2
        jobs_wob = [P(job_wob, i, n, r) for r in range(0, 64, 16) for n in range(2) for i in range(7)]
        jobs_wo = [P(job_wo, i, n) for n in range(2) for i in range(7)]
        jobs_wa = []
        for mat in range(3):
            jobs_wa += [P(job_permute, mat)] + pause
            jobs_wa += [P(job_wa, mat, i, n) for n in range(2) for i in range(7)]

        q, k, v = {}, {}, {}

        def product(dot, share, left, right):
            token = background(left.shape[0] // 2, share, JOB_CYCLES, pace["recent"])
            pace["recent"] = dot(pltpu.bitcast(_after(token, left), BF16), right)
            return pace["recent"]

        def project_q(c):
            inner = []
            for first_product in range(0, 49, 7):
                inner.append(_combine([_sum([
                    product(_dot_nt, pace["q"], _words(wq_t, (i, n), 0, RO), _load(bx_t, (i, n), c * T, T))
                    for n in range(2)]) for i in range(first_product, first_product + 7)]))
                if len(inner) <= 4:
                    due.append([400, tok.of(*[x[RO - 8:] for x in inner[-1]])])
            blocks = _combine_outer(inner)
            for h in range(2):
                for col in range(4):
                    val = _cat([blocks[2 * h, col], blocks[2 * h + 1, col]], axis=0) * SCALE_B
                    q[4 * c + (col ^ 2), h] = val.T.astype(BF16)

        def project_kv(c):
            m = [product(_dot, pace["kv"], _words(c_t, (i,), c * T, T), _load(wkv_t, (i,), 0, T))
                 for i in range(49)]
            for (row, col), val in sorted(_combine_outer([_combine(m[i:i + 7]) for i in range(0, 49, 7)]).items()):
                (k, v)[col % 2][4 * c + row, col // 2] = val.astype(BF16)

        def plain(raw, c, weights):
            def part(r, col):
                left = raw[pl.ds(c * CH + r, 32), pl.ds(col, 4 * T)]
                token = background(32, 1.0, 128)
                if token is None:
                    return left
                return _cat([_after(_cat([token, token]), left[:, :2 * T]), left[:, 2 * T:]])
            return [_dot(_cat([_cat([part(r, col) for r in range(0, CH, 32)], axis=0)
                               for col in range(0, raw.shape[1], 4 * T)]), w) for w in weights]

        def plain_kv(c, weights):
            for n, val in enumerate(plain(c_raw, c, weights)):
                for r in range(4):
                    (k, v)[n // 2][4 * c + r, n % 2] = val[r * T:(r + 1) * T].astype(BF16)

        def plain_q(c, weights):
            for h, val in enumerate(plain(bx_raw, c, weights)):
                for r in range(4):
                    q[4 * c + r, h] = (val[r * T:(r + 1) * T] * SCALE_B).astype(BF16)

        in_flight, partial, ctx, spread, checks = [], {}, {}, {}, []

        def finish(i, h):
            l, o = partial.pop((i, h))
            l = jnp.sum(l, axis=1, keepdims=True)
            r = _inverse(l)
            ctx[i, h] = o * r
            spread[i, h] = _fold(jnp.maximum, jnp.broadcast_to(l + r, (T, T)))
            b = i // 2
            quad = [(2 * b, 0), (2 * b, 1), (2 * b + 1, 0), (2 * b + 1, 1)]
            if all(u in ctx for u in quad):
                terms = _terms(LHS, lambda m: ctx.pop(quad[m]))
                for n, val in enumerate(terms):
                    ctx_t[n, j, pl.ds(b * T, T), :] = val.astype(BF16)
                checks.append((_fold(jnp.add, terms[0] + terms[5] + terms[6]),
                               functools.reduce(jnp.maximum, [spread.pop(u) for u in quad])))
                due.append([CTX_CYCLES[first], tok.stored(ctx_t, (6, j), b * T) | tok.of(*checks[-1])])

        def weigh(i, h, t, p):
            l, o = partial.get((i, h), (None, None))
            l = p if l is None else l + p
            d = _dot(_after(background(64, pace["attention"], JOB_CYCLES, p), p).astype(BF16), v[t, h])
            partial[i, h] = (l, d if o is None else o + d)
            if t == i:
                finish(i, h)

        def attention(lo, hi):
            for i in range(lo, hi):
                for h in range(2):
                    for t in range(i + 1):
                        s = _dot_nt(q[i, h], k[t, h])
                        if t == i:
                            s = jnp.where(causal, s, MASKED)
                        in_flight.append((i, h, t, jnp.exp2(s)))
                        ahead = (i, h) == (S // T - 1, 1) and 8 <= t < 13 and not first
                        if len(in_flight) > DEPTH and not ahead:
                            weigh(*in_flight.pop(0))
            while hi == S // T and in_flight:
                weigh(*in_flight.pop(0))

        def cycles(lo, hi):
            return 2 * 64 * sum(range(lo + 1, hi + 1))

        if first:
            wk, wv, wq = head_copies(0, 0)
            _start(wv, wk, c_copy(0), c_copy(1))
            _wait(wv, wk, c_copy(0))
            _start(c_copy(2), c_copy(3), wq, x_copy(0))
            weights = [w.astype(BF16) for raw in (wk_raw, wv_raw) for w in _split(raw[0])]
            queue(0.98 * 2048, jobs_c(0)[:49])
            plain_kv(0, weights)
            flush()
            _wait(c_copy(1), c_copy(2))
            _start(x_copy(1), x_copy(2))
            queue(0.92 * 4096, jobs_c(0)[49:] + jobs_c(1) + jobs_c(2))
            plain_kv(1, weights)
            plain_kv(2, weights)
            flush()
            _wait(c_copy(3), wq)
            turn, terms = jobs_wq(0)
            queue(0.9 * 2048, _interleave(turn, jobs_c(3)))
            plain_kv(3, weights)
            flush()
            _wait(x_copy(0))
            weights = [w.astype(BF16) for w in _split(wq_raw[0])]
            queue(0.9 * (2048 + 0.2 * cycles(0, 4)), jobs_x(0)[:96], attention=0.2)
            plain_q(0, weights)
            attention(0, 4)
            flush()
            _wait(x_copy(1), x_copy(2))
            stage = [*side_copies(0, 0), *head_copies(1, 1)]
            _start(x_copy(3), *stage)
            lax.fori_loop(0, 16, lambda word, carry: wo_copy(word).start(), None)
            queue(0.98 * (2048 + 0.5 * cycles(4, 7)),
                  jobs_x(2) + terms + jobs_x(0)[96:] + jobs_x(1)[:14], attention=0.5)
            plain_q(1, weights)
            attention(4, 7)
            flush()
            _wait(x_copy(3))
            queue(0.85 * (1568 + cycles(7, 10)), jobs_x(3))
            project_q(2)
            attention(7, 10)
            flush()
            _wait(*stage)
            _start(ax_copy(0, 0), *head_copies(2, 0), *side_copies(1, 1))
            turn, terms = jobs_wq(1)
            queue(0.88 * (1568 + cycles(10, 14)), _interleave(
                _interleave(jobs_wob, jobs_wa), _interleave(jobs_x(1)[14:], _interleave(turn, jobs_wkv(1)))))
            attention(10, 11)
            project_q(3)
            attention(11, 14)
            flush()
            _wait(*[wo_copy(word) for word in range(16)], ax_copy(0, 0))
            _start(ax_copy(1, 1))
            queue(0.92 * cycles(14, 16), _interleave(
                jobs_wo + terms, [P(_job_ax, tok, released, ax_raw, ax_t, 0, *job) for job in AX_JOBS]))
            attention(14, 16)
            flush()
        else:
            queue(0.98 * 4 * 1568 * (0.5 + 0.3), _interleave(jobs_wob, jobs_wo + jobs_wa),
                  q=0.5, kv=0.3, attention=0)
            project_kv(0)
            project_q(0)
            project_kv(1)
            attention(0, 3)
            project_q(1)
            attention(3, 7)
            project_q(2)
            project_kv(2)
            attention(7, 10)
            project_q(3)
            project_kv(3)
            attention(10, 12)
            flush()
            turn, terms = jobs_wq(1 - slot)
            queue(0.95 * cycles(12, 16), _interleave(jobs_wkv(1 - slot), turn + pause + terms))
            attention(12, 16)
            flush()
        guard[0] = _sum([guard[0]] + [x for x, _ in checks])
        guard[1] = functools.reduce(jnp.maximum, [guard[1]] + [x for _, x in checks])

        def ahead(n):
            return j + n if first else jnp.minimum(j + n, NP - 1)
        _wait(*head_copies(ahead(2), slot), *side_copies(ahead(1), 1 - slot))

        @pl.when(j < NP - 1)
        def _():
            _start(*head_copies(ahead(3), 1 - slot), *side_copies(ahead(2), slot))

    def exact_pairs(ctx):
        def block(i):
            return pl.ds(pl.multiple_of(i * T, T), T)

        def qkv(n, h, i):
            return c_t.at[(2 * n + h) * 4 + (i >> 2), block(i & 3), :]

        def project(x, carry):
            h, i = x & 1, x >> 1

            def weight(raw):
                even, odd = _split(raw[0])
                return jnp.where(h == 0, even, odd).astype(BF16)
            qkv(0, h, i)[...] = (_dot(bx_raw[block(i), :], weight(wq_raw)) * SCALE_B).astype(BF16)
            qkv(1, h, i)[...] = _dot(c_raw[block(i), :], weight(wk_raw)).astype(BF16)
            qkv(2, h, i)[...] = _dot(c_raw[block(i), :], weight(wv_raw)).astype(BF16)

        def attend(b, x, carry):
            h, i = x & 1, 2 * b + (x >> 1)

            def scores(t):
                row = lax.broadcasted_iota(jnp.int32, (T, T), 0) + i * T
                col = lax.broadcasted_iota(jnp.int32, (T, T), 1) + t * T
                return jnp.where(col <= row, _dot_nt(qkv(0, h, i)[...], qkv(1, h, t)[...]), MASKED)

            m = lax.fori_loop(
                0, i + 1, lambda t, m: jnp.maximum(m, jnp.max(scores(t), axis=1, keepdims=True)),
                jnp.full((T, 1), -jnp.inf, F32))

            def accumulate(t, carry):
                l, o = carry
                p = jnp.exp2(scores(t) - m)
                return (l + jnp.sum(p, axis=1, keepdims=True),
                        o + _dot(p.astype(BF16), qkv(2, h, t)[...]))
            l, o = lax.fori_loop(0, i + 1, accumulate,
                                 (jnp.zeros((T, 1), F32), jnp.zeros((T, T), F32)))
            ctx[x] = o / l

        def pair(j, carry):
            _start(*head_copies(j, 0))
            _wait(*head_copies(j, 0))
            lax.fori_loop(0, 2 * S // T, project, None)

            def rows(b, carry):
                lax.fori_loop(0, 4, P(attend, b), None)
                for n, val in enumerate(_terms(LHS, lambda m: ctx[m])):
                    ctx_t[n, j, block(b), :] = val.astype(BF16)
            lax.fori_loop(0, S // T // 2, rows, None)

        lax.fori_loop(0, NP, pair, None)

    guard[...] = jnp.zeros(guard.shape, F32)
    pair_body(0, first=True)
    lax.fori_loop(1, NP, lambda j, carry: pair_body(j), None)

    safe = jnp.logical_and(jnp.abs(guard[0]) < jnp.inf, guard[1] < SAFE_SUM)

    @pl.when(jnp.max(jnp.where(safe, 0.0, 1.0)) > 0.0)
    def _():
        pl.run_scoped(exact_pairs, pltpu.VMEM((4, T, T), F32))


def _outputs(out_hbm, ax_copy, ax_raw, ax_t, ctx_t, wob_t, wa_t, wo_t, zero_smem,
             o_t, kbuf, vbuf, qbuf, acc, obuf, sem_out):
    def out_copy(c, slot):
        rows = pl.ds(_aligned(c * CO, CO), CO)
        return pltpu.make_async_copy(obuf.at[slot], out_hbm.at[rows, :], sem_out.at[slot])

    for buf in (kbuf, vbuf):
        for t in range(8):
            buf[t, pl.ds(CO, HALO), :] = jnp.zeros((HALO, T), F32)

    t_q = 2 * 49 * RO
    t_v = t_q + 21 * 4 * RO + 49 * RO
    t_o = t_v + (21 + EARLY_B) * 4 * RO

    def chunk_body(c, carry):
        slot = c & 1
        tok = _Tokens(zero_smem)
        plan, due, clock = {}, {}, [0]

        def schedule(job, begin, end, release=False):
            plan.setdefault(max(clock[0], begin // TICK), []).append((job, -(-end // TICK), release))

        def step(results, a, w):
            res = [None] * len(w)
            for x, left in enumerate(a):
                n = clock[0]
                clock[0] += 1
                if n in due:
                    left = _after(functools.reduce(jnp.bitwise_or, due.pop(n)), left)
                left = left.astype(BF16) if left.dtype == F32 else pltpu.bitcast(left, BF16)
                for y in range(len(w)):
                    d = _dot(left, w[y](x))
                    res[y] = d if res[y] is None else res[y] + d
                token = None
                for job, last, release in plan.pop(n, []):
                    if release and token is None:
                        token = tok.of(d[:8])
                    due.setdefault(max(last, n + 1), []).append(job(token) if release else job())
            results.append(res)

        def project(lhs_t, rhs_t, tile0, write):
            inner = {}

            def combine(i, y, m):
                inner[i, y] = _combine([x[y] for x in m])
                return tok.of(*[x[r + 8:r + 16] for x in inner[i, y] for r in range(0, RO, 16)])

            def finish(outer, y, r):
                vals = [_term(SUMS, outer, lambda i: inner[i, y][n][r:r + 16]) for n in range(4)]
                for n, val in enumerate(vals):
                    row, col = _block(outer, n)
                    write(row * RO + r, 2 * col + y, val)
                return tok.of(*[x[8:] for x in vals])

            for i in range(7):
                m = []
                done = clock[0] * TICK + 7 * RO
                for y in range(2):
                    schedule(P(combine, i, y, m), done, done + 400)
                for outer in FINAL[i]:
                    slabs = [(y, r) for r in range(0, RO, 16) for y in range(2)]
                    for x, slab in enumerate(slabs):
                        schedule(P(finish, outer, *slab), done, done + 300 + 40 * (x + 1))
                for n in range(7 * i, 7 * i + 7):
                    step(m, [_words(lhs_t, (n, x), 0, RO) for x in range(2)],
                         [P(lambda y, x: _load(rhs_t, (n, tile0 + y), x * T, T), y) for y in range(2)])

        for buf in (kbuf, vbuf):
            for t in range(8):
                buf[t, pl.ds(0, HALO), :] = buf[t, pl.ds(CO, HALO), :]

        def write_rows(buf, row, t, val):
            buf[t, pl.ds(HALO + row, 16), :] = val

        def write_q(row, t, val):
            qbuf[t, pl.ds(row, 16), :] = val * SCALE_A

        project(ax_t, wa_t, 2, P(write_rows, kbuf))
        project(ax_t, wa_t, 0, write_q)

        att = {}

        def job_weights(row, r, release):
            base = HALO + row * RO + r
            qs = [_after(release, qbuf[t, pl.ds(row * RO + r, 8), :]) for t in range(8)]
            logits = []
            for w in range(WIN):
                x = _sum([qs[t] * kbuf[t, pl.ds(base - DIL * w, 8), :] for t in range(8)])
                x = x + pltpu.roll(x, 64, 1)
                x = x + pltpu.roll(x, 32, 1)
                if row == 0 and r < DIL * w:
                    pos = lax.broadcasted_iota(jnp.int32, (8, T), 0) + (c * CO + r)
                    x = jnp.where(pos >= DIL * w, x, MASKED)
                logits.append(x)
            m = functools.reduce(jnp.maximum, logits)
            p = [jnp.exp2(x - m) for x in logits]
            inv = _inverse(_sum(p))
            att[row, r] = [x * inv for x in p]
            return tok.of(att[row, r][0])

        def job_values(row, r, release):
            base = HALO + row * RO + r
            p = [_after(release, x) for x in att[row, r]]
            att[row, r] = [_sum([p[w] * vbuf[t, pl.ds(base - DIL * w, 8), :] for w in range(WIN)])
                           for t in range(8)]
            return tok.of(att[row, r][-1])

        def job_o(n, r, i):
            def block(row, col):
                return _cat([att[row, r][2 * col + n], att[row, r + 8][2 * col + n]], axis=0)
            for x, val in enumerate(_terms2(LHS, i, block)):
                o_t[7 * i + x, n, pl.ds(r, 16), :] = val.astype(BF16)
            return tok.stored(o_t, (7 * i + 6, n), r)

        groups = [(row, r + x) for r in range(0, RO, 16) for row in (2, 0, 3, 1) for x in (0, 8)]
        w0, w1, v0, v1 = t_q + 1000, t_v - 1400, t_v + 400, t_o - 700
        for g, (row, r) in enumerate(groups):
            begin = w0 + (w1 - w0) * g // len(groups)
            schedule(P(job_weights, row, r), begin, begin + 500, release=True)
            begin = v0 + (v1 - v0) * g // len(groups)
            schedule(P(job_values, row, r), begin, begin + 600, release=True)
            if g % 8 == 7:
                for x, (n, i) in enumerate((n, i) for n in range(2) for i in range(7)):
                    schedule(P(job_o, n, r - 8, i), begin, min(begin + 400 + 60 * (x + 1), t_o))

        touched = {}

        def project_b(i):
            m = []

            def accumulate(y, inner):
                val = _combine([x[y] for x in m])[inner]
                token = None
                for outer, sign in OUT[i]:
                    row, col = _block(outer, inner)
                    rows, col = pl.ds(row * RO, RO), 2 * col + y
                    total = val
                    if (outer, inner, y) in touched:
                        total = acc[col, rows, :] + val if sign > 0 else acc[col, rows, :] - val
                    touched[outer, inner, y] = True
                    if outer not in FINAL[i]:
                        acc[col, rows, :] = total
                        token = tok.stored(acc, (col,), row * RO)
                    else:
                        obuf[slot, rows, pl.ds(DM + col * T, T)] = total.astype(BF16)
                        if token is None:
                            token = tok.of(_fold(jnp.add, total))
                return token

            parts = [(y, inner) for y in range(2) for inner in range(4)]
            done = clock[0] * TICK + 7 * 4 * RO
            if i < 6:
                for x, part in enumerate(parts):
                    schedule(P(accumulate, *part), done, done + 256 + 200 * x)
            for n in range(7):
                if i == 6 and n == EARLY_B:
                    yield

                def quad(kt, x):
                    return (i, 2 * kt + x % 2), (2 * c + x // 2) * RO
                if len(LHS[n]) == 1:
                    a = [_words(ctx_t, *quad(kt, LHS[n][0][0]), RO) for kt in range(8)]
                else:
                    a = [_term(LHS, n, lambda x: _load(ctx_t, (i + tok.z * n, 2 * kt + x % 2), quad(kt, x)[1], RO).astype(F32))
                         for kt in range(8)]
                step(m, a, [P(lambda y, x: _load(wob_t, (7 * i + n, y), x * T, T), y) for y in range(2)])
            if i == 6:
                for part in parts:
                    accumulate(*part)

        for i in range(6):
            if i == 3:
                project(ax_t, wa_t, 4, P(write_rows, vbuf))
            list(project_b(i))
        last_b = project_b(6)
        next(last_b)

        for x, job in enumerate(AX_JOBS):
            schedule(P(_job_ax, tok, lambda val: val, ax_raw, ax_t, 1 - slot, *job),
                     t_o, t_o + 100 + 3000 * (x + 1) // len(AX_JOBS))

        def write_out(row, t, val):
            obuf[slot, pl.ds(row, 16), pl.ds(t * T, T)] = val.astype(BF16)

        project(o_t, wo_t, 0, write_out)
        list(last_b)
        assert not plan and not due
        out_copy(c, slot).start()
        ax_copy(jnp.minimum(c + 2, NO - 1), slot).wait()

        @pl.when(c < NO - 1)
        def _():
            ax_copy(jnp.minimum(c + 3, NO - 1), 1 - slot).start()

        @pl.when(c >= 1)
        def _():
            out_copy(c - 1, 1 - slot).wait()

    ax_copy(1, 1).wait()
    ax_copy(2, 0).start()
    lax.fori_loop(0, NO, chunk_body, None)
    out_copy(NO - 1, (NO - 1) % 2).wait()


def _kernel(ax_hbm, wqkv_hbm, wo_hbm, bx_hbm, c_hbm, wq_hbm, wuk_hbm, wuv_hbm, wob_hbm, out_hbm,
            ax_raw, ax_t, ctx_t, wob_t, wa_t, wo_t, zero_smem, sem_ax):
    vmem, dma = pltpu.VMEM, pltpu.SemaphoreType.DMA

    def clear(i, carry):
        zero_smem[0] = i >> 1
    lax.fori_loop(0, 2, clear, None)

    def ax_copy(c, slot):
        rows = pl.ds(_aligned(c * CO, CO), CO)
        return pltpu.make_async_copy(ax_hbm.at[rows, :], ax_raw.at[slot], sem_ax.at[slot])

    shared = (ax_copy, ax_raw, ax_t, ctx_t, wob_t, wa_t, wo_t, zero_smem)
    pl.run_scoped(
        P(_head_pairs, wqkv_hbm, wo_hbm, bx_hbm, c_hbm, wq_hbm, wuk_hbm, wuv_hbm, wob_hbm, *shared),
        vmem((S, DM), BF16),
        vmem((S, DC), BF16),
        vmem((2, DM, T), U32),
        vmem((2, DC, T), U32),
        vmem((2, DC, T), U32),
        vmem((2, 4, 64, DM), BF16),
        vmem((2, 4, 8, 3 * DM), U32),
        vmem((16, NH, DM), U32),
        vmem((49, 2, S // 4, T), BF16),
        vmem((49, S // 4, T), BF16),
        vmem((DM // T, T, T), U32),
        vmem((49, 2, RO, T), BF16),
        vmem((49, T, T), BF16),
        vmem((2, 8, T), F32),
        dma((2 * S // CH,)), dma((11,)))
    pl.run_scoped(
        P(_outputs, out_hbm, *shared),
        vmem((49, 2, RO, T), BF16),
        vmem((8, HALO + CO, T), F32),
        vmem((8, HALO + CO, T), F32),
        vmem((8, CO, T), F32),
        vmem((8, CO, T), F32),
        vmem((2, CO, 2 * DM), BF16),
        dma((2,)))


@jax.jit
def pallas_concat_heads__sliding_local_dilated__compressed_kv_cla__prompt_kernel(
    A_x: jax.Array,
    A_wqkv: jax.Array,
    A_wo: jax.Array,
    B_x: jax.Array,
    B_c_kv: jax.Array,
    B_w_q: jax.Array,
    B_w_uk: jax.Array,
    B_w_uv: jax.Array,
    B_w_o: jax.Array,
):
    vmem = pltpu.VMEM
    out = pl.pallas_call(
        _kernel,
        out_shape=jax.ShapeDtypeStruct((S, 2 * DM), BF16),
        in_specs=[pl.BlockSpec(memory_space=pl.ANY)] * 9,
        out_specs=pl.BlockSpec(memory_space=pl.ANY),
        scratch_shapes=[
            vmem((2, CO, DM), BF16),
            vmem((49, 2, RO, T), BF16),
            vmem((7, NP, S // 2, T), BF16),
            vmem((49, 2, DM, T), BF16),
            vmem((49, 6, 2 * T, T), BF16),
            vmem((49, 2, 2 * T, T), BF16),
            pltpu.SMEM((1,), jnp.int32),
            pltpu.SemaphoreType.DMA((2,)),
        ],
        compiler_params=pltpu.CompilerParams(
            vmem_limit_bytes=127 * 2**20, disable_bounds_checks=True),
    )(
        A_x.reshape(S, DM),
        A_wqkv.reshape(4, DM // 4, 3 * DM),
        A_wo.reshape(NH, DM // NH, DM),
        B_x.reshape(S, DM),
        B_c_kv.reshape(S, DC),
        B_w_q,
        B_w_uk,
        B_w_uv,
        B_w_o,
    )
    return out.reshape(1, S, 2 * DM)
```

```python
import functools
import math

import jax
import jax.numpy as jnp
from jax import lax
import jax.experimental.pallas as pl
import jax.experimental.pallas.tpu as pltpu

S = 2048
DM = 1024
DC = 512
NH = 32
NP = NH // 2
T = 128
CH = 4 * T
RO = 64
CO = 4 * RO
NO = S // CO
WIN, DIL = 8, 2
HALO = 16

LOG2E = math.log2(math.e)
SCALE_A = (DM // NH) ** -0.5 * LOG2E
SCALE_B = T ** -0.5 * LOG2E
MASKED = -1e9 * LOG2E
SAFE_SUM = 2.0 ** 40

DEPTH = 3
JOB_CYCLES = 896
CTX_CYCLES = 1024, 768

NX0, NX3 = 49, 84
TICK = RO // 2
EARLY_B = 4
F32, BF16, U32 = jnp.float32, jnp.bfloat16, jnp.uint32
P = functools.partial


def _dot(a, b):
    return jnp.dot(a, b, preferred_element_type=F32)


def _dot_nt(a, b):
    return lax.dot_general(a, b, (((1,), (1,)), ((), ())), preferred_element_type=F32)


def _cat(xs, axis=1):
    return xs[0] if len(xs) == 1 else jnp.concatenate(xs, axis=axis)


def _sum(xs):
    return functools.reduce(jnp.add, xs)


def _fold(op, x):
    return functools.reduce(op, [x[r:r + 8] for r in range(0, x.shape[0], 8)])


def _aligned(x, n):
    return x if isinstance(x, int) else pl.multiple_of(x, n)


def _rows(start, n):
    return pl.ds(_aligned(start, 16), n)


def _words(ref, lead, start, n):
    return ref.bitcast(U32)[(*lead, pl.ds(_aligned(start >> 1, 8), n // 2), slice(None))]


def _load(ref, lead, start, n):
    return pltpu.bitcast(_words(ref, lead, start, n), BF16)


def _split(w):
    return (pltpu.bitcast(w << 16, F32), pltpu.bitcast(w & jnp.uint32(0xFFFF0000), F32))


def _inverse(l):
    r = pl.reciprocal(l, approx=True)
    return r * (2.0 - l * r)


def _interleave(x, y):
    order = [((n + 0.5) / len(z), m, job) for m, z in enumerate((x, y)) for n, job in enumerate(z)]
    return [job for _, _, job in sorted(order, key=lambda e: e[:2])]


def _start(*copies):
    for cp in copies:
        cp.start()


def _wait(*copies):
    for cp in copies:
        cp.wait()


LHS = (((0, 1), (3, 1)), ((2, 1), (3, 1)), ((0, 1),), ((3, 1),),
       ((0, 1), (1, 1)), ((2, 1), (0, -1)), ((1, 1), (3, -1)))
RHS = (((0, 1), (3, 1)), ((0, 1),), ((1, 1), (3, -1)), ((2, 1), (0, -1)),
       ((3, 1),), ((0, 1), (1, 1)), ((2, 1), (3, 1)))
OUT = (((0, 1), (3, 1)), ((2, 1), (3, -1)), ((1, 1), (3, 1)), ((0, 1), (2, 1)),
       ((0, -1), (1, 1)), ((3, 1),), ((0, 1),))
SUMS = tuple(tuple((i, sign) for i in range(7) for m, sign in OUT[i] if m == n) for n in range(4))
FINAL = tuple(tuple(n for n in range(4) if SUMS[n][-1][0] == i) for i in range(7))


def _term(table, i, quad):
    (n, _), *rest = table[i]
    val = quad(n)
    for n, sign in rest:
        val = val + quad(n) if sign > 0 else val - quad(n)
    return val


def _terms(table, quad):
    blocks = [quad(n) for n in range(4)]
    return [_term(table, i, blocks.__getitem__) for i in range(7)]


def _block(outer, inner):
    return 2 * (outer // 2) + inner // 2, 2 * (outer % 2) + inner % 2


def _terms2(table, i, block):
    return _terms(table, lambda n: _term(table, i, lambda m: block(*_block(m, n))))


def _combine(m):
    return [_term(SUMS, n, m.__getitem__) for n in range(4)]


def _combine_outer(inner):
    return {_block(outer, n): val for n in range(4)
            for outer, val in enumerate(_combine([x[n] for x in inner]))}


class _Tokens:
    def __init__(self, zero_smem):
        self.z = zero_smem[0]
        self.zero = jnp.full((8, T), self.z, jnp.int32).astype(U32)

    def stored(self, ref, lead, start):
        first, *rest = lead
        if ref.dtype == BF16:
            return _words(ref, (first - (self.z & 1), *rest), start, 16) & self.zero
        return self.of(ref[(*lead, pl.ds(_aligned(start + 8 * (self.z & 1), 8), 8), slice(None))])

    def of(self, *vals):
        return pltpu.bitcast(_sum(vals), U32) & self.zero


def _after(token, x, everywhere=False):
    if token is None:
        return x
    bits = x if x.dtype == U32 else pltpu.bitcast(x, U32)
    cut = bits.shape[0] if everywhere else 8
    parts = [bits[r:r + 8] | token for r in range(0, cut, 8)]
    bits = _cat(parts + ([bits[cut:]] if cut < bits.shape[0] else []), axis=0)
    return bits if x.dtype == U32 else pltpu.bitcast(bits, x.dtype)


AX_JOBS = [(i, n, r) for n in range(2) for r in range(0, RO, 16) for i in range(7)]


def _job_ax(tok, released, ax_raw, ax_t, src, i, n, r):
    terms = _terms2(LHS, i, lambda row, col: released(
        ax_raw[src, pl.ds(row * RO + r, 16), pl.ds((2 * col + n) * T, T)].astype(F32)))
    for x, val in enumerate(terms):
        ax_t[7 * i + x, n, pl.ds(r, 16), :] = val.astype(BF16)
    return tok.stored(ax_t, (7 * i + 6, n), r)


def _head_pairs(wqkv_hbm, wo_hbm, bx_hbm, c_hbm, wq_hbm, wuk_hbm, wuv_hbm, wob_hbm,
                ax_copy, ax_raw, ax_t, ctx_t, wob_t, wa_t, wo_t, zero_smem,
                bx_raw, c_raw, wq_raw, wk_raw, wv_raw, wob_raw, wqkv_raw, wo_raw,
                bx_t, c_t, wq_turned, wq_t, wkv_t, guard, sem_in, sem_w):
    def head_copies(j, slot):
        return [pltpu.make_async_copy(src.bitcast(U32).at[:, j, :], dst.at[slot], sem_w.at[3 * slot + n])
                for n, (src, dst) in enumerate(((wuk_hbm, wk_raw), (wuv_hbm, wv_raw), (wq_hbm, wq_raw)))]

    def side_copies(j, slot):
        wob = wob_hbm.at[pl.ds(4 * (j >> 1), 4), pl.ds(_aligned((j & 1) * 64, 64), 64), :]
        wqkv = wqkv_hbm.bitcast(U32).at[:, pl.ds(_aligned(8 * j, 8), 8), :]
        return [pltpu.make_async_copy(wob, wob_raw.at[slot], sem_w.at[6 + 2 * slot]),
                pltpu.make_async_copy(wqkv, wqkv_raw.at[slot], sem_w.at[7 + 2 * slot])]

    def wo_copy(word):
        return pltpu.make_async_copy(wo_hbm.bitcast(U32).at[:, word, :], wo_raw.at[word], sem_w.at[10])

    def c_copy(c):
        rows = pl.ds(c * CH, CH)
        return pltpu.make_async_copy(c_hbm.at[rows, :], c_raw.at[rows, :], sem_in.at[2 * c])

    def x_copy(c):
        rows = pl.ds(c * CH, CH)
        return pltpu.make_async_copy(bx_hbm.at[rows, :], bx_raw.at[rows, :], sem_in.at[2 * c + 1])

    def pair_body(j, first=False):
        slot = j & 1
        tok = _Tokens(zero_smem)
        causal = (lax.broadcasted_iota(jnp.int32, (T, T), 1)
                  <= lax.broadcasted_iota(jnp.int32, (T, T), 0))

        jobs, due, pace = [], [], dict(release=None, recent=None)

        def queue(cycles, more, q=1.0, kv=1.0, attention=1.0):
            pace.update(period=cycles / len(more), clock=0, q=q, kv=kv, attention=attention)
            jobs.extend(more)

        def flush():
            while jobs:
                jobs.pop(0)()

        def background(cycles, share, delay, recent=None):
            pace["clock"] += cycles * share
            token = None
            while jobs and pace["clock"] >= pace["period"]:
                pace["clock"] -= pace["period"]
                pace["release"] = None if recent is None else tok.of(recent[:8])
                new = jobs.pop(0)()
                pace["release"] = None
                token = new if token is None else token | new
            if token is not None:
                due.append([delay, token])
            for entry in due:
                entry[0] -= cycles
            now = [token for left, token in due if left <= 0]
            due[:] = [entry for entry in due if entry[0] > 0]
            return functools.reduce(jnp.bitwise_or, now) if now else None

        def released(x):
            return _after(pace["release"], x, everywhere=True)

        def store_terms(dst, first_term, lead, row, terms):
            for i, val in enumerate(terms):
                dst[(first_term + i, *lead, _rows(row, 16), slice(None))] = val.astype(BF16)
            return tok.stored(dst, (first_term + 6, *lead), row)

        def job_x(c, i, n, r):
            terms = _terms2(RHS, i, lambda row, col: bx_raw[
                pl.ds(c * CH + (col ^ 2) * T + r, 16), pl.ds((2 * row + n) * T, T)].astype(F32))
            return store_terms(bx_t, 7 * i, (n,), c * T + r, terms)

        def job_c(c, i, r):
            terms = _terms2(LHS, i, lambda row, col: c_raw[
                pl.ds(c * CH + row * T + r, 16), pl.ds(col * T, T)].astype(F32))
            return store_terms(c_t, 7 * i, (), c * T + r, terms)

        def jobs_x(c):
            return [P(job_x, c, i, n, r) for r in range(0, T, 16) for n in range(2) for i in range(7)]

        def jobs_c(c):
            return [P(job_c, c, i, r) for r in range(0, T, 16) for i in range(7)]

        def job_wkv(src, i, r):
            def block(row, col):
                raw = (wk_raw, wv_raw)[col % 2]
                return _split(released(raw[src, pl.ds(row * T + r, 16), :]))[col // 2]
            return store_terms(wkv_t, 7 * i, (), r, _terms2(RHS, i, block))

        def job_turn(src, n):
            words = released(wq_raw[src, pl.ds(n * T, T), :])
            wq_turned[n] = pltpu.bitcast(pltpu.bitcast(words, F32).T, U32)
            return tok.stored(wq_turned, (n,), T - 16)

        def job_wq(i, n, r):
            def block(row, col):
                return _split(released(wq_turned[2 * col + n, pl.ds((row % 2) * RO + r, 16), :]))[row // 2]
            return store_terms(wq_t, 7 * i, (n,), r, _terms2(LHS, i, block))

        def jobs_wkv(src):
            return [P(job_wkv, src, i, r) for r in range(0, T, 16) for i in range(7)]

        def jobs_wq(src):
            return ([P(job_turn, src, n) for n in range(DM // T)],
                    [P(job_wq, i, n, r) for n in range(2) for r in range(0, RO, 16) for i in range(7)])

        def job_wob(i, n, r):
            def block(row, col):
                head = 2 * (row % 2) + row // 2
                return released(wob_raw[slot, head, pl.ds(r, 16), pl.ds((2 * col + n) * T, T)].astype(F32))
            return store_terms(wob_t, 7 * i, (n,), j * 64 + r, _terms2(RHS, i, block))

        def job_wo(i, n):
            e, odd, head = j & 3, (j >> 2) & 1, 16 * (j >> 3)

            def block(row, col):
                even_t, odd_t = _split(released(
                    wo_raw[4 * e + row, _rows(head, 16), pl.ds((2 * col + n) * T, T)]))
                return jnp.where(odd == 1, odd_t, even_t)
            return store_terms(wo_t, 7 * i, (n,), odd * T + e * NH + head, _terms2(RHS, i, block))

        permuted = {}

        def job_permute(mat):
            lane = lax.broadcasted_iota(jnp.int32, (32, T), 1)
            e, grp, sub = lane >> 5, (lane >> 2) & 7, lane & 3

            def gather(x, index):
                return jnp.take_along_axis(x, index, axis=1, mode="promise_in_bounds")
            x = [released(wqkv_raw[slot, :, :, pl.ds(mat * DM + t * T, T)].reshape(32, T))
                 for t in range(8)]
            y = [gather(x[t], sub * 32 + e * 8 + ((grp - t) & 7)) for t in range(8)]
            u = [y[-s % 8] for s in range(8)]
            for bit in (1, 2, 4):
                u = [jnp.where((grp & bit) != 0, u[(s - bit) % 8], u[s]) for s in range(8)]
            u = [u[0]] + [gather(u[t], e * 32 + ((grp + t) & 7) * 4 + sub) for t in range(1, 8)]
            permuted[mat] = u
            return _fold(jnp.bitwise_or, functools.reduce(jnp.bitwise_or, u)) & tok.zero

        def column(mat, row, t):
            return pltpu.bitcast(released(permuted[mat][t][8 * row:8 * row + 8]), BF16).astype(F32)

        def job_wa(mat, i, n):
            terms = _terms2(RHS, i, lambda row, col: column(mat, row, 2 * col + n))
            return store_terms(wa_t, 7 * i, (2 * mat + n,), 16 * j, terms)

        pause = [P(lambda: tok.zero)] * 2
        jobs_wob = [P(job_wob, i, n, r) for r in range(0, 64, 16) for n in range(2) for i in range(7)]
        jobs_wo = [P(job_wo, i, n) for n in range(2) for i in range(7)]
        jobs_wa = []
        for mat in range(3):
            jobs_wa += [P(job_permute, mat)] + pause
            jobs_wa += [P(job_wa, mat, i, n) for n in range(2) for i in range(7)]

        q, k, v = {}, {}, {}

        def product(dot, share, left, right):
            token = background(left.shape[0] // 2, share, JOB_CYCLES, pace["recent"])
            pace["recent"] = dot(pltpu.bitcast(_after(token, left), BF16), right)
            return pace["recent"]

        def project_q(c):
            inner = []
            for first_product in range(0, 49, 7):
                inner.append(_combine([_sum([
                    product(_dot_nt, pace["q"], _words(wq_t, (i, n), 0, RO), _load(bx_t, (i, n), c * T, T))
                    for n in range(2)]) for i in range(first_product, first_product + 7)]))
                if len(inner) <= 4:
                    due.append([400, tok.of(*[x[RO - 8:] for x in inner[-1]])])
            blocks = _combine_outer(inner)
            for h in range(2):
                for col in range(4):
                    val = _cat([blocks[2 * h, col], blocks[2 * h + 1, col]], axis=0) * SCALE_B
                    q[4 * c + (col ^ 2), h] = val.T.astype(BF16)

        def project_kv(c):
            m = [product(_dot, pace["kv"], _words(c_t, (i,), c * T, T), _load(wkv_t, (i,), 0, T))
                 for i in range(49)]
            for (row, col), val in sorted(_combine_outer([_combine(m[i:i + 7]) for i in range(0, 49, 7)]).items()):
                (k, v)[col % 2][4 * c + row, col // 2] = val.astype(BF16)

        def plain(raw, c, weights):
            def part(r, col):
                left = raw[pl.ds(c * CH + r, 32), pl.ds(col, 4 * T)]
                token = background(32, 1.0, 128)
                if token is None:
                    return left
                return _cat([_after(_cat([token, token]), left[:, :2 * T]), left[:, 2 * T:]])
            return [_dot(_cat([_cat([part(r, col) for r in range(0, CH, 32)], axis=0)
                               for col in range(0, raw.shape[1], 4 * T)]), w) for w in weights]

        def plain_kv(c, weights):
            for n, val in enumerate(plain(c_raw, c, weights)):
                for r in range(4):
                    (k, v)[n // 2][4 * c + r, n % 2] = val[r * T:(r + 1) * T].astype(BF16)

        def plain_q(c, weights):
            for h, val in enumerate(plain(bx_raw, c, weights)):
                for r in range(4):
                    q[4 * c + r, h] = (val[r * T:(r + 1) * T] * SCALE_B).astype(BF16)

        in_flight, partial, ctx, spread, checks = [], {}, {}, {}, []

        def finish(i, h):
            l, o = partial.pop((i, h))
            l = jnp.sum(l, axis=1, keepdims=True)
            r = _inverse(l)
            ctx[i, h] = o * r
            spread[i, h] = _fold(jnp.maximum, jnp.broadcast_to(l + r, (T, T)))
            b = i // 2
            quad = [(2 * b, 0), (2 * b, 1), (2 * b + 1, 0), (2 * b + 1, 1)]
            if all(u in ctx for u in quad):
                terms = _terms(LHS, lambda m: ctx.pop(quad[m]))
                for n, val in enumerate(terms):
                    ctx_t[n, j, pl.ds(b * T, T), :] = val.astype(BF16)
                checks.append((_fold(jnp.add, terms[0] + terms[5] + terms[6]),
                               functools.reduce(jnp.maximum, [spread.pop(u) for u in quad])))
                due.append([CTX_CYCLES[first], tok.stored(ctx_t, (6, j), b * T) | tok.of(*checks[-1])])

        def weigh(i, h, t, p):
            l, o = partial.get((i, h), (None, None))
            l = p if l is None else l + p
            d = _dot(_after(background(64, pace["attention"], JOB_CYCLES, p), p).astype(BF16), v[t, h])
            partial[i, h] = (l, d if o is None else o + d)
            if t == i:
                finish(i, h)

        def attention(lo, hi):
            for i in range(lo, hi):
                for h in range(2):
                    for t in range(i + 1):
                        s = _dot_nt(q[i, h], k[t, h])
                        if t == i:
                            s = jnp.where(causal, s, MASKED)
                        in_flight.append((i, h, t, jnp.exp2(s)))
                        ahead = (i, h) == (S // T - 1, 1) and 8 <= t < 13 and not first
                        if len(in_flight) > DEPTH and not ahead:
                            weigh(*in_flight.pop(0))
            while hi == S // T and in_flight:
                weigh(*in_flight.pop(0))

        def cycles(lo, hi):
            return 2 * 64 * sum(range(lo + 1, hi + 1))

        if first:
            wk, wv, wq = head_copies(0, 0)
            _start(wv, wk, c_copy(0), c_copy(1))
            _wait(wv, wk, c_copy(0))
            _start(c_copy(2), c_copy(3), wq, x_copy(0))
            weights = [w.astype(BF16) for raw in (wk_raw, wv_raw) for w in _split(raw[0])]
            queue(0.98 * 2048, jobs_c(0)[:49])
            plain_kv(0, weights)
            flush()
            _wait(c_copy(1), c_copy(2))
            _start(x_copy(1), x_copy(2))
            queue(0.92 * 4096, jobs_c(0)[49:] + jobs_c(1) + jobs_c(2))
            plain_kv(1, weights)
            plain_kv(2, weights)
            flush()
            _wait(c_copy(3), wq)
            turn, terms = jobs_wq(0)
            queue(0.9 * 2048, _interleave(turn, jobs_c(3)))
            plain_kv(3, weights)
            flush()
            _wait(x_copy(0))
            weights = [w.astype(BF16) for w in _split(wq_raw[0])]
            queue(0.9 * (2048 + 0.2 * cycles(0, 4)), jobs_x(0)[:96], attention=0.2)
            plain_q(0, weights)
            attention(0, 4)
            flush()
            _wait(x_copy(1), x_copy(2))
            stage = [*side_copies(0, 0), *head_copies(1, 1)]
            _start(x_copy(3), *stage)
            lax.fori_loop(0, 16, lambda word, carry: wo_copy(word).start(), None)
            queue(0.98 * (2048 + 0.5 * cycles(4, 7)),
                  jobs_x(2) + terms + jobs_x(0)[96:] + jobs_x(1)[:14], attention=0.5)
            plain_q(1, weights)
            attention(4, 7)
            flush()
            _wait(x_copy(3))
            queue(0.85 * (1568 + cycles(7, 10)), jobs_x(3))
            project_q(2)
            attention(7, 10)
            flush()
            _wait(*stage)
            _start(ax_copy(0, 0), *head_copies(2, 0), *side_copies(1, 1))
            turn, terms = jobs_wq(1)
            queue(0.88 * (1568 + cycles(10, 14)), _interleave(
                _interleave(jobs_wob, jobs_wa), _interleave(jobs_x(1)[14:], _interleave(turn, jobs_wkv(1)))))
            attention(10, 11)
            project_q(3)
            attention(11, 14)
            flush()
            _wait(*[wo_copy(word) for word in range(16)], ax_copy(0, 0))
            _start(ax_copy(1, 1))
            queue(0.92 * cycles(14, 16), _interleave(
                jobs_wo + terms, [P(_job_ax, tok, released, ax_raw, ax_t, 0, *job) for job in AX_JOBS]))
            attention(14, 16)
            flush()
        else:
            queue(0.98 * 4 * 1568 * (0.5 + 0.3), _interleave(jobs_wob, jobs_wo + jobs_wa),
                  q=0.5, kv=0.3, attention=0)
            project_kv(0)
            project_q(0)
            project_kv(1)
            attention(0, 3)
            project_q(1)
            attention(3, 7)
            project_q(2)
            project_kv(2)
            attention(7, 10)
            project_q(3)
            project_kv(3)
            attention(10, 12)
            flush()
            turn, terms = jobs_wq(1 - slot)
            queue(0.95 * cycles(12, 16), _interleave(jobs_wkv(1 - slot), turn + pause + terms))
            attention(12, 16)
            flush()
        guard[0] = _sum([guard[0]] + [x for x, _ in checks])
        guard[1] = functools.reduce(jnp.maximum, [guard[1]] + [x for _, x in checks])

        def ahead(n):
            return j + n if first else jnp.minimum(j + n, NP - 1)
        _wait(*head_copies(ahead(2), slot), *side_copies(ahead(1), 1 - slot))

        @pl.when(j < NP - 1)
        def _():
            _start(*head_copies(ahead(3), 1 - slot), *side_copies(ahead(2), slot))

    def exact_pairs(ctx):
        def block(i):
            return pl.ds(pl.multiple_of(i * T, T), T)

        def qkv(n, h, i):
            return c_t.at[(2 * n + h) * 4 + (i >> 2), block(i & 3), :]

        def project(x, carry):
            h, i = x & 1, x >> 1

            def weight(raw):
                even, odd = _split(raw[0])
                return jnp.where(h == 0, even, odd).astype(BF16)
            qkv(0, h, i)[...] = (_dot(bx_raw[block(i), :], weight(wq_raw)) * SCALE_B).astype(BF16)
            qkv(1, h, i)[...] = _dot(c_raw[block(i), :], weight(wk_raw)).astype(BF16)
            qkv(2, h, i)[...] = _dot(c_raw[block(i), :], weight(wv_raw)).astype(BF16)

        def attend(b, x, carry):
            h, i = x & 1, 2 * b + (x >> 1)

            def scores(t):
                row = lax.broadcasted_iota(jnp.int32, (T, T), 0) + i * T
                col = lax.broadcasted_iota(jnp.int32, (T, T), 1) + t * T
                return jnp.where(col <= row, _dot_nt(qkv(0, h, i)[...], qkv(1, h, t)[...]), MASKED)

            m = lax.fori_loop(
                0, i + 1, lambda t, m: jnp.maximum(m, jnp.max(scores(t), axis=1, keepdims=True)),
                jnp.full((T, 1), -jnp.inf, F32))

            def accumulate(t, carry):
                l, o = carry
                p = jnp.exp2(scores(t) - m)
                return (l + jnp.sum(p, axis=1, keepdims=True),
                        o + _dot(p.astype(BF16), qkv(2, h, t)[...]))
            l, o = lax.fori_loop(0, i + 1, accumulate,
                                 (jnp.zeros((T, 1), F32), jnp.zeros((T, T), F32)))
            ctx[x] = o / l

        def pair(j, carry):
            _start(*head_copies(j, 0))
            _wait(*head_copies(j, 0))
            lax.fori_loop(0, 2 * S // T, project, None)

            def rows(b, carry):
                lax.fori_loop(0, 4, P(attend, b), None)
                for n, val in enumerate(_terms(LHS, lambda m: ctx[m])):
                    ctx_t[n, j, block(b), :] = val.astype(BF16)
            lax.fori_loop(0, S // T // 2, rows, None)

        lax.fori_loop(0, NP, pair, None)

    guard[...] = jnp.zeros(guard.shape, F32)
    pair_body(0, first=True)
    lax.fori_loop(1, NP, lambda j, carry: pair_body(j), None)

    safe = jnp.logical_and(jnp.abs(guard[0]) < jnp.inf, guard[1] < SAFE_SUM)

    @pl.when(jnp.max(jnp.where(safe, 0.0, 1.0)) > 0.0)
    def _():
        pl.run_scoped(exact_pairs, pltpu.VMEM((4, T, T), F32))


def _outputs(out_hbm, ax_copy, ax_raw, ax_t, ctx_t, wob_t, wa_t, wo_t, zero_smem,
             o_t, kbuf, vbuf, qbuf, acc, obuf, sem_out):
    def out_copy(c, slot):
        rows = pl.ds(_aligned(c * CO, CO), CO)
        return pltpu.make_async_copy(obuf.at[slot], out_hbm.at[rows, :], sem_out.at[slot])

    for buf in (kbuf, vbuf):
        for t in range(8):
            buf[t, pl.ds(CO, HALO), :] = jnp.zeros((HALO, T), F32)

    t_q = 2 * 49 * RO
    t_v = t_q + 21 * 4 * RO + 49 * RO
    t_o = t_v + (21 + EARLY_B) * 4 * RO

    def chunk_body(c, carry):
        slot = c & 1
        tok = _Tokens(zero_smem)
        plan, due, clock = {}, {}, [0]

        def schedule(job, begin, end, release=False):
            plan.setdefault(max(clock[0], begin // TICK), []).append((job, -(-end // TICK), release))

        def step(results, a, w):
            res = [None] * len(w)
            for x, left in enumerate(a):
                n = clock[0]
                clock[0] += 1
                if n in due:
                    left = _after(functools.reduce(jnp.bitwise_or, due.pop(n)), left)
                left = left.astype(BF16) if left.dtype == F32 else pltpu.bitcast(left, BF16)
                for y in range(len(w)):
                    d = _dot(left, w[y](x))
                    res[y] = d if res[y] is None else res[y] + d
                token = None
                for job, last, release in plan.pop(n, []):
                    if release and token is None:
                        token = tok.of(d[:8])
                    due.setdefault(max(last, n + 1), []).append(job(token) if release else job())
            results.append(res)

        def project(lhs_t, rhs_t, tile0, write):
            inner = {}

            def combine(i, y, m):
                inner[i, y] = _combine([x[y] for x in m])
                return tok.of(*[x[r + 8:r + 16] for x in inner[i, y] for r in range(0, RO, 16)])

            def finish(outer, y, r):
                vals = [_term(SUMS, outer, lambda i: inner[i, y][n][r:r + 16]) for n in range(4)]
                for n, val in enumerate(vals):
                    row, col = _block(outer, n)
                    write(row * RO + r, 2 * col + y, val)
                return tok.of(*[x[8:] for x in vals])

            for i in range(7):
                m = []
                done = clock[0] * TICK + 7 * RO
                for y in range(2):
                    schedule(P(combine, i, y, m), done, done + 400)
                for outer in FINAL[i]:
                    slabs = [(y, r) for r in range(0, RO, 16) for y in range(2)]
                    for x, slab in enumerate(slabs):
                        schedule(P(finish, outer, *slab), done, done + 300 + 40 * (x + 1))
                for n in range(7 * i, 7 * i + 7):
                    step(m, [_words(lhs_t, (n, x), 0, RO) for x in range(2)],
                         [P(lambda y, x: _load(rhs_t, (n, tile0 + y), x * T, T), y) for y in range(2)])

        for buf in (kbuf, vbuf):
            for t in range(8):
                buf[t, pl.ds(0, HALO), :] = buf[t, pl.ds(CO, HALO), :]

        def write_rows(buf, row, t, val):
            buf[t, pl.ds(HALO + row, 16), :] = val

        def write_q(row, t, val):
            qbuf[t, pl.ds(row, 16), :] = val * SCALE_A

        project(ax_t, wa_t, 2, P(write_rows, kbuf))
        project(ax_t, wa_t, 0, write_q)

        att = {}

        def job_weights(row, r, release):
            base = HALO + row * RO + r
            qs = [_after(release, qbuf[t, pl.ds(row * RO + r, 8), :]) for t in range(8)]
            logits = []
            for w in range(WIN):
                x = _sum([qs[t] * kbuf[t, pl.ds(base - DIL * w, 8), :] for t in range(8)])
                x = x + pltpu.roll(x, 64, 1)
                x = x + pltpu.roll(x, 32, 1)
                if row == 0 and r < DIL * w:
                    pos = lax.broadcasted_iota(jnp.int32, (8, T), 0) + (c * CO + r)
                    x = jnp.where(pos >= DIL * w, x, MASKED)
                logits.append(x)
            m = functools.reduce(jnp.maximum, logits)
            p = [jnp.exp2(x - m) for x in logits]
            att[row, r] = p + [_inverse(_sum(p))]
            return tok.of(att[row, r][-1])

        def job_values(row, r, release):
            base = HALO + row * RO + r
            *p, inv = [_after(release, x) for x in att[row, r]]
            att[row, r] = [_sum([p[w] * vbuf[t, pl.ds(base - DIL * w, 8), :] for w in range(WIN)]) * inv
                           for t in range(8)]
            return tok.of(att[row, r][-1])

        def job_o(n, r, i):
            def block(row, col):
                return _cat([att[row, r][2 * col + n], att[row, r + 8][2 * col + n]], axis=0)
            for x, val in enumerate(_terms2(LHS, i, block)):
                o_t[7 * i + x, n, pl.ds(r, 16), :] = val.astype(BF16)
            return tok.stored(o_t, (7 * i + 6, n), r)

        groups = [(row, r + x) for r in range(0, RO, 16) for row in (2, 0, 3, 1) for x in (0, 8)]
        w0, w1, v0, v1 = t_q + 1000, t_v - 1700, t_v + 400, t_o - 700
        for g, (row, r) in enumerate(groups):
            begin = w0 + (w1 - w0) * g // len(groups)
            schedule(P(job_weights, row, r), begin, begin + 500, release=True)
            begin = v0 + (v1 - v0) * g // len(groups)
            schedule(P(job_values, row, r), begin, begin + 600, release=True)
            if g % 8 == 7:
                for x, (n, i) in enumerate((n, i) for n in range(2) for i in range(7)):
                    schedule(P(job_o, n, r - 8, i), begin, min(begin + 300 + 60 * (x + 1), t_o))

        touched = {}

        def project_b(i):
            m = []

            def accumulate(y, inner):
                val = _combine([x[y] for x in m])[inner]
                token = None
                for outer, sign in OUT[i]:
                    row, col = _block(outer, inner)
                    rows, col = pl.ds(row * RO, RO), 2 * col + y
                    total = val
                    if (outer, inner, y) in touched:
                        total = acc[col, rows, :] + val if sign > 0 else acc[col, rows, :] - val
                    touched[outer, inner, y] = True
                    if outer not in FINAL[i]:
                        acc[col, rows, :] = total
                        token = tok.stored(acc, (col,), row * RO)
                    else:
                        obuf[slot, rows, pl.ds(DM + col * T, T)] = total.astype(BF16)
                        if token is None:
                            token = tok.of(_fold(jnp.add, total))
                return token

            parts = [(y, inner) for y in range(2) for inner in range(4)]
            done = clock[0] * TICK + 7 * 4 * RO
            if i < 6:
                for x, part in enumerate(parts):
                    schedule(P(accumulate, *part), done, done + 256 + 170 * x)
            for n in range(7):
                if i == 6 and n == EARLY_B:
                    yield

                def quad(kt, x):
                    return (i, 2 * kt + x % 2), (2 * c + x // 2) * RO
                if len(LHS[n]) == 1:
                    a = [_words(ctx_t, *quad(kt, LHS[n][0][0]), RO) for kt in range(8)]
                else:
                    a = [_term(LHS, n, lambda x: _load(ctx_t, (i + tok.z * n, 2 * kt + x % 2), quad(kt, x)[1], RO).astype(F32))
                         for kt in range(8)]
                step(m, a, [P(lambda y, x: _load(wob_t, (7 * i + n, y), x * T, T), y) for y in range(2)])
            if i == 6:
                for part in parts:
                    accumulate(*part)

        for i in range(6):
            if i == 3:
                project(ax_t, wa_t, 4, P(write_rows, vbuf))
            list(project_b(i))
        last_b = project_b(6)
        next(last_b)

        for x, job in enumerate(AX_JOBS):
            schedule(P(_job_ax, tok, lambda val: val, ax_raw, ax_t, 1 - slot, *job),
                     t_o, t_o + 100 + 3300 * (x + 1) // len(AX_JOBS))

        def write_out(row, t, val):
            obuf[slot, pl.ds(row, 16), pl.ds(t * T, T)] = val.astype(BF16)

        project(o_t, wo_t, 0, write_out)
        list(last_b)
        assert not plan and not due
        out_copy(c, slot).start()
        ax_copy(jnp.minimum(c + 2, NO - 1), slot).wait()

        @pl.when(c < NO - 1)
        def _():
            ax_copy(jnp.minimum(c + 3, NO - 1), 1 - slot).start()

        @pl.when(c >= 1)
        def _():
            out_copy(c - 1, 1 - slot).wait()

    ax_copy(1, 1).wait()
    ax_copy(2, 0).start()
    lax.fori_loop(0, NO, chunk_body, None)
    out_copy(NO - 1, (NO - 1) % 2).wait()


def _kernel(ax_hbm, wqkv_hbm, wo_hbm, bx_hbm, c_hbm, wq_hbm, wuk_hbm, wuv_hbm, wob_hbm, out_hbm,
            ax_raw, ax_t, ctx_t, wob_t, wa_t, wo_t, zero_smem, sem_ax):
    vmem, dma = pltpu.VMEM, pltpu.SemaphoreType.DMA

    def clear(i, carry):
        zero_smem[0] = i >> 1
    lax.fori_loop(0, 2, clear, None)

    def ax_copy(c, slot):
        rows = pl.ds(_aligned(c * CO, CO), CO)
        return pltpu.make_async_copy(ax_hbm.at[rows, :], ax_raw.at[slot], sem_ax.at[slot])

    shared = (ax_copy, ax_raw, ax_t, ctx_t, wob_t, wa_t, wo_t, zero_smem)
    pl.run_scoped(
        P(_head_pairs, wqkv_hbm, wo_hbm, bx_hbm, c_hbm, wq_hbm, wuk_hbm, wuv_hbm, wob_hbm, *shared),
        vmem((S, DM), BF16),
        vmem((S, DC), BF16),
        vmem((2, DM, T), U32),
        vmem((2, DC, T), U32),
        vmem((2, DC, T), U32),
        vmem((2, 4, 64, DM), BF16),
        vmem((2, 4, 8, 3 * DM), U32),
        vmem((16, NH, DM), U32),
        vmem((49, 2, S // 4, T), BF16),
        vmem((49, S // 4, T), BF16),
        vmem((DM // T, T, T), U32),
        vmem((49, 2, RO, T), BF16),
        vmem((49, T, T), BF16),
        vmem((2, 8, T), F32),
        dma((2 * S // CH,)), dma((11,)))
    pl.run_scoped(
        P(_outputs, out_hbm, *shared),
        vmem((49, 2, RO, T), BF16),
        vmem((8, HALO + CO, T), F32),
        vmem((8, HALO + CO, T), F32),
        vmem((8, CO, T), F32),
        vmem((8, CO, T), F32),
        vmem((2, CO, 2 * DM), BF16),
        dma((2,)))


@jax.jit
def pallas_concat_heads__sliding_local_dilated__compressed_kv_cla__prompt_kernel(
    A_x: jax.Array,
    A_wqkv: jax.Array,
    A_wo: jax.Array,
    B_x: jax.Array,
    B_c_kv: jax.Array,
    B_w_q: jax.Array,
    B_w_uk: jax.Array,
    B_w_uv: jax.Array,
    B_w_o: jax.Array,
):
    vmem = pltpu.VMEM
    out = pl.pallas_call(
        _kernel,
        out_shape=jax.ShapeDtypeStruct((S, 2 * DM), BF16),
        in_specs=[pl.BlockSpec(memory_space=pl.ANY)] * 9,
        out_specs=pl.BlockSpec(memory_space=pl.ANY),
        scratch_shapes=[
            vmem((2, CO, DM), BF16),
            vmem((49, 2, RO, T), BF16),
            vmem((7, NP, S // 2, T), BF16),
            vmem((49, 2, DM, T), BF16),
            vmem((49, 6, 2 * T, T), BF16),
            vmem((49, 2, 2 * T, T), BF16),
            pltpu.SMEM((1,), jnp.int32),
            pltpu.SemaphoreType.DMA((2,)),
        ],
        compiler_params=pltpu.CompilerParams(
            vmem_limit_bytes=127 * 2**20, disable_bounds_checks=True),
    )(
        A_x.reshape(S, DM),
        A_wqkv.reshape(4, DM // 4, 3 * DM),
        A_wo.reshape(NH, DM // NH, DM),
        B_x.reshape(S, DM),
        B_c_kv.reshape(S, DC),
        B_w_q,
        B_w_uk,
        B_w_uv,
        B_w_o,
    )
    return out.reshape(1, S, 2 * DM)
```

```python
import functools
import math

import jax
import jax.numpy as jnp
from jax import lax
import jax.experimental.pallas as pl
import jax.experimental.pallas.tpu as pltpu

S = 2048
DM = 1024
DC = 512
NH = 32
NP = NH // 2
T = 128
CH = 4 * T
RO = 64
CO = 4 * RO
NO = S // CO
WIN, DIL = 8, 2
HALO = 16

LOG2E = math.log2(math.e)
SCALE_A = (DM // NH) ** -0.5 * LOG2E
SCALE_B = T ** -0.5 * LOG2E
MASKED = -1e9 * LOG2E
SAFE_SUM = 2.0 ** 40

DEPTH = 3
JOB_CYCLES = 896
CTX_CYCLES = 1024, 768
TICK = RO // 2
EARLY_B = 4

F32, BF16, U32 = jnp.float32, jnp.bfloat16, jnp.uint32
P = functools.partial


def _dot(a, b):
    return jnp.dot(a, b, preferred_element_type=F32)


def _dot_nt(a, b):
    return lax.dot_general(a, b, (((1,), (1,)), ((), ())), preferred_element_type=F32)


def _cat(xs, axis=1):
    return xs[0] if len(xs) == 1 else jnp.concatenate(xs, axis=axis)


def _sum(xs):
    return functools.reduce(jnp.add, xs)


def _fold(op, x):
    return functools.reduce(op, [x[r:r + 8] for r in range(0, x.shape[0], 8)])


def _aligned(x, n):
    return x if isinstance(x, int) else pl.multiple_of(x, n)


def _rows(start, n):
    return pl.ds(_aligned(start, 16), n)


def _words(ref, lead, start, n):
    return ref.bitcast(U32)[(*lead, pl.ds(_aligned(start >> 1, 8), n // 2), slice(None))]


def _load(ref, lead, start, n):
    return pltpu.bitcast(_words(ref, lead, start, n), BF16)


def _split(w):
    return (pltpu.bitcast(w << 16, F32), pltpu.bitcast(w & jnp.uint32(0xFFFF0000), F32))


def _inverse(l):
    r = pl.reciprocal(l, approx=True)
    return r * (2.0 - l * r)


def _interleave(x, y):
    order = [((n + 0.5) / len(z), m, job) for m, z in enumerate((x, y)) for n, job in enumerate(z)]
    return [job for _, _, job in sorted(order, key=lambda e: e[:2])]


def _start(*copies):
    for cp in copies:
        cp.start()


def _wait(*copies):
    for cp in copies:
        cp.wait()


LHS = (((0, 1), (3, 1)), ((2, 1), (3, 1)), ((0, 1),), ((3, 1),),
       ((0, 1), (1, 1)), ((2, 1), (0, -1)), ((1, 1), (3, -1)))
RHS = (((0, 1), (3, 1)), ((0, 1),), ((1, 1), (3, -1)), ((2, 1), (0, -1)),
       ((3, 1),), ((0, 1), (1, 1)), ((2, 1), (3, 1)))
OUT = (((0, 1), (3, 1)), ((2, 1), (3, -1)), ((1, 1), (3, 1)), ((0, 1), (2, 1)),
       ((0, -1), (1, 1)), ((3, 1),), ((0, 1),))
SUMS = tuple(tuple((i, sign) for i in range(7) for m, sign in OUT[i] if m == n) for n in range(4))
FINAL = tuple(tuple(n for n in range(4) if SUMS[n][-1][0] == i) for i in range(7))


def _term(table, i, quad):
    (n, _), *rest = table[i]
    val = quad(n)
    for n, sign in rest:
        val = val + quad(n) if sign > 0 else val - quad(n)
    return val


def _terms(table, quad):
    blocks = [quad(n) for n in range(4)]
    return [_term(table, i, blocks.__getitem__) for i in range(7)]


def _block(outer, inner):
    return 2 * (outer // 2) + inner // 2, 2 * (outer % 2) + inner % 2


def _terms2(table, i, block):
    return _terms(table, lambda n: _term(table, i, lambda m: block(*_block(m, n))))


def _combine(m):
    return [_term(SUMS, n, m.__getitem__) for n in range(4)]


def _combine_outer(inner):
    return {_block(outer, n): val for n in range(4)
            for outer, val in enumerate(_combine([x[n] for x in inner]))}


class _Tokens:
    def __init__(self, zero_smem):
        self.z = zero_smem[0]
        self.zero = jnp.full((8, T), self.z, jnp.int32).astype(U32)

    def stored(self, ref, lead, start):
        first, *rest = lead
        if ref.dtype == BF16:
            return _words(ref, (first - (self.z & 1), *rest), start, 16) & self.zero
        return self.of(ref[(*lead, pl.ds(_aligned(start + 8 * (self.z & 1), 8), 8), slice(None))])

    def of(self, *vals):
        return pltpu.bitcast(_sum(vals), U32) & self.zero


def _after(token, x, everywhere=False):
    if token is None:
        return x
    bits = x if x.dtype == U32 else pltpu.bitcast(x, U32)
    cut = bits.shape[0] if everywhere else 8
    parts = [bits[r:r + 8] | token for r in range(0, cut, 8)]
    bits = _cat(parts + ([bits[cut:]] if cut < bits.shape[0] else []), axis=0)
    return bits if x.dtype == U32 else pltpu.bitcast(bits, x.dtype)


AX_JOBS = [(i, n, r) for n in range(2) for r in range(0, RO, 16) for i in range(7)]


def _job_ax(tok, released, ax_raw, ax_t, src, i, n, r):
    terms = _terms2(LHS, i, lambda row, col: released(
        ax_raw[src, pl.ds(row * RO + r, 16), pl.ds((2 * col + n) * T, T)].astype(F32)))
    for x, val in enumerate(terms):
        ax_t[7 * i + x, n, pl.ds(r, 16), :] = val.astype(BF16)
    return tok.stored(ax_t, (7 * i + 6, n), r)


def _head_pairs(wqkv_hbm, wo_hbm, bx_hbm, c_hbm, wq_hbm, wuk_hbm, wuv_hbm, wob_hbm,
                ax_copy, ax_raw, ax_t, ctx_t, wob_t, wa_t, wo_t, zero_smem,
                bx_raw, c_raw, wq_raw, wk_raw, wv_raw, wob_raw, wqkv_raw, wo_raw,
                bx_t, c_t, wq_turned, wq_t, wkv_t, guard, sem_in, sem_w):
    def head_copies(j, slot):
        return [pltpu.make_async_copy(src.bitcast(U32).at[:, j, :], dst.at[slot], sem_w.at[3 * slot + n])
                for n, (src, dst) in enumerate(((wuk_hbm, wk_raw), (wuv_hbm, wv_raw), (wq_hbm, wq_raw)))]

    def side_copies(j, slot):
        wob = wob_hbm.at[pl.ds(4 * (j >> 1), 4), pl.ds(_aligned((j & 1) * 64, 64), 64), :]
        wqkv = wqkv_hbm.bitcast(U32).at[:, pl.ds(_aligned(8 * j, 8), 8), :]
        return [pltpu.make_async_copy(wob, wob_raw.at[slot], sem_w.at[6 + 2 * slot]),
                pltpu.make_async_copy(wqkv, wqkv_raw.at[slot], sem_w.at[7 + 2 * slot])]

    def wo_copy(word):
        return pltpu.make_async_copy(wo_hbm.bitcast(U32).at[:, word, :], wo_raw.at[word], sem_w.at[10])

    def c_copy(c):
        rows = pl.ds(c * CH, CH)
        return pltpu.make_async_copy(c_hbm.at[rows, :], c_raw.at[rows, :], sem_in.at[2 * c])

    def x_copy(c):
        rows = pl.ds(c * CH, CH)
        return pltpu.make_async_copy(bx_hbm.at[rows, :], bx_raw.at[rows, :], sem_in.at[2 * c + 1])

    def pair_body(j, first=False):
        slot = j & 1
        tok = _Tokens(zero_smem)
        causal = (lax.broadcasted_iota(jnp.int32, (T, T), 1)
                  <= lax.broadcasted_iota(jnp.int32, (T, T), 0))

        jobs, due, pace = [], [], dict(release=None, recent=None)

        def queue(cycles, more, q=1.0, kv=1.0, attention=1.0):
            pace.update(period=cycles / len(more), clock=0, q=q, kv=kv, attention=attention)
            jobs.extend(more)

        def flush():
            while jobs:
                jobs.pop(0)()

        def background(cycles, share, delay, recent=None):
            pace["clock"] += cycles * share
            token = None
            while jobs and pace["clock"] >= pace["period"]:
                pace["clock"] -= pace["period"]
                pace["release"] = None if recent is None else tok.of(recent[:8])
                new = jobs.pop(0)()
                pace["release"] = None
                token = new if token is None else token | new
            if token is not None:
                due.append([delay, token])
            for entry in due:
                entry[0] -= cycles
            now = [token for left, token in due if left <= 0]
            due[:] = [entry for entry in due if entry[0] > 0]
            return functools.reduce(jnp.bitwise_or, now) if now else None

        def released(x):
            return _after(pace["release"], x, everywhere=True)

        def store_terms(dst, first_term, lead, row, terms):
            for i, val in enumerate(terms):
                dst[(first_term + i, *lead, _rows(row, 16), slice(None))] = val.astype(BF16)
            return tok.stored(dst, (first_term + 6, *lead), row)

        def job_x(c, i, n, r):
            terms = _terms2(RHS, i, lambda row, col: bx_raw[
                pl.ds(c * CH + (col ^ 2) * T + r, 16), pl.ds((2 * row + n) * T, T)].astype(F32))
            return store_terms(bx_t, 7 * i, (n,), c * T + r, terms)

        def job_c(c, i, r):
            terms = _terms2(LHS, i, lambda row, col: c_raw[
                pl.ds(c * CH + row * T + r, 16), pl.ds(col * T, T)].astype(F32))
            return store_terms(c_t, 7 * i, (), c * T + r, terms)

        def jobs_x(c):
            return [P(job_x, c, i, n, r) for r in range(0, T, 16) for n in range(2) for i in range(7)]

        def jobs_c(c):
            return [P(job_c, c, i, r) for r in range(0, T, 16) for i in range(7)]

        def job_wkv(src, i, r):
            def block(row, col):
                raw = (wk_raw, wv_raw)[col % 2]
                return _split(released(raw[src, pl.ds(row * T + r, 16), :]))[col // 2]
            return store_terms(wkv_t, 7 * i, (), r, _terms2(RHS, i, block))

        def job_turn(src, n):
            words = released(wq_raw[src, pl.ds(n * T, T), :])
            wq_turned[n] = pltpu.bitcast(pltpu.bitcast(words, F32).T, U32)
            return tok.stored(wq_turned, (n,), T - 16)

        def job_wq(i, n, r):
            def block(row, col):
                return _split(released(wq_turned[2 * col + n, pl.ds((row % 2) * RO + r, 16), :]))[row // 2]
            return store_terms(wq_t, 7 * i, (n,), r, _terms2(LHS, i, block))

        def jobs_wkv(src):
            return [P(job_wkv, src, i, r) for r in range(0, T, 16) for i in range(7)]

        def jobs_wq(src):
            return ([P(job_turn, src, n) for n in range(DM // T)],
                    [P(job_wq, i, n, r) for n in range(2) for r in range(0, RO, 16) for i in range(7)])

        def job_wob(i, n, r):
            def block(row, col):
                head = 2 * (row % 2) + row // 2
                return released(wob_raw[slot, head, pl.ds(r, 16), pl.ds((2 * col + n) * T, T)].astype(F32))
            return store_terms(wob_t, 7 * i, (n,), j * 64 + r, _terms2(RHS, i, block))

        def job_wo(i, n):
            e, odd, head = j & 3, (j >> 2) & 1, 16 * (j >> 3)

            def block(row, col):
                even_t, odd_t = _split(released(
                    wo_raw[4 * e + row, _rows(head, 16), pl.ds((2 * col + n) * T, T)]))
                return jnp.where(odd == 1, odd_t, even_t)
            return store_terms(wo_t, 7 * i, (n,), odd * T + e * NH + head, _terms2(RHS, i, block))

        permuted = {}

        def job_permute(mat):
            lane = lax.broadcasted_iota(jnp.int32, (32, T), 1)
            e, grp, sub = lane >> 5, (lane >> 2) & 7, lane & 3

            def gather(x, index):
                return jnp.take_along_axis(x, index, axis=1, mode="promise_in_bounds")
            x = [released(wqkv_raw[slot, :, :, pl.ds(mat * DM + t * T, T)].reshape(32, T))
                 for t in range(8)]
            y = [gather(x[t], sub * 32 + e * 8 + ((grp - t) & 7)) for t in range(8)]
            u = [y[-s % 8] for s in range(8)]
            for bit in (1, 2, 4):
                u = [jnp.where((grp & bit) != 0, u[(s - bit) % 8], u[s]) for s in range(8)]
            u = [u[0]] + [gather(u[t], e * 32 + ((grp + t) & 7) * 4 + sub) for t in range(1, 8)]
            permuted[mat] = u
            return _fold(jnp.bitwise_or, functools.reduce(jnp.bitwise_or, u)) & tok.zero

        def column(mat, row, t):
            return pltpu.bitcast(released(permuted[mat][t][8 * row:8 * row + 8]), BF16).astype(F32)

        def job_wa(mat, i, n):
            terms = _terms2(RHS, i, lambda row, col: column(mat, row, 2 * col + n))
            return store_terms(wa_t, 7 * i, (2 * mat + n,), 16 * j, terms)

        pause = [P(lambda: tok.zero)] * 2
        jobs_wob = [P(job_wob, i, n, r) for r in range(0, 64, 16) for n in range(2) for i in range(7)]
        jobs_wo = [P(job_wo, i, n) for n in range(2) for i in range(7)]
        jobs_wa = []
        for mat in range(3):
            jobs_wa += [P(job_permute, mat)] + pause
            jobs_wa += [P(job_wa, mat, i, n) for n in range(2) for i in range(7)]

        q, k, v = {}, {}, {}

        def product(dot, share, left, right):
            token = background(left.shape[0] // 2, share, JOB_CYCLES, pace["recent"])
            pace["recent"] = dot(pltpu.bitcast(_after(token, left), BF16), right)
            return pace["recent"]

        def project_q(c):
            inner = []
            for first_product in range(0, 49, 7):
                inner.append(_combine([_sum([
                    product(_dot_nt, pace["q"], _words(wq_t, (i, n), 0, RO), _load(bx_t, (i, n), c * T, T))
                    for n in range(2)]) for i in range(first_product, first_product + 7)]))
                if len(inner) <= 4:
                    due.append([400, tok.of(*[x[RO - 8:] for x in inner[-1]])])
            blocks = _combine_outer(inner)
            for h in range(2):
                for col in range(4):
                    val = _cat([blocks[2 * h, col], blocks[2 * h + 1, col]], axis=0) * SCALE_B
                    q[4 * c + (col ^ 2), h] = val.T.astype(BF16)

        def project_kv(c):
            m = [product(_dot, pace["kv"], _words(c_t, (i,), c * T, T), _load(wkv_t, (i,), 0, T))
                 for i in range(49)]
            blocks = _combine_outer([_combine(m[i:i + 7]) for i in range(0, 49, 7)])
            for (row, col), val in sorted(blocks.items()):
                (k, v)[col % 2][4 * c + row, col // 2] = val.astype(BF16)

        def plain(raw, c, weights):
            def part(r, col):
                left = raw[pl.ds(c * CH + r, 32), pl.ds(col, 4 * T)]
                token = background(32, 1.0, 128)
                if token is None:
                    return left
                return _cat([_after(_cat([token, token]), left[:, :2 * T]), left[:, 2 * T:]])
            return [_dot(_cat([_cat([part(r, col) for r in range(0, CH, 32)], axis=0)
                               for col in range(0, raw.shape[1], 4 * T)]), w) for w in weights]

        def plain_kv(c, weights):
            for n, val in enumerate(plain(c_raw, c, weights)):
                for r in range(4):
                    (k, v)[n // 2][4 * c + r, n % 2] = val[r * T:(r + 1) * T].astype(BF16)

        def plain_q(c, weights):
            for h, val in enumerate(plain(bx_raw, c, weights)):
                for r in range(4):
                    q[4 * c + r, h] = (val[r * T:(r + 1) * T] * SCALE_B).astype(BF16)

        in_flight, partial, ctx, spread, checks = [], {}, {}, {}, []

        def finish(i, h):
            l, o = partial.pop((i, h))
            l = jnp.sum(l, axis=1, keepdims=True)
            r = _inverse(l)
            ctx[i, h] = o * r
            spread[i, h] = _fold(jnp.maximum, jnp.broadcast_to(l + r, (T, T)))
            b = i // 2
            quad = [(2 * b, 0), (2 * b, 1), (2 * b + 1, 0), (2 * b + 1, 1)]
            if all(u in ctx for u in quad):
                terms = _terms(LHS, lambda m: ctx.pop(quad[m]))
                for n, val in enumerate(terms):
                    ctx_t[n, j, pl.ds(b * T, T), :] = val.astype(BF16)
                checks.append((_fold(jnp.add, terms[0] + terms[5] + terms[6]),
                               functools.reduce(jnp.maximum, [spread.pop(u) for u in quad])))
                due.append([CTX_CYCLES[first], tok.stored(ctx_t, (6, j), b * T) | tok.of(*checks[-1])])

        def weigh(i, h, t, p):
            l, o = partial.get((i, h), (None, None))
            l = p if l is None else l + p
            d = _dot(_after(background(64, pace["attention"], JOB_CYCLES, p), p).astype(BF16), v[t, h])
            partial[i, h] = (l, d if o is None else o + d)
            if t == i:
                finish(i, h)

        def attention(lo, hi):
            for i in range(lo, hi):
                for h in range(2):
                    for t in range(i + 1):
                        s = _dot_nt(q[i, h], k[t, h])
                        if t == i:
                            s = jnp.where(causal, s, MASKED)
                        in_flight.append((i, h, t, jnp.exp2(s)))
                        ahead = (i, h) == (S // T - 1, 1) and 8 <= t < 13 and not first
                        if len(in_flight) > DEPTH and not ahead:
                            weigh(*in_flight.pop(0))
            while hi == S // T and in_flight:
                weigh(*in_flight.pop(0))

        def cycles(lo, hi):
            return 2 * 64 * sum(range(lo + 1, hi + 1))

        if first:
            wk, wv, wq = head_copies(0, 0)
            _start(wv, wk, c_copy(0), c_copy(1))
            _wait(wv, wk, c_copy(0))
            _start(c_copy(2), c_copy(3), wq, x_copy(0))
            weights = [w.astype(BF16) for raw in (wk_raw, wv_raw) for w in _split(raw[0])]
            queue(0.98 * 2048, jobs_c(0)[:49])
            plain_kv(0, weights)
            flush()
            _wait(c_copy(1), c_copy(2))
            _start(x_copy(1), x_copy(2))
            queue(0.92 * 4096, jobs_c(0)[49:] + jobs_c(1) + jobs_c(2))
            plain_kv(1, weights)
            plain_kv(2, weights)
            flush()
            _wait(c_copy(3), wq)
            turn, terms = jobs_wq(0)
            queue(0.9 * 2048, _interleave(turn, jobs_c(3)))
            plain_kv(3, weights)
            flush()
            _wait(x_copy(0))
            weights = [w.astype(BF16) for w in _split(wq_raw[0])]
            queue(0.9 * (2048 + 0.2 * cycles(0, 4)), jobs_x(0)[:96], attention=0.2)
            plain_q(0, weights)
            attention(0, 4)
            flush()
            _wait(x_copy(1), x_copy(2))
            stage = [*side_copies(0, 0), *head_copies(1, 1)]
            _start(x_copy(3), *stage)
            lax.fori_loop(0, 16, lambda word, carry: wo_copy(word).start(), None)
            queue(0.98 * (2048 + 0.5 * cycles(4, 7)),
                  jobs_x(2) + terms + jobs_x(0)[96:] + jobs_x(1)[:14], attention=0.5)
            plain_q(1, weights)
            attention(4, 7)
            flush()
            _wait(x_copy(3))
            queue(0.85 * (1568 + cycles(7, 10)), jobs_x(3))
            project_q(2)
            attention(7, 10)
            flush()
            _wait(*stage)
            _start(ax_copy(0, 0), *head_copies(2, 0), *side_copies(1, 1))
            turn, terms = jobs_wq(1)
            queue(0.88 * (1568 + cycles(10, 14)), _interleave(
                _interleave(jobs_wob, jobs_wa), _interleave(jobs_x(1)[14:], _interleave(turn, jobs_wkv(1)))))
            attention(10, 11)
            project_q(3)
            attention(11, 14)
            flush()
            _wait(*[wo_copy(word) for word in range(16)], ax_copy(0, 0))
            _start(ax_copy(1, 1))
            queue(0.92 * cycles(14, 16), _interleave(
                jobs_wo + terms, [P(_job_ax, tok, released, ax_raw, ax_t, 0, *job) for job in AX_JOBS]))
            attention(14, 16)
            flush()
        else:
            queue(0.98 * 4 * 1568 * (0.5 + 0.3), _interleave(jobs_wob, jobs_wo + jobs_wa),
                  q=0.5, kv=0.3, attention=0)
            project_kv(0)
            project_q(0)
            project_kv(1)
            attention(0, 3)
            project_q(1)
            attention(3, 7)
            project_q(2)
            project_kv(2)
            attention(7, 10)
            project_q(3)
            project_kv(3)
            attention(10, 12)
            flush()
            turn, terms = jobs_wq(1 - slot)
            queue(0.95 * cycles(12, 16), _interleave(jobs_wkv(1 - slot), turn + pause + terms))
            attention(12, 16)
            flush()
        guard[0] = _sum([guard[0]] + [x for x, _ in checks])
        guard[1] = functools.reduce(jnp.maximum, [guard[1]] + [x for _, x in checks])

        def ahead(n):
            return j + n if first else jnp.minimum(j + n, NP - 1)
        _wait(*head_copies(ahead(2), slot), *side_copies(ahead(1), 1 - slot))

        @pl.when(j < NP - 1)
        def _():
            _start(*head_copies(ahead(3), 1 - slot), *side_copies(ahead(2), slot))

    def exact_pairs(ctx):
        def block(i):
            return pl.ds(pl.multiple_of(i * T, T), T)

        def qkv(n, h, i):
            return c_t.at[(2 * n + h) * 4 + (i >> 2), block(i & 3), :]

        def project(x, carry):
            h, i = x & 1, x >> 1

            def weight(raw):
                even, odd = _split(raw[0])
                return jnp.where(h == 0, even, odd).astype(BF16)
            qkv(0, h, i)[...] = (_dot(bx_raw[block(i), :], weight(wq_raw)) * SCALE_B).astype(BF16)
            qkv(1, h, i)[...] = _dot(c_raw[block(i), :], weight(wk_raw)).astype(BF16)
            qkv(2, h, i)[...] = _dot(c_raw[block(i), :], weight(wv_raw)).astype(BF16)

        def attend(b, x, carry):
            h, i = x & 1, 2 * b + (x >> 1)

            def scores(t):
                row = lax.broadcasted_iota(jnp.int32, (T, T), 0) + i * T
                col = lax.broadcasted_iota(jnp.int32, (T, T), 1) + t * T
                return jnp.where(col <= row, _dot_nt(qkv(0, h, i)[...], qkv(1, h, t)[...]), MASKED)

            m = lax.fori_loop(
                0, i + 1, lambda t, m: jnp.maximum(m, jnp.max(scores(t), axis=1, keepdims=True)),
                jnp.full((T, 1), -jnp.inf, F32))

            def accumulate(t, carry):
                l, o = carry
                p = jnp.exp2(scores(t) - m)
                return (l + jnp.sum(p, axis=1, keepdims=True),
                        o + _dot(p.astype(BF16), qkv(2, h, t)[...]))
            l, o = lax.fori_loop(0, i + 1, accumulate,
                                 (jnp.zeros((T, 1), F32), jnp.zeros((T, T), F32)))
            ctx[x] = o / l

        def pair(j, carry):
            _start(*head_copies(j, 0))
            _wait(*head_copies(j, 0))
            lax.fori_loop(0, 2 * S // T, project, None)

            def rows(b, carry):
                lax.fori_loop(0, 4, P(attend, b), None)
                for n, val in enumerate(_terms(LHS, lambda m: ctx[m])):
                    ctx_t[n, j, block(b), :] = val.astype(BF16)
            lax.fori_loop(0, S // T // 2, rows, None)

        lax.fori_loop(0, NP, pair, None)

    guard[...] = jnp.zeros(guard.shape, F32)
    pair_body(0, first=True)
    lax.fori_loop(1, NP, lambda j, carry: pair_body(j), None)

    safe = jnp.logical_and(jnp.abs(guard[0]) < jnp.inf, guard[1] < SAFE_SUM)

    @pl.when(jnp.max(jnp.where(safe, 0.0, 1.0)) > 0.0)
    def _():
        pl.run_scoped(exact_pairs, pltpu.VMEM((4, T, T), F32))


def _outputs(out_hbm, ax_copy, ax_raw, ax_t, ctx_t, wob_t, wa_t, wo_t, zero_smem,
             o_t, kbuf, vbuf, qbuf, acc, obuf, sem_out):
    def out_copy(c, slot):
        rows = pl.ds(_aligned(c * CO, CO), CO)
        return pltpu.make_async_copy(obuf.at[slot], out_hbm.at[rows, :], sem_out.at[slot])

    for buf in (kbuf, vbuf):
        for t in range(8):
            buf[t, pl.ds(CO, HALO), :] = jnp.zeros((HALO, T), F32)

    t_q = 2 * 49 * RO
    t_v = t_q + 21 * 4 * RO + 49 * RO
    t_o = t_v + (21 + EARLY_B) * 4 * RO

    def chunk_body(c, carry):
        slot = c & 1
        tok = _Tokens(zero_smem)
        plan, due, clock = {}, {}, [0]

        def schedule(job, begin, end, release=False):
            plan.setdefault(max(clock[0], begin // TICK), []).append((job, -(-end // TICK), release))

        def step(results, a, w):
            res = [None] * len(w)
            for x, left in enumerate(a):
                n = clock[0]
                clock[0] += 1
                if n in due:
                    left = _after(functools.reduce(jnp.bitwise_or, due.pop(n)), left)
                left = left.astype(BF16) if left.dtype == F32 else pltpu.bitcast(left, BF16)
                for y in range(len(w)):
                    d = _dot(left, w[y](x))
                    res[y] = d if res[y] is None else res[y] + d
                token = None
                for job, last, release in plan.pop(n, []):
                    if release and token is None:
                        token = tok.of(d[:8])
                    due.setdefault(max(last, n + 1), []).append(job(token) if release else job())
            results.append(res)

        def project(lhs_t, rhs_t, tile0, write):
            inner = {}

            def combine(i, y, m):
                inner[i, y] = _combine([x[y] for x in m])
                return tok.of(*[x[r + 8:r + 16] for x in inner[i, y] for r in range(0, RO, 16)])

            def finish(outer, y, r):
                vals = [_term(SUMS, outer, lambda i: inner[i, y][n][r:r + 16]) for n in range(4)]
                for n, val in enumerate(vals):
                    row, col = _block(outer, n)
                    write(row * RO + r, 2 * col + y, val)
                return tok.of(*[x[8:] for x in vals])

            for i in range(7):
                m = []
                done = clock[0] * TICK + 7 * RO
                for y in range(2):
                    schedule(P(combine, i, y, m), done, done + 400)
                for outer in FINAL[i]:
                    slabs = [(y, r) for r in range(0, RO, 16) for y in range(2)]
                    for x, slab in enumerate(slabs):
                        schedule(P(finish, outer, *slab), done, done + 300 + 40 * (x + 1))
                for n in range(7 * i, 7 * i + 7):
                    step(m, [_words(lhs_t, (n, x), 0, RO) for x in range(2)],
                         [P(lambda y, x: _load(rhs_t, (n, tile0 + y), x * T, T), y) for y in range(2)])

        for buf in (kbuf, vbuf):
            for t in range(8):
                buf[t, pl.ds(0, HALO), :] = buf[t, pl.ds(CO, HALO), :]

        def write_rows(buf, row, t, val):
            buf[t, pl.ds(HALO + row, 16), :] = val

        def write_q(row, t, val):
            qbuf[t, pl.ds(row, 16), :] = val * SCALE_A

        project(ax_t, wa_t, 2, P(write_rows, kbuf))
        project(ax_t, wa_t, 0, write_q)

        att = {}

        def job_weights(row, r, release):
            base = HALO + row * RO + r
            qs = [_after(release, qbuf[t, pl.ds(row * RO + r, 8), :]) for t in range(8)]
            logits = []
            for w in range(WIN):
                x = _sum([qs[t] * kbuf[t, pl.ds(base - DIL * w, 8), :] for t in range(8)])
                x = x + pltpu.roll(x, 64, 1)
                x = x + pltpu.roll(x, 32, 1)
                if row == 0 and r < DIL * w:
                    pos = lax.broadcasted_iota(jnp.int32, (8, T), 0) + (c * CO + r)
                    x = jnp.where(pos >= DIL * w, x, MASKED)
                logits.append(x)
            m = functools.reduce(jnp.maximum, logits)
            p = [jnp.exp2(x - m) for x in logits]
            att[row, r] = p + [_inverse(_sum(p))]
            return tok.of(att[row, r][-1])

        def job_values(row, r, release):
            base = HALO + row * RO + r
            *p, inv = [_after(release, x) for x in att[row, r]]
            att[row, r] = [_sum([p[w] * vbuf[t, pl.ds(base - DIL * w, 8), :] for w in range(WIN)]) * inv
                           for t in range(8)]
            return tok.of(att[row, r][-1])

        def job_o(n, r, i):
            def block(row, col):
                return _cat([att[row, r][2 * col + n], att[row, r + 8][2 * col + n]], axis=0)
            for x, val in enumerate(_terms2(LHS, i, block)):
                o_t[7 * i + x, n, pl.ds(r, 16), :] = val.astype(BF16)
            return tok.stored(o_t, (7 * i + 6, n), r)

        groups = [(row, r + x) for r in range(0, RO, 16) for row in (2, 0, 3, 1) for x in (0, 8)]
        w0, w1, v0, v1 = t_q + 1000, t_v - 1700, t_v + 400, t_o - 700
        for g, (row, r) in enumerate(groups):
            begin = w0 + (w1 - w0) * g // len(groups)
            schedule(P(job_weights, row, r), begin, begin + 500, release=True)
            begin = v0 + (v1 - v0) * g // len(groups)
            schedule(P(job_values, row, r), begin, begin + 600, release=True)
            if g % 8 == 7:
                for x, (n, i) in enumerate((n, i) for n in range(2) for i in range(7)):
                    schedule(P(job_o, n, r - 8, i), begin, min(begin + 300 + 60 * (x + 1), t_o))

        touched = {}

        def project_b(i):
            m = []

            def accumulate(y, inner):
                val = _combine([x[y] for x in m])[inner]
                token = None
                for outer, sign in OUT[i]:
                    row, col = _block(outer, inner)
                    rows, col = pl.ds(row * RO, RO), 2 * col + y
                    total = val
                    if (outer, inner, y) in touched:
                        total = acc[col, rows, :] + val if sign > 0 else acc[col, rows, :] - val
                    touched[outer, inner, y] = True
                    if outer not in FINAL[i]:
                        acc[col, rows, :] = total
                        token = tok.stored(acc, (col,), row * RO)
                    else:
                        obuf[slot, rows, pl.ds(DM + col * T, T)] = total.astype(BF16)
                        if token is None:
                            token = tok.of(_fold(jnp.add, total))
                return token

            parts = [(y, inner) for y in range(2) for inner in range(4)]
            done = clock[0] * TICK + 7 * 4 * RO
            if i < 6:
                for x, part in enumerate(parts):
                    schedule(P(accumulate, *part), done, done + 256 + 170 * x)
            for n in range(7):
                if i == 6 and n == EARLY_B:
                    yield

                def quad(kt, x):
                    term = i if len(LHS[n]) == 1 else i + tok.z * n
                    return (term, 2 * kt + x % 2), (2 * c + x // 2) * RO
                if len(LHS[n]) == 1:
                    a = [_words(ctx_t, *quad(kt, LHS[n][0][0]), RO) for kt in range(8)]
                else:
                    a = [_term(LHS, n, lambda x: _load(ctx_t, *quad(kt, x), RO).astype(F32))
                         for kt in range(8)]
                step(m, a, [P(lambda y, x: _load(wob_t, (7 * i + n, y), x * T, T), y) for y in range(2)])
            if i == 6:
                for part in parts:
                    accumulate(*part)

        for i in range(6):
            if i == 3:
                project(ax_t, wa_t, 4, P(write_rows, vbuf))
            list(project_b(i))
        last_b = project_b(6)
        next(last_b)

        for x, job in enumerate(AX_JOBS):
            schedule(P(_job_ax, tok, lambda val: val, ax_raw, ax_t, 1 - slot, *job),
                     t_o, t_o + 100 + 3300 * (x + 1) // len(AX_JOBS))

        def write_out(row, t, val):
            obuf[slot, pl.ds(row, 16), pl.ds(t * T, T)] = val.astype(BF16)

        project(o_t, wo_t, 0, write_out)
        list(last_b)
        assert not plan and not due
        out_copy(c, slot).start()
        ax_copy(jnp.minimum(c + 2, NO - 1), slot).wait()

        @pl.when(c < NO - 1)
        def _():
            ax_copy(jnp.minimum(c + 3, NO - 1), 1 - slot).start()

        @pl.when(c >= 1)
        def _():
            out_copy(c - 1, 1 - slot).wait()

    ax_copy(1, 1).wait()
    ax_copy(2, 0).start()
    lax.fori_loop(0, NO, chunk_body, None)
    out_copy(NO - 1, (NO - 1) % 2).wait()


def _kernel(ax_hbm, wqkv_hbm, wo_hbm, bx_hbm, c_hbm, wq_hbm, wuk_hbm, wuv_hbm, wob_hbm, out_hbm,
            ax_raw, ax_t, ctx_t, wob_t, wa_t, wo_t, zero_smem, sem_ax):
    vmem, dma = pltpu.VMEM, pltpu.SemaphoreType.DMA

    def clear(i, carry):
        zero_smem[0] = i >> 1
    lax.fori_loop(0, 2, clear, None)

    def ax_copy(c, slot):
        rows = pl.ds(_aligned(c * CO, CO), CO)
        return pltpu.make_async_copy(ax_hbm.at[rows, :], ax_raw.at[slot], sem_ax.at[slot])

    shared = (ax_copy, ax_raw, ax_t, ctx_t, wob_t, wa_t, wo_t, zero_smem)
    pl.run_scoped(
        P(_head_pairs, wqkv_hbm, wo_hbm, bx_hbm, c_hbm, wq_hbm, wuk_hbm, wuv_hbm, wob_hbm, *shared),
        vmem((S, DM), BF16),
        vmem((S, DC), BF16),
        vmem((2, DM, T), U32),
        vmem((2, DC, T), U32),
        vmem((2, DC, T), U32),
        vmem((2, 4, 64, DM), BF16),
        vmem((2, 4, 8, 3 * DM), U32),
        vmem((16, NH, DM), U32),
        vmem((49, 2, S // 4, T), BF16),
        vmem((49, S // 4, T), BF16),
        vmem((DM // T, T, T), U32),
        vmem((49, 2, RO, T), BF16),
        vmem((49, T, T), BF16),
        vmem((2, 8, T), F32),
        dma((2 * S // CH,)), dma((11,)))
    pl.run_scoped(
        P(_outputs, out_hbm, *shared),
        vmem((49, 2, RO, T), BF16),
        vmem((8, HALO + CO, T), F32),
        vmem((8, HALO + CO, T), F32),
        vmem((8, CO, T), F32),
        vmem((8, CO, T), F32),
        vmem((2, CO, 2 * DM), BF16),
        dma((2,)))


@jax.jit
def pallas_concat_heads__sliding_local_dilated__compressed_kv_cla__prompt_kernel(
    A_x: jax.Array,
    A_wqkv: jax.Array,
    A_wo: jax.Array,
    B_x: jax.Array,
    B_c_kv: jax.Array,
    B_w_q: jax.Array,
    B_w_uk: jax.Array,
    B_w_uv: jax.Array,
    B_w_o: jax.Array,
):
    vmem = pltpu.VMEM
    out = pl.pallas_call(
        _kernel,
        out_shape=jax.ShapeDtypeStruct((S, 2 * DM), BF16),
        in_specs=[pl.BlockSpec(memory_space=pl.ANY)] * 9,
        out_specs=pl.BlockSpec(memory_space=pl.ANY),
        scratch_shapes=[
            vmem((2, CO, DM), BF16),
            vmem((49, 2, RO, T), BF16),
            vmem((7, NP, S // 2, T), BF16),
            vmem((49, 2, DM, T), BF16),
            vmem((49, 6, 2 * T, T), BF16),
            vmem((49, 2, 2 * T, T), BF16),
            pltpu.SMEM((1,), jnp.int32),
            pltpu.SemaphoreType.DMA((2,)),
        ],
        compiler_params=pltpu.CompilerParams(
            vmem_limit_bytes=127 * 2**20, disable_bounds_checks=True),
    )(
        A_x.reshape(S, DM),
        A_wqkv.reshape(4, DM // 4, 3 * DM),
        A_wo.reshape(NH, DM // NH, DM),
        B_x.reshape(S, DM),
        B_c_kv.reshape(S, DC),
        B_w_q,
        B_w_uk,
        B_w_uv,
        B_w_o,
    )
    return out.reshape(1, S, 2 * DM)
```

```python
import functools
import math

import jax
import jax.numpy as jnp
from jax import lax
import jax.experimental.pallas as pl
import jax.experimental.pallas.tpu as pltpu

S = 2048
DM = 1024
DC = 512
NH = 32
NP = NH // 2
T = 128
CH = 4 * T
RO = 64
CO = 4 * RO
NO = S // CO
WIN, DIL = 8, 2
HALO = 16

LOG2E = math.log2(math.e)
SCALE_A = (DM // NH) ** -0.5 * LOG2E
SCALE_B = T ** -0.5 * LOG2E
MASKED = -1e9 * LOG2E
SAFE_SUM = 2.0 ** 40

DEPTH = 3
JOB_CYCLES = 896
CTX_CYCLES = 1152, 768
TICK = RO // 2
EARLY_B = 4

F32, BF16, U32 = jnp.float32, jnp.bfloat16, jnp.uint32
P = functools.partial


def _dot(a, b):
    return jnp.dot(a, b, preferred_element_type=F32)


def _dot_nt(a, b):
    return lax.dot_general(a, b, (((1,), (1,)), ((), ())), preferred_element_type=F32)


def _cat(xs, axis=1):
    return xs[0] if len(xs) == 1 else jnp.concatenate(xs, axis=axis)


def _sum(xs):
    return functools.reduce(jnp.add, xs)


def _fold(op, x):
    return functools.reduce(op, [x[r:r + 8] for r in range(0, x.shape[0], 8)])


def _aligned(x, n):
    return x if isinstance(x, int) else pl.multiple_of(x, n)


def _rows(start, n):
    return pl.ds(_aligned(start, 16), n)


def _words(ref, lead, start, n):
    return ref.bitcast(U32)[(*lead, pl.ds(_aligned(start >> 1, 8), n // 2), slice(None))]


def _load(ref, lead, start, n):
    return pltpu.bitcast(_words(ref, lead, start, n), BF16)


def _split(w):
    return (pltpu.bitcast(w << 16, F32), pltpu.bitcast(w & jnp.uint32(0xFFFF0000), F32))


def _inverse(l):
    r = pl.reciprocal(l, approx=True)
    return r * (2.0 - l * r)


def _interleave(x, y):
    order = [((n + 0.5) / len(z), m, job) for m, z in enumerate((x, y)) for n, job in enumerate(z)]
    return [job for _, _, job in sorted(order, key=lambda e: e[:2])]


def _start(*copies):
    for cp in copies:
        cp.start()


def _wait(*copies):
    for cp in copies:
        cp.wait()


LHS = (((0, 1), (3, 1)), ((2, 1), (3, 1)), ((0, 1),), ((3, 1),),
       ((0, 1), (1, 1)), ((2, 1), (0, -1)), ((1, 1), (3, -1)))
RHS = (((0, 1), (3, 1)), ((0, 1),), ((1, 1), (3, -1)), ((2, 1), (0, -1)),
       ((3, 1),), ((0, 1), (1, 1)), ((2, 1), (3, 1)))
OUT = (((0, 1), (3, 1)), ((2, 1), (3, -1)), ((1, 1), (3, 1)), ((0, 1), (2, 1)),
       ((0, -1), (1, 1)), ((3, 1),), ((0, 1),))
SUMS = tuple(tuple((i, sign) for i in range(7) for m, sign in OUT[i] if m == n) for n in range(4))
FINAL = tuple(tuple(n for n in range(4) if SUMS[n][-1][0] == i) for i in range(7))


def _term(table, i, quad):
    (n, _), *rest = table[i]
    val = quad(n)
    for n, sign in rest:
        val = val + quad(n) if sign > 0 else val - quad(n)
    return val


def _terms(table, quad):
    blocks = [quad(n) for n in range(4)]
    return [_term(table, i, blocks.__getitem__) for i in range(7)]


def _block(outer, inner):
    return 2 * (outer // 2) + inner // 2, 2 * (outer % 2) + inner % 2


def _terms2(table, i, block):
    return _terms(table, lambda n: _term(table, i, lambda m: block(*_block(m, n))))


def _combine(m):
    return [_term(SUMS, n, m.__getitem__) for n in range(4)]


def _combine2(m):
    inner = [_combine(m[i:i + 7]) for i in range(0, 49, 7)]
    return {_block(outer, n): val for n in range(4)
            for outer, val in enumerate(_combine([x[n] for x in inner]))}


class _Tokens:
    def __init__(self, zero_smem):
        self.z = zero_smem[0]
        self.zero = jnp.full((8, T), self.z, jnp.int32).astype(U32)

    def stored(self, ref, lead, start):
        first, *rest = lead
        if ref.dtype == BF16:
            return _words(ref, (first - (self.z & 1), *rest), start, 16) & self.zero
        return self.of(ref[(*lead, pl.ds(_aligned(start + 8 * (self.z & 1), 8), 8), slice(None))])

    def of(self, *vals):
        return pltpu.bitcast(_sum(vals), U32) & self.zero


def _after(token, x, everywhere=False):
    if token is None:
        return x
    bits = x if x.dtype == U32 else pltpu.bitcast(x, U32)
    cut = bits.shape[0] if everywhere else 8
    parts = [bits[r:r + 8] | token for r in range(0, cut, 8)]
    bits = _cat(parts + ([bits[cut:]] if cut < bits.shape[0] else []), axis=0)
    return bits if x.dtype == U32 else pltpu.bitcast(bits, x.dtype)


AX_JOBS = [(i, n, r) for n in range(2) for r in range(0, RO, 16) for i in range(7)]


def _job_ax(tok, released, ax_raw, ax_t, src, i, n, r):
    terms = _terms2(LHS, i, lambda row, col: released(
        ax_raw[src, pl.ds(row * RO + r, 16), pl.ds((2 * col + n) * T, T)].astype(F32)))
    for x, val in enumerate(terms):
        ax_t[7 * i + x, n, pl.ds(r, 16), :] = val.astype(BF16)
    return tok.stored(ax_t, (7 * i + 6, n), r)


def _head_pairs(wqkv_hbm, wo_hbm, bx_hbm, c_hbm, wq_hbm, wuk_hbm, wuv_hbm, wob_hbm,
                ax_copy, ax_raw, ax_t, ctx_t, wob_t, wa_t, wo_t, zero_smem,
                bx_raw, c_raw, wq_raw, wk_raw, wv_raw, wob_raw, wqkv_raw, wo_raw,
                bx_t, c_t, wq_turned, wq_t, wkv_t, guard, sem_in, sem_w):
    def head_copies(j, slot):
        return [pltpu.make_async_copy(src.bitcast(U32).at[:, j, :], dst.at[slot], sem_w.at[3 * slot + n])
                for n, (src, dst) in enumerate(((wuk_hbm, wk_raw), (wuv_hbm, wv_raw), (wq_hbm, wq_raw)))]

    def side_copies(j, slot):
        wob = wob_hbm.at[pl.ds(4 * (j >> 1), 4), pl.ds(_aligned((j & 1) * 64, 64), 64), :]
        wqkv = wqkv_hbm.bitcast(U32).at[:, pl.ds(_aligned(8 * j, 8), 8), :]
        return [pltpu.make_async_copy(wob, wob_raw.at[slot], sem_w.at[6 + 2 * slot]),
                pltpu.make_async_copy(wqkv, wqkv_raw.at[slot], sem_w.at[7 + 2 * slot])]

    def wo_copy(word):
        return pltpu.make_async_copy(wo_hbm.bitcast(U32).at[:, word, :], wo_raw.at[word], sem_w.at[10])

    def c_copy(c):
        rows = pl.ds(c * CH, CH)
        return pltpu.make_async_copy(c_hbm.at[rows, :], c_raw.at[rows, :], sem_in.at[2 * c])

    def x_copy(c):
        rows = pl.ds(c * CH, CH)
        return pltpu.make_async_copy(bx_hbm.at[rows, :], bx_raw.at[rows, :], sem_in.at[2 * c + 1])

    def pair_body(j, first=False):
        slot = j & 1
        tok = _Tokens(zero_smem)
        causal = (lax.broadcasted_iota(jnp.int32, (T, T), 1)
                  <= lax.broadcasted_iota(jnp.int32, (T, T), 0))

        jobs, due, pace = [], [], dict(release=None, recent=None)

        def queue(cycles, more, q=1.0, kv=1.0, attention=1.0):
            pace.update(period=cycles / len(more), clock=0, q=q, kv=kv, attention=attention)
            jobs.extend(more)

        def flush():
            while jobs:
                jobs.pop(0)()

        def background(cycles, share, delay, recent=None):
            pace["clock"] += cycles * share
            token = None
            while jobs and pace["clock"] >= pace["period"]:
                pace["clock"] -= pace["period"]
                pace["release"] = None if recent is None else tok.of(recent[:8])
                new = jobs.pop(0)()
                pace["release"] = None
                token = new if token is None else token | new
            if token is not None:
                due.append([delay, token])
            for entry in due:
                entry[0] -= cycles
            now = [token for left, token in due if left <= 0]
            due[:] = [entry for entry in due if entry[0] > 0]
            return functools.reduce(jnp.bitwise_or, now) if now else None

        def released(x):
            return _after(pace["release"], x, everywhere=True)

        def store_terms(dst, first_term, lead, row, terms):
            for i, val in enumerate(terms):
                dst[(first_term + i, *lead, _rows(row, 16), slice(None))] = val.astype(BF16)
            return tok.stored(dst, (first_term + 6, *lead), row)

        def job_x(c, i, n, r):
            terms = _terms2(RHS, i, lambda row, col: bx_raw[
                pl.ds(c * CH + (col ^ 2) * T + r, 16), pl.ds((2 * row + n) * T, T)].astype(F32))
            return store_terms(bx_t, 7 * i, (n,), c * T + r, terms)

        def job_c(c, i, r):
            terms = _terms2(LHS, i, lambda row, col: c_raw[
                pl.ds(c * CH + row * T + r, 16), pl.ds(col * T, T)].astype(F32))
            return store_terms(c_t, 7 * i, (), c * T + r, terms)

        def jobs_x(c):
            return [P(job_x, c, i, n, r) for r in range(0, T, 16) for n in range(2) for i in range(7)]

        def jobs_c(c):
            return [P(job_c, c, i, r) for r in range(0, T, 16) for i in range(7)]

        def job_wkv(src, i, r):
            def block(row, col):
                raw = (wk_raw, wv_raw)[col % 2]
                return _split(released(raw[src, pl.ds(row * T + r, 16), :]))[col // 2]
            return store_terms(wkv_t, 7 * i, (), r, _terms2(RHS, i, block))

        def job_turn(src, n):
            words = released(wq_raw[src, pl.ds(n * T, T), :])
            wq_turned[n] = pltpu.bitcast(pltpu.bitcast(words, F32).T, U32)
            return tok.stored(wq_turned, (n,), T - 16)

        def job_wq(i, n, r):
            def block(row, col):
                return _split(released(wq_turned[2 * col + n, pl.ds((row % 2) * RO + r, 16), :]))[row // 2]
            return store_terms(wq_t, 7 * i, (n,), r, _terms2(LHS, i, block))

        def jobs_wkv(src):
            return [P(job_wkv, src, i, r) for r in range(0, T, 16) for i in range(7)]

        def jobs_wq(src):
            return ([P(job_turn, src, n) for n in range(DM // T)],
                    [P(job_wq, i, n, r) for n in range(2) for r in range(0, RO, 16) for i in range(7)])

        def job_wob(i, n, r):
            def block(row, col):
                head = 2 * (row % 2) + row // 2
                return released(wob_raw[slot, head, pl.ds(r, 16), pl.ds((2 * col + n) * T, T)].astype(F32))
            return store_terms(wob_t, 7 * i, (n,), j * 64 + r, _terms2(RHS, i, block))

        def job_wo(i, n):
            e, odd, head = j & 3, (j >> 2) & 1, 16 * (j >> 3)

            def block(row, col):
                even_t, odd_t = _split(released(
                    wo_raw[4 * e + row, _rows(head, 16), pl.ds((2 * col + n) * T, T)]))
                return jnp.where(odd == 1, odd_t, even_t)
            return store_terms(wo_t, 7 * i, (n,), odd * T + e * NH + head, _terms2(RHS, i, block))

        permuted = {}

        def job_permute(mat):
            lane = lax.broadcasted_iota(jnp.int32, (32, T), 1)
            e, grp, sub = lane >> 5, (lane >> 2) & 7, lane & 3

            def gather(x, index):
                return jnp.take_along_axis(x, index, axis=1, mode="promise_in_bounds")
            x = [released(wqkv_raw[slot, :, :, pl.ds(mat * DM + t * T, T)].reshape(32, T))
                 for t in range(8)]
            y = [gather(x[t], sub * 32 + e * 8 + ((grp - t) & 7)) for t in range(8)]
            u = [y[-s % 8] for s in range(8)]
            for bit in (1, 2, 4):
                u = [jnp.where((grp & bit) != 0, u[(s - bit) % 8], u[s]) for s in range(8)]
            u = [u[0]] + [gather(u[t], e * 32 + ((grp + t) & 7) * 4 + sub) for t in range(1, 8)]
            permuted[mat] = u
            return _fold(jnp.bitwise_or, functools.reduce(jnp.bitwise_or, u)) & tok.zero

        def column(mat, row, t):
            return pltpu.bitcast(released(permuted[mat][t][8 * row:8 * row + 8]), BF16).astype(F32)

        def job_wa(mat, i, n):
            terms = _terms2(RHS, i, lambda row, col: column(mat, row, 2 * col + n))
            return store_terms(wa_t, 7 * i, (2 * mat + n,), 16 * j, terms)

        pause = [P(lambda: tok.zero)] * 2
        jobs_wob = [P(job_wob, i, n, r) for r in range(0, 64, 16) for n in range(2) for i in range(7)]
        jobs_wo = [P(job_wo, i, n) for n in range(2) for i in range(7)]
        jobs_wa = []
        for mat in range(3):
            jobs_wa += [P(job_permute, mat)] + pause
            jobs_wa += [P(job_wa, mat, i, n) for n in range(2) for i in range(7)]

        q, k, v = {}, {}, {}

        def product(dot, share, left, right):
            token = background(left.shape[0] // 2, share, JOB_CYCLES, pace["recent"])
            pace["recent"] = dot(pltpu.bitcast(_after(token, left), BF16), right)
            return pace["recent"]

        def project_q(c):
            blocks = _combine2([_sum([
                product(_dot_nt, pace["q"], _words(wq_t, (i, n), 0, RO), _load(bx_t, (i, n), c * T, T))
                for n in range(2)]) for i in range(49)])
            for h in range(2):
                for col in range(4):
                    val = _cat([blocks[2 * h, col], blocks[2 * h + 1, col]], axis=0) * SCALE_B
                    q[4 * c + (col ^ 2), h] = val.T.astype(BF16)

        def project_kv(c):
            m = [product(_dot, pace["kv"], _words(c_t, (i,), c * T, T), _load(wkv_t, (i,), 0, T))
                 for i in range(49)]
            for (row, col), val in sorted(_combine2(m).items()):
                (k, v)[col % 2][4 * c + row, col // 2] = val.astype(BF16)

        def plain(raw, c, weights):
            def part(r, col):
                left = raw[pl.ds(c * CH + r, 32), pl.ds(col, 4 * T)]
                token = background(32, 1.0, 128)
                if token is None:
                    return left
                return _cat([_after(_cat([token, token]), left[:, :2 * T]), left[:, 2 * T:]])
            return [_dot(_cat([_cat([part(r, col) for r in range(0, CH, 32)], axis=0)
                               for col in range(0, raw.shape[1], 4 * T)]), w) for w in weights]

        def plain_kv(c, weights):
            for n, val in enumerate(plain(c_raw, c, weights)):
                for r in range(4):
                    (k, v)[n // 2][4 * c + r, n % 2] = val[r * T:(r + 1) * T].astype(BF16)

        def plain_q(c, weights):
            for h, val in enumerate(plain(bx_raw, c, weights)):
                for r in range(4):
                    q[4 * c + r, h] = (val[r * T:(r + 1) * T] * SCALE_B).astype(BF16)

        in_flight, partial, ctx, spread, checks = [], {}, {}, {}, []

        def finish(i, h):
            l, o = partial.pop((i, h))
            l = jnp.sum(l, axis=1, keepdims=True)
            r = _inverse(l)
            ctx[i, h] = o * r
            spread[i, h] = _fold(jnp.maximum, jnp.broadcast_to(l + r, (T, T)))
            b = i // 2
            quad = [(2 * b, 0), (2 * b, 1), (2 * b + 1, 0), (2 * b + 1, 1)]
            if all(u in ctx for u in quad):
                terms = _terms(LHS, lambda m: ctx.pop(quad[m]))
                for n, val in enumerate(terms):
                    ctx_t[n, j, pl.ds(b * T, T), :] = val.astype(BF16)
                checks.append((_fold(jnp.add, terms[0] + terms[5] + terms[6]),
                               functools.reduce(jnp.maximum, [spread.pop(u) for u in quad])))
                due.append([CTX_CYCLES[first], tok.stored(ctx_t, (6, j), b * T) | tok.of(*checks[-1])])

        def weigh(i, h, t, p):
            l, o = partial.get((i, h), (None, None))
            l = p if l is None else l + p
            d = _dot(_after(background(64, pace["attention"], JOB_CYCLES, p), p).astype(BF16), v[t, h])
            partial[i, h] = (l, d if o is None else o + d)
            if t == i:
                finish(i, h)

        def attention(lo, hi):
            for i in range(lo, hi):
                for h in range(2):
                    for t in range(i + 1):
                        s = _dot_nt(q[i, h], k[t, h])
                        if t == i:
                            s = jnp.where(causal, s, MASKED)
                        in_flight.append((i, h, t, jnp.exp2(s)))
                        ahead = (i, h) == (S // T - 1, 1) and 8 <= t < 13 and not first
                        if len(in_flight) > DEPTH and not ahead:
                            weigh(*in_flight.pop(0))
            while hi == S // T and in_flight:
                weigh(*in_flight.pop(0))

        def cycles(lo, hi):
            return 2 * 64 * sum(range(lo + 1, hi + 1))

        if first:
            wk, wv, wq = head_copies(0, 0)
            _start(wv, wk, c_copy(0), c_copy(1))
            _wait(wv, wk, c_copy(0))
            _start(c_copy(2), c_copy(3), wq, x_copy(0))
            weights = [w.astype(BF16) for raw in (wk_raw, wv_raw) for w in _split(raw[0])]
            queue(0.98 * 2048, jobs_c(0)[:49])
            plain_kv(0, weights)
            flush()
            _wait(c_copy(1), c_copy(2))
            _start(x_copy(1), x_copy(2))
            queue(0.92 * 4096, jobs_c(0)[49:] + jobs_c(1) + jobs_c(2))
            plain_kv(1, weights)
            plain_kv(2, weights)
            flush()
            _wait(c_copy(3), wq)
            turn, terms = jobs_wq(0)
            queue(0.9 * 2048, _interleave(turn, jobs_c(3)))
            plain_kv(3, weights)
            flush()
            _wait(x_copy(0))
            weights = [w.astype(BF16) for w in _split(wq_raw[0])]
            queue(0.9 * (2048 + 0.1 * cycles(0, 4)), jobs_x(0)[:96], attention=0.1)
            plain_q(0, weights)
            attention(0, 4)
            flush()
            _wait(x_copy(1), x_copy(2))
            stage = [*side_copies(0, 0), *head_copies(1, 1)]
            _start(x_copy(3), *stage)
            lax.fori_loop(0, 16, lambda word, carry: wo_copy(word).start(), None)
            queue(0.98 * (2048 + 0.5 * cycles(4, 7)),
                  jobs_x(2) + terms + jobs_x(0)[96:] + jobs_x(1)[:14], attention=0.5)
            plain_q(1, weights)
            attention(4, 7)
            flush()
            _wait(x_copy(3))
            queue(0.85 * (1568 + cycles(7, 10)), jobs_x(3))
            project_q(2)
            attention(7, 10)
            flush()
            _wait(*stage)
            _start(ax_copy(0, 0), *head_copies(2, 0), *side_copies(1, 1))
            turn, terms = jobs_wq(1)
            queue(0.88 * (1568 + cycles(10, 14)), _interleave(
                _interleave(jobs_wob, jobs_wa), _interleave(jobs_x(1)[14:], _interleave(turn, jobs_wkv(1)))))
            attention(10, 11)
            project_q(3)
            attention(11, 14)
            flush()
            _wait(*[wo_copy(word) for word in range(16)], ax_copy(0, 0))
            _start(ax_copy(1, 1))
            queue(0.92 * cycles(14, 16), _interleave(
                jobs_wo + terms, [P(_job_ax, tok, released, ax_raw, ax_t, 0, *job) for job in AX_JOBS]))
            attention(14, 16)
            flush()
        else:
            queue(0.98 * 4 * 1568 * (0.5 + 0.3), _interleave(jobs_wob, jobs_wo + jobs_wa),
                  q=0.5, kv=0.3, attention=0)
            project_kv(0)
            project_q(0)
            project_q(1)
            project_kv(1)
            attention(0, 7)
            project_q(2)
            project_kv(2)
            attention(7, 11)
            project_q(3)
            project_kv(3)
            attention(11, 12)
            flush()
            turn, terms = jobs_wq(1 - slot)
            queue(0.95 * cycles(12, 16), _interleave(jobs_wkv(1 - slot), turn + pause + terms))
            attention(12, 16)
            flush()
        guard[0] = _sum([guard[0]] + [x for x, _ in checks])
        guard[1] = functools.reduce(jnp.maximum, [guard[1]] + [x for _, x in checks])

        def ahead(n):
            return j + n if first else jnp.minimum(j + n, NP - 1)
        _wait(*head_copies(ahead(2), slot), *side_copies(ahead(1), 1 - slot))

        @pl.when(j < NP - 1)
        def _():
            _start(*head_copies(ahead(3), 1 - slot), *side_copies(ahead(2), slot))

    def exact_pairs(ctx):
        def block(i):
            return pl.ds(pl.multiple_of(i * T, T), T)

        def qkv(n, h, i):
            return c_t.at[(2 * n + h) * 4 + (i >> 2), block(i & 3), :]

        def project(x, carry):
            h, i = x & 1, x >> 1

            def weight(raw):
                even, odd = _split(raw[0])
                return jnp.where(h == 0, even, odd).astype(BF16)
            qkv(0, h, i)[...] = (_dot(bx_raw[block(i), :], weight(wq_raw)) * SCALE_B).astype(BF16)
            qkv(1, h, i)[...] = _dot(c_raw[block(i), :], weight(wk_raw)).astype(BF16)
            qkv(2, h, i)[...] = _dot(c_raw[block(i), :], weight(wv_raw)).astype(BF16)

        def attend(b, x, carry):
            h, i = x & 1, 2 * b + (x >> 1)

            def scores(t):
                row = lax.broadcasted_iota(jnp.int32, (T, T), 0) + i * T
                col = lax.broadcasted_iota(jnp.int32, (T, T), 1) + t * T
                return jnp.where(col <= row, _dot_nt(qkv(0, h, i)[...], qkv(1, h, t)[...]), MASKED)

            m = lax.fori_loop(
                0, i + 1, lambda t, m: jnp.maximum(m, jnp.max(scores(t), axis=1, keepdims=True)),
                jnp.full((T, 1), -jnp.inf, F32))

            def accumulate(t, carry):
                l, o = carry
                p = jnp.exp2(scores(t) - m)
                return (l + jnp.sum(p, axis=1, keepdims=True),
                        o + _dot(p.astype(BF16), qkv(2, h, t)[...]))
            l, o = lax.fori_loop(0, i + 1, accumulate,
                                 (jnp.zeros((T, 1), F32), jnp.zeros((T, T), F32)))
            ctx[x] = o / l

        def pair(j, carry):
            _start(*head_copies(j, 0))
            _wait(*head_copies(j, 0))
            lax.fori_loop(0, 2 * S // T, project, None)

            def rows(b, carry):
                lax.fori_loop(0, 4, P(attend, b), None)
                for n, val in enumerate(_terms(LHS, lambda m: ctx[m])):
                    ctx_t[n, j, block(b), :] = val.astype(BF16)
            lax.fori_loop(0, S // T // 2, rows, None)

        lax.fori_loop(0, NP, pair, None)

    guard[...] = jnp.zeros(guard.shape, F32)
    pair_body(0, first=True)
    lax.fori_loop(1, NP, lambda j, carry: pair_body(j), None)

    safe = jnp.logical_and(jnp.abs(guard[0]) < jnp.inf, guard[1] < SAFE_SUM)

    @pl.when(jnp.max(jnp.where(safe, 0.0, 1.0)) > 0.0)
    def _():
        pl.run_scoped(exact_pairs, pltpu.VMEM((4, T, T), F32))


def _outputs(out_hbm, ax_copy, ax_raw, ax_t, ctx_t, wob_t, wa_t, wo_t, zero_smem,
             o_t, kbuf, vbuf, qbuf, acc, obuf, sem_out):
    def out_copy(c, slot):
        rows = pl.ds(_aligned(c * CO, CO), CO)
        return pltpu.make_async_copy(obuf.at[slot], out_hbm.at[rows, :], sem_out.at[slot])

    for buf in (kbuf, vbuf):
        for t in range(8):
            buf[t, pl.ds(CO, HALO), :] = jnp.zeros((HALO, T), F32)

    t_q = 2 * 49 * RO
    t_v = t_q + 21 * 4 * RO + 49 * RO
    t_o = t_v + (21 + EARLY_B) * 4 * RO

    def chunk_body(c, carry):
        slot = c & 1
        tok = _Tokens(zero_smem)
        plan, due, clock = {}, {}, [0]

        def schedule(job, begin, end, release=False):
            plan.setdefault(max(clock[0], begin // TICK), []).append((job, -(-end // TICK), release))

        def step(results, a, w):
            res = [None] * len(w)
            for x, left in enumerate(a):
                n = clock[0]
                clock[0] += 1
                if n in due:
                    left = _after(functools.reduce(jnp.bitwise_or, due.pop(n)), left)
                left = left.astype(BF16) if left.dtype == F32 else pltpu.bitcast(left, BF16)
                for y in range(len(w)):
                    d = _dot(left, w[y](x))
                    res[y] = d if res[y] is None else res[y] + d
                token = None
                for job, last, release in plan.pop(n, []):
                    if release and token is None:
                        token = tok.of(d[:8])
                    due.setdefault(max(last, n + 1), []).append(job(token) if release else job())
            results.append(res)

        def project(lhs_t, rhs_t, tile0, write):
            inner = {}

            def combine(i, y, m):
                inner[i, y] = _combine([x[y] for x in m])
                return tok.of(*[x[r + 8:r + 16] for x in inner[i, y] for r in range(0, RO, 16)])

            def finish(outer, y, r):
                vals = [_term(SUMS, outer, lambda i: inner[i, y][n][r:r + 16]) for n in range(4)]
                for n, val in enumerate(vals):
                    row, col = _block(outer, n)
                    write(row * RO + r, 2 * col + y, val)
                return tok.of(*[x[8:] for x in vals])

            for i in range(7):
                m = []
                done = clock[0] * TICK + 7 * RO
                for y in range(2):
                    schedule(P(combine, i, y, m), done, done + 400)
                for outer in FINAL[i]:
                    slabs = [(y, r) for r in range(0, RO, 16) for y in range(2)]
                    for x, slab in enumerate(slabs):
                        schedule(P(finish, outer, *slab), done, done + 300 + 40 * (x + 1))
                for n in range(7 * i, 7 * i + 7):
                    step(m, [_words(lhs_t, (n, x), 0, RO) for x in range(2)],
                         [P(lambda y, x: _load(rhs_t, (n, tile0 + y), x * T, T), y) for y in range(2)])

        for buf in (kbuf, vbuf):
            for t in range(8):
                buf[t, pl.ds(0, HALO), :] = buf[t, pl.ds(CO, HALO), :]

        def write_rows(buf, row, t, val):
            buf[t, pl.ds(HALO + row, 16), :] = val

        def write_q(row, t, val):
            qbuf[t, pl.ds(row, 16), :] = val * SCALE_A

        project(ax_t, wa_t, 2, P(write_rows, kbuf))
        project(ax_t, wa_t, 0, write_q)

        att = {}

        def job_weights(row, r, release):
            base = HALO + row * RO + r
            qs = [_after(release, qbuf[t, pl.ds(row * RO + r, 8), :]) for t in range(8)]
            logits = []
            for w in range(WIN):
                x = _sum([qs[t] * kbuf[t, pl.ds(base - DIL * w, 8), :] for t in range(8)])
                x = x + pltpu.roll(x, 64, 1)
                x = x + pltpu.roll(x, 32, 1)
                if row == 0 and r < DIL * w:
                    pos = lax.broadcasted_iota(jnp.int32, (8, T), 0) + (c * CO + r)
                    x = jnp.where(pos >= DIL * w, x, MASKED)
                logits.append(x)
            m = functools.reduce(jnp.maximum, logits)
            p = [jnp.exp2(x - m) for x in logits]
            att[row, r] = p + [_inverse(_sum(p))]
            return tok.of(att[row, r][-1])

        def job_values(row, r, release):
            base = HALO + row * RO + r
            *p, inv = [_after(release, x) for x in att[row, r]]
            att[row, r] = [_sum([p[w] * vbuf[t, pl.ds(base - DIL * w, 8), :] for w in range(WIN)]) * inv
                           for t in range(8)]
            return tok.of(att[row, r][-1])

        def job_o(n, r, i):
            def block(row, col):
                return _cat([att[row, r][2 * col + n], att[row, r + 8][2 * col + n]], axis=0)
            for x, val in enumerate(_terms2(LHS, i, block)):
                o_t[7 * i + x, n, pl.ds(r, 16), :] = val.astype(BF16)
            return tok.stored(o_t, (7 * i + 6, n), r)

        groups = [(row, r + x) for r in range(0, RO, 16) for row in (2, 0, 3, 1) for x in (0, 8)]
        w0, w1, v0, v1 = t_q + 1000, t_v - 1700, t_v + 200, t_o - 700
        for g, (row, r) in enumerate(groups):
            begin = w0 + (w1 - w0) * g // len(groups)
            schedule(P(job_weights, row, r), begin, begin + 500, release=True)
            begin = v0 + (v1 - v0) * g // len(groups)
            schedule(P(job_values, row, r), begin, begin + 600, release=True)
            if g % 8 == 7:
                for x, (n, i) in enumerate((n, i) for n in range(2) for i in range(7)):
                    schedule(P(job_o, n, r - 8, i), begin, min(begin + 300 + 60 * (x + 1), t_o))

        touched = {}

        def project_b(i):
            m = []

            def accumulate(y, inner):
                val = _combine([x[y] for x in m])[inner]
                token = None
                for outer, sign in OUT[i]:
                    row, col = _block(outer, inner)
                    rows, col = pl.ds(row * RO, RO), 2 * col + y
                    total = val
                    if (outer, inner, y) in touched:
                        total = acc[col, rows, :] + val if sign > 0 else acc[col, rows, :] - val
                    touched[outer, inner, y] = True
                    if outer not in FINAL[i]:
                        acc[col, rows, :] = total
                        token = tok.stored(acc, (col,), row * RO)
                    else:
                        obuf[slot, rows, pl.ds(DM + col * T, T)] = total.astype(BF16)
                        if token is None:
                            token = tok.of(_fold(jnp.add, total))
                return token

            parts = [(y, inner) for y in range(2) for inner in range(4)]
            done = clock[0] * TICK + 7 * 4 * RO
            if i < 6:
                for x, part in enumerate(parts):
                    schedule(P(accumulate, *part), done, done + 256 + 170 * x)
            for n in range(7):
                if i == 6 and n == EARLY_B:
                    yield

                def quad(kt, x):
                    term = i if len(LHS[n]) == 1 else i + tok.z * n
                    return (term, 2 * kt + x % 2), (2 * c + x // 2) * RO
                if len(LHS[n]) == 1:
                    a = [_words(ctx_t, *quad(kt, LHS[n][0][0]), RO) for kt in range(8)]
                else:
                    a = [_term(LHS, n, lambda x: _load(ctx_t, *quad(kt, x), RO).astype(F32))
                         for kt in range(8)]
                step(m, a, [P(lambda y, x: _load(wob_t, (7 * i + n, y), x * T, T), y) for y in range(2)])
            if i == 6:
                for part in parts:
                    accumulate(*part)

        for i in range(6):
            if i == 3:
                project(ax_t, wa_t, 4, P(write_rows, vbuf))
            list(project_b(i))
        last_b = project_b(6)
        next(last_b)

        for x, job in enumerate(AX_JOBS):
            schedule(P(_job_ax, tok, lambda val: val, ax_raw, ax_t, 1 - slot, *job),
                     t_o, t_o + 100 + 3300 * (x + 1) // len(AX_JOBS))

        def write_out(row, t, val):
            obuf[slot, pl.ds(row, 16), pl.ds(t * T, T)] = val.astype(BF16)

        project(o_t, wo_t, 0, write_out)
        list(last_b)
        assert not plan and not due
        out_copy(c, slot).start()
        ax_copy(jnp.minimum(c + 2, NO - 1), slot).wait()

        @pl.when(c < NO - 1)
        def _():
            ax_copy(jnp.minimum(c + 3, NO - 1), 1 - slot).start()

        @pl.when(c >= 1)
        def _():
            out_copy(c - 1, 1 - slot).wait()

    ax_copy(1, 1).wait()
    ax_copy(2, 0).start()
    lax.fori_loop(0, NO, chunk_body, None)
    out_copy(NO - 1, (NO - 1) % 2).wait()


def _kernel(ax_hbm, wqkv_hbm, wo_hbm, bx_hbm, c_hbm, wq_hbm, wuk_hbm, wuv_hbm, wob_hbm, out_hbm,
            ax_raw, ax_t, ctx_t, wob_t, wa_t, wo_t, zero_smem, sem_ax):
    vmem, dma = pltpu.VMEM, pltpu.SemaphoreType.DMA

    def clear(i, carry):
        zero_smem[0] = i >> 1
    lax.fori_loop(0, 2, clear, None)

    def ax_copy(c, slot):
        rows = pl.ds(_aligned(c * CO, CO), CO)
        return pltpu.make_async_copy(ax_hbm.at[rows, :], ax_raw.at[slot], sem_ax.at[slot])

    shared = (ax_copy, ax_raw, ax_t, ctx_t, wob_t, wa_t, wo_t, zero_smem)
    pl.run_scoped(
        P(_head_pairs, wqkv_hbm, wo_hbm, bx_hbm, c_hbm, wq_hbm, wuk_hbm, wuv_hbm, wob_hbm, *shared),
        vmem((S, DM), BF16),
        vmem((S, DC), BF16),
        vmem((2, DM, T), U32),
        vmem((2, DC, T), U32),
        vmem((2, DC, T), U32),
        vmem((2, 4, 64, DM), BF16),
        vmem((2, 4, 8, 3 * DM), U32),
        vmem((16, NH, DM), U32),
        vmem((49, 2, S // 4, T), BF16),
        vmem((49, S // 4, T), BF16),
        vmem((DM // T, T, T), U32),
        vmem((49, 2, RO, T), BF16),
        vmem((49, T, T), BF16),
        vmem((2, 8, T), F32),
        dma((2 * S // CH,)), dma((11,)))
    pl.run_scoped(
        P(_outputs, out_hbm, *shared),
        vmem((49, 2, RO, T), BF16),
        vmem((8, HALO + CO, T), F32),
        vmem((8, HALO + CO, T), F32),
        vmem((8, CO, T), F32),
        vmem((8, CO, T), F32),
        vmem((2, CO, 2 * DM), BF16),
        dma((2,)))


@jax.jit
def pallas_concat_heads__sliding_local_dilated__compressed_kv_cla__prompt_kernel(
    A_x: jax.Array,
    A_wqkv: jax.Array,
    A_wo: jax.Array,
    B_x: jax.Array,
    B_c_kv: jax.Array,
    B_w_q: jax.Array,
    B_w_uk: jax.Array,
    B_w_uv: jax.Array,
    B_w_o: jax.Array,
):
    vmem = pltpu.VMEM
    out = pl.pallas_call(
        _kernel,
        out_shape=jax.ShapeDtypeStruct((S, 2 * DM), BF16),
        in_specs=[pl.BlockSpec(memory_space=pl.ANY)] * 9,
        out_specs=pl.BlockSpec(memory_space=pl.ANY),
        scratch_shapes=[
            vmem((2, CO, DM), BF16),
            vmem((49, 2, RO, T), BF16),
            vmem((7, NP, S // 2, T), BF16),
            vmem((49, 2, DM, T), BF16),
            vmem((49, 6, 2 * T, T), BF16),
            vmem((49, 2, 2 * T, T), BF16),
            pltpu.SMEM((1,), jnp.int32),
            pltpu.SemaphoreType.DMA((2,)),
        ],
        compiler_params=pltpu.CompilerParams(
            vmem_limit_bytes=127 * 2**20, disable_bounds_checks=True),
    )(
        A_x.reshape(S, DM),
        A_wqkv.reshape(4, DM // 4, 3 * DM),
        A_wo.reshape(NH, DM // NH, DM),
        B_x.reshape(S, DM),
        B_c_kv.reshape(S, DC),
        B_w_q,
        B_w_uk,
        B_w_uv,
        B_w_o,
    )
    return out.reshape(1, S, 2 * DM)
```
